```python
import jax
import jax.numpy as jnp

def _softmax(x, axis=-1):
    return jax.nn.softmax(x, axis=axis)

def _gelu(x):
    return jax.nn.gelu(x, approximate=True)

def _silu(x):
    return jax.nn.silu(x)

def _sigmoid(x):
    return jax.nn.sigmoid(x)

def _layernorm(x, axis=-1, eps=1e-05):
    m = jnp.mean(x, axis=axis, keepdims=True)
    v = jnp.var(x, axis=axis, keepdims=True)
    return (x - m) / jnp.sqrt(v + eps)

def _scatter_add(tgt, idx, src, axis=0):
    return tgt.at[idx].add(src)

def _segment_sum(src, seg, n):
    return jax.ops.segment_sum(src, seg, n)

class _Rng:

    def __init__(self, key):
        self._k = key

    def _next(self):
        self._k, sub = jax.random.split(self._k)
        return sub

    def normal(self, shape):
        return jax.random.normal(self._next(), shape, dtype=jnp.bfloat16)

    def randint(self, lo, hi, shape):
        return jax.random.randint(self._next(), shape, lo, hi, dtype=jnp.int32)

    def uniform(self, shape, lo=0.0, hi=1.0):
        return jax.random.uniform(self._next(), shape, jnp.bfloat16, lo, hi)

    def permutation(self, n):
        return jax.random.permutation(self._next(), n)
kernel_name = 'adaLN_cond__memory_aug_recurrent_mem_tr__moe_arch_mod__prompt'

def setup_inputs():
    _rng = _Rng(jax.random.key(int.from_bytes(__import__("os").urandom(4), "little")))
    _w = lambda a: (lambda t: t.astype(jnp.bfloat16) if jnp.issubdtype(t.dtype, jnp.floating) else t)(jnp.asarray(a))

    def _A_setup():
        B, S, Dm = (1, 2048, 1024)
        H, Dh = (32, 128)
        M, seg = (8, 32)
        seg = min(seg, S)
        S = S // seg * seg
        return {'x': _w((lambda *s: _rng.normal(s) * 0.05)(B, S, Dm)), 'mem0': _w((lambda *s: _rng.normal(s) * 0.05)(B, M, Dm)), 'Wq': _w((lambda *s: _rng.normal(s) * 0.05)(Dm, H, Dh) * Dm ** (-0.5)), 'Wk': _w((lambda *s: _rng.normal(s) * 0.05)(Dm, H, Dh) * Dm ** (-0.5)), 'Wv': _w((lambda *s: _rng.normal(s) * 0.05)(Dm, H, Dh) * Dm ** (-0.5)), 'Wo': _w((lambda *s: _rng.normal(s) * 0.05)(H, Dh, Dm) * (H * Dh) ** (-0.5)), 'seg_len': seg}
    _A_in = _A_setup()

    def _B_setup():
        B, S, D, F, C = (1, 2048, 1024, 3584, 2)
        return {'x': _w((lambda *s: _rng.normal(s) * 0.05)(B, S, D)), 'w_r': _w((lambda *s: _rng.normal(s) * 0.05)(D)), 'w_gate': _w((lambda *s: _rng.normal(s) * 0.05)(D, F)), 'w_up': _w((lambda *s: _rng.normal(s) * 0.05)(D, F)), 'w_down': _w((lambda *s: _rng.normal(s) * 0.05)(F, D))}
    _B_in = _B_setup()
    return {'A_x': _A_in['x'], 'A_mem0': _A_in['mem0'], 'A_Wq': _A_in['Wq'], 'A_Wk': _A_in['Wk'], 'A_Wv': _A_in['Wv'], 'A_Wo': _A_in['Wo'], 'A_seg_len': _A_in['seg_len'], 'B_x': _B_in['x'], 'B_w_r': _B_in['w_r'], 'B_w_gate': _B_in['w_gate'], 'B_w_up': _B_in['w_up'], 'B_w_down': _B_in['w_down'], 'c': _w((lambda *s: _rng.normal(s) * 0.05)(1, 1024)), 'w_mod': _w((lambda *s: _rng.normal(s) * 0.05)(1024, 6 * 1024) * 1024 ** (-0.5))}

def reference(A_x, A_mem0, A_Wq, A_Wk, A_Wv, A_Wo, A_seg_len, B_x, B_w_r, B_w_gate, B_w_up, B_w_down, c, w_mod):

    def _A_ref(x, mem0, Wq, Wk, Wv, Wo, seg_len):
        B, S, Dm = x.shape
        H, Dh = (Wq.shape[1], Wq.shape[2])
        M = mem0.shape[1]
        scale = Dh ** (-0.5)
        n_seg = S // seg_len
        L = M + seg_len
        idx = jnp.arange(L)
        mask = (idx[:, None] < M) | (idx[:, None] >= idx[None, :])
        mem = mem0
        outs = []
        for s in range(n_seg):
            xs = x[:, s * seg_len:(s + 1) * seg_len, :].copy()
            h = jnp.concatenate([mem, xs], axis=1)
            q = jnp.einsum('btd,dhe->bhte', h, Wq)
            k = jnp.einsum('btd,dhe->bhte', h, Wk)
            v = jnp.einsum('btd,dhe->bhte', h, Wv)
            scores = jnp.einsum('bhqe,bhke->bhqk', q, k) * scale
            scores = jnp.where(mask[None, None], scores, -1000000000.0)
            p = _softmax(scores, axis=-1)
            o = jnp.einsum('bhqk,bhke->bhqe', p, v)
            o = jnp.einsum('bhte,hed->btd', o, Wo)
            mem = o[:, :M, :].copy()
            outs.append(o[:, M:, :])
        return jnp.concatenate(outs, axis=1)

    def _B_ref(x, w_r, w_gate, w_up, w_down):
        B, S, D = x.shape
        C = 2
        r = x @ w_r
        idx = jnp.argsort(-r, axis=-1)[:, :C]
        idx_e = jnp.repeat(idx.reshape(B, C, 1), D, axis=2)
        x_sel = jnp.take_along_axis(x, idx_e, axis=1)
        g = _silu(x_sel @ w_gate)
        u = x_sel @ w_up
        y = g * u @ w_down
        r_sel = _sigmoid(jnp.take_along_axis(r, idx, axis=1))
        y = y * r_sel.reshape(B, C, 1)
        b_off = (jnp.arange(B) * S).reshape(B, 1)
        flat_idx = (idx + b_off).reshape(B * C)
        zero = (x * 0.0).reshape(B * S, D)
        upd = _scatter_add(zero, flat_idx, y.reshape(B * C, D), axis=0)
        return x + upd.reshape(B, S, D)
    x = A_x
    mod = (_silu(c) @ w_mod).reshape(c.shape[0], 6, 1, -1)
    sa, ca, ga, sb, cb, gb = (mod[:, 0].copy(), mod[:, 1].copy(), mod[:, 2].copy(), mod[:, 3].copy(), mod[:, 4].copy(), mod[:, 5].copy())
    h = _layernorm(x, axis=-1) * (1 + ca) + sa
    x = x + ga * _A_ref(h, A_mem0, A_Wq, A_Wk, A_Wv, A_Wo, A_seg_len)
    h = _layernorm(x, axis=-1) * (1 + cb) + sb
    x = x + gb * _B_ref(h, B_w_r, B_w_gate, B_w_up, B_w_down)
    return x
```

```python
import jax
import jax.numpy as jnp
from jax import lax
import jax.experimental.pallas as pl
import jax.experimental.pallas.tpu as pltpu

BF = jnp.bfloat16
F32 = jnp.float32
U32 = jnp.uint32

S = 2048
D = 1024
H = 32
DH = 128
M = 8
SEG = 32
NSEG = S // SEG
FF = 3584
RIDE = 24
BULK = S - RIDE * NSEG
RING = 576
PITCH = 520
NSTAGE = 4
TAIL0 = RIDE * NSEG
TCH = 128
EPS = 1e-5
NEG = -3.0e38


def _rb(v):
    return v.astype(BF).astype(F32)


def _layernorm(xf):
    mu = jnp.mean(xf, axis=-1, keepdims=True)
    dv = xf - mu
    var = jnp.mean(dv * dv, axis=-1, keepdims=True)
    sd = _rb(jnp.sqrt(_rb(_rb(var) + EPS)))
    return _rb(_rb(xf - _rb(mu)) * (1.0 / sd))


def _kernel(x_hbm, mem0_hbm, wq_hbm, wk_hbm, wv_hbm, wo_hbm, wr_hbm, wg_hbm, wu_hbm, wd_hbm,
            c_hbm, wmod_hbm, out_hbm,
            x_v, h_v, att_v, h2_v, out_v, wqkv_v, wo_v, ring, oring, stage, wmod_v,
            wg_v, wu_v, wd_v, mem_v, c_v, wr_v, mod_v, r1_v, r2_v,
            sem_small, sem_x, sem_stage, sem_wmod, sem_wo, sem_ffn, sem_out):
    w_hbm = (wq_hbm, wk_hbm, wv_hbm)

    def piece_copy(m, hh, j, slot):
        return pltpu.make_async_copy(
            w_hbm[m].at[pl.ds(j * 512, 512), pl.ds(hh * 16, 16), :], stage.at[slot],
            sem_stage.at[slot])

    def piece_wait(slot):
        pltpu.make_async_copy(stage.at[slot], stage.at[slot], sem_stage.at[slot]).wait()

    def wmod_copy(k):
        return pltpu.make_async_copy(wmod_hbm.at[:, pl.ds(k * 512, 512)], wmod_v.at[k],
                                     sem_wmod.at[k])

    def wo_copy(n):
        return pltpu.make_async_copy(wo_hbm.at[:, pl.ds(n * 128, 128)], wo_v.at[n], sem_wo.at[n])

    x0_copy = pltpu.make_async_copy(x_hbm.at[0, pl.ds(0, BULK), :], x_v.at[pl.ds(0, BULK), :],
                                    sem_x.at[0])
    x1_copy = pltpu.make_async_copy(x_hbm.at[0, pl.ds(BULK, S - BULK), :],
                                    x_v.at[pl.ds(BULK, S - BULK), :], sem_x.at[1])
    c_copy = pltpu.make_async_copy(c_hbm, c_v, sem_small.at[0])
    mem_copy = pltpu.make_async_copy(mem0_hbm.at[0], mem_v, sem_small.at[1])
    wr_copy = pltpu.make_async_copy(wr_hbm, wr_v, sem_small.at[2])
    wg_copy = pltpu.make_async_copy(wg_hbm, wg_v, sem_ffn.at[0])
    wu_copy = pltpu.make_async_copy(wu_hbm, wu_v, sem_ffn.at[1])
    wd_copies = [pltpu.make_async_copy(wd_hbm.at[:, pl.ds(k * 512, 512)], wd_v.at[k],
                                       sem_ffn.at[2 + k]) for k in range(2)]

    def slab_row(m, h):
        chunk = 2 * m + h // 16
        return (chunk * 16 + (h % 2) * 8 + (h % 16) // 2) * PITCH

    def relayout(slot, chunk, j, lo, n):
        base = chunk * (16 * PITCH) + j * 256 + lo // 2
        u = pltpu.bitcast(stage[slot, pl.ds(lo, n)], U32)
        for i in range(n // 2):
            a = u[2 * i]
            b = u[2 * i + 1]
            even = (a & jnp.uint32(0xFFFF)) | (b << 16)
            odd = (a >> 16) | (b & jnp.uint32(0xFFFF0000))
            wqkv_v[pl.ds(base + i, 8, stride=PITCH), :] = even
            wqkv_v[pl.ds(base + 8 * PITCH + i, 8, stride=PITCH), :] = odd

    def mod_row(k):
        return mod_v[pl.ds(k, 1), :]

    def modulate(ln, k_scale, k_shift):
        return _rb(ln * mod_row(k_scale)) + mod_row(k_shift)

    def post(row0, n, r_ref, lane):
        xf = x_v[pl.ds(row0, n), :].astype(F32)
        a = att_v[pl.ds(row0, n), :].astype(F32)
        x2 = _rb(xf + _rb(mod_row(2) * a))
        h2b = modulate(_layernorm(x2), 4, 3).astype(BF)
        h2 = h2b.astype(F32)
        h2_v[pl.ds(row0, n), :] = h2b
        out_v[pl.ds(row0, n), :] = (x2 + mod_row(5) * h2).astype(BF)
        r = jnp.sum(h2 * mod_row(6), axis=-1, keepdims=True)
        lanes = lax.broadcasted_iota(jnp.int32, (n, 128), 1)
        r_ref[...] = jnp.where(lanes == lane, r, r_ref[...])

    piece_copy(0, 0, 0, 0).start()
    x0_copy.start()
    c_copy.start()
    piece_copy(0, 0, 1, 1).start()
    for k in range(4):
        wmod_copy(k).start()
    mem_copy.start()
    wr_copy.start()

    r1_v[...] = jnp.full(r1_v.shape, NEG, F32)
    r2_v[...] = jnp.full(r2_v.shape, NEG, F32)
    att_v[pl.ds(0, RIDE), :] = jnp.zeros((RIDE, D), BF)

    piece_wait(0)

    def relayout0(i, carry):
        relayout(0, 0, 0, pl.multiple_of(i * 64, 64), 64)
        return carry
    lax.fori_loop(0, 8, relayout0, 0)

    x0_copy.wait()

    def ln0(i, carry):
        r0 = pl.multiple_of(i * 64, 64)
        h_v[pl.ds(r0, 64), :] = _layernorm(x_v[pl.ds(r0, 64), :].astype(F32)).astype(BF)
        return carry
    lax.fori_loop(0, BULK // 64, ln0, 0)

    piece_wait(1)

    def relayout1(i, carry):
        relayout(1, 0, 1, pl.multiple_of(i * 64, 64), 64)
        return carry
    lax.fori_loop(0, 8, relayout1, 0)

    c_copy.wait()
    cf = c_v[...].astype(F32)
    sc = jnp.broadcast_to((cf * jax.nn.sigmoid(cf)).astype(BF), (16, D))

    def mod_slab(k):
        y = _rb(jnp.dot(sc, wmod_v[k], preferred_element_type=F32)[0:1])
        if k // 2 in (1, 4):
            y = _rb(1.0 + y)
        mod_v[pl.ds(k // 2, 1), pl.ds((k % 2) * 512, 512)] = y

    for k in range(4):
        wmod_copy(k).wait()
        if k == 3:
            piece_copy(0, 1, 0, 2).start()
            piece_copy(0, 1, 1, 3).start()
            x1_copy.start()
        mod_slab(k)

    def mod0(i, carry):
        r0 = pl.multiple_of(i * 64, 64)
        h_v[pl.ds(r0, 64), :] = modulate(h_v[pl.ds(r0, 64), :].astype(F32), 1, 0).astype(BF)
        return carry
    lax.fori_loop(0, BULK // 64, mod0, 0)

    def bulk_qkv(i, carry):
        @pl.when(i == 0)
        def _():
            x1_copy.wait()

        @pl.when(i < 10)
        def _():
            piece_wait((i + 2) % NSTAGE)

        for t in range(4, 12):
            @pl.when(i == t - 4)
            def _():
                piece_copy(t // 4, (t // 2) % 2, t % 2, t % NSTAGE).start()
                wo_copy(t - 4).start()
                wmod_copy(t).start()

        t = jnp.minimum(i + 2, 11)
        slot = t % NSTAGE
        hb = h_v[pl.ds(0, BULK), :]
        for k in range(8):
            sl = 8 * i + k
            w = pltpu.bitcast(wqkv_v[pl.ds(pl.multiple_of(sl * PITCH, 8), 512), :], BF)
            y = jnp.dot(hb, w, preferred_element_type=F32)
            ring[sl, pl.ds(RING - BULK, BULK), :] = y.astype(BF)
            relayout(slot, t // 2, t % 2, k * 64, 64)
            r0 = pl.multiple_of(BULK + i * 128 + k * 16, 16)
            ln = _layernorm(x_v[pl.ds(r0, 16), :].astype(F32))
            att_dummy = modulate(ln, 1, 0).astype(BF)
            h2_v[pl.ds(r0, 16), :] = att_dummy
        return carry
    lax.fori_loop(0, 12, bulk_qkv, 0)

    wg_copy.start()
    wu_copy.start()
    for cp in wd_copies:
        cp.start()

    for k in range(4, 12):
        wmod_copy(k).wait()
    for k in range(4, 12):
        mod_slab(k)
    wr_copy.wait()
    mod_v[pl.ds(6, 1), :] = wr_v[...].astype(F32)
    mem_copy.wait()
    for n in range(8):
        wo_copy(n).wait()

    scale = DH ** -0.5
    rr = lax.broadcasted_iota(jnp.int32, (80, 80), 0)
    cc = lax.broadcasted_iota(jnp.int32, (80, 80), 1)

    def second(i):
        return ((i >= 8) & (i < 16)) | (i >= 48)
    same = second(rr) == second(cc)
    allowed = same & ((rr < 16) | (cc <= rr))
    fill = jnp.where(same, -1e9, NEG).astype(F32)

    def ring_slab(m, h):
        return slab_row(m, h) // PITCH

    def step(s, carry):
        wr = pl.multiple_of(lax.rem(RIDE * s, RING), 8)
        rd = pl.multiple_of(lax.rem(SEG * s + RING - BULK, RING), SEG)
        ow = pl.multiple_of(lax.rem(SEG * s + 192, RING), SEG)
        orr = pl.multiple_of(lax.rem(RIDE * s + 192, RING), 8)
        hx = h2_v[pl.ds(pl.multiple_of(BULK + RIDE * s, 8), RIDE), :]
        xin = jnp.concatenate([mem_v[...], hx], axis=0)

        prev = jnp.maximum(s - 1, 0)
        post(pl.multiple_of(RIDE * prev, 8), RIDE, r1_v, prev)

        memqkv, tok, probs, rinv, omem, otok = {}, {}, {}, {}, {}, {}
        acc = []

        def qkv(p):
            for m in range(3):
                ys = []
                for h in (2 * p, 2 * p + 1):
                    w = pltpu.bitcast(wqkv_v[pl.ds(slab_row(m, h), 512), :], BF)
                    y = jnp.dot(xin, w, preferred_element_type=F32)
                    ring[ring_slab(m, h), pl.ds(wr, RIDE), :] = y[M:].astype(BF)
                    ys.append(y[:M])
                memqkv[(m, p)] = jnp.concatenate(ys, axis=0).astype(BF)

        def gather(m, p):
            tok[(m, p)] = [ring[ring_slab(m, h), pl.ds(rd, SEG), :] for h in (2 * p, 2 * p + 1)]

        def cat(m, p):
            return jnp.concatenate([memqkv[(m, p)]] + tok[(m, p)], axis=0)

        def scores(p):
            sc_ = lax.dot_general(cat(0, p), cat(1, p), (((1,), (1,)), ((), ())),
                                  preferred_element_type=F32)
            sc_ = jnp.where(allowed, sc_ * scale, fill)
            e = jnp.exp(sc_ - jnp.max(sc_, axis=1, keepdims=True))
            l = jnp.sum(e, axis=1, keepdims=True)
            rc = pl.reciprocal(l, approx=True)
            rinv[p] = rc * (2.0 - l * rc)
            probs[p] = e.astype(BF)

        def pv(p):
            o = jnp.dot(probs[p], cat(2, p), preferred_element_type=F32) * rinv[p]
            omem[2 * p] = o[0:8]
            omem[2 * p + 1] = o[8:16]
            oring[2 * p, pl.ds(ow, SEG), :] = o[16:48].astype(BF)
            oring[2 * p + 1, pl.ds(ow, SEG), :] = o[48:80].astype(BF)

        def wo_load(g):
            for h in range(4 * g, 4 * g + 4):
                otok[h] = oring[h, pl.ds(orr, RIDE), :]

        def wo(g):
            lhs = jnp.concatenate(
                [jnp.concatenate([omem[h].astype(BF), otok[h]], axis=0)
                 for h in range(4 * g, 4 * g + 4)], axis=1)
            w = jnp.concatenate([wo_v[n, pl.ds(512 * g, 512), :] for n in range(8)], axis=1)
            y = jnp.dot(lhs, w, preferred_element_type=F32)
            acc[:] = [y if not acc else acc[0] + y]

        ng = 8
        pend = list(range(ng))
        for g in range(ng + 2):
            if 0 <= g - 1 < ng:
                for p in (2 * g - 2, 2 * g - 1):
                    gather(0, p)
                    gather(1, p)
            if 0 <= g - 2 < ng:
                for p in (2 * g - 4, 2 * g - 3):
                    gather(2, p)
            if g == 7:
                wo_load(0), wo_load(1)
            if g == 8:
                wo_load(2), wo_load(3)
            if g == 9:
                wo_load(4), wo_load(5), wo_load(6)
            if g < ng:
                qkv(2 * g)
                qkv(2 * g + 1)
            else:
                wo(pend.pop(0))
                wo(pend.pop(0))
            if 0 <= g - 1 < ng:
                scores(2 * g - 2)
                scores(2 * g - 1)
            if 0 <= g - 2 < ng:
                pv(2 * g - 4)
                pv(2 * g - 3)
        wo_load(7)
        for g in pend:
            wo(g)
        y = acc[0].astype(BF)
        mem_v[...] = y[:M]
        att_v[pl.ds(pl.multiple_of(RIDE * s, 8), RIDE), :] = y[M:]
        return carry
    lax.fori_loop(0, NSEG, step, 0)

    P0 = TAIL0 - TCH

    def out_copy(row0, n, k):
        return pltpu.make_async_copy(out_v.at[pl.ds(row0, n), :],
                                     out_hbm.at[0, pl.ds(row0, n), :], sem_out.at[k])
    out_copy(0, P0, 0).start()

    def tail(j, carry):
        r0 = pl.multiple_of(j * TCH, TCH)
        lhs = jnp.concatenate([oring[h, pl.ds(r0, TCH), :] for h in range(H)], axis=1)
        for k in range(8):
            post(pl.multiple_of(P0 + j * TCH + k * 16, 16), 16, r2_v, j * 8 + k)
            y = jnp.dot(lhs, wo_v[k], preferred_element_type=F32)
            att_v[pl.ds(pl.multiple_of(TAIL0 + j * TCH, TCH), TCH), pl.ds(k * 128, 128)] = (
                y.astype(BF))
        out_copy(pl.multiple_of(P0 + j * TCH, TCH), TCH, 1 + j).start()
        return carry
    ntail = BULK // TCH
    lax.fori_loop(0, ntail, tail, 0)
    for k in range(8):
        post(P0 + ntail * TCH + k * 16, 16, r2_v, ntail * 8 + k)
    out_copy(P0 + ntail * TCH, TCH, 1 + ntail).start()

    sub1 = lax.broadcasted_iota(jnp.int32, (RIDE, 128), 0)
    lan1 = lax.broadcasted_iota(jnp.int32, (RIDE, 128), 1)
    idx1 = lan1 * RIDE + sub1
    sub2 = lax.broadcasted_iota(jnp.int32, (16, 128), 0)
    lan2 = lax.broadcasted_iota(jnp.int32, (16, 128), 1)
    idx2 = P0 + lan2 * 16 + sub2
    idx = jnp.concatenate([idx1, idx2], axis=0)
    valid = jnp.concatenate([idx1 < P0, idx2 < S], axis=0)
    rall = _rb(jnp.concatenate([r1_v[...], r2_v[...]], axis=0))
    big = jnp.int32(2 ** 30)

    def argtop(ok):
        v = jnp.where(ok, rall, -jnp.inf)
        m = jnp.max(jnp.max(v, axis=0, keepdims=True), axis=1, keepdims=True)
        cand = jnp.where(ok & (v >= m), idx, big)
        i = jnp.min(jnp.min(cand, axis=0, keepdims=True), axis=1, keepdims=True)
        return m, i
    m_a, i_a = argtop(valid)
    m_b, i_b = argtop(valid & (idx != i_a))
    ia = jnp.clip(i_a[0, 0], 0, S - 1)
    ib = jnp.clip(i_b[0, 0], 0, S - 1)
    blk_a = pl.multiple_of((ia // 8) * 8, 8)
    blk_b = pl.multiple_of((ib // 8) * 8, 8)

    def two(ref):
        return jnp.concatenate([ref[pl.ds(blk_a, 8), :], ref[pl.ds(blk_b, 8), :]], axis=0)

    hs = two(h2_v)
    wg_copy.wait()
    wu_copy.wait()
    for cp in wd_copies:
        cp.wait()
    g = _rb(jnp.dot(hs, wg_v[...], preferred_element_type=F32))
    u = _rb(jnp.dot(hs, wu_v[...], preferred_element_type=F32))
    act = (_rb(g * jax.nn.sigmoid(g)) * u).astype(BF)
    y = jnp.concatenate(
        [jnp.dot(act, wd_v[k], preferred_element_type=F32) for k in range(2)], axis=1)
    sub = lax.broadcasted_iota(jnp.int32, (16, 1), 0)
    rows = jnp.where(sub < 8, blk_a + sub, blk_b + sub - 8)
    gate = jnp.where(rows == ia, jax.nn.sigmoid(m_a),
                     jnp.where(rows == ib, jax.nn.sigmoid(m_b), 0.0))
    upd = jnp.where((rows == ia) | (rows == ib), y * gate, 0.0)
    x2 = _rb(two(x_v).astype(F32) + _rb(mod_row(2) * two(att_v).astype(F32)))
    fin = (x2 + mod_row(5) * (hs.astype(F32) + upd)).astype(BF)

    out_copy(0, P0, 0).wait()
    for j in range(ntail + 1):
        out_copy(P0 + j * TCH, TCH, 1 + j).wait()
    out_v[pl.ds(blk_a, 8), :] = fin[0:8]
    out_v[pl.ds(blk_b, 8), :] = fin[8:16]
    out_copy(blk_a, 8, 0).start()

    @pl.when(blk_a != blk_b)
    def _():
        out_copy(blk_b, 8, 1).start()
        out_copy(blk_b, 8, 1).wait()
    out_copy(blk_a, 8, 0).wait()


@jax.jit
def pallas_adaLN_cond__memory_aug_recurrent_mem_tr__moe_arch_mod__prompt_kernel(
    A_x, A_mem0, A_Wq, A_Wk, A_Wv, A_Wo, A_seg_len, B_x, B_w_r, B_w_gate, B_w_up, B_w_down, c,
    w_mod,
):
    del B_x
    del A_seg_len
    assert A_x.shape == (1, S, D) and A_Wq.shape == (D, H, DH) and A_mem0.shape == (1, M, D)
    any_spec = pl.BlockSpec(memory_space=pl.ANY)
    scratch = [
        pltpu.VMEM((S, D), BF),
        pltpu.VMEM((BULK, D), BF),
        pltpu.VMEM((S, D), BF),
        pltpu.VMEM((S, D), BF),
        pltpu.VMEM((S, D), BF),
        pltpu.VMEM((96 * PITCH, 128), U32),
        pltpu.VMEM((8, H * DH, 128), BF),
        pltpu.VMEM((96, RING, 128), BF),
        pltpu.VMEM((H, RING, 128), BF),
        pltpu.VMEM((NSTAGE, 512, 16, 128), BF),
        pltpu.VMEM((12, D, 512), BF),
        pltpu.VMEM((D, FF), BF),
        pltpu.VMEM((D, FF), BF),
        pltpu.VMEM((2, FF, 512), BF),
        pltpu.VMEM((M, D), BF),
        pltpu.VMEM((1, D), BF),
        pltpu.VMEM((1, D), BF),
        pltpu.VMEM((8, D), F32),
        pltpu.VMEM((RIDE, 128), F32),
        pltpu.VMEM((16, 128), F32),
        pltpu.SemaphoreType.DMA((3,)),
        pltpu.SemaphoreType.DMA((2,)),
        pltpu.SemaphoreType.DMA((NSTAGE,)),
        pltpu.SemaphoreType.DMA((12,)),
        pltpu.SemaphoreType.DMA((8,)),
        pltpu.SemaphoreType.DMA((4,)),
        pltpu.SemaphoreType.DMA((8,)),
    ]
    return pl.pallas_call(
        _kernel,
        out_shape=jax.ShapeDtypeStruct((1, S, D), BF),
        in_specs=[any_spec] * 12,
        out_specs=any_spec,
        scratch_shapes=scratch,
        compiler_params=pltpu.CompilerParams(vmem_limit_bytes=120 * 1024 * 1024),
    )(A_x, A_mem0, A_Wq, A_Wk, A_Wv, A_Wo.reshape(H * DH, D), B_w_r.reshape(1, D), B_w_gate,
      B_w_up, B_w_down, c, w_mod)
```

```python
import jax
import jax.numpy as jnp
from jax import lax
import jax.experimental.pallas as pl
import jax.experimental.pallas.tpu as pltpu

BF = jnp.bfloat16
F32 = jnp.float32
U32 = jnp.uint32

S = 2048
D = 1024
H = 32
DH = 128
M = 8
SEG = 32
NSEG = S // SEG
FF = 3584
RIDE = 24
BULK = S - RIDE * NSEG
X0 = BULK + 32
RING = 576
PITCH = 520
TAIL0 = RIDE * NSEG
TCH = 128
UNROLL = 2
EPS = 1e-5
NEG = -3.0e38
PERM = (0, 2, 4, 6, 1, 3, 5, 7)


def _rb(v):
    return v.astype(BF).astype(F32)


def _layernorm(xf):
    mu = jnp.mean(xf, axis=-1, keepdims=True)
    dv = xf - mu
    var = jnp.mean(dv * dv, axis=-1, keepdims=True)
    sd = _rb(jnp.sqrt(_rb(_rb(var) + EPS)))
    return _rb(_rb(xf - _rb(mu)) * (1.0 / sd))


def _f3(v):
    return v.astype(F32).reshape(v.shape[0] // 8, 8, D)


def _b2(v):
    return v.reshape(v.shape[0] * 8, D).astype(BF)


def _kernel(x_hbm, mem0_hbm, wq_hbm, wk_hbm, wv_hbm, wo_hbm, wr_hbm, wg_hbm, wu_hbm, wd_hbm,
            c_hbm, wmod_hbm, out_hbm,
            x_v, h_v, att_v, ho_v, wqkv_v, wo_v, stage, wmod_v,
            wg_v, wu_v, wd_v, mem_v, c_v, wr_v, mod_v, r1_v, r2_v,
            sem_small, sem_x, sem_stage, sem_wmod, sem_wo, sem_ffn, sem_out, *rings):
    w_hbm = (wq_hbm, wk_hbm, wv_hbm)
    ring = rings[:8]
    oring = rings[8:]

    def piece_copy(t, lo=0, n=D, sem=None):
        slot = t % 2
        return pltpu.make_async_copy(
            w_hbm[t // 4].at[pl.ds(lo, n), pl.ds((t % 4) * 8, 8), :],
            stage.at[slot, pl.ds(lo, n)], sem_stage.at[slot if sem is None else sem])

    def piece_wait(slot):
        pltpu.make_async_copy(stage.at[slot], stage.at[slot], sem_stage.at[slot]).wait()

    def wmod_copy(k):
        return pltpu.make_async_copy(wmod_hbm.at[:, pl.ds(k * 512, 512)], wmod_v.at[k],
                                     sem_wmod.at[k])

    def wo_copy(n):
        return pltpu.make_async_copy(wo_hbm.at[:, pl.ds(n * 128, 128)], wo_v.at[n], sem_wo.at[n])

    x0_copy = pltpu.make_async_copy(x_hbm.at[0, pl.ds(0, X0), :], x_v.at[pl.ds(0, X0), :],
                                    sem_x.at[0])
    x1_copy = pltpu.make_async_copy(x_hbm.at[0, pl.ds(X0, S - X0), :],
                                    x_v.at[pl.ds(X0, S - X0), :], sem_x.at[1])
    c_copy = pltpu.make_async_copy(c_hbm, c_v, sem_small.at[0])
    mem_copy = pltpu.make_async_copy(mem0_hbm.at[0], mem_v, sem_small.at[1])
    wr_copy = pltpu.make_async_copy(wr_hbm, wr_v, sem_small.at[2])
    wg_copy = pltpu.make_async_copy(wg_hbm, wg_v, sem_ffn.at[0])
    wu_copy = pltpu.make_async_copy(wu_hbm, wu_v, sem_ffn.at[1])
    wd_copies = [pltpu.make_async_copy(wd_hbm.at[:, pl.ds(k * 512, 512)], wd_v.at[k],
                                       sem_ffn.at[2 + k]) for k in range(2)]

    def relayout(slot, t, lo, n):
        base = t * (8 * PITCH) + lo // 2
        u = pltpu.bitcast(stage[slot, pl.ds(lo, n)], U32)
        for i in range(n // 2):
            a = u[2 * i]
            b = u[2 * i + 1]
            even = (a & jnp.uint32(0xFFFF)) | (b << 16)
            odd = (a >> 16) | (b & jnp.uint32(0xFFFF0000))
            wqkv_v[pl.ds(base + i, 4, stride=PITCH), :] = even
            wqkv_v[pl.ds(base + 4 * PITCH + i, 4, stride=PITCH), :] = odd

    def relayout_loop(slot, t, lo, n):
        def body(i, carry):
            relayout(slot, t, pl.multiple_of(lo + i * 128, 128), 128)
            return carry
        lax.fori_loop(0, n // 128, body, 0)

    def modulate(ln, k_scale, k_shift):
        return _rb(ln * mod_v[k_scale]) + mod_v[k_shift]

    def post(row0, n, r_ref, lane):
        x2 = _rb(_f3(x_v[pl.ds(row0, n), :]) + _rb(mod_v[2] * _f3(att_v[pl.ds(row0, n), :])))
        h2 = _rb(modulate(_layernorm(x2), 4, 3))
        ho_v[0, pl.ds(row0, n), :] = _b2(h2)
        ho_v[1, pl.ds(row0, n), :] = _b2(x2 + mod_v[5] * h2)
        r = jnp.sum(h2 * mod_v[6], axis=-1, keepdims=True)
        lanes = lax.broadcasted_iota(jnp.int32, r_ref.shape, 2)
        r_ref[...] = jnp.where(lanes == lane, r, r_ref[...])

    x0_copy.start()
    c_copy.start()
    wmod_copy(0).start()
    mem_copy.start()
    wr_copy.start()

    r1_v[...] = jnp.full(r1_v.shape, NEG, F32)
    r2_v[...] = jnp.full(r2_v.shape, NEG, F32)
    att_v[pl.ds(0, RIDE), :] = jnp.zeros((RIDE, D), BF)

    x0_copy.wait()
    wmod_copy(1).start()
    wmod_copy(2).start()

    LNB = X0 // 4

    def ln0(i, carry):
        r0 = pl.multiple_of(i * LNB, 8)
        h_v[pl.ds(r0, LNB), :] = _b2(_layernorm(_f3(x_v[pl.ds(r0, LNB), :])))
        return carry
    lax.fori_loop(0, 4, ln0, 0)

    wmod_copy(3).start()
    piece_copy(0, 0, 512, 0).start()
    c_copy.wait()
    cf = c_v[...].astype(F32)
    sc = jnp.broadcast_to((cf * jax.nn.sigmoid(cf)).astype(BF), (16, D))

    def mod_slab(k):
        y = _rb(jnp.dot(sc, wmod_v[k], preferred_element_type=F32)[0:8])
        if k // 2 in (1, 4):
            y = _rb(1.0 + y)
        mod_v[k // 2, :, pl.ds((k % 2) * 512, 512)] = y

    for k in range(4):
        wmod_copy(k).wait()
        if k == 2:
            piece_copy(0, 512, 256, 2).start()
            piece_copy(0, 768, 256, 3).start()
        mod_slab(k)

    def mod0(i, carry):
        r0 = pl.multiple_of(i * LNB, 8)
        h_v[pl.ds(r0, LNB), :] = _b2(modulate(_f3(h_v[pl.ds(r0, LNB), :]), 1, 0))
        return carry
    lax.fori_loop(0, 4, mod0, 0)
    ho_v[0, pl.ds(BULK, RIDE), :] = h_v[pl.ds(BULK, RIDE), :]

    piece_copy(0, 0, 512, 0).wait()
    relayout_loop(0, 0, 0, 512)
    piece_copy(0, 512, 256, 2).wait()
    piece_copy(1).start()
    relayout_loop(0, 0, 512, 256)
    piece_copy(0, 768, 256, 3).wait()
    relayout_loop(0, 0, 768, 256)

    def bulk_qkv(i, carry):
        t = jnp.minimum(i + 1, 11)
        hb = h_v[pl.ds(0, BULK), :]
        for k in range(8):
            if k == 4:
                @pl.when(i < 11)
                def _():
                    piece_wait((i + 1) % 2)

                for j in range(11):
                    @pl.when(i == j)
                    def _():
                        if j < 10:
                            piece_copy(j + 2).start()
                        if j < 8:
                            wo_copy(j).start()
                        if 2 <= j < 10:
                            wmod_copy(j + 2).start()
                        if j == 10:
                            x1_copy.start()
            w = pltpu.bitcast(wqkv_v[pl.ds(pl.multiple_of((8 * i + k) * PITCH, 8), 512), :], BF)
            y = jnp.dot(hb, w, preferred_element_type=F32)
            ring[k][i, pl.ds(RING - BULK, BULK), :] = y.astype(BF)
            if k >= 4:
                relayout(t % 2, t, (k - 4) * 256, 256)
        return carry
    lax.fori_loop(0, 12, bulk_qkv, 0)

    wg_copy.start()
    wu_copy.start()
    for cp in wd_copies:
        cp.start()

    for k in range(4, 12):
        wmod_copy(k).wait()
    for k in range(4, 12):
        mod_slab(k)
    wr_copy.wait()
    mod_v[6] = jnp.broadcast_to(wr_v[...].astype(F32), (8, D))
    mem_copy.wait()
    for n in range(8):
        wo_copy(n).wait()
    x1_copy.wait()

    scale = DH ** -0.5
    rr = lax.broadcasted_iota(jnp.int32, (80, 80), 0)
    cc = lax.broadcasted_iota(jnp.int32, (80, 80), 1)

    def second(i):
        return ((i >= 8) & (i < 16)) | (i >= 48)
    same = second(rr) == second(cc)
    allowed = same & ((rr < 16) | (cc <= rr))
    fill = jnp.where(same, -1e9, NEG).astype(F32)

    def w_slab(t, g, lo=0, n=512):
        return pltpu.bitcast(wqkv_v[pl.ds((8 * t + g) * PITCH + lo, n), :], BF)

    def step(s, mem, chained):
        wr = pl.multiple_of(lax.rem(RIDE * s, RING), 8)
        rd = pl.multiple_of(lax.rem(SEG * s + RING - BULK, RING), SEG)
        ow = pl.multiple_of(lax.rem(SEG * s + 192, RING), SEG)
        orr = pl.multiple_of(lax.rem(RIDE * s + 192, RING), 8)
        hrow = pl.multiple_of(BULK + RIDE * s, 8)

        def lhs():
            return jnp.concatenate([mem, ho_v[0, pl.ds(hrow, RIDE), :]], axis=0)

        memqkv, probs, omem = {}, {}, {}
        acc = []

        def qkv(g, xin, split=False):
            part = {}
            if split:
                for t in range(6):
                    part[t] = jnp.dot(xin[:, :512], w_slab(t, g, 0, 256),
                                      preferred_element_type=F32)
            for t0 in range(0, 12, 2):
                ys = []
                for t in (t0, t0 + 1):
                    if t in part:
                        y = jnp.dot(xin[:, 512:], w_slab(t, g, 256, 256),
                                    preferred_element_type=F32) + part[t]
                    else:
                        y = jnp.dot(xin, w_slab(t, g), preferred_element_type=F32)
                    ring[g][t, pl.ds(wr, RIDE), :] = y[M:].astype(BF)
                    ys.append(y[:M])
                memqkv[(t0, g)] = jnp.concatenate(ys, axis=0).astype(BF)

        def cat(t0, g):
            return jnp.concatenate([memqkv[(t0, g)], ring[g][t0, pl.ds(rd, SEG), :],
                                    ring[g][t0 + 1, pl.ds(rd, SEG), :]], axis=0)

        def scores(g):
            for p in (0, 2):
                sc_ = lax.dot_general(cat(p, g), cat(4 + p, g), (((1,), (1,)), ((), ())),
                                      preferred_element_type=F32)
                sc_ = jnp.where(allowed, sc_ * scale, fill)
                e = jnp.exp(sc_ - jnp.max(sc_, axis=1, keepdims=True))
                l = jnp.sum(e, axis=1, keepdims=True)
                rc = pl.reciprocal(l, approx=True)
                rc = rc * (2.0 - l * rc)
                probs[(p, g)] = (e * rc).astype(BF)

        def pv(g):
            for p in (0, 2):
                o = jnp.dot(probs[(p, g)], cat(8 + p, g), preferred_element_type=F32)
                omem[(p, g)] = o[0:8]
                omem[(p + 1, g)] = o[8:16]
                oring[g][p, pl.ds(ow, SEG), :] = o[16:48].astype(BF)
                oring[g][p + 1, pl.ds(ow, SEG), :] = o[48:80].astype(BF)

        def wo(g):
            a = jnp.concatenate(
                [jnp.concatenate([omem[(o, g)].astype(BF), oring[g][o, pl.ds(orr, RIDE), :]],
                                 axis=0) for o in range(4)], axis=1)
            w = jnp.concatenate(
                [jnp.concatenate([wo_v[n, pl.ds((8 * o + PERM[g]) * DH, DH), :]
                                  for o in range(4)], axis=0) for n in range(8)], axis=1)
            y = jnp.dot(a, w, preferred_element_type=F32)
            acc[:] = [y if not acc else y + acc[0]]

        x_a = lhs()
        prev = jnp.maximum(s - 1, 0)
        post(pl.multiple_of(RIDE * prev, 8), RIDE, r1_v, prev)
        nrow = pl.multiple_of(BULK + RIDE * jnp.minimum(s + 1, NSEG - 1), 8)
        ho_v[0, pl.ds(nrow, RIDE), :] = _b2(
            modulate(_layernorm(_f3(x_v[pl.ds(nrow, RIDE), :])), 1, 0))
        x_b = lhs()

        qkv(0, x_a, chained), qkv(1, x_a), qkv(2, x_b)
        scores(0), scores(1)
        qkv(3, x_b), qkv(4, x_b)
        pv(0), pv(1), scores(2), scores(3)
        qkv(5, x_b), qkv(6, x_b)
        pv(2), pv(3), scores(4), scores(5)
        qkv(7, x_b), wo(0)
        pv(4), pv(5), scores(6), scores(7)
        wo(1), wo(2), wo(3)
        pv(6), pv(7)
        wo(4), wo(5), wo(6), wo(7)
        y = acc[0].astype(BF)
        att_v[pl.ds(pl.multiple_of(RIDE * s, 8), RIDE), :] = y[M:]
        return y[:M]

    def steps(i, carry):
        mem = mem_v[...]
        for u in range(UNROLL):
            mem = step(i * UNROLL + u, mem, u > 0)
        mem_v[...] = mem
        return carry
    lax.fori_loop(0, NSEG // UNROLL, steps, 0)

    P0 = TAIL0 - TCH

    def out_copy(row0, n, k):
        return pltpu.make_async_copy(ho_v.at[1, pl.ds(row0, n), :],
                                     out_hbm.at[0, pl.ds(row0, n), :], sem_out.at[k])
    out_copy(0, P0, 0).start()

    def tail(j, carry):
        r0 = pl.multiple_of(j * TCH, TCH)
        a = jnp.concatenate([oring[PERM.index(h % 8)][h // 8, pl.ds(r0, TCH), :]
                             for h in range(H)], axis=1)
        for k in range(8):
            post(pl.multiple_of(P0 + j * TCH + k * 16, 16), 16, r2_v, j * 8 + k)
            y = jnp.dot(a, wo_v[k], preferred_element_type=F32)
            att_v[pl.ds(pl.multiple_of(TAIL0 + j * TCH, TCH), TCH), pl.ds(k * 128, 128)] = (
                y.astype(BF))
        out_copy(pl.multiple_of(P0 + j * TCH, TCH), TCH, 1 + j).start()
        return carry
    ntail = BULK // TCH
    lax.fori_loop(0, ntail, tail, 0)
    for k in range(8):
        post(P0 + ntail * TCH + k * 16, 16, r2_v, ntail * 8 + k)
    out_copy(P0 + ntail * TCH, TCH, 1 + ntail).start()

    sub1 = lax.broadcasted_iota(jnp.int32, (RIDE, 128), 0)
    lan1 = lax.broadcasted_iota(jnp.int32, (RIDE, 128), 1)
    idx1 = lan1 * RIDE + sub1
    sub2 = lax.broadcasted_iota(jnp.int32, (16, 128), 0)
    lan2 = lax.broadcasted_iota(jnp.int32, (16, 128), 1)
    idx2 = P0 + lan2 * 16 + sub2
    idx = jnp.concatenate([idx1, idx2], axis=0)
    valid = jnp.concatenate([idx1 < P0, idx2 < S], axis=0)
    rall = _rb(jnp.concatenate([r1_v[...].reshape(RIDE, 128), r2_v[...].reshape(16, 128)],
                               axis=0))
    big = jnp.int32(2 ** 30)

    def argtop(ok):
        v = jnp.where(ok, rall, -jnp.inf)
        m = jnp.max(jnp.max(v, axis=0, keepdims=True), axis=1, keepdims=True)
        cand = jnp.where(ok & (v >= m), idx, big)
        i = jnp.min(jnp.min(cand, axis=0, keepdims=True), axis=1, keepdims=True)
        return m, i
    m_a, i_a = argtop(valid)
    m_b, i_b = argtop(valid & (idx != i_a))
    ia = jnp.clip(i_a[0, 0], 0, S - 1)
    ib = jnp.clip(i_b[0, 0], 0, S - 1)
    blk_a = pl.multiple_of((ia // 8) * 8, 8)
    blk_b = pl.multiple_of((ib // 8) * 8, 8)

    def two(ref):
        return jnp.concatenate([ref[pl.ds(blk_a, 8), :], ref[pl.ds(blk_b, 8), :]], axis=0)

    hs = two(ho_v.at[0])
    wg_copy.wait()
    wu_copy.wait()
    for cp in wd_copies:
        cp.wait()
    g = _rb(jnp.dot(hs, wg_v[...], preferred_element_type=F32))
    u = _rb(jnp.dot(hs, wu_v[...], preferred_element_type=F32))
    act = (_rb(g * jax.nn.sigmoid(g)) * u).astype(BF)
    y = jnp.concatenate(
        [jnp.dot(act, wd_v[k], preferred_element_type=F32) for k in range(2)], axis=1)
    sub = lax.broadcasted_iota(jnp.int32, (16, 1), 0)
    rows = jnp.where(sub < 8, blk_a + sub, blk_b + sub - 8)
    gate = jnp.where(rows == ia, jax.nn.sigmoid(m_a),
                     jnp.where(rows == ib, jax.nn.sigmoid(m_b), 0.0))
    upd = jnp.where((rows == ia) | (rows == ib), y * gate, 0.0).reshape(2, 8, D)
    x2 = _rb(_f3(two(x_v)) + _rb(mod_v[2] * _f3(two(att_v))))
    fin = _b2(x2 + mod_v[5] * (_f3(hs) + upd))

    out_copy(0, P0, 0).wait()
    for j in range(ntail + 1):
        out_copy(P0 + j * TCH, TCH, 1 + j).wait()
    ho_v[1, pl.ds(blk_a, 8), :] = fin[0:8]
    ho_v[1, pl.ds(blk_b, 8), :] = fin[8:16]
    out_copy(blk_a, 8, 0).start()

    @pl.when(blk_a != blk_b)
    def _():
        out_copy(blk_b, 8, 1).start()
        out_copy(blk_b, 8, 1).wait()
    out_copy(blk_a, 8, 0).wait()


@jax.jit
def pallas_adaLN_cond__memory_aug_recurrent_mem_tr__moe_arch_mod__prompt_kernel(
    A_x, A_mem0, A_Wq, A_Wk, A_Wv, A_Wo, A_seg_len, B_x, B_w_r, B_w_gate, B_w_up, B_w_down, c,
    w_mod,
):
    del B_x
    del A_seg_len
    assert A_x.shape == (1, S, D) and A_Wq.shape == (D, H, DH) and A_mem0.shape == (1, M, D)
    any_spec = pl.BlockSpec(memory_space=pl.ANY)
    scratch = [
        pltpu.VMEM((S, D), BF),
        pltpu.VMEM((X0, D), BF),
        pltpu.VMEM((S, D), BF),
        pltpu.VMEM((2, S, D), BF),
        pltpu.VMEM((96 * PITCH, 128), U32),
        pltpu.VMEM((8, H * DH, 128), BF),
        pltpu.VMEM((2, D, 8, 128), BF),
        pltpu.VMEM((12, D, 512), BF),
        pltpu.VMEM((D, FF), BF),
        pltpu.VMEM((D, FF), BF),
        pltpu.VMEM((2, FF, 512), BF),
        pltpu.VMEM((M, D), BF),
        pltpu.VMEM((1, D), BF),
        pltpu.VMEM((1, D), BF),
        pltpu.VMEM((7, 8, D), F32),
        pltpu.VMEM((RIDE // 8, 8, 128), F32),
        pltpu.VMEM((2, 8, 128), F32),
        pltpu.SemaphoreType.DMA((3,)),
        pltpu.SemaphoreType.DMA((2,)),
        pltpu.SemaphoreType.DMA((4,)),
        pltpu.SemaphoreType.DMA((12,)),
        pltpu.SemaphoreType.DMA((8,)),
        pltpu.SemaphoreType.DMA((4,)),
        pltpu.SemaphoreType.DMA((8,)),
    ] + [pltpu.VMEM((12, RING, 128), BF)] * 8 + [pltpu.VMEM((4, RING, 128), BF)] * 8
    return pl.pallas_call(
        _kernel,
        out_shape=jax.ShapeDtypeStruct((1, S, D), BF),
        in_specs=[any_spec] * 12,
        out_specs=any_spec,
        scratch_shapes=scratch,
        compiler_params=pltpu.CompilerParams(vmem_limit_bytes=120 * 1024 * 1024),
    )(A_x, A_mem0, A_Wq, A_Wk, A_Wv, A_Wo.reshape(H * DH, D), B_w_r.reshape(1, D), B_w_gate,
      B_w_up, B_w_down, c, w_mod)
```

```python
import functools

import jax
import jax.numpy as jnp
from jax import lax
import jax.experimental.pallas as pl
import jax.experimental.pallas.tpu as pltpu

BF = jnp.bfloat16
F32 = jnp.float32
U32 = jnp.uint32

S = 2048
D = 1024
H = 32
DH = 128
M = 8
SEG = 32
NSEG = S // SEG
FF = 3584
RIDE = 24
BULK = S - RIDE * NSEG
X0 = BULK + 32
RING = 576
PITCH = 520
X1 = 1024
UNROLL = 4
EPS = 1e-5
SIDE0, SIDE_LAT, SIDE_DUE = 2, 6, 6
NEG = -3.0e38
PERM = (0, 2, 4, 6, 1, 3, 5, 7)


def _rb(v):
    return v.astype(BF).astype(F32)


def _layernorm(xf):
    mu = jnp.mean(xf, axis=-1, keepdims=True)
    dv = xf - mu
    var = jnp.mean(dv * dv, axis=-1, keepdims=True)
    sd = _rb(jnp.sqrt(_rb(_rb(var) + EPS)))
    return _rb(_rb(xf - _rb(mu)) * (1.0 / sd))


def _f3(v):
    return v.astype(F32).reshape(v.shape[0] // 8, 8, D)


def _b2(v):
    return v.reshape(v.shape[0] * 8, D).astype(BF)


def _kernel(x_hbm, mem0_hbm, wq_hbm, wk_hbm, wv_hbm, wo_hbm, wr_hbm, wg_hbm, wu_hbm, wd_hbm,
            c_hbm, wmod_hbm, out_hbm,
            x_v, h_v, hp_v, att_v, ho_v, wqkv_v, wo_v, stage, wmod_v,
            wg_v, wu_v, wd_v, mem_v, c_v, wr_v, mod_v, r_v,
            sem_small, sem_x, sem_stage, sem_wmod, sem_wo, sem_ffn, sem_out, *rings):
    w_hbm = (wq_hbm, wk_hbm, wv_hbm)
    ring = rings

    def piece_copy(t, lo=0, n=D, sem=None):
        slot = t % 2
        return pltpu.make_async_copy(
            w_hbm[t // 4].at[pl.ds(lo, n), pl.ds((t % 4) * 8, 8), :],
            stage.at[slot, pl.ds(lo, n)], sem_stage.at[slot if sem is None else sem])

    def piece_wait(slot):
        pltpu.make_async_copy(stage.at[slot], stage.at[slot], sem_stage.at[slot]).wait()

    def wmod_copy(k):
        return pltpu.make_async_copy(wmod_hbm.at[:, pl.ds(k * 512, 512)], wmod_v.at[k],
                                     sem_wmod.at[k])

    def wo_copy(n):
        return pltpu.make_async_copy(wo_hbm.at[:, pl.ds(n * 512, 512)], wo_v.at[n], sem_wo.at[n])

    x0_copy = pltpu.make_async_copy(x_hbm.at[0, pl.ds(0, X0), :], x_v.at[pl.ds(0, X0), :],
                                    sem_x.at[0])
    x1_copy = pltpu.make_async_copy(x_hbm.at[0, pl.ds(X0, X1 - X0), :],
                                    x_v.at[pl.ds(X0, X1 - X0), :], sem_x.at[1])
    x2_copy = pltpu.make_async_copy(x_hbm.at[0, pl.ds(X1, S - X1), :],
                                    x_v.at[pl.ds(X1, S - X1), :], sem_x.at[2])
    c_copy = pltpu.make_async_copy(c_hbm, c_v, sem_small.at[0])
    mem_copy = pltpu.make_async_copy(mem0_hbm.at[0], mem_v, sem_small.at[1])
    wr_copy = pltpu.make_async_copy(wr_hbm, wr_v, sem_small.at[2])
    wg_copy = pltpu.make_async_copy(wg_hbm, wg_v, sem_ffn.at[0])
    wu_copy = pltpu.make_async_copy(wu_hbm, wu_v, sem_ffn.at[1])
    wd_copies = [pltpu.make_async_copy(wd_hbm.at[:, pl.ds(k * 512, 512)], wd_v.at[k],
                                       sem_ffn.at[2 + k]) for k in range(2)]

    def relayout(slot, t, lo, n):
        base = t * (8 * PITCH) + lo // 2
        u = pltpu.bitcast(stage[slot, pl.ds(lo, n)], U32)
        tok = None
        for i in range(n // 2):
            a = u[2 * i]
            b = u[2 * i + 1]
            even = (a & jnp.uint32(0xFFFF)) | (b << 16)
            odd = (a >> 16) | (b & jnp.uint32(0xFFFF0000))
            wqkv_v[pl.ds(base + i, 4, stride=PITCH), :] = even
            wqkv_v[pl.ds(base + 4 * PITCH + i, 4, stride=PITCH), :] = odd
            tok = even ^ odd if tok is None else tok ^ even ^ odd
        return jnp.concatenate([tok, tok], axis=0)

    def relayout_loop(slot, t, lo, n):
        def body(i, carry):
            relayout(slot, t, pl.multiple_of(lo + i * 128, 128), 128)
            return carry
        lax.fori_loop(0, n // 128, body, 0)

    def modulate(ln, k_scale, k_shift):
        return _rb(ln * mod_v[k_scale]) + mod_v[k_shift]

    CW = 256

    def ln_stats(xf):
        mu = jnp.mean(xf, axis=-1, keepdims=True)
        dv = xf - mu
        var = jnp.mean(dv * dv, axis=-1, keepdims=True)
        sd = _rb(jnp.sqrt(_rb(_rb(var) + EPS)))
        return _rb(mu), 1.0 / sd

    def mod_c(k, c):
        return mod_v[k, :, pl.ds(c * CW, CW)]

    def token(v):
        return pltpu.bitcast(v[:, :128] + v[:, 128:], U32)

    def after(v, trig):
        if trig is None:
            return v
        return jnp.concatenate([jnp.where(trig[0], trig[1], v[:, :128]), v[:, 128:]], axis=1)

    def post_work(row0, att):
        st = {}

        def head(trig):
            a = after(att().astype(F32), trig)
            st["x2"] = _rb(x_v[pl.ds(row0, 8), :].astype(F32) + _rb(mod_v[2] * a))
            st["mu"], st["inv"] = ln_stats(st["x2"])

        def chunk(c, trig):
            xc = after(st["x2"][:, c * CW:(c + 1) * CW], trig)
            h2b = (_rb(_rb(_rb(xc - st["mu"]) * st["inv"]) * mod_c(4, c))
                   + mod_c(3, c)).astype(BF)
            h2 = h2b.astype(F32)
            ho_v[0, pl.ds(row0, 8), pl.ds(c * CW, CW)] = h2b
            o = xc + mod_c(5, c) * h2
            ho_v[1, pl.ds(row0, 8), pl.ds(c * CW, CW)] = o.astype(BF)
            rp = h2 * mod_c(6, c)
            st["r"] = rp if c == 0 else st["r"] + rp
            if c == D // CW - 1:
                r = jnp.sum(st["r"], axis=-1, keepdims=True)
                grp = row0 // 8
                lanes = lax.broadcasted_iota(jnp.int32, (8, 128), 1)
                r_v[grp // 128] = jnp.where(lanes == grp % 128, r, r_v[grp // 128])
            return token(o + st["r"])
        return [head] + [functools.partial(chunk, c) for c in range(D // CW)]

    def ln1_work(row0):
        st = {}

        def head(trig):
            st["x"] = after(x_v[pl.ds(row0, 8), :].astype(F32), trig)
            st["mu"], st["inv"] = ln_stats(st["x"])

        def chunk(c, trig):
            xc = after(st["x"][:, c * CW:(c + 1) * CW], trig)
            h = _rb(_rb(_rb(xc - st["mu"]) * st["inv"]) * mod_c(1, c)) + mod_c(0, c)
            ho_v[0, pl.ds(row0, 8), pl.ds(c * CW, CW)] = h.astype(BF)
            return token(h)
        return [head] + [functools.partial(chunk, c) for c in range(D // CW)]

    x0_copy.start()
    c_copy.start()
    wmod_copy(0).start()
    mem_copy.start()
    wr_copy.start()

    r_v[...] = jnp.full(r_v.shape, NEG, F32)
    att_v[...] = jnp.zeros(att_v.shape, BF)

    x0_copy.wait()
    wmod_copy(1).start()
    wmod_copy(2).start()

    LNB = X0 // 4

    def ln0(i, carry):
        r0 = pl.multiple_of(i * LNB, 8)
        h_v[pl.ds(r0, LNB), :] = _b2(_layernorm(_f3(x_v[pl.ds(r0, LNB), :])))
        return carry
    lax.fori_loop(0, 4, ln0, 0)

    wmod_copy(3).start()
    piece_copy(0, 0, 512, 0).start()
    c_copy.wait()
    cf = c_v[...].astype(F32)
    sc = jnp.broadcast_to((cf * jax.nn.sigmoid(cf)).astype(BF), (16, D))

    def mod_slab(k):
        y = _rb(jnp.dot(sc, wmod_v[k], preferred_element_type=F32)[0:8])
        if k // 2 in (1, 4):
            y = _rb(1.0 + y)
        mod_v[k // 2, :, pl.ds((k % 2) * 512, 512)] = y

    for k in range(4):
        wmod_copy(k).wait()
        if k == 2:
            piece_copy(0, 512, 256, 2).start()
            piece_copy(0, 768, 256, 3).start()
        mod_slab(k)

    def mod0(i, carry):
        r0 = pl.multiple_of(i * 128, 128)
        hb = _b2(modulate(_f3(h_v[pl.ds(r0, 128), :]), 1, 0))
        hp_v[pl.ds(pl.multiple_of(i * 64, 64), 64), :] = pltpu.bitcast(hb, U32)
        return carry
    lax.fori_loop(0, BULK // 128, mod0, 0)
    ho_v[0, pl.ds(BULK, RIDE), :] = _b2(modulate(_f3(h_v[pl.ds(BULK, RIDE), :]), 1, 0))

    piece_copy(0, 0, 512, 0).wait()
    relayout_loop(0, 0, 0, 512)
    piece_copy(0, 512, 256, 2).wait()
    piece_copy(1).start()
    relayout_loop(0, 0, 512, 256)
    piece_copy(0, 768, 256, 3).wait()
    relayout_loop(0, 0, 768, 256)

    def bulk_dot(i, k, never=None, rl=None):
        w = pltpu.bitcast(wqkv_v[pl.ds(pl.multiple_of((8 * i + k) * PITCH, 8), 512), :], BF)
        cols = [hp_v[:, pl.ds(128 * c, 128)] for c in range(8)]
        if rl is not None:
            slot, t, lo, n = rl
            g = n // 16
            spots = [(12 + (q * 48) // g) for q in range(g)]
            toks = {sp: relayout(slot, t, lo + 16 * q, 16) for q, sp in enumerate(spots)}
            for c in (0, 4):
                cols[c] = jnp.concatenate(
                    [jnp.where(never, toks[8 * c + j], cols[c][8 * j:8 * j + 8])
                     if 8 * c + j in toks else cols[c][8 * j:8 * j + 8]
                     for j in range(32)], axis=0)
        hb = pltpu.bitcast(jnp.concatenate(cols, axis=1), BF)
        y = jnp.dot(hb, w, preferred_element_type=F32)
        ring[k][i, pl.ds(RING - BULK, BULK), :] = y.astype(BF)

    never0 = r_v[0] > 0.0
    piece_copy(2).start()
    for k in range(8):
        if k == 6:
            piece_wait(1)
        bulk_dot(0, k, never0, (1, 1, (k - 6) * 512, 512) if k >= 6 else None)

    def bulk_qkv(i, carry):
        @pl.when(i < 11)
        def _():
            piece_wait((i + 1) % 2)

        for j in range(1, 11):
            @pl.when(i == j)
            def _():
                if j < 10:
                    piece_copy(j + 2).start()
                if j < 9:
                    wmod_copy(j + 3).start()
                if j == 9:
                    x1_copy.start()
                if j == 10:
                    for n in range(2):
                        wo_copy(n).start()
        t = jnp.minimum(i + 1, 11)
        never = jnp.full((8, 128), i, jnp.int32) < 0
        for k in range(8):
            bulk_dot(i, k, never, (t % 2, t, k * 128, 128))
        return carry
    lax.fori_loop(1, 12, bulk_qkv, 0)

    for k in range(4, 12):
        wmod_copy(k).wait()
    for k in range(4, 12):
        mod_slab(k)
    wr_copy.wait()
    mod_v[6] = jnp.broadcast_to(wr_v[...].astype(F32), (8, D))
    mem_copy.wait()
    for n in range(2):
        wo_copy(n).wait()
    x1_copy.wait()
    x2_copy.start()
    wg_copy.start()
    wu_copy.start()
    for cp in wd_copies:
        cp.start()

    scale = DH ** -0.5
    rr = lax.broadcasted_iota(jnp.int32, (80, 80), 0)
    cc = lax.broadcasted_iota(jnp.int32, (80, 80), 1)

    def second(i):
        return ((i >= 8) & (i < 16)) | (i >= 48)
    same = second(rr) == second(cc)
    allowed = same & ((rr < 16) | (cc <= rr))
    fill = jnp.where(same, -1e9, NEG).astype(F32)

    def w_slab(t, g, lo=0, n=512, tok=None):
        u = wqkv_v[pl.ds((8 * t + g) * PITCH + lo, n), :]
        if tok is not None:
            u = jnp.concatenate([jnp.where(tok[0], tok[1], u[:8]), u[8:]], axis=0)
        return pltpu.bitcast(u, BF)

    def step(s, mem, chained, left, att_prev):
        odd = left is not None
        wr = pl.multiple_of(lax.rem(RIDE * s, RING), 8)
        rd = pl.multiple_of(lax.rem(SEG * s + RING - BULK, RING), SEG)
        xin = jnp.concatenate(
            [mem, ho_v[0, pl.ds(pl.multiple_of(BULK + RIDE * s, 8), RIDE), :]], axis=0)

        prow = SEG * (s - 1) if odd else jnp.maximum(SEG * s - 40, 0)
        nrow = BULK + RIDE * jnp.minimum(s + 1, NSEG - 1)
        works = [post_work(pl.multiple_of(prow + 8 * q, 8), functools.partial(att_prev, q))
                 for q in range(3 if odd else 5)]
        works += [ln1_work(pl.multiple_of(nrow + 8 * q, 8)) for q in range(RIDE // 8)]
        never = jnp.full((8, 128), s, jnp.int32) < 0
        gap = (96 - SIDE0 - SIDE_LAT - SIDE_DUE) // len(works)
        sched = {}
        for q, wk in enumerate(works):
            sched.setdefault(SIDE0 + gap * q, []).append(wk[0])
            for c in range(1, len(wk)):
                sched.setdefault(SIDE0 + SIDE_LAT + gap * q + ((c - 1) * gap) // 4,
                                 []).append(wk[c])

        memqkv, probs, wl, new_left, toks = {}, {}, {}, {}, {}
        acc = []

        def qkv(g, split=False):
            part = {}
            if split:
                for t in range(6):
                    part[t] = jnp.dot(xin[:, :512], w_slab(t, g, 0, 256),
                                      preferred_element_type=F32)
            for t0 in range(0, 12, 2):
                ys = []
                for t in (t0, t0 + 1):
                    if t in part:
                        y = jnp.dot(xin[:, 512:], w_slab(t, g, 256, 256),
                                    preferred_element_type=F32) + part[t]
                    else:
                        y = jnp.dot(xin, w_slab(t, g, tok=toks.get(12 * g + t)),
                                    preferred_element_type=F32)
                    ring[g][t, pl.ds(wr, RIDE), :] = y[M:].astype(BF)
                    ys.append(y[:M])
                    for item in sched.get(12 * g + t, ()):
                        tk = item((never, y[:M]))
                        if tk is not None:
                            toks[12 * g + t + SIDE_DUE] = (never, tk)
                memqkv[(t0, g)] = jnp.concatenate(ys, axis=0).astype(BF)

        def cat(t0, g):
            return jnp.concatenate([memqkv[(t0, g)], ring[g][t0, pl.ds(rd, SEG), :],
                                    ring[g][t0 + 1, pl.ds(rd, SEG), :]], axis=0)

        def scores(g):
            for p in (0, 2):
                sc_ = lax.dot_general(cat(p, g), cat(4 + p, g), (((1,), (1,)), ((), ())),
                                      preferred_element_type=F32)
                sc_ = jnp.where(allowed, sc_ * scale, fill)
                e = jnp.exp(sc_ - jnp.max(sc_, axis=1, keepdims=True))
                l = jnp.sum(e, axis=1, keepdims=True)
                rc = pl.reciprocal(l, approx=True)
                rc = rc * (2.0 - l * rc)
                probs[(p, g)] = (e * rc).astype(BF)

        def pv(g):
            for p in (0, 2):
                o = jnp.dot(probs[(p, g)], cat(8 + p, g), preferred_element_type=F32)
                for j in range(2):
                    om, ot = o[8 * j:8 * j + 8], o[16 + 32 * j:48 + 32 * j]
                    if odd:
                        rows = [om, left[(p + j, g)], ot]
                    else:
                        rows = [om, ot[:RIDE]]
                        new_left[(p + j, g)] = ot[RIDE:]
                    wl[(p + j, g)] = jnp.concatenate(rows, axis=0).astype(BF)

        def wo(g):
            a = jnp.concatenate([wl[(o, g)] for o in range(4)], axis=1)
            w = jnp.concatenate(
                [jnp.concatenate([wo_v[n, pl.ds((8 * o + PERM[g]) * DH, DH), :]
                                  for o in range(4)], axis=0) for n in range(2)], axis=1)
            y = jnp.dot(a, w, preferred_element_type=F32)
            acc[:] = [y if not acc else y + acc[0]]

        qkv(0, chained), qkv(1), qkv(2)
        scores(0), scores(1)
        qkv(3), qkv(4)
        pv(0), pv(1), scores(2), scores(3)
        qkv(5), qkv(6)
        pv(2), pv(3), scores(4), scores(5)
        qkv(7), wo(0)
        pv(4), pv(5), scores(6), scores(7)
        wo(1), wo(2), wo(3)
        pv(6), pv(7)
        wo(4), wo(5), wo(6), wo(7)
        y = acc[0].astype(BF)
        return y[:M], y[M:], (None if odd else new_left)

    def out_copy(row0, n, k):
        return pltpu.make_async_copy(ho_v.at[1, pl.ds(row0, n), :],
                                     out_hbm.at[0, pl.ds(row0, n), :], sem_out.at[k])

    OB = SEG * UNROLL

    def carried(q):
        return att_v[pl.ds(8 * q, 8), :]

    def steps(i, carry):
        @pl.when(i == 16 // UNROLL)
        def _():
            x2_copy.wait()

        @pl.when(i >= 3)
        def _():
            out_copy(0, OB, 0).wait()

        @pl.when(i >= 2)
        def _():
            out_copy(pl.multiple_of((i - 2) * OB, OB), OB, 0).start()

        mem, left, att_prev = mem_v[...], None, carried
        for u in range(UNROLL):
            mem, att, left = step(i * UNROLL + u, mem, u > 0, left, att_prev)
            att_prev = (lambda a: lambda q: a[8 * q:8 * q + 8])(att)
        mem_v[...] = mem
        att_v[...] = att
        return carry
    lax.fori_loop(0, NSEG // UNROLL, steps, 0)

    out_copy(S - 2 * OB, OB, 1).start()
    for q in range(5):
        for item in post_work(S - 40 + 8 * q, functools.partial(carried, q)):
            item(None)
    out_copy(S - OB, OB, 2).start()

    sub1 = lax.broadcasted_iota(jnp.int32, (16, 128), 0)
    lan1 = lax.broadcasted_iota(jnp.int32, (16, 128), 1)
    idx = (sub1 // 8) * 1024 + lan1 * 8 + sub1 % 8
    valid = idx >= 0
    rall = _rb(r_v[...].reshape(16, 128))
    big = jnp.int32(2 ** 30)

    def argtop(ok):
        v = jnp.where(ok, rall, -jnp.inf)
        m = jnp.max(jnp.max(v, axis=0, keepdims=True), axis=1, keepdims=True)
        cand = jnp.where(ok & (v >= m), idx, big)
        i = jnp.min(jnp.min(cand, axis=0, keepdims=True), axis=1, keepdims=True)
        return m, i
    m_a, i_a = argtop(valid)
    m_b, i_b = argtop(valid & (idx != i_a))
    ia = jnp.clip(i_a[0, 0], 0, S - 1)
    ib = jnp.clip(i_b[0, 0], 0, S - 1)
    blk_a = pl.multiple_of((ia // 8) * 8, 8)
    blk_b = pl.multiple_of((ib // 8) * 8, 8)

    def two(ref):
        return jnp.concatenate([ref[pl.ds(blk_a, 8), :], ref[pl.ds(blk_b, 8), :]], axis=0)

    hs = two(ho_v.at[0])
    wg_copy.wait()
    wu_copy.wait()
    for cp in wd_copies:
        cp.wait()
    g = _rb(jnp.dot(hs, wg_v[...], preferred_element_type=F32))
    u = _rb(jnp.dot(hs, wu_v[...], preferred_element_type=F32))
    act = (_rb(g * jax.nn.sigmoid(g)) * u).astype(BF)
    y = jnp.concatenate(
        [jnp.dot(act, wd_v[k], preferred_element_type=F32) for k in range(2)], axis=1)
    sub = lax.broadcasted_iota(jnp.int32, (16, 1), 0)
    rows = jnp.where(sub < 8, blk_a + sub, blk_b + sub - 8)
    gate = jnp.where(rows == ia, jax.nn.sigmoid(m_a),
                     jnp.where(rows == ib, jax.nn.sigmoid(m_b), 0.0))
    upd = jnp.where((rows == ia) | (rows == ib), y * gate, 0.0).reshape(2, 8, D)
    fin = _b2(_f3(two(ho_v.at[1])) + mod_v[5] * upd)

    for k in range(3):
        out_copy(0, OB, k).wait()
    ho_v[1, pl.ds(blk_a, 8), :] = fin[0:8]
    ho_v[1, pl.ds(blk_b, 8), :] = fin[8:16]
    out_copy(blk_a, 8, 0).start()

    @pl.when(blk_a != blk_b)
    def _():
        out_copy(blk_b, 8, 1).start()
        out_copy(blk_b, 8, 1).wait()
    out_copy(blk_a, 8, 0).wait()


@jax.jit
def pallas_adaLN_cond__memory_aug_recurrent_mem_tr__moe_arch_mod__prompt_kernel(
    A_x, A_mem0, A_Wq, A_Wk, A_Wv, A_Wo, A_seg_len, B_x, B_w_r, B_w_gate, B_w_up, B_w_down, c,
    w_mod,
):
    del B_x
    del A_seg_len
    assert A_x.shape == (1, S, D) and A_Wq.shape == (D, H, DH) and A_mem0.shape == (1, M, D)
    any_spec = pl.BlockSpec(memory_space=pl.ANY)
    scratch = [
        pltpu.VMEM((S, D), BF),
        pltpu.VMEM((X0, D), BF),
        pltpu.VMEM((BULK // 2, D), U32),
        pltpu.VMEM((40, D), BF),
        pltpu.VMEM((2, S, D), BF),
        pltpu.VMEM((96 * PITCH, 128), U32),
        pltpu.VMEM((2, H * DH, 512), BF),
        pltpu.VMEM((2, D, 8, 128), BF),
        pltpu.VMEM((12, D, 512), BF),
        pltpu.VMEM((D, FF), BF),
        pltpu.VMEM((D, FF), BF),
        pltpu.VMEM((2, FF, 512), BF),
        pltpu.VMEM((M, D), BF),
        pltpu.VMEM((1, D), BF),
        pltpu.VMEM((1, D), BF),
        pltpu.VMEM((7, 8, D), F32),
        pltpu.VMEM((2, 8, 128), F32),
        pltpu.SemaphoreType.DMA((3,)),
        pltpu.SemaphoreType.DMA((3,)),
        pltpu.SemaphoreType.DMA((4,)),
        pltpu.SemaphoreType.DMA((12,)),
        pltpu.SemaphoreType.DMA((8,)),
        pltpu.SemaphoreType.DMA((4,)),
        pltpu.SemaphoreType.DMA((8,)),
    ] + [pltpu.VMEM((12, RING, 128), BF)] * 8
    return pl.pallas_call(
        _kernel,
        out_shape=jax.ShapeDtypeStruct((1, S, D), BF),
        in_specs=[any_spec] * 12,
        out_specs=any_spec,
        scratch_shapes=scratch,
        compiler_params=pltpu.CompilerParams(vmem_limit_bytes=120 * 1024 * 1024),
    )(A_x, A_mem0, A_Wq, A_Wk, A_Wv, A_Wo.reshape(H * DH, D), B_w_r.reshape(1, D), B_w_gate,
      B_w_up, B_w_down, c, w_mod)
```

```python
import functools

import jax
import jax.numpy as jnp
from jax import lax
import jax.experimental.pallas as pl
import jax.experimental.pallas.tpu as pltpu

BF = jnp.bfloat16
F32 = jnp.float32
U32 = jnp.uint32

S = 2048
D = 1024
H = 32
DH = 128
M = 8
SEG = 32
NSEG = S // SEG
FF = 3584
RIDE = 24
BULK = S - RIDE * NSEG
X0 = BULK + 32
RING = 576
PITCH = 520
X1 = 1024
UNROLL = 4
EPS = 1e-5
SIDE0, SIDE_LAT, SIDE_DUE = 2, 6, 6
NEG = -3.0e38
PERM = (0, 2, 4, 6, 1, 3, 5, 7)


def _rb(v):
    return v.astype(BF).astype(F32)


def _layernorm(xf):
    mu = jnp.mean(xf, axis=-1, keepdims=True)
    dv = xf - mu
    var = jnp.mean(dv * dv, axis=-1, keepdims=True)
    sd = _rb(jnp.sqrt(_rb(_rb(var) + EPS)))
    return _rb(_rb(xf - _rb(mu)) * (1.0 / sd))


def _f3(v):
    return v.astype(F32).reshape(v.shape[0] // 8, 8, D)


def _b2(v):
    return v.reshape(v.shape[0] * 8, D).astype(BF)


def _kernel(x_hbm, mem0_hbm, wq_hbm, wk_hbm, wv_hbm, wo_hbm, wr_hbm, wg_hbm, wu_hbm, wd_hbm,
            c_hbm, wmod_hbm, out_hbm,
            x_v, h_v, hp_v, att_v, ho_v, wqkv_v, wo_v, stage, wmod_v,
            wg_v, wu_v, wd_v, mem_v, c_v, wr_v, mod_v, r_v,
            sem_small, sem_x, sem_stage, sem_wmod, sem_wo, sem_ffn, sem_out, *rings):
    w_hbm = (wq_hbm, wk_hbm, wv_hbm)
    ring = rings

    def piece_copy(t, lo=0, n=D, sem=None):
        slot = t % 2
        return pltpu.make_async_copy(
            w_hbm[t // 4].at[pl.ds(lo, n), pl.ds((t % 4) * 8, 8), :],
            stage.at[slot, pl.ds(lo, n)], sem_stage.at[slot if sem is None else sem])

    def piece_wait(slot):
        pltpu.make_async_copy(stage.at[slot], stage.at[slot], sem_stage.at[slot]).wait()

    def wmod_copy(k):
        return pltpu.make_async_copy(wmod_hbm.at[:, pl.ds(k * 512, 512)], wmod_v.at[k],
                                     sem_wmod.at[k])

    def wo_copy(n):
        return pltpu.make_async_copy(wo_hbm.at[:, pl.ds(n * 512, 512)], wo_v.at[n], sem_wo.at[n])

    x0_copy = pltpu.make_async_copy(x_hbm.at[0, pl.ds(0, X0), :], x_v.at[pl.ds(0, X0), :],
                                    sem_x.at[0])
    x1_copy = pltpu.make_async_copy(x_hbm.at[0, pl.ds(X0, X1 - X0), :],
                                    x_v.at[pl.ds(X0, X1 - X0), :], sem_x.at[1])
    x2_copy = pltpu.make_async_copy(x_hbm.at[0, pl.ds(X1, S - X1), :],
                                    x_v.at[pl.ds(X1, S - X1), :], sem_x.at[2])
    c_copy = pltpu.make_async_copy(c_hbm, c_v, sem_small.at[0])
    mem_copy = pltpu.make_async_copy(mem0_hbm.at[0], mem_v, sem_small.at[1])
    wr_copy = pltpu.make_async_copy(wr_hbm, wr_v, sem_small.at[2])
    wg_copy = pltpu.make_async_copy(wg_hbm, wg_v, sem_ffn.at[0])
    wu_copy = pltpu.make_async_copy(wu_hbm, wu_v, sem_ffn.at[1])
    wd_copies = [pltpu.make_async_copy(wd_hbm.at[:, pl.ds(k * 512, 512)], wd_v.at[k],
                                       sem_ffn.at[2 + k]) for k in range(2)]

    def relayout(slot, t, lo, n):
        base = t * (8 * PITCH) + lo // 2
        u = pltpu.bitcast(stage[slot, pl.ds(lo, n)], U32)
        tok = None
        for i in range(n // 2):
            a = u[2 * i]
            b = u[2 * i + 1]
            even = (a & jnp.uint32(0xFFFF)) | (b << 16)
            odd = (a >> 16) | (b & jnp.uint32(0xFFFF0000))
            wqkv_v[pl.ds(base + i, 4, stride=PITCH), :] = even
            wqkv_v[pl.ds(base + 4 * PITCH + i, 4, stride=PITCH), :] = odd
            tok = even ^ odd if tok is None else tok ^ even ^ odd
        return jnp.concatenate([tok, tok], axis=0)

    def relayout_loop(slot, t, lo, n):
        def body(i, carry):
            relayout(slot, t, pl.multiple_of(lo + i * 128, 128), 128)
            return carry
        lax.fori_loop(0, n // 128, body, 0)

    def modulate(ln, k_scale, k_shift):
        return _rb(ln * mod_v[k_scale]) + mod_v[k_shift]

    CW = 256

    def ln_stats(xf):
        mu = jnp.mean(xf, axis=-1, keepdims=True)
        dv = xf - mu
        var = jnp.mean(dv * dv, axis=-1, keepdims=True)
        sd = _rb(jnp.sqrt(_rb(_rb(var) + EPS)))
        return _rb(mu), 1.0 / sd

    def mod_c(k, c):
        return mod_v[k, :, pl.ds(c * CW, CW)]

    def token(v):
        return pltpu.bitcast(v[:, :128] + v[:, 128:], U32)

    def after(v, trig):
        if trig is None:
            return v
        return jnp.concatenate([jnp.where(trig[0], trig[1], v[:, :128]), v[:, 128:]], axis=1)

    def post_work(row0, att):
        st = {}

        def head(trig):
            a = after(att().astype(F32), trig)
            st["x2"] = _rb(x_v[pl.ds(row0, 8), :].astype(F32) + _rb(mod_v[2] * a))
            st["mu"], st["inv"] = ln_stats(st["x2"])

        def chunk(c, trig):
            xc = after(st["x2"][:, c * CW:(c + 1) * CW], trig)
            h2b = (_rb(_rb(_rb(xc - st["mu"]) * st["inv"]) * mod_c(4, c))
                   + mod_c(3, c)).astype(BF)
            h2 = h2b.astype(F32)
            ho_v[0, pl.ds(row0, 8), pl.ds(c * CW, CW)] = h2b
            o = xc + mod_c(5, c) * h2
            ho_v[1, pl.ds(row0, 8), pl.ds(c * CW, CW)] = o.astype(BF)
            rp = h2 * mod_c(6, c)
            st["r"] = rp if c == 0 else st["r"] + rp
            if c == D // CW - 1:
                r = jnp.sum(st["r"], axis=-1, keepdims=True)
                grp = row0 // 8
                lanes = lax.broadcasted_iota(jnp.int32, (8, 128), 1)
                r_v[grp // 128] = jnp.where(lanes == grp % 128, r, r_v[grp // 128])
            return token(o + st["r"])
        return [head] + [functools.partial(chunk, c) for c in range(D // CW)]

    def ln1_work(row0):
        st = {}

        def head(trig):
            st["x"] = after(x_v[pl.ds(row0, 8), :].astype(F32), trig)
            st["mu"], st["inv"] = ln_stats(st["x"])

        def chunk(c, trig):
            xc = after(st["x"][:, c * CW:(c + 1) * CW], trig)
            h = _rb(_rb(_rb(xc - st["mu"]) * st["inv"]) * mod_c(1, c)) + mod_c(0, c)
            ho_v[0, pl.ds(row0, 8), pl.ds(c * CW, CW)] = h.astype(BF)
            return token(h)
        return [head] + [functools.partial(chunk, c) for c in range(D // CW)]

    x0_copy.start()
    c_copy.start()
    wmod_copy(0).start()
    mem_copy.start()
    wr_copy.start()

    r_v[...] = jnp.full(r_v.shape, NEG, F32)
    att_v[...] = jnp.zeros(att_v.shape, BF)

    x0_copy.wait()
    wmod_copy(1).start()
    wmod_copy(2).start()

    LNB = X0 // 4

    def ln0(i, carry):
        r0 = pl.multiple_of(i * LNB, 8)
        h_v[pl.ds(r0, LNB), :] = _b2(_layernorm(_f3(x_v[pl.ds(r0, LNB), :])))
        return carry
    lax.fori_loop(0, 4, ln0, 0)

    wmod_copy(3).start()
    piece_copy(0, 0, 512, 0).start()
    c_copy.wait()
    cf = c_v[...].astype(F32)
    sc = jnp.broadcast_to((cf * jax.nn.sigmoid(cf)).astype(BF), (16, D))

    def mod_slab(k):
        y = _rb(jnp.dot(sc, wmod_v[k], preferred_element_type=F32)[0:8])
        if k // 2 in (1, 4):
            y = _rb(1.0 + y)
        mod_v[k // 2, :, pl.ds((k % 2) * 512, 512)] = y

    for k in range(4):
        wmod_copy(k).wait()
        if k == 2:
            piece_copy(0, 512, 256, 2).start()
            piece_copy(0, 768, 256, 3).start()
        mod_slab(k)

    def mod0(i, carry):
        r0 = pl.multiple_of(i * 128, 128)
        hb = _b2(modulate(_f3(h_v[pl.ds(r0, 128), :]), 1, 0))
        hp_v[pl.ds(pl.multiple_of(i * 64, 64), 64), :] = pltpu.bitcast(hb, U32)
        return carry
    lax.fori_loop(0, BULK // 128, mod0, 0)
    ho_v[0, pl.ds(BULK, RIDE), :] = _b2(modulate(_f3(h_v[pl.ds(BULK, RIDE), :]), 1, 0))

    piece_copy(0, 0, 512, 0).wait()
    relayout_loop(0, 0, 0, 512)
    piece_copy(0, 512, 256, 2).wait()
    piece_copy(1).start()
    relayout_loop(0, 0, 512, 256)
    piece_copy(0, 768, 256, 3).wait()
    relayout_loop(0, 0, 768, 256)

    def bulk_dot(i, k, never=None, rl=None):
        w = pltpu.bitcast(wqkv_v[pl.ds(pl.multiple_of((8 * i + k) * PITCH, 8), 512), :], BF)
        cols = [hp_v[:, pl.ds(128 * c, 128)] for c in range(8)]
        if rl is not None:
            slot, t, lo, n = rl
            g = n // 16
            spots = [(12 + (q * 48) // g) for q in range(g)]
            toks = {sp: relayout(slot, t, lo + 16 * q, 16) for q, sp in enumerate(spots)}
            for c in (0, 4):
                cols[c] = jnp.concatenate(
                    [jnp.where(never, toks[8 * c + j], cols[c][8 * j:8 * j + 8])
                     if 8 * c + j in toks else cols[c][8 * j:8 * j + 8]
                     for j in range(32)], axis=0)
        hb = pltpu.bitcast(jnp.concatenate(cols, axis=1), BF)
        y = jnp.dot(hb, w, preferred_element_type=F32)
        ring[k][i, pl.ds(RING - BULK, BULK), :] = y.astype(BF)

    never0 = r_v[0] > 0.0
    piece_copy(2).start()
    for k in range(8):
        if k == 6:
            piece_wait(1)
        bulk_dot(0, k, never0, (1, 1, (k - 6) * 512, 512) if k >= 6 else None)

    def bulk_qkv(i, carry):
        @pl.when(i < 11)
        def _():
            piece_wait((i + 1) % 2)

        for j in range(1, 10):
            @pl.when(i == j)
            def _():
                piece_copy(j + 2).start()
        t = jnp.minimum(i + 1, 11)
        never = jnp.full((8, 128), i, jnp.int32) < 0
        for k in range(8):
            bulk_dot(i, k, never, (t % 2, t, k * 128, 128))

        for j in range(1, 10):
            @pl.when(i == j)
            def _():
                if j < 8:
                    wmod_copy(j + 4).start()
                if j == 8:
                    x1_copy.start()
                if j == 9:
                    for n in range(2):
                        wo_copy(n).start()
        return carry
    wmod_copy(4).start()
    lax.fori_loop(1, 12, bulk_qkv, 0)

    for k in range(4, 12):
        wmod_copy(k).wait()
    for k in range(4, 12):
        mod_slab(k)
    wr_copy.wait()
    mod_v[6] = jnp.broadcast_to(wr_v[...].astype(F32), (8, D))
    mem_copy.wait()
    for n in range(2):
        wo_copy(n).wait()
    x1_copy.wait()
    x2_copy.start()
    wg_copy.start()
    wu_copy.start()
    for cp in wd_copies:
        cp.start()

    scale = DH ** -0.5
    rr = lax.broadcasted_iota(jnp.int32, (80, 80), 0)
    cc = lax.broadcasted_iota(jnp.int32, (80, 80), 1)

    def second(i):
        return ((i >= 8) & (i < 16)) | (i >= 48)
    same = second(rr) == second(cc)
    allowed = same & ((rr < 16) | (cc <= rr))
    fill = jnp.where(same, -1e9, NEG).astype(F32)

    def w_slab(t, g, lo=0, n=512, tok=None):
        u = wqkv_v[pl.ds((8 * t + g) * PITCH + lo, n), :]
        if tok is not None:
            u = jnp.concatenate([jnp.where(tok[0], tok[1], u[:8]), u[8:]], axis=0)
        return pltpu.bitcast(u, BF)

    def step(s, mem, chained, left, att_prev):
        odd = left is not None
        wr = pl.multiple_of(lax.rem(RIDE * s, RING), 8)
        rd = pl.multiple_of(lax.rem(SEG * s + RING - BULK, RING), SEG)
        xin = jnp.concatenate(
            [mem, ho_v[0, pl.ds(pl.multiple_of(BULK + RIDE * s, 8), RIDE), :]], axis=0)

        prow = SEG * (s - 1) if odd else jnp.maximum(SEG * s - 40, 0)
        nrow = BULK + RIDE * jnp.minimum(s + 1, NSEG - 1)
        works = [post_work(pl.multiple_of(prow + 8 * q, 8), functools.partial(att_prev, q))
                 for q in range(3 if odd else 5)]
        works += [ln1_work(pl.multiple_of(nrow + 8 * q, 8)) for q in range(RIDE // 8)]
        never = jnp.full((8, 128), s, jnp.int32) < 0
        gap = (96 - SIDE0 - SIDE_LAT - SIDE_DUE) // len(works)
        sched = {}
        for q, wk in enumerate(works):
            sched.setdefault(SIDE0 + gap * q, []).append(wk[0])
            for c in range(1, len(wk)):
                sched.setdefault(SIDE0 + SIDE_LAT + gap * q + ((c - 1) * gap) // 4,
                                 []).append(wk[c])

        memqkv, probs, wl, new_left, toks = {}, {}, {}, {}, {}
        acc = []

        def qkv(g, split=False):
            part = {}
            if split:
                for t in range(6):
                    part[t] = jnp.dot(xin[:, :512], w_slab(t, g, 0, 256),
                                      preferred_element_type=F32)
            for t0 in range(0, 12, 2):
                ys = []
                for t in (t0, t0 + 1):
                    if t in part:
                        y = jnp.dot(xin[:, 512:], w_slab(t, g, 256, 256),
                                    preferred_element_type=F32) + part[t]
                    else:
                        y = jnp.dot(xin, w_slab(t, g, tok=toks.get(12 * g + t)),
                                    preferred_element_type=F32)
                    ring[g][t, pl.ds(wr, RIDE), :] = y[M:].astype(BF)
                    ys.append(y[:M])
                    for item in sched.get(12 * g + t, ()):
                        tk = item((never, y[:M]))
                        if tk is not None:
                            toks[12 * g + t + SIDE_DUE] = (never, tk)
                memqkv[(t0, g)] = jnp.concatenate(ys, axis=0).astype(BF)

        def cat(t0, g):
            return jnp.concatenate([memqkv[(t0, g)], ring[g][t0, pl.ds(rd, SEG), :],
                                    ring[g][t0 + 1, pl.ds(rd, SEG), :]], axis=0)

        def scores(g):
            for p in (0, 2):
                sc_ = lax.dot_general(cat(p, g), cat(4 + p, g), (((1,), (1,)), ((), ())),
                                      preferred_element_type=F32)
                sc_ = jnp.where(allowed, sc_ * scale, fill)
                e = jnp.exp(sc_ - jnp.max(sc_, axis=1, keepdims=True))
                l = jnp.sum(e, axis=1, keepdims=True)
                rc = pl.reciprocal(l, approx=True)
                rc = rc * (2.0 - l * rc)
                probs[(p, g)] = (e * rc).astype(BF)

        def pv(g):
            for p in (0, 2):
                o = jnp.dot(probs[(p, g)], cat(8 + p, g), preferred_element_type=F32)
                for j in range(2):
                    om, ot = o[8 * j:8 * j + 8], o[16 + 32 * j:48 + 32 * j]
                    if odd:
                        rows = [om, left[(p + j, g)], ot]
                    else:
                        rows = [om, ot[:RIDE]]
                        new_left[(p + j, g)] = ot[RIDE:]
                    wl[(p + j, g)] = jnp.concatenate(rows, axis=0).astype(BF)

        def wo(g):
            a = jnp.concatenate([wl[(o, g)] for o in range(4)], axis=1)
            w = jnp.concatenate(
                [jnp.concatenate([wo_v[n, pl.ds((8 * o + PERM[g]) * DH, DH), :]
                                  for o in range(4)], axis=0) for n in range(2)], axis=1)
            y = jnp.dot(a, w, preferred_element_type=F32)
            acc[:] = [y if not acc else y + acc[0]]

        qkv(0, chained), qkv(1), qkv(2)
        scores(0), scores(1)
        qkv(3), qkv(4)
        pv(0), pv(1), scores(2), scores(3)
        qkv(5), qkv(6)
        pv(2), pv(3), scores(4), scores(5)
        qkv(7), wo(0)
        pv(4), pv(5), scores(6), scores(7)
        wo(1), wo(2), wo(3)
        pv(6), pv(7)
        wo(4), wo(5), wo(6), wo(7)
        y = acc[0].astype(BF)
        return y[:M], y[M:], (None if odd else new_left)

    def out_copy(row0, n, k):
        return pltpu.make_async_copy(ho_v.at[1, pl.ds(row0, n), :],
                                     out_hbm.at[0, pl.ds(row0, n), :], sem_out.at[k])

    OB = SEG * UNROLL

    def carried(q):
        return att_v[pl.ds(8 * q, 8), :]

    def steps(i, carry):
        @pl.when(i == 16 // UNROLL)
        def _():
            x2_copy.wait()

        @pl.when(i >= 3)
        def _():
            out_copy(0, OB, 0).wait()

        @pl.when(i >= 2)
        def _():
            out_copy(pl.multiple_of((i - 2) * OB, OB), OB, 0).start()

        mem, left, att_prev = mem_v[...], None, carried
        for u in range(UNROLL):
            mem, att, left = step(i * UNROLL + u, mem, u > 0, left, att_prev)
            att_prev = (lambda a: lambda q: a[8 * q:8 * q + 8])(att)
        mem_v[...] = mem
        att_v[...] = att
        return carry
    lax.fori_loop(0, NSEG // UNROLL, steps, 0)

    out_copy(S - 2 * OB, OB, 1).start()
    for q in range(5):
        for item in post_work(S - 40 + 8 * q, functools.partial(carried, q)):
            item(None)
    out_copy(S - OB, OB, 2).start()

    sub1 = lax.broadcasted_iota(jnp.int32, (16, 128), 0)
    lan1 = lax.broadcasted_iota(jnp.int32, (16, 128), 1)
    idx = (sub1 // 8) * 1024 + lan1 * 8 + sub1 % 8
    valid = idx >= 0
    rall = _rb(r_v[...].reshape(16, 128))
    big = jnp.int32(2 ** 30)

    def argtop(ok):
        v = jnp.where(ok, rall, -jnp.inf)
        m = jnp.max(jnp.max(v, axis=0, keepdims=True), axis=1, keepdims=True)
        cand = jnp.where(ok & (v >= m), idx, big)
        i = jnp.min(jnp.min(cand, axis=0, keepdims=True), axis=1, keepdims=True)
        return m, i
    m_a, i_a = argtop(valid)
    m_b, i_b = argtop(valid & (idx != i_a))
    ia = jnp.clip(i_a[0, 0], 0, S - 1)
    ib = jnp.clip(i_b[0, 0], 0, S - 1)
    blk_a = pl.multiple_of((ia // 8) * 8, 8)
    blk_b = pl.multiple_of((ib // 8) * 8, 8)

    def two(ref):
        return jnp.concatenate([ref[pl.ds(blk_a, 8), :], ref[pl.ds(blk_b, 8), :]], axis=0)

    hs = two(ho_v.at[0])
    wg_copy.wait()
    wu_copy.wait()
    for cp in wd_copies:
        cp.wait()
    g = _rb(jnp.dot(hs, wg_v[...], preferred_element_type=F32))
    u = _rb(jnp.dot(hs, wu_v[...], preferred_element_type=F32))
    act = (_rb(g * jax.nn.sigmoid(g)) * u).astype(BF)
    y = jnp.concatenate(
        [jnp.dot(act, wd_v[k], preferred_element_type=F32) for k in range(2)], axis=1)
    sub = lax.broadcasted_iota(jnp.int32, (16, 1), 0)
    rows = jnp.where(sub < 8, blk_a + sub, blk_b + sub - 8)
    gate = jnp.where(rows == ia, jax.nn.sigmoid(m_a),
                     jnp.where(rows == ib, jax.nn.sigmoid(m_b), 0.0))
    upd = jnp.where((rows == ia) | (rows == ib), y * gate, 0.0).reshape(2, 8, D)
    fin = _b2(_f3(two(ho_v.at[1])) + mod_v[5] * upd)

    for k in range(3):
        out_copy(0, OB, k).wait()
    ho_v[1, pl.ds(blk_a, 8), :] = fin[0:8]
    ho_v[1, pl.ds(blk_b, 8), :] = fin[8:16]
    out_copy(blk_a, 8, 0).start()

    @pl.when(blk_a != blk_b)
    def _():
        out_copy(blk_b, 8, 1).start()
        out_copy(blk_b, 8, 1).wait()
    out_copy(blk_a, 8, 0).wait()


@jax.jit
def pallas_adaLN_cond__memory_aug_recurrent_mem_tr__moe_arch_mod__prompt_kernel(
    A_x, A_mem0, A_Wq, A_Wk, A_Wv, A_Wo, A_seg_len, B_x, B_w_r, B_w_gate, B_w_up, B_w_down, c,
    w_mod,
):
    del B_x
    del A_seg_len
    assert A_x.shape == (1, S, D) and A_Wq.shape == (D, H, DH) and A_mem0.shape == (1, M, D)
    any_spec = pl.BlockSpec(memory_space=pl.ANY)
    scratch = [
        pltpu.VMEM((S, D), BF),
        pltpu.VMEM((X0, D), BF),
        pltpu.VMEM((BULK // 2, D), U32),
        pltpu.VMEM((40, D), BF),
        pltpu.VMEM((2, S, D), BF),
        pltpu.VMEM((96 * PITCH, 128), U32),
        pltpu.VMEM((2, H * DH, 512), BF),
        pltpu.VMEM((2, D, 8, 128), BF),
        pltpu.VMEM((12, D, 512), BF),
        pltpu.VMEM((D, FF), BF),
        pltpu.VMEM((D, FF), BF),
        pltpu.VMEM((2, FF, 512), BF),
        pltpu.VMEM((M, D), BF),
        pltpu.VMEM((1, D), BF),
        pltpu.VMEM((1, D), BF),
        pltpu.VMEM((7, 8, D), F32),
        pltpu.VMEM((2, 8, 128), F32),
        pltpu.SemaphoreType.DMA((3,)),
        pltpu.SemaphoreType.DMA((3,)),
        pltpu.SemaphoreType.DMA((4,)),
        pltpu.SemaphoreType.DMA((12,)),
        pltpu.SemaphoreType.DMA((8,)),
        pltpu.SemaphoreType.DMA((4,)),
        pltpu.SemaphoreType.DMA((8,)),
    ] + [pltpu.VMEM((12, RING, 128), BF)] * 8
    return pl.pallas_call(
        _kernel,
        out_shape=jax.ShapeDtypeStruct((1, S, D), BF),
        in_specs=[any_spec] * 12,
        out_specs=any_spec,
        scratch_shapes=scratch,
        compiler_params=pltpu.CompilerParams(vmem_limit_bytes=120 * 1024 * 1024),
    )(A_x, A_mem0, A_Wq, A_Wk, A_Wv, A_Wo.reshape(H * DH, D), B_w_r.reshape(1, D), B_w_gate,
      B_w_up, B_w_down, c, w_mod)
```

```python
import functools

import jax
import jax.numpy as jnp
from jax import lax
import jax.experimental.pallas as pl
import jax.experimental.pallas.tpu as pltpu

BF = jnp.bfloat16
F32 = jnp.float32
U32 = jnp.uint32

S = 2048
D = 1024
H = 32
DH = 128
M = 8
SEG = 32
NSEG = S // SEG
FF = 3584
RIDE = 24
BULK = S - RIDE * NSEG
X0 = BULK + 32
RING = 576
PITCH = 520
X1 = 1024
UNROLL = 4
EPS = 1e-5
SIDE0, SIDE_LAT, SIDE_DUE, SIDE_END = 2, 6, 6, 96
NEG = -3.0e38
ORDER = ("q0 q1 q2 q3 q4 q5 q6 s0 s1 s2 s3 s4 s5 q7 p0 p1 p2 p3 p4 p5 s6 s7 w0 w1 w2 p6 p7 w3 "
         "w4 w5 w6 w7")
PERM = (0, 2, 4, 6, 1, 3, 5, 7)


def _rb(v):
    return v.astype(BF).astype(F32)


def _layernorm(xf):
    mu = jnp.mean(xf, axis=-1, keepdims=True)
    dv = xf - mu
    var = jnp.mean(dv * dv, axis=-1, keepdims=True)
    sd = _rb(jnp.sqrt(_rb(_rb(var) + EPS)))
    return _rb(_rb(xf - _rb(mu)) * (1.0 / sd))


def _f3(v):
    return v.astype(F32).reshape(v.shape[0] // 8, 8, D)


def _b2(v):
    return v.reshape(v.shape[0] * 8, D).astype(BF)


def _kernel(x_hbm, mem0_hbm, wq_hbm, wk_hbm, wv_hbm, wo_hbm, wr_hbm, wg_hbm, wu_hbm, wd_hbm,
            c_hbm, wmod_hbm, out_hbm,
            x_v, h_v, hp_v, att_v, ho_v, wqkv_v, wo_v, stage, wmod_v,
            wg_v, wu_v, wd_v, mem_v, c_v, wr_v, mod_v, r_v,
            sem_small, sem_x, sem_stage, sem_wmod, sem_wo, sem_ffn, sem_out, *rings):
    w_hbm = (wq_hbm, wk_hbm, wv_hbm)
    ring = rings

    def piece_copy(t, lo=0, n=D, sem=None):
        slot = t % 2
        return pltpu.make_async_copy(
            w_hbm[t // 4].at[pl.ds(lo, n), pl.ds((t % 4) * 8, 8), :],
            stage.at[slot, pl.ds(lo, n)], sem_stage.at[slot if sem is None else sem])

    def piece_wait(slot):
        pltpu.make_async_copy(stage.at[slot], stage.at[slot], sem_stage.at[slot]).wait()

    def wmod_copy(k):
        return pltpu.make_async_copy(wmod_hbm.at[:, pl.ds(k * 512, 512)], wmod_v.at[k],
                                     sem_wmod.at[k])

    def wo_copy(n):
        return pltpu.make_async_copy(wo_hbm.at[:, pl.ds(n * 512, 512)], wo_v.at[n], sem_wo.at[n])

    x0_copy = pltpu.make_async_copy(x_hbm.at[0, pl.ds(0, X0), :], x_v.at[pl.ds(0, X0), :],
                                    sem_x.at[0])
    x1_copy = pltpu.make_async_copy(x_hbm.at[0, pl.ds(X0, X1 - X0), :],
                                    x_v.at[pl.ds(X0, X1 - X0), :], sem_x.at[1])
    x2_copy = pltpu.make_async_copy(x_hbm.at[0, pl.ds(X1, S - X1), :],
                                    x_v.at[pl.ds(X1, S - X1), :], sem_x.at[2])
    c_copy = pltpu.make_async_copy(c_hbm, c_v, sem_small.at[0])
    mem_copy = pltpu.make_async_copy(mem0_hbm.at[0], mem_v, sem_small.at[1])
    wr_copy = pltpu.make_async_copy(wr_hbm, wr_v, sem_small.at[2])
    wg_copy = pltpu.make_async_copy(wg_hbm, wg_v, sem_ffn.at[0])
    wu_copy = pltpu.make_async_copy(wu_hbm, wu_v, sem_ffn.at[1])
    wd_copies = [pltpu.make_async_copy(wd_hbm.at[:, pl.ds(k * 512, 512)], wd_v.at[k],
                                       sem_ffn.at[2 + k]) for k in range(2)]

    def relayout(slot, t, lo, n):
        base = t * (8 * PITCH) + lo // 2
        u = pltpu.bitcast(stage[slot, pl.ds(lo, n)], U32)
        tok = None
        for i in range(n // 2):
            a = u[2 * i]
            b = u[2 * i + 1]
            even = (a & jnp.uint32(0xFFFF)) | (b << 16)
            odd = (a >> 16) | (b & jnp.uint32(0xFFFF0000))
            wqkv_v[pl.ds(base + i, 4, stride=PITCH), :] = even
            wqkv_v[pl.ds(base + 4 * PITCH + i, 4, stride=PITCH), :] = odd
            tok = even ^ odd if tok is None else tok ^ even ^ odd
        return jnp.concatenate([tok, tok], axis=0)

    def relayout_loop(slot, t, lo, n):
        def body(i, carry):
            relayout(slot, t, pl.multiple_of(lo + i * 128, 128), 128)
            return carry
        lax.fori_loop(0, n // 128, body, 0)

    def modulate(ln, k_scale, k_shift):
        return _rb(ln * mod_v[k_scale]) + mod_v[k_shift]

    CW = 256

    def ln_stats(xf):
        mu = jnp.mean(xf, axis=-1, keepdims=True)
        dv = xf - mu
        var = jnp.mean(dv * dv, axis=-1, keepdims=True)
        sd = _rb(jnp.sqrt(_rb(_rb(var) + EPS)))
        return _rb(mu), 1.0 / sd

    def mod_c(k, c):
        return mod_v[k, :, pl.ds(c * CW, CW)]

    def token(v):
        return pltpu.bitcast(v[:, :128] + v[:, 128:], U32)

    def after(v, trig):
        if trig is None:
            return v
        return jnp.concatenate([jnp.where(trig[0], trig[1], v[:, :128]), v[:, 128:]], axis=1)

    def post_work(row0, att):
        st = {}

        def head(trig):
            a = after(att().astype(F32), trig)
            st["x2"] = _rb(x_v[pl.ds(row0, 8), :].astype(F32) + _rb(mod_v[2] * a))
            st["mu"], st["inv"] = ln_stats(st["x2"])

        def chunk(c, trig):
            xc = after(st["x2"][:, c * CW:(c + 1) * CW], trig)
            h2b = (_rb(_rb(_rb(xc - st["mu"]) * st["inv"]) * mod_c(4, c))
                   + mod_c(3, c)).astype(BF)
            h2 = h2b.astype(F32)
            ho_v[0, pl.ds(row0, 8), pl.ds(c * CW, CW)] = h2b
            o = xc + mod_c(5, c) * h2
            ho_v[1, pl.ds(row0, 8), pl.ds(c * CW, CW)] = o.astype(BF)
            rp = h2 * mod_c(6, c)
            st["r"] = rp if c == 0 else st["r"] + rp
            if c == D // CW - 1:
                r = jnp.sum(st["r"], axis=-1, keepdims=True)
                grp = row0 // 8
                lanes = lax.broadcasted_iota(jnp.int32, (8, 128), 1)
                r_v[grp // 128] = jnp.where(lanes == grp % 128, r, r_v[grp // 128])
            return token(o + st["r"])
        return [head] + [functools.partial(chunk, c) for c in range(D // CW)]

    def ln1_work(row0):
        st = {}

        def head(trig):
            st["x"] = after(x_v[pl.ds(row0, 8), :].astype(F32), trig)
            st["mu"], st["inv"] = ln_stats(st["x"])

        def chunk(c, trig):
            xc = after(st["x"][:, c * CW:(c + 1) * CW], trig)
            h = _rb(_rb(_rb(xc - st["mu"]) * st["inv"]) * mod_c(1, c)) + mod_c(0, c)
            ho_v[0, pl.ds(row0, 8), pl.ds(c * CW, CW)] = h.astype(BF)
            return token(h)
        return [head] + [functools.partial(chunk, c) for c in range(D // CW)]

    x0_copy.start()
    c_copy.start()
    wmod_copy(0).start()
    mem_copy.start()
    wr_copy.start()

    r_v[...] = jnp.full(r_v.shape, NEG, F32)
    att_v[...] = jnp.zeros(att_v.shape, BF)

    x0_copy.wait()
    wmod_copy(1).start()
    wmod_copy(2).start()

    LNB = X0 // 4

    def ln0(i, carry):
        r0 = pl.multiple_of(i * LNB, 8)
        h_v[pl.ds(r0, LNB), :] = _b2(_layernorm(_f3(x_v[pl.ds(r0, LNB), :])))
        return carry
    lax.fori_loop(0, 4, ln0, 0)

    wmod_copy(3).start()
    piece_copy(0, 0, 512, 0).start()
    c_copy.wait()
    cf = c_v[...].astype(F32)
    sc = jnp.broadcast_to((cf * jax.nn.sigmoid(cf)).astype(BF), (16, D))

    def mod_slab(k):
        y = _rb(jnp.dot(sc, wmod_v[k], preferred_element_type=F32)[0:8])
        if k // 2 in (1, 4):
            y = _rb(1.0 + y)
        mod_v[k // 2, :, pl.ds((k % 2) * 512, 512)] = y

    for k in range(4):
        wmod_copy(k).wait()
        if k == 2:
            piece_copy(0, 512, 256, 2).start()
            piece_copy(0, 768, 256, 3).start()
        mod_slab(k)

    def mod0(i, carry):
        r0 = pl.multiple_of(i * 128, 128)
        hb = _b2(modulate(_f3(h_v[pl.ds(r0, 128), :]), 1, 0))
        hp_v[pl.ds(pl.multiple_of(i * 64, 64), 64), :] = pltpu.bitcast(hb, U32)
        return carry
    lax.fori_loop(0, BULK // 128, mod0, 0)
    ho_v[0, pl.ds(BULK, RIDE), :] = _b2(modulate(_f3(h_v[pl.ds(BULK, RIDE), :]), 1, 0))

    piece_copy(0, 0, 512, 0).wait()
    relayout_loop(0, 0, 0, 512)
    piece_copy(0, 512, 256, 2).wait()
    piece_copy(1).start()
    relayout_loop(0, 0, 512, 256)
    piece_copy(0, 768, 256, 3).wait()
    relayout_loop(0, 0, 768, 256)

    def bulk_dot(i, k, never=None, rl=None):
        w = pltpu.bitcast(wqkv_v[pl.ds(pl.multiple_of((8 * i + k) * PITCH, 8), 512), :], BF)
        cols = [hp_v[:, pl.ds(128 * c, 128)] for c in range(8)]
        if rl is not None:
            slot, t, lo, n = rl
            g = n // 16
            spots = [(12 + (q * 48) // g) for q in range(g)]
            toks = {sp: relayout(slot, t, lo + 16 * q, 16) for q, sp in enumerate(spots)}
            for c in (0, 4):
                cols[c] = jnp.concatenate(
                    [jnp.where(never, toks[8 * c + j], cols[c][8 * j:8 * j + 8])
                     if 8 * c + j in toks else cols[c][8 * j:8 * j + 8]
                     for j in range(32)], axis=0)
        hb = pltpu.bitcast(jnp.concatenate(cols, axis=1), BF)
        y = jnp.dot(hb, w, preferred_element_type=F32)
        ring[k][i, pl.ds(RING - BULK, BULK), :] = y.astype(BF)

    never0 = r_v[0] > 0.0
    piece_copy(2).start()
    for k in range(8):
        if k == 6:
            piece_wait(1)
        bulk_dot(0, k, never0, (1, 1, (k - 6) * 512, 512) if k >= 6 else None)

    def bulk_qkv(i, carry):
        @pl.when(i < 11)
        def _():
            piece_wait((i + 1) % 2)

        for j in range(1, 10):
            @pl.when(i == j)
            def _():
                piece_copy(j + 2).start()
        t = jnp.minimum(i + 1, 11)
        never = jnp.full((8, 128), i, jnp.int32) < 0
        for k in range(8):
            bulk_dot(i, k, never, (t % 2, t, k * 128, 128))

        for j in range(1, 10):
            @pl.when(i == j)
            def _():
                if j < 8:
                    wmod_copy(j + 4).start()
                if j == 8:
                    x1_copy.start()
                if j == 9:
                    for n in range(2):
                        wo_copy(n).start()
        return carry
    wmod_copy(4).start()
    lax.fori_loop(1, 12, bulk_qkv, 0)

    for k in range(4, 12):
        wmod_copy(k).wait()
    for k in range(4, 12):
        mod_slab(k)
    wr_copy.wait()
    mod_v[6] = jnp.broadcast_to(wr_v[...].astype(F32), (8, D))
    mem_copy.wait()
    for n in range(2):
        wo_copy(n).wait()
    x1_copy.wait()
    x2_copy.start()
    wg_copy.start()
    wu_copy.start()
    for cp in wd_copies:
        cp.start()

    scale = DH ** -0.5
    rr = lax.broadcasted_iota(jnp.int32, (80, 80), 0)
    cc = lax.broadcasted_iota(jnp.int32, (80, 80), 1)

    def second(i):
        return ((i >= 8) & (i < 16)) | (i >= 48)
    same = second(rr) == second(cc)
    allowed = same & ((rr < 16) | (cc <= rr))
    fill = jnp.where(same, -1e9, NEG).astype(F32)

    def tied(u, never, toks):
        if not toks:
            return u
        parts, at = [], 0
        for j, tk in enumerate(toks):
            r = 64 * j
            if r > at:
                parts.append(u[at:r])
            w = tk.shape[1]
            sel = jnp.where(never[:, :w], tk, u[r:r + 8, :w])
            parts.append(sel if w == 128 else jnp.concatenate([sel, u[r:r + 8, w:]], axis=1))
            at = r + 8
        return jnp.concatenate(parts + [u[at:]], axis=0)

    def w_slab(t, g, lo=0, n=512, never=None, toks=()):
        return pltpu.bitcast(
            tied(wqkv_v[pl.ds((8 * t + g) * PITCH + lo, n), :], never, toks), BF)

    def step(s, mem, chained, left, att_prev):
        odd = left is not None
        wr = pl.multiple_of(lax.rem(RIDE * s, RING), 8)
        rd = pl.multiple_of(lax.rem(SEG * s + RING - BULK, RING), SEG)
        xin = jnp.concatenate(
            [mem, ho_v[0, pl.ds(pl.multiple_of(BULK + RIDE * s, 8), RIDE), :]], axis=0)

        prow = SEG * (s - 1) if odd else jnp.maximum(SEG * s - 40, 0)
        nrow = BULK + RIDE * jnp.minimum(s + 1, NSEG - 1)
        works = [post_work(pl.multiple_of(prow + 8 * q, 8), functools.partial(att_prev, q))
                 for q in range(3 if odd else 5)]
        works += [ln1_work(pl.multiple_of(nrow + 8 * q, 8)) for q in range(RIDE // 8)]
        never = jnp.full((8, 128), s, jnp.int32) < 0
        gap = (SIDE_END - SIDE0 - SIDE_LAT - SIDE_DUE) // len(works)
        sched = {}
        for q, wk in enumerate(works):
            sched.setdefault(SIDE0 + gap * q, []).append(wk[0])
            for c in range(1, len(wk)):
                sched.setdefault(SIDE0 + SIDE_LAT + gap * q + ((c - 1) * gap) // 4,
                                 []).append(wk[c])

        memqkv, probs, wl, new_left, toks = {}, {}, {}, {}, {}
        acc = []

        ndot = [0]

        def proj(g, t_lo, t_hi):
            part = {}
            if chained and ndot[0] == 0:
                for t in range(t_lo, t_lo + 6):
                    part[t] = jnp.dot(xin[:, :512], w_slab(t, g, 0, 256),
                                      preferred_element_type=F32)
            for t0 in range(t_lo, t_hi, 2):
                ys = []
                for t in (t0, t0 + 1):
                    n = ndot[0]
                    ndot[0] += 1
                    if t in part:
                        y = jnp.dot(xin[:, 512:], w_slab(t, g, 256, 256),
                                    preferred_element_type=F32) + part[t]
                    else:
                        y = jnp.dot(xin, w_slab(t, g, 0, 512, never, toks.get(n)),
                                    preferred_element_type=F32)
                    ring[g][t, pl.ds(wr, RIDE), :] = y[M:].astype(BF)
                    ys.append(y[:M])
                    for item in sched.get(n, ()):
                        tk = item((never, y[:M]))
                        if tk is not None:
                            toks.setdefault(n + SIDE_DUE, []).append(tk)
                memqkv[(t0, g)] = jnp.concatenate(ys, axis=0).astype(BF)

        def cat(t0, g):
            return jnp.concatenate([memqkv[(t0, g)], ring[g][t0, pl.ds(rd, SEG), :],
                                    ring[g][t0 + 1, pl.ds(rd, SEG), :]], axis=0)

        def scores(g):
            for p in (0, 2):
                sc_ = lax.dot_general(cat(p, g), cat(4 + p, g), (((1,), (1,)), ((), ())),
                                      preferred_element_type=F32)
                sc_ = jnp.where(allowed, sc_ * scale, fill)
                e = jnp.exp(sc_ - jnp.max(sc_, axis=1, keepdims=True))
                l = jnp.sum(e, axis=1, keepdims=True)
                rc = pl.reciprocal(l, approx=True)
                rc = rc * (2.0 - l * rc)
                probs[(p, g)] = (e * rc).astype(BF)

        def pv(g):
            for p in (0, 2):
                o = jnp.dot(probs[(p, g)], cat(8 + p, g), preferred_element_type=F32)
                for j in range(2):
                    om, ot = o[8 * j:8 * j + 8], o[16 + 32 * j:48 + 32 * j]
                    if odd:
                        rows = [om, left[(p + j, g)], ot]
                    else:
                        rows = [om, ot[:RIDE]]
                        new_left[(p + j, g)] = ot[RIDE:]
                    wl[(p + j, g)] = jnp.concatenate(rows, axis=0).astype(BF)

        def wo(g):
            a = jnp.concatenate([wl[(o, g)] for o in range(4)], axis=1)
            w = jnp.concatenate(
                [jnp.concatenate([wo_v[n, pl.ds((8 * o + PERM[g]) * DH, DH), :]
                                  for o in range(4)], axis=0) for n in range(2)], axis=1)
            y = jnp.dot(a, w, preferred_element_type=F32)
            acc[:] = [y if not acc else y + acc[0]]

        for op in ORDER.split():
            g = int(op[1])
            if op[0] in "qkv":
                proj(g, *{"q": (0, 12), "k": (0, 8), "v": (8, 12)}[op[0]])
            else:
                {"s": scores, "p": pv, "w": wo}[op[0]](g)
        y = acc[0].astype(BF)
        return y[:M], y[M:], (None if odd else new_left)

    def out_copy(row0, n, k):
        return pltpu.make_async_copy(ho_v.at[1, pl.ds(row0, n), :],
                                     out_hbm.at[0, pl.ds(row0, n), :], sem_out.at[k])

    OB = SEG * UNROLL

    def carried(q):
        return att_v[pl.ds(8 * q, 8), :]

    def steps(i, carry):
        @pl.when(i == 16 // UNROLL)
        def _():
            x2_copy.wait()

        @pl.when(i >= 3)
        def _():
            out_copy(0, OB, 0).wait()

        @pl.when(i >= 2)
        def _():
            out_copy(pl.multiple_of((i - 2) * OB, OB), OB, 0).start()

        mem, left, att_prev = mem_v[...], None, carried
        for u in range(UNROLL):
            mem, att, left = step(i * UNROLL + u, mem, u > 0, left, att_prev)
            att_prev = (lambda a: lambda q: a[8 * q:8 * q + 8])(att)
        mem_v[...] = mem
        att_v[...] = att
        return carry
    lax.fori_loop(0, NSEG // UNROLL, steps, 0)

    out_copy(S - 2 * OB, OB, 1).start()
    for q in range(5):
        for item in post_work(S - 40 + 8 * q, functools.partial(carried, q)):
            item(None)
    out_copy(S - OB, OB, 2).start()

    sub1 = lax.broadcasted_iota(jnp.int32, (16, 128), 0)
    lan1 = lax.broadcasted_iota(jnp.int32, (16, 128), 1)
    idx = (sub1 // 8) * 1024 + lan1 * 8 + sub1 % 8
    valid = idx >= 0
    rall = _rb(r_v[...].reshape(16, 128))
    big = jnp.int32(2 ** 30)

    def argtop(ok):
        v = jnp.where(ok, rall, -jnp.inf)
        m = jnp.max(jnp.max(v, axis=0, keepdims=True), axis=1, keepdims=True)
        cand = jnp.where(ok & (v >= m), idx, big)
        i = jnp.min(jnp.min(cand, axis=0, keepdims=True), axis=1, keepdims=True)
        return m, i
    m_a, i_a = argtop(valid)
    m_b, i_b = argtop(valid & (idx != i_a))
    ia = jnp.clip(i_a[0, 0], 0, S - 1)
    ib = jnp.clip(i_b[0, 0], 0, S - 1)
    blk_a = pl.multiple_of((ia // 8) * 8, 8)
    blk_b = pl.multiple_of((ib // 8) * 8, 8)

    def two(ref):
        return jnp.concatenate([ref[pl.ds(blk_a, 8), :], ref[pl.ds(blk_b, 8), :]], axis=0)

    hs = two(ho_v.at[0])
    wg_copy.wait()
    wu_copy.wait()
    for cp in wd_copies:
        cp.wait()
    g = _rb(jnp.dot(hs, wg_v[...], preferred_element_type=F32))
    u = _rb(jnp.dot(hs, wu_v[...], preferred_element_type=F32))
    act = (_rb(g * jax.nn.sigmoid(g)) * u).astype(BF)
    y = jnp.concatenate(
        [jnp.dot(act, wd_v[k], preferred_element_type=F32) for k in range(2)], axis=1)
    sub = lax.broadcasted_iota(jnp.int32, (16, 1), 0)
    rows = jnp.where(sub < 8, blk_a + sub, blk_b + sub - 8)
    gate = jnp.where(rows == ia, jax.nn.sigmoid(m_a),
                     jnp.where(rows == ib, jax.nn.sigmoid(m_b), 0.0))
    upd = jnp.where((rows == ia) | (rows == ib), y * gate, 0.0).reshape(2, 8, D)
    fin = _b2(_f3(two(ho_v.at[1])) + mod_v[5] * upd)

    for k in range(3):
        out_copy(0, OB, k).wait()
    ho_v[1, pl.ds(blk_a, 8), :] = fin[0:8]
    ho_v[1, pl.ds(blk_b, 8), :] = fin[8:16]
    out_copy(blk_a, 8, 0).start()

    @pl.when(blk_a != blk_b)
    def _():
        out_copy(blk_b, 8, 1).start()
        out_copy(blk_b, 8, 1).wait()
    out_copy(blk_a, 8, 0).wait()


@jax.jit
def pallas_adaLN_cond__memory_aug_recurrent_mem_tr__moe_arch_mod__prompt_kernel(
    A_x, A_mem0, A_Wq, A_Wk, A_Wv, A_Wo, A_seg_len, B_x, B_w_r, B_w_gate, B_w_up, B_w_down, c,
    w_mod,
):
    del B_x
    del A_seg_len
    assert A_x.shape == (1, S, D) and A_Wq.shape == (D, H, DH) and A_mem0.shape == (1, M, D)
    any_spec = pl.BlockSpec(memory_space=pl.ANY)
    scratch = [
        pltpu.VMEM((S, D), BF),
        pltpu.VMEM((X0, D), BF),
        pltpu.VMEM((BULK // 2, D), U32),
        pltpu.VMEM((40, D), BF),
        pltpu.VMEM((2, S, D), BF),
        pltpu.VMEM((96 * PITCH, 128), U32),
        pltpu.VMEM((2, H * DH, 512), BF),
        pltpu.VMEM((2, D, 8, 128), BF),
        pltpu.VMEM((12, D, 512), BF),
        pltpu.VMEM((D, FF), BF),
        pltpu.VMEM((D, FF), BF),
        pltpu.VMEM((2, FF, 512), BF),
        pltpu.VMEM((M, D), BF),
        pltpu.VMEM((1, D), BF),
        pltpu.VMEM((1, D), BF),
        pltpu.VMEM((7, 8, D), F32),
        pltpu.VMEM((2, 8, 128), F32),
        pltpu.SemaphoreType.DMA((3,)),
        pltpu.SemaphoreType.DMA((3,)),
        pltpu.SemaphoreType.DMA((4,)),
        pltpu.SemaphoreType.DMA((12,)),
        pltpu.SemaphoreType.DMA((8,)),
        pltpu.SemaphoreType.DMA((4,)),
        pltpu.SemaphoreType.DMA((8,)),
    ] + [pltpu.VMEM((12, RING, 128), BF)] * 8
    return pl.pallas_call(
        _kernel,
        out_shape=jax.ShapeDtypeStruct((1, S, D), BF),
        in_specs=[any_spec] * 12,
        out_specs=any_spec,
        scratch_shapes=scratch,
        compiler_params=pltpu.CompilerParams(vmem_limit_bytes=120 * 1024 * 1024),
    )(A_x, A_mem0, A_Wq, A_Wk, A_Wv, A_Wo.reshape(H * DH, D), B_w_r.reshape(1, D), B_w_gate,
      B_w_up, B_w_down, c, w_mod)
```

```python
import functools

import jax
import jax.numpy as jnp
from jax import lax
import jax.experimental.pallas as pl
import jax.experimental.pallas.tpu as pltpu

BF = jnp.bfloat16
F32 = jnp.float32
U32 = jnp.uint32

S = 2048
D = 1024
H = 32
DH = 128
M = 8
SEG = 32
NSEG = S // SEG
FF = 3584
RIDE = 24
BULK = S - RIDE * NSEG
X0 = BULK + 32
RING = 576
PITCH = 520
X1 = 1024
UNROLL = 4
EPS = 1e-5
SIDE0, SIDE_LAT, SIDE_DUE, SIDE_END = 2, 6, 6, 96
NEG = -3.0e38
ORDER = ("q0 q1 q2 q3 q4 q5 q6 s0 s1 s2 s3 s4 s5 q7 p0 p1 p2 p3 p4 p5 s6 s7 w0 w1 w2 p6 p7 w3 "
         "w4 w5 w6 w7")
PERM = (0, 2, 4, 6, 1, 3, 5, 7)


def _rb(v):
    return v.astype(BF).astype(F32)


def _layernorm(xf):
    mu = jnp.mean(xf, axis=-1, keepdims=True)
    dv = xf - mu
    var = jnp.mean(dv * dv, axis=-1, keepdims=True)
    sd = _rb(jnp.sqrt(_rb(_rb(var) + EPS)))
    return _rb(_rb(xf - _rb(mu)) * (1.0 / sd))


def _f3(v):
    return v.astype(F32).reshape(v.shape[0] // 8, 8, D)


def _b2(v):
    return v.reshape(v.shape[0] * 8, D).astype(BF)


def _kernel(x_hbm, mem0_hbm, wq_hbm, wk_hbm, wv_hbm, wo_hbm, wr_hbm, wg_hbm, wu_hbm, wd_hbm,
            c_hbm, wmod_hbm, out_hbm,
            x_v, h_v, hp_v, att_v, ho_v, wqkv_v, wo_v, stage, wmod_v,
            wg_v, wu_v, wd_v, mem_v, c_v, wr_v, mod_v, r_v, sb_v, macc_v,
            sem_small, sem_x, sem_stage, sem_wmod, sem_wo, sem_ffn, sem_out, *rings):
    w_hbm = (wq_hbm, wk_hbm, wv_hbm)
    ring = rings

    def piece_copy(t, lo=0, n=D, sem=None):
        slot = t % 2
        return pltpu.make_async_copy(
            w_hbm[t // 4].at[pl.ds(lo, n), pl.ds((t % 4) * 8, 8), :],
            stage.at[slot, pl.ds(lo, n)], sem_stage.at[slot if sem is None else sem])

    def piece_wait(slot):
        pltpu.make_async_copy(stage.at[slot], stage.at[slot], sem_stage.at[slot]).wait()

    def wmod_copy(k):
        col = k * 512 if isinstance(k, int) else pl.multiple_of(k * 512, 512)
        return pltpu.make_async_copy(wmod_hbm.at[:, pl.ds(col, 512)], wmod_v.at[k],
                                     sem_wmod.at[k])

    def wo_copy(n):
        lo, rows = ((n // 2) * 512, 512) if n < 4 else (1024, 3072)
        return pltpu.make_async_copy(wo_hbm.at[pl.ds(lo, rows), pl.ds((n % 2) * 512, 512)],
                                     wo_v.at[n % 2, pl.ds(lo, rows)], sem_wo.at[n])

    x0_copy = pltpu.make_async_copy(x_hbm.at[0, pl.ds(0, X0), :], x_v.at[pl.ds(0, X0), :],
                                    sem_x.at[0])
    x1_copy = pltpu.make_async_copy(x_hbm.at[0, pl.ds(X0, X1 - X0), :],
                                    x_v.at[pl.ds(X0, X1 - X0), :], sem_x.at[1])
    x2_copy = pltpu.make_async_copy(x_hbm.at[0, pl.ds(X1, S - X1), :],
                                    x_v.at[pl.ds(X1, S - X1), :], sem_x.at[2])
    c_copy = pltpu.make_async_copy(c_hbm, c_v, sem_small.at[0])
    mem_copy = pltpu.make_async_copy(mem0_hbm.at[0], mem_v, sem_small.at[1])
    wr_copy = pltpu.make_async_copy(wr_hbm, wr_v, sem_small.at[2])
    wg_copy = pltpu.make_async_copy(wg_hbm, wg_v, sem_ffn.at[0])
    wu_copy = pltpu.make_async_copy(wu_hbm, wu_v, sem_ffn.at[1])
    wd_copies = [pltpu.make_async_copy(wd_hbm.at[:, pl.ds(k * 512, 512)], wd_v.at[k],
                                       sem_ffn.at[2 + k]) for k in range(2)]

    def relayout(slot, t, lo, n):
        base = t * (8 * PITCH) + lo // 2
        u = pltpu.bitcast(stage[slot, pl.ds(lo, n)], U32)
        tok = None
        for i in range(n // 2):
            a = u[2 * i]
            b = u[2 * i + 1]
            even = (a & jnp.uint32(0xFFFF)) | (b << 16)
            odd = (a >> 16) | (b & jnp.uint32(0xFFFF0000))
            wqkv_v[pl.ds(base + i, 4, stride=PITCH), :] = even
            wqkv_v[pl.ds(base + 4 * PITCH + i, 4, stride=PITCH), :] = odd
            tok = even ^ odd if tok is None else tok ^ even ^ odd
        return jnp.concatenate([tok, tok], axis=0)

    def relayout_loop(slot, t, lo, n):
        def body(i, carry):
            relayout(slot, t, pl.multiple_of(lo + i * 128, 128), 128)
            return carry
        lax.fori_loop(0, n // 128, body, 0)

    def modulate(ln, k_scale, k_shift):
        return _rb(ln * mod_v[k_scale]) + mod_v[k_shift]

    CW = 256

    def ln_stats(xf):
        mu = jnp.mean(xf, axis=-1, keepdims=True)
        dv = xf - mu
        var = jnp.mean(dv * dv, axis=-1, keepdims=True)
        sd = _rb(jnp.sqrt(_rb(_rb(var) + EPS)))
        return _rb(mu), 1.0 / sd

    def mod_c(k, c):
        return mod_v[k, :, pl.ds(c * CW, CW)]

    def token(v):
        return pltpu.bitcast(v[:, :128] + v[:, 128:], U32)

    def after(v, trig):
        if trig is None:
            return v
        return jnp.concatenate([jnp.where(trig[0], trig[1], v[:, :128]), v[:, 128:]], axis=1)

    def post_work(row0, att, scores_out=None):
        st = {}

        def head(trig):
            a = after(att().astype(F32), trig)
            st["x2"] = _rb(x_v[pl.ds(row0, 8), :].astype(F32) + _rb(mod_v[2] * a))
            st["mu"], st["inv"] = ln_stats(st["x2"])

        def chunk(c, trig):
            xc = after(st["x2"][:, c * CW:(c + 1) * CW], trig)
            h2b = (_rb(_rb(_rb(xc - st["mu"]) * st["inv"]) * mod_c(4, c))
                   + mod_c(3, c)).astype(BF)
            h2 = h2b.astype(F32)
            ho_v[0, pl.ds(row0, 8), pl.ds(c * CW, CW)] = h2b
            o = xc + mod_c(5, c) * h2
            ho_v[1, pl.ds(row0, 8), pl.ds(c * CW, CW)] = o.astype(BF)
            rp = h2 * mod_c(6, c)
            st["r"] = rp if c == 0 else st["r"] + rp
            if c == D // CW - 1:
                r = jnp.sum(st["r"], axis=-1, keepdims=True)
                if scores_out is not None:
                    scores_out.append(r)
                    return None
                grp = row0 // 8
                lanes = lax.broadcasted_iota(jnp.int32, (8, 128), 1)
                r_v[grp // 128] = jnp.where(lanes == grp % 128, r, r_v[grp // 128])
            return token(o + st["r"])
        return [head] + [functools.partial(chunk, c) for c in range(D // CW)]

    def ln1_work(row0):
        st = {}

        def head(trig):
            st["x"] = after(x_v[pl.ds(row0, 8), :].astype(F32), trig)
            st["mu"], st["inv"] = ln_stats(st["x"])

        def chunk(c, trig):
            xc = after(st["x"][:, c * CW:(c + 1) * CW], trig)
            h = _rb(_rb(_rb(xc - st["mu"]) * st["inv"]) * mod_c(1, c)) + mod_c(0, c)
            ho_v[0, pl.ds(row0, 8), pl.ds(c * CW, CW)] = h.astype(BF)
            return token(h)
        return [head] + [functools.partial(chunk, c) for c in range(D // CW)]

    x0_copy.start()
    c_copy.start()
    wmod_copy(0).start()
    mem_copy.start()
    wr_copy.start()

    r_v[...] = jnp.full(r_v.shape, NEG, F32)
    att_v[...] = jnp.zeros(att_v.shape, BF)

    c_copy.wait()
    cf = c_v[...].astype(F32)
    sil = (cf * jax.nn.sigmoid(cf)).astype(BF)
    sc = jnp.broadcast_to(sil, (16, D))
    for k in range(8):
        sb_v[pl.ds(128 * k, 128), :] = jnp.broadcast_to(
            sil[:, 128 * k:128 * k + 128].astype(F32), (128, 128)).T

    x0_copy.wait()
    wmod_copy(1).start()
    wmod_copy(2).start()

    LNB = X0 // 4

    def ln0(i, carry):
        r0 = pl.multiple_of(i * LNB, 8)
        h_v[pl.ds(r0, LNB), :] = _b2(_layernorm(_f3(x_v[pl.ds(r0, LNB), :])))
        return carry
    lax.fori_loop(0, 4, ln0, 0)

    wmod_copy(3).start()
    piece_copy(0, 0, 512, 0).start()

    def mod_slab(k):
        y = _rb(jnp.dot(sc, wmod_v[k], preferred_element_type=F32)[0:8])
        if k // 2 in (1, 4):
            y = _rb(1.0 + y)
        mod_v[k // 2, :, pl.ds((k % 2) * 512, 512)] = y

    for k in range(4):
        wmod_copy(k).wait()
        if k == 2:
            piece_copy(0, 512, 256, 2).start()
            piece_copy(0, 768, 256, 3).start()
        mod_slab(k)

    def mod0(i, carry):
        r0 = pl.multiple_of(i * 128, 128)
        hb = _b2(modulate(_f3(h_v[pl.ds(r0, 128), :]), 1, 0))
        hp_v[pl.ds(pl.multiple_of(i * 64, 64), 64), :] = pltpu.bitcast(hb, U32)
        return carry
    lax.fori_loop(0, BULK // 128, mod0, 0)
    ho_v[0, pl.ds(BULK, RIDE), :] = _b2(modulate(_f3(h_v[pl.ds(BULK, RIDE), :]), 1, 0))

    piece_copy(0, 0, 512, 0).wait()
    relayout_loop(0, 0, 0, 512)
    piece_copy(0, 512, 256, 2).wait()
    piece_copy(1).start()
    relayout_loop(0, 0, 512, 256)
    piece_copy(0, 768, 256, 3).wait()
    relayout_loop(0, 0, 768, 256)

    def mod_rows(slab, r0, n, acc):
        for r in range(r0, r0 + n, 8):
            sv = sb_v[pl.ds(r, 8), :]
            t = wmod_v[slab, pl.ds(r, 8), :].astype(F32) * jnp.concatenate([sv] * 4, axis=1)
            acc = t if acc is None else acc + t
        return acc

    def bulk_dot(i, k, never=None, rl=None, md=None):
        w = pltpu.bitcast(wqkv_v[pl.ds(pl.multiple_of((8 * i + k) * PITCH, 8), 512), :], BF)
        cols = [hp_v[:, pl.ds(128 * c, 128)] for c in range(8)]
        if rl is not None:
            slot, t, lo, n = rl
            g = n // 16
            spots = [(12 + (q * 48) // g) for q in range(g)]
            toks = {sp: relayout(slot, t, lo + 16 * q, 16) for q, sp in enumerate(spots)}
            if md is not None:
                for q, sp in enumerate(spots):
                    md[1] = mod_rows(md[0], 128 * k + 16 * q, 16, md[1])
                    toks[sp] = toks[sp] ^ token(md[1][:, :256] + md[1][:, 256:])
            for c in (0, 4):
                cols[c] = jnp.concatenate(
                    [jnp.where(never, toks[8 * c + j], cols[c][8 * j:8 * j + 8])
                     if 8 * c + j in toks else cols[c][8 * j:8 * j + 8]
                     for j in range(32)], axis=0)
        hb = pltpu.bitcast(jnp.concatenate(cols, axis=1), BF)
        y = jnp.dot(hb, w, preferred_element_type=F32)
        ring[k][i, pl.ds(RING - BULK, BULK), :] = y.astype(BF)

    never0 = r_v[0] > 0.0
    piece_copy(2).start()
    for k in range(8):
        if k == 6:
            piece_wait(1)
        bulk_dot(0, k, never0, (1, 1, (k - 6) * 512, 512) if k >= 6 else None)

    def bulk_qkv(i, carry):
        @pl.when(i < 11)
        def _():
            piece_wait((i + 1) % 2)

        @pl.when((i >= 2) & (i < 10))
        def _():
            wmod_copy(i + 2).wait()

        for j in range(1, 10):
            @pl.when(i == j)
            def _():
                piece_copy(j + 2).start()

        t = jnp.minimum(i + 1, 11)
        never = jnp.full((8, 128), i, jnp.int32) < 0
        md = [jnp.minimum(i + 2, 11), None]
        for k in range(8):
            bulk_dot(i, k, never, (t % 2, t, k * 128, 128), md)
        macc_v[md[0]] = md[1]

        for j in range(1, 10):
            @pl.when(i == j)
            def _():
                if j < 8:
                    wmod_copy(j + 4).start()
                if j == 8:
                    x1_copy.start()
                if j in (1, 3, 5, 7):
                    wo_copy(j // 2).start()
                if j == 9:
                    wo_copy(4).start()
                    wo_copy(5).start()
        return carry
    wmod_copy(4).start()
    lax.fori_loop(1, 12, bulk_qkv, 0)

    for k in range(4, 12):
        y = _rb(jnp.sum(macc_v[k], axis=0, keepdims=True))
        if k // 2 == 4:
            y = _rb(1.0 + y)
        mod_v[k // 2, :, pl.ds((k % 2) * 512, 512)] = jnp.broadcast_to(y, (8, 512))
    wr_copy.wait()
    mod_v[6] = jnp.broadcast_to(wr_v[...].astype(F32), (8, D))
    mem_copy.wait()
    for n in range(6):
        wo_copy(n).wait()
    x1_copy.wait()
    x2_copy.start()
    wg_copy.start()
    wu_copy.start()
    for cp in wd_copies:
        cp.start()

    scale = DH ** -0.5
    rr = lax.broadcasted_iota(jnp.int32, (80, 80), 0)
    cc = lax.broadcasted_iota(jnp.int32, (80, 80), 1)

    def second(i):
        return ((i >= 8) & (i < 16)) | (i >= 48)
    same = second(rr) == second(cc)
    allowed = same & ((rr < 16) | (cc <= rr))
    fill = jnp.where(same, -1e9, NEG).astype(F32)

    def tied(u, never, toks):
        if not toks:
            return u
        parts, at = [], 0
        for j, tk in enumerate(toks):
            r = 64 * j
            if r > at:
                parts.append(u[at:r])
            w = tk.shape[1]
            sel = jnp.where(never[:, :w], tk, u[r:r + 8, :w])
            parts.append(sel if w == 128 else jnp.concatenate([sel, u[r:r + 8, w:]], axis=1))
            at = r + 8
        return jnp.concatenate(parts + [u[at:]], axis=0)

    def w_slab(t, g, lo=0, n=512, never=None, toks=()):
        return pltpu.bitcast(
            tied(wqkv_v[pl.ds((8 * t + g) * PITCH + lo, n), :], never, toks), BF)

    def step(s, mem, chained, left, att_prev):
        odd = left is not None
        wr = pl.multiple_of(lax.rem(RIDE * s, RING), 8)
        rd = pl.multiple_of(lax.rem(SEG * s + RING - BULK, RING), SEG)
        xin = jnp.concatenate(
            [mem, ho_v[0, pl.ds(pl.multiple_of(BULK + RIDE * s, 8), RIDE), :]], axis=0)

        prow = SEG * (s - 1) if odd else jnp.maximum(SEG * s - 40, 0)
        nrow = BULK + RIDE * jnp.minimum(s + 1, NSEG - 1)
        works = [post_work(pl.multiple_of(prow + 8 * q, 8), functools.partial(att_prev, q))
                 for q in range(3 if odd else 5)]
        works += [ln1_work(pl.multiple_of(nrow + 8 * q, 8)) for q in range(RIDE // 8)]
        never = jnp.full((8, 128), s, jnp.int32) < 0
        gap = (SIDE_END - SIDE0 - SIDE_LAT - SIDE_DUE) // len(works)
        sched = {}
        for q, wk in enumerate(works):
            sched.setdefault(SIDE0 + gap * q, []).append(wk[0])
            for c in range(1, len(wk)):
                sched.setdefault(SIDE0 + SIDE_LAT + gap * q + ((c - 1) * gap) // 4,
                                 []).append(wk[c])

        memqkv, probs, wl, new_left, toks = {}, {}, {}, {}, {}
        acc = []

        ndot = [0]

        def proj(g, t_lo, t_hi):
            part = {}
            if chained and ndot[0] == 0:
                for t in range(t_lo, t_lo + 6):
                    part[t] = jnp.dot(xin[:, :512], w_slab(t, g, 0, 256),
                                      preferred_element_type=F32)
            for t0 in range(t_lo, t_hi, 2):
                ys = []
                for t in (t0, t0 + 1):
                    n = ndot[0]
                    ndot[0] += 1
                    if t in part:
                        y = jnp.dot(xin[:, 512:], w_slab(t, g, 256, 256),
                                    preferred_element_type=F32) + part[t]
                    else:
                        y = jnp.dot(xin, w_slab(t, g, 0, 512, never, toks.get(n)),
                                    preferred_element_type=F32)
                    ring[g][t, pl.ds(wr, RIDE), :] = y[M:].astype(BF)
                    ys.append(y[:M])
                    for item in sched.get(n, ()):
                        tk = item((never, y[:M]))
                        if tk is not None:
                            toks.setdefault(n + SIDE_DUE, []).append(tk)
                memqkv[(t0, g)] = jnp.concatenate(ys, axis=0).astype(BF)

        def cat(t0, g):
            return jnp.concatenate([memqkv[(t0, g)], ring[g][t0, pl.ds(rd, SEG), :],
                                    ring[g][t0 + 1, pl.ds(rd, SEG), :]], axis=0)

        def scores(g):
            for p in (0, 2):
                sc_ = lax.dot_general(cat(p, g), cat(4 + p, g), (((1,), (1,)), ((), ())),
                                      preferred_element_type=F32)
                sc_ = jnp.where(allowed, sc_ * scale, fill)
                e = jnp.exp(sc_ - jnp.max(sc_, axis=1, keepdims=True))
                l = jnp.sum(e, axis=1, keepdims=True)
                rc = pl.reciprocal(l, approx=True)
                rc = rc * (2.0 - l * rc)
                probs[(p, g)] = (e * rc).astype(BF)

        def pv(g):
            for p in (0, 2):
                o = jnp.dot(probs[(p, g)], cat(8 + p, g), preferred_element_type=F32)
                for j in range(2):
                    om, ot = o[8 * j:8 * j + 8], o[16 + 32 * j:48 + 32 * j]
                    if odd:
                        rows = [om, left[(p + j, g)], ot]
                    else:
                        rows = [om, ot[:RIDE]]
                        new_left[(p + j, g)] = ot[RIDE:]
                    wl[(p + j, g)] = jnp.concatenate(rows, axis=0).astype(BF)

        def wo(g):
            a = jnp.concatenate([wl[(o, g)] for o in range(4)], axis=1)
            w = jnp.concatenate(
                [jnp.concatenate([wo_v[n, pl.ds((8 * o + PERM[g]) * DH, DH), :]
                                  for o in range(4)], axis=0) for n in range(2)], axis=1)
            y = jnp.dot(a, w, preferred_element_type=F32)
            acc[:] = [y if not acc else y + acc[0]]

        for op in ORDER.split():
            g = int(op[1])
            if op[0] in "qkv":
                proj(g, *{"q": (0, 12), "k": (0, 8), "v": (8, 12)}[op[0]])
            else:
                {"s": scores, "p": pv, "w": wo}[op[0]](g)
        y = acc[0].astype(BF)
        return y[:M], y[M:], (None if odd else new_left)

    def out_copy(row0, n, k):
        return pltpu.make_async_copy(ho_v.at[1, pl.ds(row0, n), :],
                                     out_hbm.at[0, pl.ds(row0, n), :], sem_out.at[k])

    OB = SEG * UNROLL

    def carried(q):
        return att_v[pl.ds(8 * q, 8), :]

    def steps(i, carry):
        @pl.when(i == 16 // UNROLL)
        def _():
            x2_copy.wait()

        @pl.when(i >= 3)
        def _():
            out_copy(0, OB, 0).wait()

        @pl.when(i >= 2)
        def _():
            out_copy(pl.multiple_of((i - 2) * OB, OB), OB, 0).start()

        mem, left, att_prev = mem_v[...], None, carried
        for u in range(UNROLL):
            mem, att, left = step(i * UNROLL + u, mem, u > 0, left, att_prev)
            att_prev = (lambda a: lambda q: a[8 * q:8 * q + 8])(att)
        mem_v[...] = mem
        att_v[...] = att
        return carry
    lax.fori_loop(0, NSEG // UNROLL, steps, 0)

    wg_copy.wait()
    wu_copy.wait()
    for cp in wd_copies:
        cp.wait()
    out_copy(S - 2 * OB, OB, 1).start()
    last = []
    for q in range(5):
        for item in post_work(S - 40 + 8 * q, functools.partial(carried, q), last):
            item(None)
    out_copy(S - OB, OB, 2).start()

    def top2(val, idx, valid):
        def reduce(f, v):
            v = f(v, axis=0, keepdims=True)
            return v if v.shape[1] == 1 else f(v, axis=1, keepdims=True)

        def argtop(ok):
            v = jnp.where(ok, val, -jnp.inf)
            m = reduce(jnp.max, v)
            return m, reduce(jnp.min, jnp.where(ok & (v >= m), idx, float(S)))
        m1, i1 = argtop(valid)
        return (m1, i1), argtop(valid & (idx != i1))

    sub1 = lax.broadcasted_iota(jnp.int32, (16, 128), 0)
    lan1 = lax.broadcasted_iota(jnp.int32, (16, 128), 1)
    idx = (sub1 // 8) * 1024 + lan1 * 8 + sub1 % 8
    c_a, c_b = top2(_rb(r_v[...].reshape(16, 128)), idx.astype(F32), idx < S - 40)
    sub2 = lax.broadcasted_iota(jnp.int32, (48, 1), 0)
    val2 = jnp.concatenate([_rb(r) for r in last] + [jnp.where(sub2[:8] == 0, c_a[0], c_b[0])],
                           axis=0)
    idx2 = jnp.where(sub2 < 40, (sub2 + (S - 40)).astype(F32),
                     jnp.where(sub2 == 40, c_a[1], c_b[1]))
    (m_a, i_a), (m_b, i_b) = top2(val2, idx2, sub2 < 42)
    i_a = i_a.astype(jnp.int32)
    i_b = i_b.astype(jnp.int32)
    ia = jnp.clip(i_a[0, 0], 0, S - 1)
    ib = jnp.clip(i_b[0, 0], 0, S - 1)
    blk_a = pl.multiple_of((ia // 8) * 8, 8)
    blk_b = pl.multiple_of((ib // 8) * 8, 8)

    def two(ref):
        return jnp.concatenate([ref[pl.ds(blk_a, 8), :], ref[pl.ds(blk_b, 8), :]], axis=0)

    hs = two(ho_v.at[0])
    g = _rb(jnp.dot(hs, wg_v[...], preferred_element_type=F32))
    u = _rb(jnp.dot(hs, wu_v[...], preferred_element_type=F32))
    act = (_rb(g * jax.nn.sigmoid(g)) * u).astype(BF)
    y = jnp.concatenate(
        [jnp.dot(act, wd_v[k], preferred_element_type=F32) for k in range(2)], axis=1)
    sub = lax.broadcasted_iota(jnp.int32, (16, 1), 0)
    rows = jnp.where(sub < 8, blk_a + sub, blk_b + sub - 8)
    gate = jnp.where(rows == ia, jax.nn.sigmoid(m_a),
                     jnp.where(rows == ib, jax.nn.sigmoid(m_b), 0.0))
    upd = jnp.where((rows == ia) | (rows == ib), y * gate, 0.0).reshape(2, 8, D)
    fin = _b2(_f3(two(ho_v.at[1])) + mod_v[5] * upd)

    for k in range(3):
        out_copy(0, OB, k).wait()
    ho_v[1, pl.ds(blk_a, 8), :] = fin[0:8]
    ho_v[1, pl.ds(blk_b, 8), :] = fin[8:16]
    out_copy(blk_a, 8, 0).start()

    @pl.when(blk_a != blk_b)
    def _():
        out_copy(blk_b, 8, 1).start()
        out_copy(blk_b, 8, 1).wait()
    out_copy(blk_a, 8, 0).wait()


@jax.jit
def pallas_adaLN_cond__memory_aug_recurrent_mem_tr__moe_arch_mod__prompt_kernel(
    A_x, A_mem0, A_Wq, A_Wk, A_Wv, A_Wo, A_seg_len, B_x, B_w_r, B_w_gate, B_w_up, B_w_down, c,
    w_mod,
):
    del B_x
    del A_seg_len
    assert A_x.shape == (1, S, D) and A_Wq.shape == (D, H, DH) and A_mem0.shape == (1, M, D)
    any_spec = pl.BlockSpec(memory_space=pl.ANY)
    scratch = [
        pltpu.VMEM((S, D), BF),
        pltpu.VMEM((X0, D), BF),
        pltpu.VMEM((BULK // 2, D), U32),
        pltpu.VMEM((40, D), BF),
        pltpu.VMEM((2, S, D), BF),
        pltpu.VMEM((96 * PITCH, 128), U32),
        pltpu.VMEM((2, H * DH, 512), BF),
        pltpu.VMEM((2, D, 8, 128), BF),
        pltpu.VMEM((12, D, 512), BF),
        pltpu.VMEM((D, FF), BF),
        pltpu.VMEM((D, FF), BF),
        pltpu.VMEM((2, FF, 512), BF),
        pltpu.VMEM((M, D), BF),
        pltpu.VMEM((1, D), BF),
        pltpu.VMEM((1, D), BF),
        pltpu.VMEM((7, 8, D), F32),
        pltpu.VMEM((2, 8, 128), F32),
        pltpu.VMEM((D, 128), F32),
        pltpu.VMEM((12, 8, 512), F32),
        pltpu.SemaphoreType.DMA((3,)),
        pltpu.SemaphoreType.DMA((3,)),
        pltpu.SemaphoreType.DMA((4,)),
        pltpu.SemaphoreType.DMA((12,)),
        pltpu.SemaphoreType.DMA((8,)),
        pltpu.SemaphoreType.DMA((4,)),
        pltpu.SemaphoreType.DMA((8,)),
    ] + [pltpu.VMEM((12, RING, 128), BF)] * 8
    return pl.pallas_call(
        _kernel,
        out_shape=jax.ShapeDtypeStruct((1, S, D), BF),
        in_specs=[any_spec] * 12,
        out_specs=any_spec,
        scratch_shapes=scratch,
        compiler_params=pltpu.CompilerParams(vmem_limit_bytes=120 * 1024 * 1024),
    )(A_x, A_mem0, A_Wq, A_Wk, A_Wv, A_Wo.reshape(H * DH, D), B_w_r.reshape(1, D), B_w_gate,
      B_w_up, B_w_down, c, w_mod)
```

```python
import functools

import jax
import jax.numpy as jnp
from jax import lax
import jax.experimental.pallas as pl
import jax.experimental.pallas.tpu as pltpu

BF = jnp.bfloat16
F32 = jnp.float32
U32 = jnp.uint32

S = 2048
D = 1024
H = 32
DH = 128
M = 8
SEG = 32
NSEG = S // SEG
FF = 3584
RIDE = 24
BULK = S - RIDE * NSEG
X0 = BULK + 32
RING = 576
PITCH = 520
X1 = 1024
UNROLL = 4
EPS = 1e-5
SIDE0, SIDE_LAT, SIDE_DUE, SIDE_END = 2, 6, 6, 96
NEG = -3.0e38
ORDER = ("q0 q1 q2 q3 q4 q5 q6 s0 s1 s2 s3 s4 s5 q7 p0 p1 p2 p3 p4 p5 s6 s7 w0 w1 w2 p6 p7 w3 "
         "w4 w5 w6 w7")
PERM = (0, 2, 4, 6, 1, 3, 5, 7)


def _rb(v):
    return v.astype(BF).astype(F32)


def _layernorm(xf):
    mu = jnp.mean(xf, axis=-1, keepdims=True)
    dv = xf - mu
    var = jnp.mean(dv * dv, axis=-1, keepdims=True)
    sd = _rb(jnp.sqrt(_rb(_rb(var) + EPS)))
    return _rb(_rb(xf - _rb(mu)) * (1.0 / sd))


def _f3(v):
    return v.astype(F32).reshape(v.shape[0] // 8, 8, D)


def _b2(v):
    return v.reshape(v.shape[0] * 8, D).astype(BF)


def _kernel(x_hbm, mem0_hbm, wq_hbm, wk_hbm, wv_hbm, wo_hbm, wr_hbm, wg_hbm, wu_hbm, wd_hbm,
            c_hbm, wmod_hbm, out_hbm,
            x_v, h_v, hp_v, att_v, ho_v, wqkv_v, wo_v, stage, wmod_v,
            wg_v, wu_v, wd_v, mem_v, c_v, wr_v, mod_v, r_v, sb_v, macc_v,
            part_v, sems, *rings):
    w_hbm = (wq_hbm, wk_hbm, wv_hbm)
    ring = rings

    def piece_copy(t, sem, lo=0, n=D):
        return pltpu.make_async_copy(
            w_hbm[t // 4].at[pl.ds(lo, n), pl.ds((t % 4) * 8, 8), :],
            stage.at[t % 2, pl.ds(lo, n)], sems.at[sem])

    def stage_wait(slot, sem, lo=0, n=D):
        dst = stage.at[slot, pl.ds(lo, n)]
        pltpu.make_async_copy(dst, dst, sems.at[sem]).wait()

    def wmod_copy(k, sem):
        col = k * 512 if isinstance(k, int) else pl.multiple_of(k * 512, 512)
        return pltpu.make_async_copy(wmod_hbm.at[:, pl.ds(col, 512)], wmod_v.at[k], sems.at[sem])

    def x_copy(lo, hi, sem):
        return pltpu.make_async_copy(x_hbm.at[0, pl.ds(lo, hi - lo), :],
                                     x_v.at[pl.ds(lo, hi - lo), :], sems.at[sem])

    def wo_copy(n):
        lo, rows = ((n // 2) * 512, 512) if n < 6 else (1536, 2560)
        return pltpu.make_async_copy(wo_hbm.at[pl.ds(lo, rows), pl.ds((n % 2) * 512, 512)],
                                     wo_v.at[n % 2, pl.ds(lo, rows)], sems.at[0])

    small_copies = [pltpu.make_async_copy(c_hbm, c_v, sems.at[0]),
                    pltpu.make_async_copy(mem0_hbm.at[0], mem_v, sems.at[0]),
                    pltpu.make_async_copy(wr_hbm, wr_v, sems.at[0])]
    x0_copy = x_copy(0, X0, 1)
    mid_copies = ([x_copy(X0, (X0 + X1) // 2, 0), x_copy((X0 + X1) // 2, X1, 0)]
                  + [wo_copy(n) for n in range(8)])
    x2_copy = x_copy(X1, S, 1)
    ffn_copies = [pltpu.make_async_copy(wg_hbm, wg_v, sems.at[2]),
                  pltpu.make_async_copy(wu_hbm, wu_v, sems.at[2])] + [
        pltpu.make_async_copy(wd_hbm.at[:, pl.ds(k * 512, 512)], wd_v.at[k], sems.at[2])
        for k in range(2)]

    def relayout(slot, t, lo, n):
        base = t * (8 * PITCH) + lo // 2
        u = pltpu.bitcast(stage[slot, pl.ds(lo, n)], U32)
        tok = None
        for i in range(n // 2):
            a = u[2 * i]
            b = u[2 * i + 1]
            even = (a & jnp.uint32(0xFFFF)) | (b << 16)
            odd = (a >> 16) | (b & jnp.uint32(0xFFFF0000))
            wqkv_v[pl.ds(base + i, 4, stride=PITCH), :] = even
            wqkv_v[pl.ds(base + 4 * PITCH + i, 4, stride=PITCH), :] = odd
            tok = even ^ odd if tok is None else tok ^ even ^ odd
        return jnp.concatenate([tok, tok], axis=0)

    def relayout_loop(slot, t, lo, n):
        def body(i, carry):
            relayout(slot, t, pl.multiple_of(lo + i * 128, 128), 128)
            return carry
        lax.fori_loop(0, n // 128, body, 0)

    CW = 256

    def ln_stats(xf):
        mu = jnp.mean(xf, axis=-1, keepdims=True)
        dv = xf - mu
        var = jnp.mean(dv * dv, axis=-1, keepdims=True)
        sd = _rb(jnp.sqrt(_rb(_rb(var) + EPS)))
        return _rb(mu), 1.0 / sd

    def mod_c(k, c):
        return mod_v[k, :, pl.ds(c * CW, CW)]

    def token(v):
        return pltpu.bitcast(v[:, :128] + v[:, 128:], U32)

    def after(v, trig):
        if trig is None:
            return v
        return jnp.concatenate([jnp.where(trig[0], trig[1], v[:, :128]), v[:, 128:]], axis=1)

    def post_work(row0, att, scores_out=None):
        st = {}

        def head(trig):
            a = after(att().astype(F32), trig)
            st["x2"] = _rb(x_v[pl.ds(row0, 8), :].astype(F32) + _rb(mod_v[2] * a))
            st["mu"], st["inv"] = ln_stats(st["x2"])

        def chunk(c, trig):
            xc = after(st["x2"][:, c * CW:(c + 1) * CW], trig)
            h2b = (_rb(_rb(_rb(xc - st["mu"]) * st["inv"]) * mod_c(4, c))
                   + mod_c(3, c)).astype(BF)
            h2 = h2b.astype(F32)
            ho_v[0, pl.ds(row0, 8), pl.ds(c * CW, CW)] = h2b
            o = xc + mod_c(5, c) * h2
            ho_v[1, pl.ds(row0, 8), pl.ds(c * CW, CW)] = o.astype(BF)
            rp = h2 * mod_c(6, c)
            st["r"] = rp if c == 0 else st["r"] + rp
            if c == D // CW - 1:
                r = jnp.sum(st["r"], axis=-1, keepdims=True)
                if scores_out is not None:
                    scores_out.append(r)
                    return None
                grp = row0 // 8
                lanes = lax.broadcasted_iota(jnp.int32, (8, 128), 1)
                r_v[grp // 128] = jnp.where(lanes == grp % 128, r, r_v[grp // 128])
            return token(o + st["r"])
        return [head] + [functools.partial(chunk, c) for c in range(D // CW)]

    def ln1_work(row0):
        st = {}

        def head(trig):
            st["x"] = after(x_v[pl.ds(row0, 8), :].astype(F32), trig)
            st["mu"], st["inv"] = ln_stats(st["x"])

        def chunk(c, trig):
            xc = after(st["x"][:, c * CW:(c + 1) * CW], trig)
            h = _rb(_rb(_rb(xc - st["mu"]) * st["inv"]) * mod_c(1, c)) + mod_c(0, c)
            ho_v[0, pl.ds(row0, 8), pl.ds(c * CW, CW)] = h.astype(BF)
            return token(h)
        return [head] + [functools.partial(chunk, c) for c in range(D // CW)]

    x0_copy.start()
    for cp in small_copies:
        cp.start()
    wmod_copy(0, 2).start()

    r_v[...] = jnp.full(r_v.shape, NEG, F32)
    att_v[...] = jnp.zeros(att_v.shape, BF)

    for cp in small_copies:
        cp.wait()
    mod_v[6] = jnp.broadcast_to(wr_v[...].astype(F32), (8, D))
    cf = c_v[...].astype(F32)
    sil = (cf * jax.nn.sigmoid(cf)).astype(BF)
    sc = jnp.broadcast_to(sil, (16, D))
    for k in range(8):
        sb_v[pl.ds(128 * k, 128), :] = jnp.broadcast_to(
            sil[:, 128 * k:128 * k + 128].astype(F32), (128, 128)).T

    x0_copy.wait()
    wmod_copy(2, 3).start()

    LNB = X0 // 4

    def ln0(i, carry):
        r0 = pl.multiple_of(i * LNB, 8)
        h_v[pl.ds(r0, LNB), :] = _b2(_layernorm(_f3(x_v[pl.ds(r0, LNB), :])))
        return carry
    lax.fori_loop(0, 4, ln0, 0)

    piece_copy(0, 0, 0, 256).start()
    piece_copy(0, 1, 256, 256).start()

    def mod_slab(k):
        y = _rb(jnp.dot(sc, wmod_v[k], preferred_element_type=F32)[0:8])
        if k // 2 == 1:
            y = _rb(1.0 + y)
        mod_v[k // 2, :, pl.ds((k % 2) * 512, 512)] = y

    def modulate_half(half):
        cols = pl.ds(half * 512, 512)

        def f(r0, n):
            ln = h_v[pl.ds(r0, n), cols].astype(F32).reshape(n // 8, 8, 512)
            h = _rb(ln * mod_v[1, :, cols]) + mod_v[0, :, cols]
            return h.reshape(n, 512).astype(BF)

        def mod0(i, carry):
            hp_v[pl.ds(pl.multiple_of(i * 128, 128), 128), cols] = pltpu.bitcast(
                f(pl.multiple_of(i * 256, 256), 256), U32)
            return carry
        lax.fori_loop(0, BULK // 256, mod0, 0)
        ho_v[0, pl.ds(BULK, RIDE), cols] = f(BULK, RIDE)

    wmod_copy(0, 2).wait()
    mod_slab(0)
    wmod_copy(2, 3).wait()
    mod_slab(2)
    modulate_half(0)
    piece_copy(0, 0, 0, 256).wait()
    piece_copy(1, 4, 0, 512).start()
    relayout_loop(0, 0, 0, 256)
    wmod_copy(1, 2).start()
    piece_copy(0, 1, 256, 256).wait()
    relayout_loop(0, 0, 256, 256)

    def mod_rows(slab, r0, n, acc):
        for r in range(r0, r0 + n, 8):
            sv = sb_v[pl.ds(r, 8), :]
            t = wmod_v[slab, pl.ds(r, 8), :].astype(F32) * jnp.concatenate([sv] * 4, axis=1)
            acc = t if acc is None else acc + t
        return acc

    def bulk_dot(i, k, never, rl=None, md=None, half=None):
        tiles = range(8) if half is None else range(4 * half, 4 * half + 4)
        w = pltpu.bitcast(
            wqkv_v[pl.ds(pl.multiple_of((8 * i + k) * PITCH + 64 * tiles[0], 8),
                         64 * len(tiles)), :], BF)
        cols = [hp_v[:, pl.ds(128 * c, 128)] for c in tiles]
        if rl is not None:
            slot, t, lo = rl
            spots = [12 + 6 * q if half is None else 4 + 3 * q for q in range(8)]
            toks = {sp: relayout(slot, t, lo + 16 * q, 16) for q, sp in enumerate(spots)}
            if md is not None:
                for q, sp in enumerate(spots):
                    md[1] = mod_rows(md[0], 128 * k + 16 * q, 16, md[1])
                    toks[sp] = toks[sp] ^ token(md[1][:, :256] + md[1][:, 256:])
            for c in range(0, len(tiles), 4):
                cols[c] = jnp.concatenate(
                    [jnp.where(never, toks[8 * c + j], cols[c][8 * j:8 * j + 8])
                     if 8 * c + j in toks else cols[c][8 * j:8 * j + 8]
                     for j in range(32)], axis=0)
        hb = pltpu.bitcast(jnp.concatenate(cols, axis=1), BF)
        y = jnp.dot(hb, w, preferred_element_type=F32)
        if half == 0:
            part_v[i, k] = y
            return
        if half == 1:
            y = y + part_v[i, k]
        ring[k][i, pl.ds(RING - BULK, BULK), :] = y.astype(BF)

    def bulk_a(a, carry):
        never = jnp.full((8, 128), a, jnp.int32) < 0
        for k in range(4):
            bulk_dot(a, k, never, half=0)

        @pl.when(a == 0)
        def _():
            piece_copy(0, 5, 512, 512).start()

        @pl.when(a == 1)
        def _():
            piece_copy(1, 4, 512, 512).start()
        lo = pl.multiple_of(512 * a, 512)
        stage_wait(1 - a, 4 + a, lo, 512)
        for k in range(4, 8):
            bulk_dot(a, k, never, (1 - a, 1 - a, lo + 128 * (k - 4)), half=0)

        @pl.when(a == 0)
        def _():
            wmod_copy(3, 3).start()
        return carry
    lax.fori_loop(0, 2, bulk_a, 0)

    piece_copy(2, 0, 0, 512).start()
    wmod_copy(1, 2).wait()
    wmod_copy(3, 3).wait()
    mod_slab(1)
    mod_slab(3)
    modulate_half(1)

    def bulk_b(b, carry):
        never = jnp.full((8, 128), b, jnp.int32) < 0

        @pl.when(b == 1)
        def _():
            piece_copy(2, 0, 0, 512).wait()
        for k in range(4):
            bulk_dot(b, k, never, (1 - b, 1 + b, 128 * k), half=1)

        @pl.when(b == 0)
        def _():
            piece_copy(2, 1, 512, 512).start()
        stage_wait(1 - b, 4 - 3 * b, 512, 512)
        for k in range(4, 8):
            bulk_dot(b, k, never, (1 - b, 1 + b, 128 * k), half=1)

        @pl.when(b == 0)
        def _():
            piece_copy(3, 5).start()
        return carry
    lax.fori_loop(0, 2, bulk_b, 0)

    def bulk_qkv(i, carry):
        @pl.when(i < 11)
        def _():
            stage_wait((i + 1) % 2, 4 + (i + 1) % 2)

        @pl.when((i >= 3) & (i < 11))
        def _():
            wmod_copy(i + 1, 2 + (i + 1) % 2).wait()

        for j in range(2, 10):
            @pl.when(i == j)
            def _():
                piece_copy(j + 2, 4 + j % 2).start()

        t = jnp.minimum(i + 1, 11)
        never = jnp.full((8, 128), i, jnp.int32) < 0
        md = [t, None]
        for k in range(8):
            bulk_dot(i, k, never, (t % 2, t, k * 128), md)
        macc_v[t] = md[1]

        for j in range(2, 10):
            @pl.when(i == j)
            def _():
                if j < 9:
                    wmod_copy(j + 3, 2 + (j + 3) % 2).start()
                    mid_copies[j - 2].start()
                else:
                    for cp in mid_copies[7:]:
                        cp.start()
        return carry
    wmod_copy(4, 2).start()
    lax.fori_loop(2, 12, bulk_qkv, 0)

    for k in range(4, 12):
        y = _rb(jnp.sum(macc_v[k], axis=0, keepdims=True))
        if k // 2 == 4:
            y = _rb(1.0 + y)
        mod_v[k // 2, :, pl.ds((k % 2) * 512, 512)] = jnp.broadcast_to(y, (8, 512))
    for cp in mid_copies:
        cp.wait()
    x2_copy.start()
    for cp in ffn_copies:
        cp.start()

    scale = DH ** -0.5
    rr = lax.broadcasted_iota(jnp.int32, (80, 80), 0)
    cc = lax.broadcasted_iota(jnp.int32, (80, 80), 1)

    def second(i):
        return ((i >= 8) & (i < 16)) | (i >= 48)
    same = second(rr) == second(cc)
    allowed = same & ((rr < 16) | (cc <= rr))
    fill = jnp.where(same, -1e9, NEG).astype(F32)

    def tied(u, never, toks):
        if not toks:
            return u
        parts, at = [], 0
        for j, tk in enumerate(toks):
            r = 64 * j
            if r > at:
                parts.append(u[at:r])
            w = tk.shape[1]
            sel = jnp.where(never[:, :w], tk, u[r:r + 8, :w])
            parts.append(sel if w == 128 else jnp.concatenate([sel, u[r:r + 8, w:]], axis=1))
            at = r + 8
        return jnp.concatenate(parts + [u[at:]], axis=0)

    def w_slab(t, g, lo=0, n=512, never=None, toks=()):
        return pltpu.bitcast(
            tied(wqkv_v[pl.ds((8 * t + g) * PITCH + lo, n), :], never, toks), BF)

    def step(s, mem, chained, left, att_prev):
        odd = left is not None
        wr = pl.multiple_of(lax.rem(RIDE * s, RING), 8)
        rd = pl.multiple_of(lax.rem(SEG * s + RING - BULK, RING), SEG)
        xin = jnp.concatenate(
            [mem, ho_v[0, pl.ds(pl.multiple_of(BULK + RIDE * s, 8), RIDE), :]], axis=0)

        prow = SEG * (s - 1) if odd else jnp.maximum(SEG * s - 40, 0)
        nrow = BULK + RIDE * jnp.minimum(s + 1, NSEG - 1)
        works = [post_work(pl.multiple_of(prow + 8 * q, 8), functools.partial(att_prev, q))
                 for q in range(3 if odd else 5)]
        works += [ln1_work(pl.multiple_of(nrow + 8 * q, 8)) for q in range(RIDE // 8)]
        never = jnp.full((8, 128), s, jnp.int32) < 0
        gap = (SIDE_END - SIDE0 - SIDE_LAT - SIDE_DUE) // len(works)
        sched = {}
        for q, wk in enumerate(works):
            sched.setdefault(SIDE0 + gap * q, []).append(wk[0])
            for c in range(1, len(wk)):
                sched.setdefault(SIDE0 + SIDE_LAT + gap * q + ((c - 1) * gap) // 4,
                                 []).append(wk[c])

        memqkv, probs, wl, new_left, toks = {}, {}, {}, {}, {}
        acc = []

        ndot = [0]

        def proj(g, t_lo, t_hi):
            part = {}
            if chained and ndot[0] == 0:
                for t in range(t_lo, t_lo + 6):
                    part[t] = jnp.dot(xin[:, :512], w_slab(t, g, 0, 256),
                                      preferred_element_type=F32)
            for t0 in range(t_lo, t_hi, 2):
                ys = []
                for t in (t0, t0 + 1):
                    n = ndot[0]
                    ndot[0] += 1
                    if t in part:
                        y = jnp.dot(xin[:, 512:], w_slab(t, g, 256, 256),
                                    preferred_element_type=F32) + part[t]
                    else:
                        y = jnp.dot(xin, w_slab(t, g, 0, 512, never, toks.get(n)),
                                    preferred_element_type=F32)
                    ring[g][t, pl.ds(wr, RIDE), :] = y[M:].astype(BF)
                    ys.append(y[:M])
                    for item in sched.get(n, ()):
                        tk = item((never, y[:M]))
                        if tk is not None:
                            toks.setdefault(n + SIDE_DUE, []).append(tk)
                memqkv[(t0, g)] = jnp.concatenate(ys, axis=0).astype(BF)

        def cat(t0, g):
            return jnp.concatenate([memqkv[(t0, g)], ring[g][t0, pl.ds(rd, SEG), :],
                                    ring[g][t0 + 1, pl.ds(rd, SEG), :]], axis=0)

        def scores(g):
            for p in (0, 2):
                sc_ = lax.dot_general(cat(p, g), cat(4 + p, g), (((1,), (1,)), ((), ())),
                                      preferred_element_type=F32)
                sc_ = jnp.where(allowed, sc_ * scale, fill)
                e = jnp.exp(sc_ - jnp.max(sc_, axis=1, keepdims=True))
                l = jnp.sum(e, axis=1, keepdims=True)
                rc = pl.reciprocal(l, approx=True)
                rc = rc * (2.0 - l * rc)
                probs[(p, g)] = (e * rc).astype(BF)

        def pv(g):
            for p in (0, 2):
                o = jnp.dot(probs[(p, g)], cat(8 + p, g), preferred_element_type=F32)
                for j in range(2):
                    om, ot = o[8 * j:8 * j + 8], o[16 + 32 * j:48 + 32 * j]
                    if odd:
                        rows = [om, left[(p + j, g)], ot]
                    else:
                        rows = [om, ot[:RIDE]]
                        new_left[(p + j, g)] = ot[RIDE:]
                    wl[(p + j, g)] = jnp.concatenate(rows, axis=0).astype(BF)

        def wo(g):
            a = jnp.concatenate([wl[(o, g)] for o in range(4)], axis=1)
            w = jnp.concatenate(
                [jnp.concatenate([wo_v[n, pl.ds((8 * o + PERM[g]) * DH, DH), :]
                                  for o in range(4)], axis=0) for n in range(2)], axis=1)
            y = jnp.dot(a, w, preferred_element_type=F32)
            acc[:] = [y if not acc else y + acc[0]]

        for op in ORDER.split():
            g = int(op[1])
            if op[0] in "qkv":
                proj(g, *{"q": (0, 12), "k": (0, 8), "v": (8, 12)}[op[0]])
            else:
                {"s": scores, "p": pv, "w": wo}[op[0]](g)
        y = acc[0].astype(BF)
        return y[:M], y[M:], (None if odd else new_left)

    def out_copy(row0, n, k):
        return pltpu.make_async_copy(ho_v.at[1, pl.ds(row0, n), :],
                                     out_hbm.at[0, pl.ds(row0, n), :], sems.at[3 + k])

    OB = SEG * UNROLL

    def carried(q):
        return att_v[pl.ds(8 * q, 8), :]

    def steps(i, carry):
        @pl.when(i == 16 // UNROLL)
        def _():
            x2_copy.wait()

        @pl.when(i >= 3)
        def _():
            out_copy(pl.multiple_of((i - 3) * OB, OB), OB, 0).wait()

        @pl.when(i >= 2)
        def _():
            out_copy(pl.multiple_of((i - 2) * OB, OB), OB, 0).start()

        mem, left, att_prev = mem_v[...], None, carried
        for u in range(UNROLL):
            mem, att, left = step(i * UNROLL + u, mem, u > 0, left, att_prev)
            att_prev = (lambda a: lambda q: a[8 * q:8 * q + 8])(att)
        mem_v[...] = mem
        att_v[...] = att
        return carry
    lax.fori_loop(0, NSEG // UNROLL, steps, 0)

    for cp in ffn_copies:
        cp.wait()
    out_copy(S - 2 * OB, OB, 1).start()
    last = []
    for q in range(5):
        for item in post_work(S - 40 + 8 * q, functools.partial(carried, q), last):
            item(None)
    out_copy(S - OB, OB, 2).start()

    def top2(val, idx, valid):
        def reduce(f, v):
            v = f(v, axis=0, keepdims=True)
            return v if v.shape[1] == 1 else f(v, axis=1, keepdims=True)

        def argtop(ok):
            v = jnp.where(ok, val, -jnp.inf)
            m = reduce(jnp.max, v)
            return m, reduce(jnp.min, jnp.where(ok & (v >= m), idx, float(S)))
        m1, i1 = argtop(valid)
        return (m1, i1), argtop(valid & (idx != i1))

    sub1 = lax.broadcasted_iota(jnp.int32, (16, 128), 0)
    lan1 = lax.broadcasted_iota(jnp.int32, (16, 128), 1)
    idx = (sub1 // 8) * 1024 + lan1 * 8 + sub1 % 8
    c_a, c_b = top2(_rb(r_v[...].reshape(16, 128)), idx.astype(F32), idx < S - 40)
    sub2 = lax.broadcasted_iota(jnp.int32, (48, 1), 0)
    val2 = jnp.concatenate([_rb(r) for r in last] + [jnp.where(sub2[:8] == 0, c_a[0], c_b[0])],
                           axis=0)
    idx2 = jnp.where(sub2 < 40, (sub2 + (S - 40)).astype(F32),
                     jnp.where(sub2 == 40, c_a[1], c_b[1]))
    (m_a, i_a), (m_b, i_b) = top2(val2, idx2, sub2 < 42)
    i_a = i_a.astype(jnp.int32)
    i_b = i_b.astype(jnp.int32)
    ia = jnp.clip(i_a[0, 0], 0, S - 1)
    ib = jnp.clip(i_b[0, 0], 0, S - 1)
    blk_a = pl.multiple_of((ia // 8) * 8, 8)
    blk_b = pl.multiple_of((ib // 8) * 8, 8)

    def two(ref):
        return jnp.concatenate([ref[pl.ds(blk_a, 8), :], ref[pl.ds(blk_b, 8), :]], axis=0)

    hs = two(ho_v.at[0])
    g = _rb(jnp.dot(hs, wg_v[...], preferred_element_type=F32))
    u = _rb(jnp.dot(hs, wu_v[...], preferred_element_type=F32))
    act = (_rb(g * jax.nn.sigmoid(g)) * u).astype(BF)
    y = jnp.concatenate(
        [jnp.dot(act, wd_v[k], preferred_element_type=F32) for k in range(2)], axis=1)
    sub = lax.broadcasted_iota(jnp.int32, (16, 1), 0)
    rows = jnp.where(sub < 8, blk_a + sub, blk_b + sub - 8)
    gate = jnp.where(rows == ia, jax.nn.sigmoid(m_a),
                     jnp.where(rows == ib, jax.nn.sigmoid(m_b), 0.0))
    upd = jnp.where((rows == ia) | (rows == ib), y * gate, 0.0).reshape(2, 8, D)
    fin = _b2(_f3(two(ho_v.at[1])) + mod_v[5] * upd)

    for k in range(3):
        out_copy(S - (3 - k) * OB, OB, k).wait()
    ho_v[1, pl.ds(blk_a, 8), :] = fin[0:8]
    ho_v[1, pl.ds(blk_b, 8), :] = fin[8:16]
    out_copy(blk_a, 8, 0).start()

    @pl.when(blk_a != blk_b)
    def _():
        out_copy(blk_b, 8, 1).start()
        out_copy(blk_b, 8, 1).wait()
    out_copy(blk_a, 8, 0).wait()


@jax.jit
def pallas_adaLN_cond__memory_aug_recurrent_mem_tr__moe_arch_mod__prompt_kernel(
    A_x, A_mem0, A_Wq, A_Wk, A_Wv, A_Wo, A_seg_len, B_x, B_w_r, B_w_gate, B_w_up, B_w_down, c,
    w_mod,
):
    del B_x
    del A_seg_len
    assert A_x.shape == (1, S, D) and A_Wq.shape == (D, H, DH) and A_mem0.shape == (1, M, D)
    any_spec = pl.BlockSpec(memory_space=pl.ANY)
    scratch = [
        pltpu.VMEM((S, D), BF),
        pltpu.VMEM((X0, D), BF),
        pltpu.VMEM((BULK // 2, D), U32),
        pltpu.VMEM((40, D), BF),
        pltpu.VMEM((2, S, D), BF),
        pltpu.VMEM((96 * PITCH, 128), U32),
        pltpu.VMEM((2, H * DH, 512), BF),
        pltpu.VMEM((2, D, 8, 128), BF),
        pltpu.VMEM((12, D, 512), BF),
        pltpu.VMEM((D, FF), BF),
        pltpu.VMEM((D, FF), BF),
        pltpu.VMEM((2, FF, 512), BF),
        pltpu.VMEM((M, D), BF),
        pltpu.VMEM((1, D), BF),
        pltpu.VMEM((1, D), BF),
        pltpu.VMEM((7, 8, D), F32),
        pltpu.VMEM((2, 8, 128), F32),
        pltpu.VMEM((D, 128), F32),
        pltpu.VMEM((12, 8, 512), F32),
        pltpu.VMEM((2, 8, BULK, 128), F32),
        pltpu.SemaphoreType.DMA((6,)),
    ] + [pltpu.VMEM((12, RING, 128), BF)] * 8
    return pl.pallas_call(
        _kernel,
        out_shape=jax.ShapeDtypeStruct((1, S, D), BF),
        in_specs=[any_spec] * 12,
        out_specs=any_spec,
        scratch_shapes=scratch,
        compiler_params=pltpu.CompilerParams(vmem_limit_bytes=120 * 1024 * 1024),
    )(A_x, A_mem0, A_Wq, A_Wk, A_Wv, A_Wo.reshape(H * DH, D), B_w_r.reshape(1, D), B_w_gate,
      B_w_up, B_w_down, c, w_mod)
```

```python
import functools

import jax
import jax.numpy as jnp
from jax import lax
import jax.experimental.pallas as pl
import jax.experimental.pallas.tpu as pltpu

BF = jnp.bfloat16
F32 = jnp.float32
U32 = jnp.uint32

S = 2048
D = 1024
H = 32
DH = 128
M = 8
SEG = 32
NSEG = S // SEG
FF = 3584
RIDE = 24
BULK = S - RIDE * NSEG
X0 = BULK + 32
RING = 576
PITCH = 520
X1 = 1024
UNROLL = 4
EPS = 1e-5
SIDE0, SIDE_LAT, SIDE_DUE, SIDE_END = 2, 6, 6, 96
NEG = -3.0e38
ORDER = ("q0 q1 q2 q3 q4 q5 q6 s0 s1 s2 s3 s4 s5 q7 p0 p1 p2 p3 p4 p5 s6 s7 w0 w1 w2 p6 p7 w3 "
         "w4 w5 w6 w7")
PERM = (0, 2, 4, 6, 1, 3, 5, 7)


def _rb(v):
    return v.astype(BF).astype(F32)


def _layernorm(xf):
    mu = jnp.mean(xf, axis=-1, keepdims=True)
    dv = xf - mu
    var = jnp.mean(dv * dv, axis=-1, keepdims=True)
    sd = _rb(jnp.sqrt(_rb(_rb(var) + EPS)))
    return _rb(_rb(xf - _rb(mu)) * (1.0 / sd))


def _f3(v):
    return v.astype(F32).reshape(v.shape[0] // 8, 8, D)


def _b2(v):
    return v.reshape(v.shape[0] * 8, D).astype(BF)


def _kernel(x_hbm, mem0_hbm, wq_hbm, wk_hbm, wv_hbm, wo_hbm, wr_hbm, wg_hbm, wu_hbm, wd_hbm,
            c_hbm, wmod_hbm, out_hbm,
            x_v, h_v, hp_v, att_v, ho_v, wqkv_v, wo_v, stage, wmod_v,
            wg_v, wu_v, wd_v, mem_v, c_v, wr_v, mod_v, r_v, sb_v, macc_v,
            part_v, sems, *rings):
    w_hbm = (wq_hbm, wk_hbm, wv_hbm)
    ring = rings

    def piece_copy(t, sem, lo=0, n=D):
        return pltpu.make_async_copy(
            w_hbm[t // 4].at[pl.ds(lo, n), pl.ds((t % 4) * 8, 8), :],
            stage.at[t % 2, pl.ds(lo, n)], sems.at[sem])

    def stage_wait(slot, sem, lo=0, n=D):
        dst = stage.at[slot, pl.ds(lo, n)]
        pltpu.make_async_copy(dst, dst, sems.at[sem]).wait()

    def wmod_copy(k, sem):
        col = k * 512 if isinstance(k, int) else pl.multiple_of(k * 512, 512)
        return pltpu.make_async_copy(wmod_hbm.at[:, pl.ds(col, 512)], wmod_v.at[k], sems.at[sem])

    def x_copy(lo, hi, sem):
        return pltpu.make_async_copy(x_hbm.at[0, pl.ds(lo, hi - lo), :],
                                     x_v.at[pl.ds(lo, hi - lo), :], sems.at[sem])

    def wo_copy(n):
        lo, rows = ((n // 2) * 512, 512) if n < 6 else (1536, 2560)
        return pltpu.make_async_copy(wo_hbm.at[pl.ds(lo, rows), pl.ds((n % 2) * 512, 512)],
                                     wo_v.at[n % 2, pl.ds(lo, rows)], sems.at[0])

    small_copies = [pltpu.make_async_copy(c_hbm, c_v, sems.at[0]),
                    pltpu.make_async_copy(mem0_hbm.at[0], mem_v, sems.at[0]),
                    pltpu.make_async_copy(wr_hbm, wr_v, sems.at[0])]
    x0_copy = x_copy(0, X0, 1)
    mid_copies = ([x_copy(X0, (X0 + X1) // 2, 0), x_copy((X0 + X1) // 2, X1, 0)]
                  + [wo_copy(n) for n in range(8)])
    x2_copy = x_copy(X1, S, 1)
    ffn_copies = [pltpu.make_async_copy(wg_hbm, wg_v, sems.at[2]),
                  pltpu.make_async_copy(wu_hbm, wu_v, sems.at[2])] + [
        pltpu.make_async_copy(wd_hbm.at[:, pl.ds(k * 512, 512)], wd_v.at[k], sems.at[2])
        for k in range(2)]

    def relayout(slot, t, lo2, n):
        base = t * (8 * PITCH) + lo2
        u = pltpu.bitcast(stage[slot, pl.ds(2 * lo2, n)], U32)
        tok = None
        for i in range(n // 2):
            a = u[2 * i]
            b = u[2 * i + 1]
            even = (a & jnp.uint32(0xFFFF)) | (b << 16)
            odd = (a >> 16) | (b & jnp.uint32(0xFFFF0000))
            wqkv_v[pl.ds(base + i, 4, stride=PITCH), :] = even
            wqkv_v[pl.ds(base + 4 * PITCH + i, 4, stride=PITCH), :] = odd
            tok = even ^ odd if tok is None else tok ^ even ^ odd
        return jnp.concatenate([tok, tok], axis=0)

    def relayout_loop(slot, t, lo, n):
        def body(i, carry):
            relayout(slot, t, lo // 2 + i * 64, 128)
            return carry
        lax.fori_loop(0, n // 128, body, 0)

    CW = 256

    def ln_stats(xf):
        mu = jnp.mean(xf, axis=-1, keepdims=True)
        dv = xf - mu
        var = jnp.mean(dv * dv, axis=-1, keepdims=True)
        sd = _rb(jnp.sqrt(_rb(_rb(var) + EPS)))
        return _rb(mu), 1.0 / sd

    def mod_c(k, c):
        return mod_v[k, :, pl.ds(c * CW, CW)]

    def token(v):
        return pltpu.bitcast(v[:, :128] + v[:, 128:], U32)

    def after(v, trig):
        if trig is None:
            return v
        return jnp.concatenate([jnp.where(trig[0], trig[1], v[:, :128]), v[:, 128:]], axis=1)

    def post_work(row0, att, scores_out=None):
        st = {}

        def head(trig):
            a = after(att().astype(F32), trig)
            st["x2"] = _rb(x_v[pl.ds(row0, 8), :].astype(F32) + _rb(mod_v[2] * a))
            st["mu"], st["inv"] = ln_stats(st["x2"])

        def chunk(c, trig):
            xc = after(st["x2"][:, c * CW:(c + 1) * CW], trig)
            h2b = (_rb(_rb(_rb(xc - st["mu"]) * st["inv"]) * mod_c(4, c))
                   + mod_c(3, c)).astype(BF)
            h2 = h2b.astype(F32)
            ho_v[0, pl.ds(row0, 8), pl.ds(c * CW, CW)] = h2b
            o = xc + mod_c(5, c) * h2
            ho_v[1, pl.ds(row0, 8), pl.ds(c * CW, CW)] = o.astype(BF)
            rp = h2 * mod_c(6, c)
            st["r"] = rp if c == 0 else st["r"] + rp
            if c == D // CW - 1:
                r = jnp.sum(st["r"], axis=-1, keepdims=True)
                if scores_out is not None:
                    scores_out.append(r)
                    return None
                grp = row0 // 8
                lanes = lax.broadcasted_iota(jnp.int32, (8, 128), 1)
                r_v[grp // 128] = jnp.where(lanes == grp % 128, r, r_v[grp // 128])
            return token(o + st["r"])
        return [head] + [functools.partial(chunk, c) for c in range(D // CW)]

    def ln1_work(row0):
        st = {}

        def head(trig):
            st["x"] = after(x_v[pl.ds(row0, 8), :].astype(F32), trig)
            st["mu"], st["inv"] = ln_stats(st["x"])

        def chunk(c, trig):
            xc = after(st["x"][:, c * CW:(c + 1) * CW], trig)
            h = _rb(_rb(_rb(xc - st["mu"]) * st["inv"]) * mod_c(1, c)) + mod_c(0, c)
            ho_v[0, pl.ds(row0, 8), pl.ds(c * CW, CW)] = h.astype(BF)
            return token(h)
        return [head] + [functools.partial(chunk, c) for c in range(D // CW)]

    x0_copy.start()
    for cp in small_copies:
        cp.start()
    wmod_copy(0, 2).start()

    r_v[...] = jnp.full(r_v.shape, NEG, F32)
    att_v[...] = jnp.zeros(att_v.shape, BF)

    for cp in small_copies:
        cp.wait()
    mod_v[6] = jnp.broadcast_to(wr_v[...].astype(F32), (8, D))
    cf = c_v[...].astype(F32)
    sil = (cf * jax.nn.sigmoid(cf)).astype(BF)
    sc = jnp.broadcast_to(sil, (16, D))
    for k in range(8):
        sb_v[pl.ds(128 * k, 128), :] = jnp.broadcast_to(
            sil[:, 128 * k:128 * k + 128].astype(F32), (128, 128)).T

    x0_copy.wait()
    wmod_copy(2, 3).start()

    LNB = X0 // 4

    def ln0(i, carry):
        r0 = pl.multiple_of(i * LNB, 8)
        h_v[pl.ds(r0, LNB), :] = _b2(_layernorm(_f3(x_v[pl.ds(r0, LNB), :])))
        return carry
    lax.fori_loop(0, 4, ln0, 0)

    piece_copy(0, 0, 0, 256).start()
    piece_copy(0, 1, 256, 256).start()

    def mod_slab(k):
        y = _rb(jnp.dot(sc, wmod_v[k], preferred_element_type=F32)[0:8])
        if k // 2 == 1:
            y = _rb(1.0 + y)
        mod_v[k // 2, :, pl.ds((k % 2) * 512, 512)] = y

    def modulate_half(half):
        cols = pl.ds(half * 512, 512)

        def f(r0, n):
            ln = h_v[pl.ds(r0, n), cols].astype(F32).reshape(n // 8, 8, 512)
            h = _rb(ln * mod_v[1, :, cols]) + mod_v[0, :, cols]
            return h.reshape(n, 512).astype(BF)

        def mod0(i, carry):
            hp_v[pl.ds(pl.multiple_of(i * 128, 128), 128), cols] = pltpu.bitcast(
                f(pl.multiple_of(i * 256, 256), 256), U32)
            return carry
        lax.fori_loop(0, BULK // 256, mod0, 0)
        ho_v[0, pl.ds(BULK, RIDE), cols] = f(BULK, RIDE)

    wmod_copy(0, 2).wait()
    mod_slab(0)
    wmod_copy(2, 3).wait()
    mod_slab(2)
    modulate_half(0)
    piece_copy(0, 0, 0, 256).wait()
    piece_copy(1, 4, 0, 512).start()
    relayout_loop(0, 0, 0, 256)
    wmod_copy(1, 2).start()
    piece_copy(0, 1, 256, 256).wait()
    relayout_loop(0, 0, 256, 256)

    def mod_rows(slab, r0, n, acc):
        for r in range(r0, r0 + n, 8):
            sv = sb_v[pl.ds(r, 8), :]
            t = wmod_v[slab, pl.ds(r, 8), :].astype(F32) * jnp.concatenate([sv] * 4, axis=1)
            acc = t if acc is None else acc + t
        return acc

    def bulk_dot(i, k, never, rl=None, md=None, half=None):
        tiles = range(8) if half is None else range(4 * half, 4 * half + 4)
        w = pltpu.bitcast(
            wqkv_v[pl.ds(pl.multiple_of((8 * i + k) * PITCH + 64 * tiles[0], 8),
                         64 * len(tiles)), :], BF)
        cols = [hp_v[:, pl.ds(128 * c, 128)] for c in tiles]
        if rl is not None:
            slot, t, lo2 = rl
            spots = [12 + 6 * q if half is None else 4 + 3 * q for q in range(8)]
            toks = {sp: relayout(slot, t, lo2 + 8 * q, 16) for q, sp in enumerate(spots)}
            if md is not None:
                for q, sp in enumerate(spots):
                    md[1] = mod_rows(md[0], 128 * k + 16 * q, 16, md[1])
                    toks[sp] = toks[sp] ^ token(md[1][:, :256] + md[1][:, 256:])
            for c in range(0, len(tiles), 4):
                cols[c] = jnp.concatenate(
                    [jnp.where(never, toks[8 * c + j], cols[c][8 * j:8 * j + 8])
                     if 8 * c + j in toks else cols[c][8 * j:8 * j + 8]
                     for j in range(32)], axis=0)
        hb = pltpu.bitcast(jnp.concatenate(cols, axis=1), BF)
        y = jnp.dot(hb, w, preferred_element_type=F32)
        if half == 0:
            part_v[i, k] = y
            return
        if half == 1:
            y = y + part_v[i, k]
        ring[k][i, pl.ds(RING - BULK, BULK), :] = y.astype(BF)

    def bulk_a(a, carry):
        never = jnp.full((8, 128), a, jnp.int32) < 0
        for k in range(4):
            bulk_dot(a, k, never, half=0)

        @pl.when(a == 0)
        def _():
            piece_copy(0, 5, 512, 512).start()

        @pl.when(a == 1)
        def _():
            piece_copy(1, 4, 512, 512).start()
        lo = pl.multiple_of(512 * a, 512)
        stage_wait(1 - a, 4 + a, lo, 512)
        for k in range(4, 8):
            bulk_dot(a, k, never, (1 - a, 1 - a, 256 * a + 64 * (k - 4)), half=0)

        @pl.when(a == 0)
        def _():
            wmod_copy(3, 3).start()
        return carry
    lax.fori_loop(0, 2, bulk_a, 0)

    piece_copy(2, 0, 0, 512).start()
    wmod_copy(1, 2).wait()
    wmod_copy(3, 3).wait()
    mod_slab(1)
    mod_slab(3)
    modulate_half(1)

    def bulk_b(b, carry):
        never = jnp.full((8, 128), b, jnp.int32) < 0

        @pl.when(b == 1)
        def _():
            piece_copy(2, 0, 0, 512).wait()
        for k in range(4):
            bulk_dot(b, k, never, (1 - b, 1 + b, 64 * k), half=1)

        @pl.when(b == 0)
        def _():
            piece_copy(2, 1, 512, 512).start()
        stage_wait(1 - b, 4 - 3 * b, 512, 512)
        for k in range(4, 8):
            bulk_dot(b, k, never, (1 - b, 1 + b, 64 * k), half=1)

        @pl.when(b == 0)
        def _():
            piece_copy(3, 5).start()
        return carry
    lax.fori_loop(0, 2, bulk_b, 0)

    def bulk_qkv(i, carry):
        @pl.when(i < 11)
        def _():
            stage_wait((i + 1) % 2, 4 + (i + 1) % 2)

        @pl.when((i >= 3) & (i < 11))
        def _():
            wmod_copy(i + 1, 2 + (i + 1) % 2).wait()

        for j in range(2, 10):
            @pl.when(i == j)
            def _():
                piece_copy(j + 2, 4 + j % 2).start()

        t = jnp.minimum(i + 1, 11)
        never = jnp.full((8, 128), i, jnp.int32) < 0
        md = [t, None]
        for k in range(8):
            bulk_dot(i, k, never, (t % 2, t, k * 64), md)
        macc_v[t] = md[1]

        for j in range(2, 10):
            @pl.when(i == j)
            def _():
                if j < 9:
                    wmod_copy(j + 3, 2 + (j + 3) % 2).start()
                    mid_copies[j - 2].start()
                else:
                    for cp in mid_copies[7:]:
                        cp.start()
        return carry
    wmod_copy(4, 2).start()
    lax.fori_loop(2, 12, bulk_qkv, 0)

    for k in range(4, 12):
        y = _rb(jnp.sum(macc_v[k], axis=0, keepdims=True))
        if k // 2 == 4:
            y = _rb(1.0 + y)
        mod_v[k // 2, :, pl.ds((k % 2) * 512, 512)] = jnp.broadcast_to(y, (8, 512))
    for cp in mid_copies:
        cp.wait()
    x2_copy.start()
    for cp in ffn_copies:
        cp.start()

    scale = DH ** -0.5
    rr = lax.broadcasted_iota(jnp.int32, (80, 80), 0)
    cc = lax.broadcasted_iota(jnp.int32, (80, 80), 1)

    def second(i):
        return ((i >= 8) & (i < 16)) | (i >= 48)
    same = second(rr) == second(cc)
    allowed = same & ((rr < 16) | (cc <= rr))
    fill = jnp.where(same, -1e9, NEG).astype(F32)

    def tied(u, never, toks):
        if not toks:
            return u
        parts, at = [], 0
        for j, tk in enumerate(toks):
            r = 64 * j
            if r > at:
                parts.append(u[at:r])
            w = tk.shape[1]
            sel = jnp.where(never[:, :w], tk, u[r:r + 8, :w])
            parts.append(sel if w == 128 else jnp.concatenate([sel, u[r:r + 8, w:]], axis=1))
            at = r + 8
        return jnp.concatenate(parts + [u[at:]], axis=0)

    def w_slab(t, g, lo=0, n=512, never=None, toks=()):
        return pltpu.bitcast(
            tied(wqkv_v[pl.ds((8 * t + g) * PITCH + lo, n), :], never, toks), BF)

    def step(s, mem, chained, left, att_prev):
        odd = left is not None
        wr = pl.multiple_of(lax.rem(RIDE * s, RING), 8)
        rd = pl.multiple_of(lax.rem(SEG * s + RING - BULK, RING), SEG)
        xin = jnp.concatenate(
            [mem, ho_v[0, pl.ds(pl.multiple_of(BULK + RIDE * s, 8), RIDE), :]], axis=0)

        prow = SEG * (s - 1) if odd else jnp.maximum(SEG * s - 40, 0)
        nrow = BULK + RIDE * jnp.minimum(s + 1, NSEG - 1)
        works = [post_work(pl.multiple_of(prow + 8 * q, 8), functools.partial(att_prev, q))
                 for q in range(3 if odd else 5)]
        works += [ln1_work(pl.multiple_of(nrow + 8 * q, 8)) for q in range(RIDE // 8)]
        never = jnp.full((8, 128), s, jnp.int32) < 0
        gap = (SIDE_END - SIDE0 - SIDE_LAT - SIDE_DUE) // len(works)
        sched = {}
        for q, wk in enumerate(works):
            sched.setdefault(SIDE0 + gap * q, []).append(wk[0])
            for c in range(1, len(wk)):
                sched.setdefault(SIDE0 + SIDE_LAT + gap * q + ((c - 1) * gap) // 4,
                                 []).append(wk[c])

        memqkv, probs, wl, new_left, toks = {}, {}, {}, {}, {}
        acc = []

        ndot = [0]

        def proj(g, t_lo, t_hi):
            part = {}
            if chained and ndot[0] == 0:
                for t in range(t_lo, t_lo + 6):
                    part[t] = jnp.dot(xin[:, :512], w_slab(t, g, 0, 256),
                                      preferred_element_type=F32)
            for t0 in range(t_lo, t_hi, 2):
                ys = []
                for t in (t0, t0 + 1):
                    n = ndot[0]
                    ndot[0] += 1
                    if t in part:
                        y = jnp.dot(xin[:, 512:], w_slab(t, g, 256, 256),
                                    preferred_element_type=F32) + part[t]
                    else:
                        y = jnp.dot(xin, w_slab(t, g, 0, 512, never, toks.get(n)),
                                    preferred_element_type=F32)
                    ring[g][t, pl.ds(wr, RIDE), :] = y[M:].astype(BF)
                    ys.append(y[:M])
                    for item in sched.get(n, ()):
                        tk = item((never, y[:M]))
                        if tk is not None:
                            toks.setdefault(n + SIDE_DUE, []).append(tk)
                memqkv[(t0, g)] = jnp.concatenate(ys, axis=0).astype(BF)

        def cat(t0, g):
            return jnp.concatenate([memqkv[(t0, g)], ring[g][t0, pl.ds(rd, SEG), :],
                                    ring[g][t0 + 1, pl.ds(rd, SEG), :]], axis=0)

        def scores(g):
            for p in (0, 2):
                sc_ = lax.dot_general(cat(p, g), cat(4 + p, g), (((1,), (1,)), ((), ())),
                                      preferred_element_type=F32)
                sc_ = jnp.where(allowed, sc_ * scale, fill)
                e = jnp.exp(sc_ - jnp.max(sc_, axis=1, keepdims=True))
                l = jnp.sum(e, axis=1, keepdims=True)
                rc = pl.reciprocal(l, approx=True)
                rc = rc * (2.0 - l * rc)
                probs[(p, g)] = (e * rc).astype(BF)

        def pv(g):
            for p in (0, 2):
                o = jnp.dot(probs[(p, g)], cat(8 + p, g), preferred_element_type=F32)
                for j in range(2):
                    om, ot = o[8 * j:8 * j + 8], o[16 + 32 * j:48 + 32 * j]
                    if odd:
                        rows = [om, left[(p + j, g)], ot]
                    else:
                        rows = [om, ot[:RIDE]]
                        new_left[(p + j, g)] = ot[RIDE:]
                    wl[(p + j, g)] = jnp.concatenate(rows, axis=0).astype(BF)

        def wo(g):
            a = jnp.concatenate([wl[(o, g)] for o in range(4)], axis=1)
            w = jnp.concatenate(
                [jnp.concatenate([wo_v[n, pl.ds((8 * o + PERM[g]) * DH, DH), :]
                                  for o in range(4)], axis=0) for n in range(2)], axis=1)
            y = jnp.dot(a, w, preferred_element_type=F32)
            acc[:] = [y if not acc else y + acc[0]]

        for op in ORDER.split():
            g = int(op[1])
            if op[0] in "qkv":
                proj(g, *{"q": (0, 12), "k": (0, 8), "v": (8, 12)}[op[0]])
            else:
                {"s": scores, "p": pv, "w": wo}[op[0]](g)
        y = acc[0].astype(BF)
        return y[:M], y[M:], (None if odd else new_left)

    def out_copy(row0, n, k):
        return pltpu.make_async_copy(ho_v.at[1, pl.ds(row0, n), :],
                                     out_hbm.at[0, pl.ds(row0, n), :], sems.at[3 + k])

    OB = SEG * UNROLL

    def carried(q):
        return att_v[pl.ds(8 * q, 8), :]

    def steps(i, carry):
        @pl.when(i == 16 // UNROLL)
        def _():
            x2_copy.wait()

        @pl.when(i >= 3)
        def _():
            out_copy(pl.multiple_of((i - 3) * OB, OB), OB, 0).wait()

        @pl.when(i >= 2)
        def _():
            out_copy(pl.multiple_of((i - 2) * OB, OB), OB, 0).start()

        mem, left, att_prev = mem_v[...], None, carried
        for u in range(UNROLL):
            mem, att, left = step(i * UNROLL + u, mem, u > 0, left, att_prev)
            att_prev = (lambda a: lambda q: a[8 * q:8 * q + 8])(att)
        mem_v[...] = mem
        att_v[...] = att
        return carry
    lax.fori_loop(0, NSEG // UNROLL, steps, 0)

    for cp in ffn_copies:
        cp.wait()
    out_copy(S - 2 * OB, OB, 1).start()
    last = []
    for q in range(5):
        for item in post_work(S - 40 + 8 * q, functools.partial(carried, q), last):
            item(None)
    out_copy(S - OB, OB, 2).start()

    def top2(val, idx, valid):
        def reduce(f, v):
            v = f(v, axis=0, keepdims=True)
            return v if v.shape[1] == 1 else f(v, axis=1, keepdims=True)

        def argtop(ok):
            v = jnp.where(ok, val, -jnp.inf)
            m = reduce(jnp.max, v)
            return m, reduce(jnp.min, jnp.where(ok & (v >= m), idx, float(S)))
        m1, i1 = argtop(valid)
        return (m1, i1), argtop(valid & (idx != i1))

    sub1 = lax.broadcasted_iota(jnp.int32, (16, 128), 0)
    lan1 = lax.broadcasted_iota(jnp.int32, (16, 128), 1)
    idx = (sub1 // 8) * 1024 + lan1 * 8 + sub1 % 8
    c_a, c_b = top2(_rb(r_v[...].reshape(16, 128)), idx.astype(F32), idx < S - 40)
    sub2 = lax.broadcasted_iota(jnp.int32, (48, 1), 0)
    val2 = jnp.concatenate([_rb(r) for r in last] + [jnp.where(sub2[:8] == 0, c_a[0], c_b[0])],
                           axis=0)
    idx2 = jnp.where(sub2 < 40, (sub2 + (S - 40)).astype(F32),
                     jnp.where(sub2 == 40, c_a[1], c_b[1]))
    (m_a, i_a), (m_b, i_b) = top2(val2, idx2, sub2 < 42)
    i_a = i_a.astype(jnp.int32)
    i_b = i_b.astype(jnp.int32)
    ia = jnp.clip(i_a[0, 0], 0, S - 1)
    ib = jnp.clip(i_b[0, 0], 0, S - 1)
    blk_a = pl.multiple_of((ia // 8) * 8, 8)
    blk_b = pl.multiple_of((ib // 8) * 8, 8)

    def two(ref):
        return jnp.concatenate([ref[pl.ds(blk_a, 8), :], ref[pl.ds(blk_b, 8), :]], axis=0)

    hs = two(ho_v.at[0])
    g = _rb(jnp.dot(hs, wg_v[...], preferred_element_type=F32))
    u = _rb(jnp.dot(hs, wu_v[...], preferred_element_type=F32))
    act = (_rb(g * jax.nn.sigmoid(g)) * u).astype(BF)
    y = jnp.concatenate(
        [jnp.dot(act, wd_v[k], preferred_element_type=F32) for k in range(2)], axis=1)
    sub = lax.broadcasted_iota(jnp.int32, (16, 1), 0)
    rows = jnp.where(sub < 8, blk_a + sub, blk_b + sub - 8)
    gate = jnp.where(rows == ia, jax.nn.sigmoid(m_a),
                     jnp.where(rows == ib, jax.nn.sigmoid(m_b), 0.0))
    upd = jnp.where((rows == ia) | (rows == ib), y * gate, 0.0).reshape(2, 8, D)
    fin = _b2(_f3(two(ho_v.at[1])) + mod_v[5] * upd)

    for k in range(3):
        out_copy(S - (3 - k) * OB, OB, k).wait()
    ho_v[1, pl.ds(blk_a, 8), :] = fin[0:8]
    ho_v[1, pl.ds(blk_b, 8), :] = fin[8:16]
    out_copy(blk_a, 8, 0).start()

    @pl.when(blk_a != blk_b)
    def _():
        out_copy(blk_b, 8, 1).start()
        out_copy(blk_b, 8, 1).wait()
    out_copy(blk_a, 8, 0).wait()


@jax.jit
def pallas_adaLN_cond__memory_aug_recurrent_mem_tr__moe_arch_mod__prompt_kernel(
    A_x, A_mem0, A_Wq, A_Wk, A_Wv, A_Wo, A_seg_len, B_x, B_w_r, B_w_gate, B_w_up, B_w_down, c,
    w_mod,
):
    del B_x
    del A_seg_len
    assert A_x.shape == (1, S, D) and A_Wq.shape == (D, H, DH) and A_mem0.shape == (1, M, D)
    any_spec = pl.BlockSpec(memory_space=pl.ANY)
    scratch = [
        pltpu.VMEM((S, D), BF),
        pltpu.VMEM((X0, D), BF),
        pltpu.VMEM((BULK // 2, D), U32),
        pltpu.VMEM((40, D), BF),
        pltpu.VMEM((2, S, D), BF),
        pltpu.VMEM((96 * PITCH, 128), U32),
        pltpu.VMEM((2, H * DH, 512), BF),
        pltpu.VMEM((2, D, 8, 128), BF),
        pltpu.VMEM((12, D, 512), BF),
        pltpu.VMEM((D, FF), BF),
        pltpu.VMEM((D, FF), BF),
        pltpu.VMEM((2, FF, 512), BF),
        pltpu.VMEM((M, D), BF),
        pltpu.VMEM((1, D), BF),
        pltpu.VMEM((1, D), BF),
        pltpu.VMEM((7, 8, D), F32),
        pltpu.VMEM((2, 8, 128), F32),
        pltpu.VMEM((D, 128), F32),
        pltpu.VMEM((12, 8, 512), F32),
        pltpu.VMEM((2, 8, BULK, 128), F32),
        pltpu.SemaphoreType.DMA((6,)),
    ] + [pltpu.VMEM((12, RING, 128), BF)] * 8
    return pl.pallas_call(
        _kernel,
        out_shape=jax.ShapeDtypeStruct((1, S, D), BF),
        in_specs=[any_spec] * 12,
        out_specs=any_spec,
        scratch_shapes=scratch,
        compiler_params=pltpu.CompilerParams(vmem_limit_bytes=120 * 1024 * 1024),
    )(A_x, A_mem0, A_Wq, A_Wk, A_Wv, A_Wo.reshape(H * DH, D), B_w_r.reshape(1, D), B_w_gate,
      B_w_up, B_w_down, c, w_mod)
```

```python
import functools

import jax
import jax.numpy as jnp
from jax import lax
import jax.experimental.pallas as pl
import jax.experimental.pallas.tpu as pltpu

BF = jnp.bfloat16
F32 = jnp.float32
U32 = jnp.uint32

S = 2048
D = 1024
H = 32
DH = 128
M = 8
SEG = 32
NSEG = S // SEG
FF = 3584
RIDE = 24
BULK = S - RIDE * NSEG
X0 = BULK + 32
RING = 576
PITCH = 520
X1 = 1024
UNROLL = 4
EPS = 1e-5
SIDE0, SIDE_LAT, SIDE_DUE, SIDE_END = 2, 6, 6, 96
NEG = -3.0e38
ORDER = ("q0 q1 q2 q3 q4 q5 q6 s0 s1 s2 s3 s4 s5 q7 p0 p1 p2 p3 p4 p5 s6 s7 w0 w1 w2 p6 p7 w3 "
         "w4 w5 w6 w7")
PERM = (0, 2, 4, 6, 1, 3, 5, 7)


def _rb(v):
    return v.astype(BF).astype(F32)


def _layernorm(xf):
    mu = jnp.mean(xf, axis=-1, keepdims=True)
    dv = xf - mu
    var = jnp.mean(dv * dv, axis=-1, keepdims=True)
    sd = _rb(jnp.sqrt(_rb(_rb(var) + EPS)))
    return _rb(_rb(xf - _rb(mu)) * (1.0 / sd))


def _f3(v):
    return v.astype(F32).reshape(v.shape[0] // 8, 8, D)


def _b2(v):
    return v.reshape(v.shape[0] * 8, D).astype(BF)


def _kernel(x_hbm, mem0_hbm, wq_hbm, wk_hbm, wv_hbm, wo_hbm, wr_hbm, wg_hbm, wu_hbm, wd_hbm,
            c_hbm, wmod_hbm, out_hbm,
            x_v, h_v, hp_v, att_v, ho_v, wqkv_v, wo_v, stage, wmod_v,
            wg_v, wu_v, wd_v, mem_v, c_v, wr_v, mod_v, r_v, sb_v, macc_v,
            part_v, sems, *rings):
    w_hbm = (wq_hbm, wk_hbm, wv_hbm)
    ring = rings

    def piece_copy(t, sem, lo=0, n=D):
        return pltpu.make_async_copy(
            w_hbm[t // 4].at[pl.ds(lo, n), pl.ds((t % 4) * 8, 8), :],
            stage.at[t % 2, pl.ds(lo, n)], sems.at[sem])

    def stage_wait(slot, sem, lo=0, n=D):
        dst = stage.at[slot, pl.ds(lo, n)]
        pltpu.make_async_copy(dst, dst, sems.at[sem]).wait()

    def wmod_copy(k, sem):
        col = k * 512 if isinstance(k, int) else pl.multiple_of(k * 512, 512)
        return pltpu.make_async_copy(wmod_hbm.at[:, pl.ds(col, 512)], wmod_v.at[k], sems.at[sem])

    def x_copy(lo, hi, sem):
        return pltpu.make_async_copy(x_hbm.at[0, pl.ds(lo, hi - lo), :],
                                     x_v.at[pl.ds(lo, hi - lo), :], sems.at[sem])

    def wo_copy(n):
        lo, rows = ((n // 2) * 512, 512) if n < 6 else (1536, 2560)
        return pltpu.make_async_copy(wo_hbm.at[pl.ds(lo, rows), pl.ds((n % 2) * 512, 512)],
                                     wo_v.at[n % 2, pl.ds(lo, rows)], sems.at[0])

    small_copies = [pltpu.make_async_copy(c_hbm, c_v, sems.at[0]),
                    pltpu.make_async_copy(mem0_hbm.at[0], mem_v, sems.at[0]),
                    pltpu.make_async_copy(wr_hbm, wr_v, sems.at[0])]
    x0_copy = x_copy(0, X0, 1)
    mid_copies = ([x_copy(X0, (X0 + X1) // 2, 0), x_copy((X0 + X1) // 2, X1, 0)]
                  + [wo_copy(n) for n in range(8)])
    x2_copy = x_copy(X1, S, 1)
    ffn_copies = [pltpu.make_async_copy(wg_hbm, wg_v, sems.at[2]),
                  pltpu.make_async_copy(wu_hbm, wu_v, sems.at[2])] + [
        pltpu.make_async_copy(wd_hbm.at[:, pl.ds(k * 512, 512)], wd_v.at[k], sems.at[2])
        for k in range(2)]

    def relayout(slot, t, lo2, n):
        base = t * (8 * PITCH) + lo2
        u = pltpu.bitcast(stage[slot, pl.ds(2 * lo2, n)], U32)
        tok = None
        for i in range(n // 2):
            a = u[2 * i]
            b = u[2 * i + 1]
            even = (a & jnp.uint32(0xFFFF)) | (b << 16)
            odd = (a >> 16) | (b & jnp.uint32(0xFFFF0000))
            wqkv_v[pl.ds(base + i, 4, stride=PITCH), :] = even
            wqkv_v[pl.ds(base + 4 * PITCH + i, 4, stride=PITCH), :] = odd
            tok = even ^ odd if tok is None else tok ^ even ^ odd
        return jnp.concatenate([tok, tok], axis=0)

    def relayout_loop(slot, t, lo, n):
        def body(i, carry):
            relayout(slot, t, lo // 2 + i * 64, 128)
            return carry
        lax.fori_loop(0, n // 128, body, 0)

    CW = 256

    def ln_stats(xf):
        mu = jnp.mean(xf, axis=-1, keepdims=True)
        dv = xf - mu
        var = jnp.mean(dv * dv, axis=-1, keepdims=True)
        sd = _rb(jnp.sqrt(_rb(_rb(var) + EPS)))
        return _rb(mu), 1.0 / sd

    def mod_c(k, c):
        return mod_v[k, :, pl.ds(c * CW, CW)]

    def token(v):
        return pltpu.bitcast(v[:, :128] + v[:, 128:], U32)

    def after(v, trig):
        if trig is None:
            return v
        return jnp.concatenate([jnp.where(trig[0], trig[1], v[:, :128]), v[:, 128:]], axis=1)

    def post_work(row0, att, scores_out=None):
        st = {}

        def head(trig):
            a = after(att().astype(F32), trig)
            st["x2"] = _rb(x_v[pl.ds(row0, 8), :].astype(F32) + _rb(mod_v[2] * a))
            st["mu"], st["inv"] = ln_stats(st["x2"])

        def chunk(c, trig):
            xc = after(st["x2"][:, c * CW:(c + 1) * CW], trig)
            h2b = (_rb(_rb(_rb(xc - st["mu"]) * st["inv"]) * mod_c(4, c))
                   + mod_c(3, c)).astype(BF)
            h2 = h2b.astype(F32)
            ho_v[0, pl.ds(row0, 8), pl.ds(c * CW, CW)] = h2b
            o = xc + mod_c(5, c) * h2
            ho_v[1, pl.ds(row0, 8), pl.ds(c * CW, CW)] = o.astype(BF)
            rp = h2 * mod_c(6, c)
            st["r"] = rp if c == 0 else st["r"] + rp
            if c == D // CW - 1:
                r = jnp.sum(st["r"], axis=-1, keepdims=True)
                if scores_out is not None:
                    scores_out.append(r)
                    return None
                grp = row0 // 8
                lanes = lax.broadcasted_iota(jnp.int32, (8, 128), 1)
                r_v[grp // 128] = jnp.where(lanes == grp % 128, r, r_v[grp // 128])
            return token(o + st["r"])
        return [head] + [functools.partial(chunk, c) for c in range(D // CW)]

    def ln1_work(row0):
        st = {}

        def head(trig):
            st["x"] = after(x_v[pl.ds(row0, 8), :].astype(F32), trig)
            st["mu"], st["inv"] = ln_stats(st["x"])

        def chunk(c, trig):
            xc = after(st["x"][:, c * CW:(c + 1) * CW], trig)
            h = _rb(_rb(_rb(xc - st["mu"]) * st["inv"]) * mod_c(1, c)) + mod_c(0, c)
            ho_v[0, pl.ds(row0, 8), pl.ds(c * CW, CW)] = h.astype(BF)
            return token(h)
        return [head] + [functools.partial(chunk, c) for c in range(D // CW)]

    for cp in small_copies:
        cp.start()
    x0_copy.start()
    wmod_copy(0, 2).start()

    r_v[...] = jnp.full(r_v.shape, NEG, F32)
    att_v[...] = jnp.zeros(att_v.shape, BF)

    for cp in small_copies:
        cp.wait()
    mod_v[6] = jnp.broadcast_to(wr_v[...].astype(F32), (8, D))
    cf = c_v[...].astype(F32)
    sil = (cf * jax.nn.sigmoid(cf)).astype(BF)
    sc = jnp.broadcast_to(sil, (16, D))
    for k in range(8):
        sb_v[pl.ds(128 * k, 128), :] = jnp.broadcast_to(
            sil[:, 128 * k:128 * k + 128].astype(F32), (128, 128)).T

    x0_copy.wait()
    wmod_copy(2, 3).start()

    LNB = X0 // 4

    def ln0(i, carry):
        r0 = pl.multiple_of(i * LNB, 8)
        h_v[pl.ds(r0, LNB), :] = _b2(_layernorm(_f3(x_v[pl.ds(r0, LNB), :])))
        return carry
    lax.fori_loop(0, 4, ln0, 0)

    piece_copy(0, 0, 0, 256).start()
    piece_copy(0, 1, 256, 256).start()

    def mod_slab(k):
        y = _rb(jnp.dot(sc, wmod_v[k], preferred_element_type=F32)[0:8])
        if k // 2 == 1:
            y = _rb(1.0 + y)
        mod_v[k // 2, :, pl.ds((k % 2) * 512, 512)] = y

    def modulate_half(half):
        cols = pl.ds(half * 512, 512)

        def f(r0, n):
            ln = h_v[pl.ds(r0, n), cols].astype(F32).reshape(n // 8, 8, 512)
            h = _rb(ln * mod_v[1, :, cols]) + mod_v[0, :, cols]
            return h.reshape(n, 512).astype(BF)

        def mod0(i, carry):
            hp_v[pl.ds(pl.multiple_of(i * 128, 128), 128), cols] = pltpu.bitcast(
                f(pl.multiple_of(i * 256, 256), 256), U32)
            return carry
        lax.fori_loop(0, BULK // 256, mod0, 0)
        ho_v[0, pl.ds(BULK, RIDE), cols] = f(BULK, RIDE)

    wmod_copy(0, 2).wait()
    mod_slab(0)
    wmod_copy(2, 3).wait()
    mod_slab(2)
    modulate_half(0)
    piece_copy(0, 0, 0, 256).wait()
    piece_copy(1, 4, 0, 512).start()
    relayout_loop(0, 0, 0, 256)
    wmod_copy(1, 2).start()
    piece_copy(0, 1, 256, 256).wait()
    relayout_loop(0, 0, 256, 256)

    def mod_rows(slab, r0, n, acc):
        for r in range(r0, r0 + n, 8):
            sv = sb_v[pl.ds(r, 8), :]
            t = wmod_v[slab, pl.ds(r, 8), :].astype(F32) * jnp.concatenate([sv] * 4, axis=1)
            acc = t if acc is None else acc + t
        return acc

    def bulk_w(i, k, half=None):
        lo, n = (0, 512) if half is None else (256 * half, 256)
        return pltpu.bitcast(
            wqkv_v[pl.ds(pl.multiple_of((8 * i + k) * PITCH + lo, 8), n), :], BF)

    def bulk_dot(i, k, never, rl=None, md=None, half=None, w=None):
        tiles = range(8) if half is None else range(4 * half, 4 * half + 4)
        if w is None:
            w = bulk_w(i, k, half)
        cols = [hp_v[:, pl.ds(128 * c, 128)] for c in tiles]
        if rl is not None:
            slot, t, lo2 = rl
            spots = [12 + 6 * q if half is None else 4 + 3 * q for q in range(8)]
            toks = {sp: relayout(slot, t, lo2 + 8 * q, 16) for q, sp in enumerate(spots)}
            if md is not None:
                for q, sp in enumerate(spots):
                    md[1] = mod_rows(md[0], 128 * k + 16 * q, 16, md[1])
                    toks[sp] = toks[sp] ^ token(md[1][:, :256] + md[1][:, 256:])
            for c in range(0, len(tiles), 4):
                cols[c] = jnp.concatenate(
                    [jnp.where(never, toks[8 * c + j], cols[c][8 * j:8 * j + 8])
                     if 8 * c + j in toks else cols[c][8 * j:8 * j + 8]
                     for j in range(32)], axis=0)
        hb = pltpu.bitcast(jnp.concatenate(cols, axis=1), BF)
        y = jnp.dot(hb, w, preferred_element_type=F32)
        if half == 0:
            part_v[i, k] = y
            return
        if half == 1:
            y = y + part_v[i, k]
        ring[k][i, pl.ds(RING - BULK, BULK), :] = y.astype(BF)

    def bulk_a(a, carry):
        never = jnp.full((8, 128), a, jnp.int32) < 0
        for k in range(4):
            bulk_dot(a, k, never, half=0)

        @pl.when(a == 0)
        def _():
            piece_copy(0, 5, 512, 512).start()

        @pl.when(a == 1)
        def _():
            piece_copy(1, 4, 512, 512).start()
        lo = pl.multiple_of(512 * a, 512)
        stage_wait(1 - a, 4 + a, lo, 512)
        w = bulk_w(a, 4, 0)
        for k in range(4, 8):
            w_next = bulk_w(a, k + 1, 0) if k < 7 else None
            bulk_dot(a, k, never, (1 - a, 1 - a, 256 * a + 64 * (k - 4)), half=0, w=w)
            w = w_next

        @pl.when(a == 0)
        def _():
            wmod_copy(3, 3).start()
        return carry
    lax.fori_loop(0, 2, bulk_a, 0)

    piece_copy(2, 0, 0, 512).start()
    wmod_copy(1, 2).wait()
    wmod_copy(3, 3).wait()
    mod_slab(1)
    mod_slab(3)
    modulate_half(1)

    def bulk_b(b, carry):
        never = jnp.full((8, 128), b, jnp.int32) < 0

        @pl.when(b == 1)
        def _():
            piece_copy(2, 0, 0, 512).wait()
        for k in range(4):
            bulk_dot(b, k, never, (1 - b, 1 + b, 64 * k), half=1)

        @pl.when(b == 0)
        def _():
            piece_copy(2, 1, 512, 512).start()
        stage_wait(1 - b, 4 - 3 * b, 512, 512)
        for k in range(4, 8):
            bulk_dot(b, k, never, (1 - b, 1 + b, 64 * k), half=1)

        @pl.when(b == 0)
        def _():
            piece_copy(3, 5).start()
        return carry
    lax.fori_loop(0, 2, bulk_b, 0)

    def bulk_qkv(i, carry):
        @pl.when(i < 11)
        def _():
            stage_wait((i + 1) % 2, 4 + (i + 1) % 2)

        @pl.when((i >= 3) & (i < 11))
        def _():
            wmod_copy(i + 1, 2 + (i + 1) % 2).wait()

        for j in range(2, 10):
            @pl.when(i == j)
            def _():
                piece_copy(j + 2, 4 + j % 2).start()

        t = jnp.minimum(i + 1, 11)
        never = jnp.full((8, 128), i, jnp.int32) < 0
        md = [t, None]
        for k in range(8):
            bulk_dot(i, k, never, (t % 2, t, k * 64), md)
        macc_v[t] = md[1]

        for j in range(2, 10):
            @pl.when(i == j)
            def _():
                if j < 9:
                    wmod_copy(j + 3, 2 + (j + 3) % 2).start()
                    mid_copies[j - 2].start()
                else:
                    for cp in mid_copies[7:]:
                        cp.start()
        return carry
    wmod_copy(4, 2).start()
    lax.fori_loop(2, 12, bulk_qkv, 0)

    for k in range(4, 12):
        y = _rb(jnp.sum(macc_v[k], axis=0, keepdims=True))
        if k // 2 == 4:
            y = _rb(1.0 + y)
        mod_v[k // 2, :, pl.ds((k % 2) * 512, 512)] = jnp.broadcast_to(y, (8, 512))
    for cp in mid_copies:
        cp.wait()
    x2_copy.start()
    for cp in ffn_copies:
        cp.start()

    scale = DH ** -0.5
    rr = lax.broadcasted_iota(jnp.int32, (80, 80), 0)
    cc = lax.broadcasted_iota(jnp.int32, (80, 80), 1)

    def second(i):
        return ((i >= 8) & (i < 16)) | (i >= 48)
    same = second(rr) == second(cc)
    allowed = same & ((rr < 16) | (cc <= rr))
    fill = jnp.where(same, -1e9, NEG).astype(F32)

    def tied(u, never, toks):
        if not toks:
            return u
        parts, at = [], 0
        for j, tk in enumerate(toks):
            r = 64 * j
            if r > at:
                parts.append(u[at:r])
            w = tk.shape[1]
            sel = jnp.where(never[:, :w], tk, u[r:r + 8, :w])
            parts.append(sel if w == 128 else jnp.concatenate([sel, u[r:r + 8, w:]], axis=1))
            at = r + 8
        return jnp.concatenate(parts + [u[at:]], axis=0)

    def w_slab(t, g, lo=0, n=512, never=None, toks=()):
        return pltpu.bitcast(
            tied(wqkv_v[pl.ds((8 * t + g) * PITCH + lo, n), :], never, toks), BF)

    def step(s, mem, chained, left, att_prev):
        odd = left is not None
        wr = pl.multiple_of(lax.rem(RIDE * s, RING), 8)
        rd = pl.multiple_of(lax.rem(SEG * s + RING - BULK, RING), SEG)
        xin = jnp.concatenate(
            [mem, ho_v[0, pl.ds(pl.multiple_of(BULK + RIDE * s, 8), RIDE), :]], axis=0)

        prow = SEG * (s - 1) if odd else jnp.maximum(SEG * s - 40, 0)
        nrow = BULK + RIDE * jnp.minimum(s + 1, NSEG - 1)
        works = [post_work(pl.multiple_of(prow + 8 * q, 8), functools.partial(att_prev, q))
                 for q in range(3 if odd else 5)]
        works += [ln1_work(pl.multiple_of(nrow + 8 * q, 8)) for q in range(RIDE // 8)]
        never = jnp.full((8, 128), s, jnp.int32) < 0
        gap = (SIDE_END - SIDE0 - SIDE_LAT - SIDE_DUE) // len(works)
        sched = {}
        for q, wk in enumerate(works):
            sched.setdefault(SIDE0 + gap * q, []).append(wk[0])
            for c in range(1, len(wk)):
                sched.setdefault(SIDE0 + SIDE_LAT + gap * q + ((c - 1) * gap) // 4,
                                 []).append(wk[c])

        memqkv, probs, wl, new_left, toks = {}, {}, {}, {}, {}
        acc = []

        ndot = [0]

        def proj(g, t_lo, t_hi):
            part = {}
            if chained and ndot[0] == 0:
                for t in range(t_lo, t_lo + 6):
                    part[t] = jnp.dot(xin[:, :512], w_slab(t, g, 0, 256),
                                      preferred_element_type=F32)
            for t0 in range(t_lo, t_hi, 2):
                ys = []
                for t in (t0, t0 + 1):
                    n = ndot[0]
                    ndot[0] += 1
                    if t in part:
                        y = jnp.dot(xin[:, 512:], w_slab(t, g, 256, 256),
                                    preferred_element_type=F32) + part[t]
                    else:
                        y = jnp.dot(xin, w_slab(t, g, 0, 512, never, toks.get(n)),
                                    preferred_element_type=F32)
                    ring[g][t, pl.ds(wr, RIDE), :] = y[M:].astype(BF)
                    ys.append(y[:M])
                    for item in sched.get(n, ()):
                        tk = item((never, y[:M]))
                        if tk is not None:
                            toks.setdefault(n + SIDE_DUE, []).append(tk)
                memqkv[(t0, g)] = jnp.concatenate(ys, axis=0).astype(BF)

        def cat(t0, g):
            return jnp.concatenate([memqkv[(t0, g)], ring[g][t0, pl.ds(rd, SEG), :],
                                    ring[g][t0 + 1, pl.ds(rd, SEG), :]], axis=0)

        def scores(g):
            for p in (0, 2):
                sc_ = lax.dot_general(cat(p, g), cat(4 + p, g), (((1,), (1,)), ((), ())),
                                      preferred_element_type=F32)
                sc_ = jnp.where(allowed, sc_ * scale, fill)
                e = jnp.exp(sc_ - jnp.max(sc_, axis=1, keepdims=True))
                l = jnp.sum(e, axis=1, keepdims=True)
                rc = pl.reciprocal(l, approx=True)
                rc = rc * (2.0 - l * rc)
                probs[(p, g)] = (e * rc).astype(BF)

        def pv(g):
            for p in (0, 2):
                o = jnp.dot(probs[(p, g)], cat(8 + p, g), preferred_element_type=F32)
                for j in range(2):
                    om, ot = o[8 * j:8 * j + 8], o[16 + 32 * j:48 + 32 * j]
                    if odd:
                        rows = [om, left[(p + j, g)], ot]
                    else:
                        rows = [om, ot[:RIDE]]
                        new_left[(p + j, g)] = ot[RIDE:]
                    wl[(p + j, g)] = jnp.concatenate(rows, axis=0).astype(BF)

        def wo(g):
            a = jnp.concatenate([wl[(o, g)] for o in range(4)], axis=1)
            w = jnp.concatenate(
                [jnp.concatenate([wo_v[n, pl.ds((8 * o + PERM[g]) * DH, DH), :]
                                  for o in range(4)], axis=0) for n in range(2)], axis=1)
            y = jnp.dot(a, w, preferred_element_type=F32)
            acc[:] = [y if not acc else y + acc[0]]

        for op in ORDER.split():
            g = int(op[1])
            if op[0] in "qkv":
                proj(g, *{"q": (0, 12), "k": (0, 8), "v": (8, 12)}[op[0]])
            else:
                {"s": scores, "p": pv, "w": wo}[op[0]](g)
        y = acc[0].astype(BF)
        return y[:M], y[M:], (None if odd else new_left)

    def out_copy(row0, n, k):
        return pltpu.make_async_copy(ho_v.at[1, pl.ds(row0, n), :],
                                     out_hbm.at[0, pl.ds(row0, n), :], sems.at[3 + k])

    OB = SEG * UNROLL

    def carried(q):
        return att_v[pl.ds(8 * q, 8), :]

    def steps(i, carry):
        @pl.when(i == 16 // UNROLL)
        def _():
            x2_copy.wait()

        @pl.when(i >= 3)
        def _():
            out_copy(pl.multiple_of((i - 3) * OB, OB), OB, 0).wait()

        @pl.when(i >= 2)
        def _():
            out_copy(pl.multiple_of((i - 2) * OB, OB), OB, 0).start()

        mem, left, att_prev = mem_v[...], None, carried
        for u in range(UNROLL):
            mem, att, left = step(i * UNROLL + u, mem, u > 0, left, att_prev)
            att_prev = (lambda a: lambda q: a[8 * q:8 * q + 8])(att)
        mem_v[...] = mem
        att_v[...] = att
        return carry
    lax.fori_loop(0, NSEG // UNROLL, steps, 0)

    for cp in ffn_copies:
        cp.wait()
    out_copy(S - 2 * OB, OB, 1).start()
    last = []
    for q in range(5):
        for item in post_work(S - 40 + 8 * q, functools.partial(carried, q), last):
            item(None)
    out_copy(S - OB, OB, 2).start()

    def top2(val, idx, valid):
        def reduce(f, v):
            v = f(v, axis=0, keepdims=True)
            return v if v.shape[1] == 1 else f(v, axis=1, keepdims=True)

        def argtop(ok):
            v = jnp.where(ok, val, -jnp.inf)
            m = reduce(jnp.max, v)
            return m, reduce(jnp.min, jnp.where(ok & (v >= m), idx, float(S)))
        m1, i1 = argtop(valid)
        return (m1, i1), argtop(valid & (idx != i1))

    sub1 = lax.broadcasted_iota(jnp.int32, (16, 128), 0)
    lan1 = lax.broadcasted_iota(jnp.int32, (16, 128), 1)
    idx = (sub1 // 8) * 1024 + lan1 * 8 + sub1 % 8
    c_a, c_b = top2(_rb(r_v[...].reshape(16, 128)), idx.astype(F32), idx < S - 40)
    sub2 = lax.broadcasted_iota(jnp.int32, (48, 1), 0)
    val2 = jnp.concatenate([_rb(r) for r in last] + [jnp.where(sub2[:8] == 0, c_a[0], c_b[0])],
                           axis=0)
    idx2 = jnp.where(sub2 < 40, (sub2 + (S - 40)).astype(F32),
                     jnp.where(sub2 == 40, c_a[1], c_b[1]))
    (m_a, i_a), (m_b, i_b) = top2(val2, idx2, sub2 < 42)
    i_a = i_a.astype(jnp.int32)
    i_b = i_b.astype(jnp.int32)
    ia = jnp.clip(i_a[0, 0], 0, S - 1)
    ib = jnp.clip(i_b[0, 0], 0, S - 1)
    blk_a = pl.multiple_of((ia // 8) * 8, 8)
    blk_b = pl.multiple_of((ib // 8) * 8, 8)

    def two(ref):
        return jnp.concatenate([ref[pl.ds(blk_a, 8), :], ref[pl.ds(blk_b, 8), :]], axis=0)

    hs = two(ho_v.at[0])
    g = _rb(jnp.dot(hs, wg_v[...], preferred_element_type=F32))
    u = _rb(jnp.dot(hs, wu_v[...], preferred_element_type=F32))
    act = (_rb(g * jax.nn.sigmoid(g)) * u).astype(BF)
    y = jnp.concatenate(
        [jnp.dot(act, wd_v[k], preferred_element_type=F32) for k in range(2)], axis=1)
    sub = lax.broadcasted_iota(jnp.int32, (16, 1), 0)
    rows = jnp.where(sub < 8, blk_a + sub, blk_b + sub - 8)
    gate = jnp.where(rows == ia, jax.nn.sigmoid(m_a),
                     jnp.where(rows == ib, jax.nn.sigmoid(m_b), 0.0))
    upd = jnp.where((rows == ia) | (rows == ib), y * gate, 0.0).reshape(2, 8, D)
    fin = _b2(_f3(two(ho_v.at[1])) + mod_v[5] * upd)

    for k in range(3):
        out_copy(S - (3 - k) * OB, OB, k).wait()
    ho_v[1, pl.ds(blk_a, 8), :] = fin[0:8]
    ho_v[1, pl.ds(blk_b, 8), :] = fin[8:16]
    out_copy(blk_a, 8, 0).start()

    @pl.when(blk_a != blk_b)
    def _():
        out_copy(blk_b, 8, 1).start()
        out_copy(blk_b, 8, 1).wait()
    out_copy(blk_a, 8, 0).wait()


@jax.jit
def pallas_adaLN_cond__memory_aug_recurrent_mem_tr__moe_arch_mod__prompt_kernel(
    A_x, A_mem0, A_Wq, A_Wk, A_Wv, A_Wo, A_seg_len, B_x, B_w_r, B_w_gate, B_w_up, B_w_down, c,
    w_mod,
):
    del B_x
    del A_seg_len
    assert A_x.shape == (1, S, D) and A_Wq.shape == (D, H, DH) and A_mem0.shape == (1, M, D)
    any_spec = pl.BlockSpec(memory_space=pl.ANY)
    scratch = [
        pltpu.VMEM((S, D), BF),
        pltpu.VMEM((X0, D), BF),
        pltpu.VMEM((BULK // 2, D), U32),
        pltpu.VMEM((40, D), BF),
        pltpu.VMEM((2, S, D), BF),
        pltpu.VMEM((96 * PITCH, 128), U32),
        pltpu.VMEM((2, H * DH, 512), BF),
        pltpu.VMEM((2, D, 8, 128), BF),
        pltpu.VMEM((12, D, 512), BF),
        pltpu.VMEM((D, FF), BF),
        pltpu.VMEM((D, FF), BF),
        pltpu.VMEM((2, FF, 512), BF),
        pltpu.VMEM((M, D), BF),
        pltpu.VMEM((1, D), BF),
        pltpu.VMEM((1, D), BF),
        pltpu.VMEM((7, 8, D), F32),
        pltpu.VMEM((2, 8, 128), F32),
        pltpu.VMEM((D, 128), F32),
        pltpu.VMEM((12, 8, 512), F32),
        pltpu.VMEM((2, 8, BULK, 128), F32),
        pltpu.SemaphoreType.DMA((6,)),
    ] + [pltpu.VMEM((12, RING, 128), BF)] * 8
    return pl.pallas_call(
        _kernel,
        out_shape=jax.ShapeDtypeStruct((1, S, D), BF),
        in_specs=[any_spec] * 12,
        out_specs=any_spec,
        scratch_shapes=scratch,
        compiler_params=pltpu.CompilerParams(vmem_limit_bytes=120 * 1024 * 1024),
    )(A_x, A_mem0, A_Wq, A_Wk, A_Wv, A_Wo.reshape(H * DH, D), B_w_r.reshape(1, D), B_w_gate,
      B_w_up, B_w_down, c, w_mod)
```

```python
import functools

import jax
import jax.numpy as jnp
from jax import lax
import jax.experimental.pallas as pl
import jax.experimental.pallas.tpu as pltpu

BF = jnp.bfloat16
F32 = jnp.float32
U32 = jnp.uint32

S = 2048
D = 1024
H = 32
DH = 128
M = 8
SEG = 32
NSEG = S // SEG
FF = 3584
RIDE = 24
BULK = S - RIDE * NSEG
X0 = BULK + 32
RING = 576
PITCH = 520
X1 = 1024
UNROLL = 4
EPS = 1e-5
SIDE0, SIDE_LAT, SIDE_DUE, SIDE_END = 2, 6, 6, 96
NEG = -3.0e38
ORDER = ("q0 q1 q2 q3 q4 q5 q6 s0 s1 s2 s3 s4 s5 q7 p0 p1 p2 p3 p4 p5 s6 s7 w0 w1 w2 p6 p7 w3 "
         "w4 w5 w6 w7")
PERM = (0, 2, 4, 6, 1, 3, 5, 7)


def _rb(v):
    return v.astype(BF).astype(F32)


def _layernorm(xf):
    mu = jnp.mean(xf, axis=-1, keepdims=True)
    dv = xf - mu
    var = jnp.mean(dv * dv, axis=-1, keepdims=True)
    sd = _rb(jnp.sqrt(_rb(_rb(var) + EPS)))
    return _rb(_rb(xf - _rb(mu)) * (1.0 / sd))


def _f3(v):
    return v.astype(F32).reshape(v.shape[0] // 8, 8, D)


def _b2(v):
    return v.reshape(v.shape[0] * 8, D).astype(BF)


def _kernel(x_hbm, mem0_hbm, wq_hbm, wk_hbm, wv_hbm, wo_hbm, wr_hbm, wg_hbm, wu_hbm, wd_hbm,
            c_hbm, wmod_hbm, out_hbm,
            x_v, h_v, hp_v, att_v, ho_v, wqkv_v, wo_v, stage, wmod_v,
            wg_v, wu_v, wd_v, mem_v, c_v, wr_v, mod_v, r_v, sb_v, macc_v,
            part_v, sems, *rings):
    w_hbm = (wq_hbm, wk_hbm, wv_hbm)
    ring = rings

    def piece_copy(t, sem, lo=0, n=D):
        return pltpu.make_async_copy(
            w_hbm[t // 4].at[pl.ds(lo, n), pl.ds((t % 4) * 8, 8), :],
            stage.at[t % 2, pl.ds(lo, n)], sems.at[sem])

    def stage_wait(slot, sem, lo=0, n=D):
        dst = stage.at[slot, pl.ds(lo, n)]
        pltpu.make_async_copy(dst, dst, sems.at[sem]).wait()

    def wmod_copy(k, sem):
        col = k * 512 if isinstance(k, int) else pl.multiple_of(k * 512, 512)
        return pltpu.make_async_copy(wmod_hbm.at[:, pl.ds(col, 512)], wmod_v.at[k], sems.at[sem])

    def x_copy(lo, hi, sem):
        return pltpu.make_async_copy(x_hbm.at[0, pl.ds(lo, hi - lo), :],
                                     x_v.at[pl.ds(lo, hi - lo), :], sems.at[sem])

    def wo_copy(n):
        lo, rows = ((n // 2) * 512, 512) if n < 6 else (1536, 2560)
        return pltpu.make_async_copy(wo_hbm.at[pl.ds(lo, rows), pl.ds((n % 2) * 512, 512)],
                                     wo_v.at[n % 2, pl.ds(lo, rows)], sems.at[0])

    small_copies = [pltpu.make_async_copy(c_hbm, c_v, sems.at[0]),
                    pltpu.make_async_copy(mem0_hbm.at[0], mem_v, sems.at[0]),
                    pltpu.make_async_copy(wr_hbm, wr_v, sems.at[0])]
    x0_copy = x_copy(0, X0, 1)
    mid_copies = ([x_copy(X0, (X0 + X1) // 2, 0), x_copy((X0 + X1) // 2, X1, 0)]
                  + [wo_copy(n) for n in range(8)])
    x2_copy = x_copy(X1, S, 1)
    ffn_copies = [pltpu.make_async_copy(wg_hbm, wg_v, sems.at[2]),
                  pltpu.make_async_copy(wu_hbm, wu_v, sems.at[2])] + [
        pltpu.make_async_copy(wd_hbm.at[:, pl.ds(k * 512, 512)], wd_v.at[k], sems.at[2])
        for k in range(2)]

    def relayout(slot, t, lo2, n):
        base = t * (8 * PITCH) + lo2
        u = pltpu.bitcast(stage[slot, pl.ds(2 * lo2, n)], U32)
        tok = None
        for i in range(n // 2):
            a = u[2 * i]
            b = u[2 * i + 1]
            even = (a & jnp.uint32(0xFFFF)) | (b << 16)
            odd = (a >> 16) | (b & jnp.uint32(0xFFFF0000))
            wqkv_v[pl.ds(base + i, 4, stride=PITCH), :] = even
            wqkv_v[pl.ds(base + 4 * PITCH + i, 4, stride=PITCH), :] = odd
            tok = even ^ odd if tok is None else tok ^ even ^ odd
        return jnp.concatenate([tok, tok], axis=0)

    def relayout_loop(slot, t, lo, n):
        def body(i, carry):
            relayout(slot, t, lo // 2 + i * 64, 128)
            return carry
        lax.fori_loop(0, n // 128, body, 0)

    CW = 256

    def ln_stats(xf):
        mu = jnp.mean(xf, axis=-1, keepdims=True)
        dv = xf - mu
        var = jnp.mean(dv * dv, axis=-1, keepdims=True)
        sd = _rb(jnp.sqrt(_rb(_rb(var) + EPS)))
        return _rb(mu), 1.0 / sd

    def mod_c(k, c):
        return mod_v[k, :, pl.ds(c * CW, CW)]

    def token(v):
        return pltpu.bitcast(v[:, :128] + v[:, 128:], U32)

    def after(v, trig):
        if trig is None:
            return v
        return jnp.concatenate([jnp.where(trig[0], trig[1], v[:, :128]), v[:, 128:]], axis=1)

    def post_work(row0, att, scores_out=None):
        st = {}

        def head(trig):
            a = after(att().astype(F32), trig)
            st["x2"] = _rb(x_v[pl.ds(row0, 8), :].astype(F32) + _rb(mod_v[2] * a))
            st["mu"], st["inv"] = ln_stats(st["x2"])

        def chunk(c, trig):
            xc = after(st["x2"][:, c * CW:(c + 1) * CW], trig)
            h2b = (_rb(_rb(_rb(xc - st["mu"]) * st["inv"]) * mod_c(4, c))
                   + mod_c(3, c)).astype(BF)
            h2 = h2b.astype(F32)
            ho_v[0, pl.ds(row0, 8), pl.ds(c * CW, CW)] = h2b
            o = xc + mod_c(5, c) * h2
            ho_v[1, pl.ds(row0, 8), pl.ds(c * CW, CW)] = o.astype(BF)
            rp = h2 * mod_c(6, c)
            st["r"] = rp if c == 0 else st["r"] + rp
            if c == D // CW - 1:
                r = jnp.sum(st["r"], axis=-1, keepdims=True)
                if scores_out is not None:
                    scores_out.append(r)
                    return None
                grp = row0 // 8
                lanes = lax.broadcasted_iota(jnp.int32, (8, 128), 1)
                r_v[grp // 128] = jnp.where(lanes == grp % 128, r, r_v[grp // 128])
            return token(o + st["r"])
        return [head] + [functools.partial(chunk, c) for c in range(D // CW)]

    def ln1_work(row0):
        st = {}

        def head(trig):
            st["x"] = after(x_v[pl.ds(row0, 8), :].astype(F32), trig)
            st["mu"], st["inv"] = ln_stats(st["x"])

        def chunk(c, trig):
            xc = after(st["x"][:, c * CW:(c + 1) * CW], trig)
            h = _rb(_rb(_rb(xc - st["mu"]) * st["inv"]) * mod_c(1, c)) + mod_c(0, c)
            ho_v[0, pl.ds(row0, 8), pl.ds(c * CW, CW)] = h.astype(BF)
            return token(h)
        return [head] + [functools.partial(chunk, c) for c in range(D // CW)]

    for cp in small_copies:
        cp.start()
    x0_copy.start()
    wmod_copy(0, 2).start()

    r_v[...] = jnp.full(r_v.shape, NEG, F32)
    att_v[...] = jnp.zeros(att_v.shape, BF)

    for cp in small_copies:
        cp.wait()
    mod_v[6] = jnp.broadcast_to(wr_v[...].astype(F32), (8, D))
    cf = c_v[...].astype(F32)
    sil = (cf * jax.nn.sigmoid(cf)).astype(BF)
    sc = jnp.broadcast_to(sil, (16, D))
    for k in range(8):
        sb_v[pl.ds(128 * k, 128), :] = jnp.broadcast_to(
            sil[:, 128 * k:128 * k + 128].astype(F32), (128, 128)).T

    x0_copy.wait()
    wmod_copy(2, 3).start()

    LNB = X0 // 4

    def ln0(i, carry):
        r0 = pl.multiple_of(i * LNB, 8)
        h_v[pl.ds(r0, LNB), :] = _b2(_layernorm(_f3(x_v[pl.ds(r0, LNB), :])))
        return carry
    lax.fori_loop(0, 4, ln0, 0)

    piece_copy(0, 0, 0, 256).start()
    piece_copy(0, 1, 256, 256).start()

    def mod_slab(k):
        y = _rb(jnp.dot(sc, wmod_v[k], preferred_element_type=F32)[0:8])
        if k // 2 == 1:
            y = _rb(1.0 + y)
        mod_v[k // 2, :, pl.ds((k % 2) * 512, 512)] = y

    def modulate_half(half):
        cols = pl.ds(half * 512, 512)

        def f(r0, n):
            ln = h_v[pl.ds(r0, n), cols].astype(F32).reshape(n // 8, 8, 512)
            h = _rb(ln * mod_v[1, :, cols]) + mod_v[0, :, cols]
            return h.reshape(n, 512).astype(BF)

        def mod0(i, carry):
            hp_v[pl.ds(pl.multiple_of(i * 128, 128), 128), cols] = pltpu.bitcast(
                f(pl.multiple_of(i * 256, 256), 256), U32)
            return carry
        lax.fori_loop(0, BULK // 256, mod0, 0)
        ho_v[0, pl.ds(BULK, RIDE), cols] = f(BULK, RIDE)

    wmod_copy(0, 2).wait()
    mod_slab(0)
    wmod_copy(2, 3).wait()
    mod_slab(2)
    modulate_half(0)
    piece_copy(0, 0, 0, 256).wait()
    piece_copy(1, 4, 0, 512).start()
    relayout_loop(0, 0, 0, 256)
    wmod_copy(1, 2).start()
    piece_copy(0, 1, 256, 256).wait()
    relayout_loop(0, 0, 256, 256)

    def mod_rows(slab, r0, n, acc):
        for r in range(r0, r0 + n, 8):
            sv = sb_v[pl.ds(r, 8), :]
            t = wmod_v[slab, pl.ds(r, 8), :].astype(F32) * jnp.concatenate([sv] * 4, axis=1)
            acc = t if acc is None else acc + t
        return acc

    def bulk_w(i, k, half=None):
        lo, n = (0, 512) if half is None else (256 * half, 256)
        return pltpu.bitcast(
            wqkv_v[pl.ds(pl.multiple_of((8 * i + k) * PITCH + lo, 8), n), :], BF)

    def bulk_dot(i, k, never, rl=None, md=None, half=None, w=None):
        tiles = range(8) if half is None else range(4 * half, 4 * half + 4)
        if w is None:
            w = bulk_w(i, k, half)
        cols = [hp_v[:, pl.ds(128 * c, 128)] for c in tiles]
        if rl is not None:
            slot, t, lo2 = rl
            spots = [12 + 6 * q if half is None else 4 + 3 * q for q in range(8)]
            toks = {sp: relayout(slot, t, lo2 + 8 * q, 16) for q, sp in enumerate(spots)}
            if md is not None:
                for q, sp in enumerate(spots):
                    md[1] = mod_rows(md[0], 128 * k + 16 * q, 16, md[1])
                    toks[sp] = toks[sp] ^ token(md[1][:, :256] + md[1][:, 256:])
            for c in range(0, len(tiles), 4):
                cols[c] = jnp.concatenate(
                    [jnp.where(never, toks[8 * c + j], cols[c][8 * j:8 * j + 8])
                     if 8 * c + j in toks else cols[c][8 * j:8 * j + 8]
                     for j in range(32)], axis=0)
        hb = pltpu.bitcast(jnp.concatenate(cols, axis=1), BF)
        y = jnp.dot(hb, w, preferred_element_type=F32)
        if half == 0:
            part_v[i, k] = y
            return
        if half == 1:
            y = y + part_v[i, k]
        ring[k][i, pl.ds(RING - BULK, BULK), :] = y.astype(BF)

    def bulk_a(a, carry):
        never = jnp.full((8, 128), a, jnp.int32) < 0
        for k in range(4):
            bulk_dot(a, k, never, half=0)

        @pl.when(a == 0)
        def _():
            piece_copy(0, 5, 512, 512).start()

        @pl.when(a == 1)
        def _():
            piece_copy(1, 4, 512, 512).start()
        lo = pl.multiple_of(512 * a, 512)
        stage_wait(1 - a, 4 + a, lo, 512)
        w = bulk_w(a, 4, 0)
        for k in range(4, 8):
            w_next = bulk_w(a, k + 1, 0) if k < 7 else None
            bulk_dot(a, k, never, (1 - a, 1 - a, 256 * a + 64 * (k - 4)), half=0, w=w)
            w = w_next

        @pl.when(a == 0)
        def _():
            wmod_copy(3, 3).start()
        return carry
    lax.fori_loop(0, 2, bulk_a, 0)

    piece_copy(2, 0, 0, 512).start()
    wmod_copy(1, 2).wait()
    wmod_copy(3, 3).wait()
    mod_slab(1)
    mod_slab(3)
    modulate_half(1)

    def bulk_b(b, carry):
        never = jnp.full((8, 128), b, jnp.int32) < 0

        @pl.when(b == 1)
        def _():
            piece_copy(2, 0, 0, 512).wait()
        for k in range(4):
            bulk_dot(b, k, never, (1 - b, 1 + b, 64 * k), half=1)

        @pl.when(b == 0)
        def _():
            piece_copy(2, 1, 512, 512).start()
        stage_wait(1 - b, 4 - 3 * b, 512, 512)
        for k in range(4, 8):
            bulk_dot(b, k, never, (1 - b, 1 + b, 64 * k), half=1)

        @pl.when(b == 0)
        def _():
            piece_copy(3, 5).start()
        return carry
    lax.fori_loop(0, 2, bulk_b, 0)

    def bulk_qkv(i, carry):
        @pl.when(i < 11)
        def _():
            stage_wait((i + 1) % 2, 4 + (i + 1) % 2)

        @pl.when((i >= 3) & (i < 11))
        def _():
            wmod_copy(i + 1, 2 + (i + 1) % 2).wait()

        for j in range(2, 10):
            @pl.when(i == j)
            def _():
                piece_copy(j + 2, 4 + j % 2).start()

        t = jnp.minimum(i + 1, 11)
        never = jnp.full((8, 128), i, jnp.int32) < 0
        md = [t, None]
        for k in range(8):
            bulk_dot(i, k, never, (t % 2, t, k * 64), md)
        macc_v[t] = md[1]

        for j in range(2, 10):
            @pl.when(i == j)
            def _():
                if j < 9:
                    wmod_copy(j + 3, 2 + (j + 3) % 2).start()
                    mid_copies[j - 2].start()
                else:
                    for cp in mid_copies[7:]:
                        cp.start()
        return carry
    wmod_copy(4, 2).start()
    lax.fori_loop(2, 12, bulk_qkv, 0)

    for k in range(4, 12):
        y = _rb(jnp.sum(macc_v[k], axis=0, keepdims=True))
        if k // 2 == 4:
            y = _rb(1.0 + y)
        mod_v[k // 2, :, pl.ds((k % 2) * 512, 512)] = jnp.broadcast_to(y, (8, 512))
    for cp in mid_copies:
        cp.wait()
    x2_copy.start()
    for cp in ffn_copies:
        cp.start()

    scale = DH ** -0.5
    kk = lax.broadcasted_iota(jnp.int32, (M + SEG, 80), 0)
    cc = lax.broadcasted_iota(jnp.int32, (M + SEG, 80), 1)
    second = ((cc >= 8) & (cc < 16)) | (cc >= 48)
    allowed = (cc < 16) | (kk <= jnp.where(second, cc - 40, cc - 8))

    def over_keys(f, fr, v):
        t = v[0:8]
        for j in range(8, M + SEG, 8):
            t = f(t, v[j:j + 8])
        return fr(t, axis=0, keepdims=True)

    def tied(u, never, toks):
        if not toks:
            return u
        parts, at = [], 0
        for j, tk in enumerate(toks):
            r = 64 * j
            if r > at:
                parts.append(u[at:r])
            w = tk.shape[1]
            sel = jnp.where(never[:, :w], tk, u[r:r + 8, :w])
            parts.append(sel if w == 128 else jnp.concatenate([sel, u[r:r + 8, w:]], axis=1))
            at = r + 8
        return jnp.concatenate(parts + [u[at:]], axis=0)

    def w_slab(t, g, lo=0, n=512, never=None, toks=()):
        return pltpu.bitcast(
            tied(wqkv_v[pl.ds((8 * t + g) * PITCH + lo, n), :], never, toks), BF)

    def step(s, mem, chained, left, att_prev):
        odd = left is not None
        wr = pl.multiple_of(lax.rem(RIDE * s, RING), 8)
        rd = pl.multiple_of(lax.rem(SEG * s + RING - BULK, RING), SEG)
        xin = jnp.concatenate(
            [mem, ho_v[0, pl.ds(pl.multiple_of(BULK + RIDE * s, 8), RIDE), :]], axis=0)

        prow = SEG * (s - 1) if odd else jnp.maximum(SEG * s - 40, 0)
        nrow = BULK + RIDE * jnp.minimum(s + 1, NSEG - 1)
        works = [post_work(pl.multiple_of(prow + 8 * q, 8), functools.partial(att_prev, q))
                 for q in range(3 if odd else 5)]
        works += [ln1_work(pl.multiple_of(nrow + 8 * q, 8)) for q in range(RIDE // 8)]
        never = jnp.full((8, 128), s, jnp.int32) < 0
        gap = (SIDE_END - SIDE0 - SIDE_LAT - SIDE_DUE) // len(works)
        sched = {}
        for q, wk in enumerate(works):
            sched.setdefault(SIDE0 + gap * q, []).append(wk[0])
            for c in range(1, len(wk)):
                sched.setdefault(SIDE0 + SIDE_LAT + gap * q + ((c - 1) * gap) // 4,
                                 []).append(wk[c])

        memqkv, probs, wl, new_left, toks = {}, {}, {}, {}, {}
        acc = []
        chain = []

        ndot = [0]

        def proj(g, t_lo, t_hi):
            part = {}
            if chained and ndot[0] == 0:
                for t in range(t_lo, t_lo + 6):
                    part[t] = jnp.dot(xin[:, :512], w_slab(t, g, 0, 256),
                                      preferred_element_type=F32)
            for t0 in range(t_lo, t_hi, 2):
                ys = []
                for t in (t0, t0 + 1):
                    n = ndot[0]
                    ndot[0] += 1
                    if t in part:
                        y = jnp.dot(xin[:, 512:], w_slab(t, g, 256, 256),
                                    preferred_element_type=F32) + part[t]
                    else:
                        y = jnp.dot(xin, w_slab(t, g, 0, 512, never, toks.get(n)),
                                    preferred_element_type=F32)
                    ring[g][t, pl.ds(wr, RIDE), :] = y[M:].astype(BF)
                    ys.append(y[:M])
                    for item in sched.get(n, ()):
                        tk = item((never, y[:M]))
                        if tk is not None:
                            toks.setdefault(n + SIDE_DUE, []).append(tk)
                memqkv[(t0, g)] = jnp.concatenate(ys, axis=0).astype(BF)

        def cat(t0, g):
            return jnp.concatenate([memqkv[(t0, g)], ring[g][t0, pl.ds(rd, SEG), :],
                                    ring[g][t0 + 1, pl.ds(rd, SEG), :]], axis=0)

        def scores(g):
            for p in (0, 2):
                st = lax.dot_general(cat(4 + p, g), cat(p, g), (((1,), (1,)), ((), ())),
                                     preferred_element_type=F32)
                st = jnp.where(second, jnp.concatenate([st[8:16], st[48:80]], axis=0),
                               jnp.concatenate([st[0:8], st[16:48]], axis=0))
                if chain:
                    st = jnp.concatenate(
                        [jnp.where(never[:, :80], chain[-1], st[0:8]), st[8:]], axis=0)
                st = jnp.where(allowed, st * scale, -1e9)
                e = jnp.exp(st - over_keys(jnp.maximum, jnp.max, st))
                l = over_keys(jnp.add, jnp.sum, e)
                chain.append(jnp.broadcast_to(l, (8, 80)))
                rc = pl.reciprocal(l, approx=True)
                e = e * (rc * (2.0 - l * rc))
                e0 = jnp.where(second, 0.0, e)
                e1 = jnp.where(second, e, 0.0)
                probs[(p, g)] = jnp.concatenate(
                    [e0[:M], e1[:M], e0[M:], e1[M:]], axis=0).astype(BF)

        def pv(g):
            for p in (0, 2):
                o = lax.dot_general(probs[(p, g)], cat(8 + p, g), (((0,), (0,)), ((), ())),
                                    preferred_element_type=F32)
                for j in range(2):
                    om, ot = o[8 * j:8 * j + 8], o[16 + 32 * j:48 + 32 * j]
                    if odd:
                        rows = [om, left[(p + j, g)], ot]
                    else:
                        rows = [om, ot[:RIDE]]
                        new_left[(p + j, g)] = ot[RIDE:]
                    wl[(p + j, g)] = jnp.concatenate(rows, axis=0).astype(BF)

        def wo(g):
            a = jnp.concatenate([wl[(o, g)] for o in range(4)], axis=1)
            w = jnp.concatenate(
                [jnp.concatenate([wo_v[n, pl.ds((8 * o + PERM[g]) * DH, DH), :]
                                  for o in range(4)], axis=0) for n in range(2)], axis=1)
            y = jnp.dot(a, w, preferred_element_type=F32)
            acc[:] = [y if not acc else y + acc[0]]

        for op in ORDER.split():
            g = int(op[1])
            if op[0] in "qkvux":
                proj(g, *{"q": (0, 12), "k": (0, 8), "v": (8, 12), "u": (0, 10), "x": (10, 12)}[op[0]])
            else:
                {"s": scores, "p": pv, "w": wo}[op[0]](g)
        y = acc[0].astype(BF)
        return y[:M], y[M:], (None if odd else new_left)

    def out_copy(row0, n, k):
        return pltpu.make_async_copy(ho_v.at[1, pl.ds(row0, n), :],
                                     out_hbm.at[0, pl.ds(row0, n), :], sems.at[3 + k])

    OB = SEG * UNROLL

    def carried(q):
        return att_v[pl.ds(8 * q, 8), :]

    def steps(i, carry):
        @pl.when(i == 16 // UNROLL)
        def _():
            x2_copy.wait()

        @pl.when(i >= 3)
        def _():
            out_copy(pl.multiple_of((i - 3) * OB, OB), OB, i % 2).wait()

        mem, left, att_prev = mem_v[...], None, carried
        for u in range(UNROLL):
            mem, att, left = step(i * UNROLL + u, mem, u > 0, left, att_prev)
            att_prev = (lambda a: lambda q: a[8 * q:8 * q + 8])(att)
        mem_v[...] = mem
        att_v[...] = att

        @pl.when(i >= 1)
        def _():
            out_copy(pl.multiple_of((i - 1) * OB, OB), OB, i % 2).start()
        return carry
    lax.fori_loop(0, NSEG // UNROLL, steps, 0)

    for cp in ffn_copies:
        cp.wait()
    last = []
    for q in range(5):
        for item in post_work(S - 40 + 8 * q, functools.partial(carried, q), last):
            item(None)
    out_copy(S - OB, OB, 2).start()

    def top2(val, idx, valid):
        def reduce(f, v):
            v = f(v, axis=0, keepdims=True)
            return v if v.shape[1] == 1 else f(v, axis=1, keepdims=True)

        def argtop(ok):
            v = jnp.where(ok, val, -jnp.inf)
            m = reduce(jnp.max, v)
            return m, reduce(jnp.min, jnp.where(ok & (v >= m), idx, float(S)))
        m1, i1 = argtop(valid)
        return (m1, i1), argtop(valid & (idx != i1))

    sub1 = lax.broadcasted_iota(jnp.int32, (16, 128), 0)
    lan1 = lax.broadcasted_iota(jnp.int32, (16, 128), 1)
    idx = (sub1 // 8) * 1024 + lan1 * 8 + sub1 % 8
    c_a, c_b = top2(_rb(r_v[...].reshape(16, 128)), idx.astype(F32), idx < S - 40)
    sub2 = lax.broadcasted_iota(jnp.int32, (48, 1), 0)
    val2 = jnp.concatenate([_rb(r) for r in last] + [jnp.where(sub2[:8] == 0, c_a[0], c_b[0])],
                           axis=0)
    idx2 = jnp.where(sub2 < 40, (sub2 + (S - 40)).astype(F32),
                     jnp.where(sub2 == 40, c_a[1], c_b[1]))
    (m_a, i_a), (m_b, i_b) = top2(val2, idx2, sub2 < 42)
    i_a = i_a.astype(jnp.int32)
    i_b = i_b.astype(jnp.int32)
    ia = jnp.clip(i_a[0, 0], 0, S - 1)
    ib = jnp.clip(i_b[0, 0], 0, S - 1)
    blk_a = pl.multiple_of((ia // 8) * 8, 8)
    blk_b = pl.multiple_of((ib // 8) * 8, 8)

    def two(ref):
        return jnp.concatenate([ref[pl.ds(blk_a, 8), :], ref[pl.ds(blk_b, 8), :]], axis=0)

    hs = two(ho_v.at[0])
    g = _rb(jnp.dot(hs, wg_v[...], preferred_element_type=F32))
    u = _rb(jnp.dot(hs, wu_v[...], preferred_element_type=F32))
    act = (_rb(g * jax.nn.sigmoid(g)) * u).astype(BF)
    y = jnp.concatenate(
        [jnp.dot(act, wd_v[k], preferred_element_type=F32) for k in range(2)], axis=1)
    sub = lax.broadcasted_iota(jnp.int32, (16, 1), 0)
    rows = jnp.where(sub < 8, blk_a + sub, blk_b + sub - 8)
    gate = jnp.where(rows == ia, jax.nn.sigmoid(m_a),
                     jnp.where(rows == ib, jax.nn.sigmoid(m_b), 0.0))
    upd = jnp.where((rows == ia) | (rows == ib), y * gate, 0.0).reshape(2, 8, D)
    fin = _b2(_f3(two(ho_v.at[1])) + mod_v[5] * upd)

    for k in range(3):
        out_copy(S - (3 - k) * OB, OB, k).wait()
    ho_v[1, pl.ds(blk_a, 8), :] = fin[0:8]
    ho_v[1, pl.ds(blk_b, 8), :] = fin[8:16]
    out_copy(blk_a, 8, 0).start()

    @pl.when(blk_a != blk_b)
    def _():
        out_copy(blk_b, 8, 1).start()
        out_copy(blk_b, 8, 1).wait()
    out_copy(blk_a, 8, 0).wait()


@jax.jit
def pallas_adaLN_cond__memory_aug_recurrent_mem_tr__moe_arch_mod__prompt_kernel(
    A_x, A_mem0, A_Wq, A_Wk, A_Wv, A_Wo, A_seg_len, B_x, B_w_r, B_w_gate, B_w_up, B_w_down, c,
    w_mod,
):
    del B_x
    del A_seg_len
    assert A_x.shape == (1, S, D) and A_Wq.shape == (D, H, DH) and A_mem0.shape == (1, M, D)
    any_spec = pl.BlockSpec(memory_space=pl.ANY)
    scratch = [
        pltpu.VMEM((S, D), BF),
        pltpu.VMEM((X0, D), BF),
        pltpu.VMEM((BULK // 2, D), U32),
        pltpu.VMEM((40, D), BF),
        pltpu.VMEM((2, S, D), BF),
        pltpu.VMEM((96 * PITCH, 128), U32),
        pltpu.VMEM((2, H * DH, 512), BF),
        pltpu.VMEM((2, D, 8, 128), BF),
        pltpu.VMEM((12, D, 512), BF),
        pltpu.VMEM((D, FF), BF),
        pltpu.VMEM((D, FF), BF),
        pltpu.VMEM((2, FF, 512), BF),
        pltpu.VMEM((M, D), BF),
        pltpu.VMEM((1, D), BF),
        pltpu.VMEM((1, D), BF),
        pltpu.VMEM((7, 8, D), F32),
        pltpu.VMEM((2, 8, 128), F32),
        pltpu.VMEM((D, 128), F32),
        pltpu.VMEM((12, 8, 512), F32),
        pltpu.VMEM((2, 8, BULK, 128), F32),
        pltpu.SemaphoreType.DMA((6,)),
    ] + [pltpu.VMEM((12, RING, 128), BF)] * 8
    return pl.pallas_call(
        _kernel,
        out_shape=jax.ShapeDtypeStruct((1, S, D), BF),
        in_specs=[any_spec] * 12,
        out_specs=any_spec,
        scratch_shapes=scratch,
        compiler_params=pltpu.CompilerParams(vmem_limit_bytes=120 * 1024 * 1024),
    )(A_x, A_mem0, A_Wq, A_Wk, A_Wv, A_Wo.reshape(H * DH, D), B_w_r.reshape(1, D), B_w_gate,
      B_w_up, B_w_down, c, w_mod)
```

```python
import functools

import jax
import jax.numpy as jnp
from jax import lax
import jax.experimental.pallas as pl
import jax.experimental.pallas.tpu as pltpu

BF = jnp.bfloat16
F32 = jnp.float32
U32 = jnp.uint32

S = 2048
D = 1024
H = 32
DH = 128
M = 8
SEG = 32
NSEG = S // SEG
FF = 3584
RIDE = 24
BULK = S - RIDE * NSEG
X0 = BULK + 32
RING = 576
PITCH = 520
X1 = 1024
UNROLL = 4
EPS = 1e-5
SIDE0, SIDE_LAT, SIDE_DUE, SIDE_END = 2, 6, 6, 96
NEG = -3.0e38
ORDER = ("q0 q1 q2 q3 q4 q5 q6 s0 s1 s2 s3 s4 s5 q7 p0 p1 p2 p3 p4 p5 s6 s7 w0 w1 w2 p6 p7 w3 "
         "w4 w5 w6 w7")
PERM = (0, 2, 4, 6, 1, 3, 5, 7)


def _rb(v):
    return v.astype(BF).astype(F32)


def _layernorm(xf):
    mu = jnp.mean(xf, axis=-1, keepdims=True)
    dv = xf - mu
    var = jnp.mean(dv * dv, axis=-1, keepdims=True)
    sd = _rb(jnp.sqrt(_rb(_rb(var) + EPS)))
    return _rb(_rb(xf - _rb(mu)) * (1.0 / sd))


def _f3(v):
    return v.astype(F32).reshape(v.shape[0] // 8, 8, D)


def _b2(v):
    return v.reshape(v.shape[0] * 8, D).astype(BF)


def _kernel(x_hbm, mem0_hbm, wq_hbm, wk_hbm, wv_hbm, wo_hbm, wr_hbm, wg_hbm, wu_hbm, wd_hbm,
            c_hbm, wmod_hbm, out_hbm,
            x_v, h_v, hp_v, att_v, ho_v, wqkv_v, wo_v, stage, wmod_v,
            wg_v, wu_v, wd_v, mem_v, c_v, wr_v, mod_v, r_v, sb_v, macc_v,
            part_v, sems, *rings):
    w_hbm = (wq_hbm, wk_hbm, wv_hbm)
    ring = rings

    def piece_copy(t, sem, lo=0, n=D):
        return pltpu.make_async_copy(
            w_hbm[t // 4].at[pl.ds(lo, n), pl.ds((t % 4) * 8, 8), :],
            stage.at[t % 2, pl.ds(lo, n)], sems.at[sem])

    def stage_wait(slot, sem, lo=0, n=D):
        dst = stage.at[slot, pl.ds(lo, n)]
        pltpu.make_async_copy(dst, dst, sems.at[sem]).wait()

    def wmod_copy(k, sem):
        col = k * 512 if isinstance(k, int) else pl.multiple_of(k * 512, 512)
        return pltpu.make_async_copy(wmod_hbm.at[:, pl.ds(col, 512)], wmod_v.at[k], sems.at[sem])

    def x_copy(lo, hi, sem):
        return pltpu.make_async_copy(x_hbm.at[0, pl.ds(lo, hi - lo), :],
                                     x_v.at[pl.ds(lo, hi - lo), :], sems.at[sem])

    def wo_copy(n):
        lo, rows = ((n // 2) * 512, 512) if n < 6 else (1536, 2560)
        return pltpu.make_async_copy(wo_hbm.at[pl.ds(lo, rows), pl.ds((n % 2) * 512, 512)],
                                     wo_v.at[n % 2, pl.ds(lo, rows)], sems.at[0])

    small_copies = [pltpu.make_async_copy(c_hbm, c_v, sems.at[0]),
                    pltpu.make_async_copy(mem0_hbm.at[0], mem_v, sems.at[0]),
                    pltpu.make_async_copy(wr_hbm, wr_v, sems.at[0])]
    x0_copy = x_copy(0, X0, 1)
    mid_copies = ([x_copy(X0, (X0 + X1) // 2, 0), x_copy((X0 + X1) // 2, X1, 0)]
                  + [wo_copy(n) for n in range(8)])
    x2_copy = x_copy(X1, S, 1)
    ffn_copies = [pltpu.make_async_copy(wg_hbm, wg_v, sems.at[2]),
                  pltpu.make_async_copy(wu_hbm, wu_v, sems.at[2])] + [
        pltpu.make_async_copy(wd_hbm.at[:, pl.ds(k * 512, 512)], wd_v.at[k], sems.at[2])
        for k in range(2)]

    def relayout(slot, t, lo2, n):
        base = t * (8 * PITCH) + lo2
        u = pltpu.bitcast(stage[slot, pl.ds(2 * lo2, n)], U32)
        tok = None
        for i in range(n // 2):
            a = u[2 * i]
            b = u[2 * i + 1]
            even = (a & jnp.uint32(0xFFFF)) | (b << 16)
            odd = (a >> 16) | (b & jnp.uint32(0xFFFF0000))
            wqkv_v[pl.ds(base + i, 4, stride=PITCH), :] = even
            wqkv_v[pl.ds(base + 4 * PITCH + i, 4, stride=PITCH), :] = odd
            tok = even ^ odd if tok is None else tok ^ even ^ odd
        return jnp.concatenate([tok, tok], axis=0)

    def relayout_loop(slot, t, lo, n):
        def body(i, carry):
            relayout(slot, t, lo // 2 + i * 64, 128)
            return carry
        lax.fori_loop(0, n // 128, body, 0)

    CW = 256

    def ln_stats(xf):
        mu = jnp.mean(xf, axis=-1, keepdims=True)
        dv = xf - mu
        var = jnp.mean(dv * dv, axis=-1, keepdims=True)
        sd = _rb(jnp.sqrt(_rb(_rb(var) + EPS)))
        return _rb(mu), 1.0 / sd

    def mod_c(k, c):
        return mod_v[k, :, pl.ds(c * CW, CW)]

    def token(v):
        return pltpu.bitcast(v[:, :128] + v[:, 128:], U32)

    def after(v, trig):
        if trig is None:
            return v
        return jnp.concatenate([jnp.where(trig[0], trig[1], v[:, :128]), v[:, 128:]], axis=1)

    def post_work(row0, att, scores_out=None):
        st = {}

        def head(trig):
            a = after(att().astype(F32), trig)
            st["x2"] = _rb(x_v[pl.ds(row0, 8), :].astype(F32) + _rb(mod_v[2] * a))
            st["mu"], st["inv"] = ln_stats(st["x2"])

        def chunk(c, trig):
            xc = after(st["x2"][:, c * CW:(c + 1) * CW], trig)
            h2b = (_rb(_rb(_rb(xc - st["mu"]) * st["inv"]) * mod_c(4, c))
                   + mod_c(3, c)).astype(BF)
            h2 = h2b.astype(F32)
            ho_v[0, pl.ds(row0, 8), pl.ds(c * CW, CW)] = h2b
            o = xc + mod_c(5, c) * h2
            ho_v[1, pl.ds(row0, 8), pl.ds(c * CW, CW)] = o.astype(BF)
            rp = h2 * mod_c(6, c)
            st["r"] = rp if c == 0 else st["r"] + rp
            if c == D // CW - 1:
                r = jnp.sum(st["r"], axis=-1, keepdims=True)
                if scores_out is not None:
                    scores_out.append(r)
                    return None
                grp = row0 >> 3
                lanes = lax.broadcasted_iota(jnp.int32, (8, 128), 1)
                r_v[grp >> 7] = jnp.where(lanes == (grp & 127), r, r_v[grp >> 7])
            return token(o + st["r"])
        return [head] + [functools.partial(chunk, c) for c in range(D // CW)]

    def ln1_work(row0):
        st = {}

        def head(trig):
            st["x"] = after(x_v[pl.ds(row0, 8), :].astype(F32), trig)
            st["mu"], st["inv"] = ln_stats(st["x"])

        def chunk(c, trig):
            xc = after(st["x"][:, c * CW:(c + 1) * CW], trig)
            h = _rb(_rb(_rb(xc - st["mu"]) * st["inv"]) * mod_c(1, c)) + mod_c(0, c)
            ho_v[0, pl.ds(row0, 8), pl.ds(c * CW, CW)] = h.astype(BF)
            return token(h)
        return [head] + [functools.partial(chunk, c) for c in range(D // CW)]

    for cp in small_copies:
        cp.start()
    x0_copy.start()
    wmod_copy(0, 2).start()

    r_v[...] = jnp.full(r_v.shape, NEG, F32)
    att_v[...] = jnp.zeros(att_v.shape, BF)

    for cp in small_copies:
        cp.wait()
    mod_v[6] = jnp.broadcast_to(wr_v[...].astype(F32), (8, D))
    cf = c_v[...].astype(F32)
    sil = (cf * jax.nn.sigmoid(cf)).astype(BF)
    sc = jnp.broadcast_to(sil, (16, D))
    for k in range(8):
        sb_v[pl.ds(128 * k, 128), :] = jnp.broadcast_to(
            sil[:, 128 * k:128 * k + 128].astype(F32), (128, 128)).T

    x0_copy.wait()
    wmod_copy(2, 3).start()

    LNB = X0 // 4

    def ln0(i, carry):
        r0 = pl.multiple_of(i * LNB, 8)
        h_v[pl.ds(r0, LNB), :] = _b2(_layernorm(_f3(x_v[pl.ds(r0, LNB), :])))
        return carry
    lax.fori_loop(0, 4, ln0, 0)

    piece_copy(0, 0, 0, 256).start()
    piece_copy(0, 1, 256, 256).start()

    def mod_slab(k):
        y = _rb(jnp.dot(sc, wmod_v[k], preferred_element_type=F32)[0:8])
        if k // 2 == 1:
            y = _rb(1.0 + y)
        mod_v[k // 2, :, pl.ds((k % 2) * 512, 512)] = y

    def modulate_half(half):
        cols = pl.ds(half * 512, 512)

        def f(r0, n):
            ln = h_v[pl.ds(r0, n), cols].astype(F32).reshape(n // 8, 8, 512)
            h = _rb(ln * mod_v[1, :, cols]) + mod_v[0, :, cols]
            return h.reshape(n, 512).astype(BF)

        def mod0(i, carry):
            hp_v[pl.ds(pl.multiple_of(i * 128, 128), 128), cols] = pltpu.bitcast(
                f(pl.multiple_of(i * 256, 256), 256), U32)
            return carry
        lax.fori_loop(0, BULK // 256, mod0, 0)
        ho_v[0, pl.ds(BULK, RIDE), cols] = f(BULK, RIDE)

    wmod_copy(0, 2).wait()
    mod_slab(0)
    wmod_copy(2, 3).wait()
    mod_slab(2)
    modulate_half(0)
    piece_copy(0, 0, 0, 256).wait()
    piece_copy(1, 4, 0, 512).start()
    relayout_loop(0, 0, 0, 256)
    wmod_copy(1, 2).start()
    piece_copy(0, 1, 256, 256).wait()
    relayout_loop(0, 0, 256, 256)

    def mod_rows(slab, r0, n, acc):
        for r in range(r0, r0 + n, 8):
            sv = sb_v[pl.ds(r, 8), :]
            t = wmod_v[slab, pl.ds(r, 8), :].astype(F32) * jnp.concatenate([sv] * 4, axis=1)
            acc = t if acc is None else acc + t
        return acc

    def bulk_w(i, k, half=None):
        lo, n = (0, 512) if half is None else (256 * half, 256)
        return pltpu.bitcast(
            wqkv_v[pl.ds(pl.multiple_of((8 * i + k) * PITCH + lo, 8), n), :], BF)

    def bulk_dot(i, k, never, rl=None, md=None, half=None, w=None):
        tiles = range(8) if half is None else range(4 * half, 4 * half + 4)
        if w is None:
            w = bulk_w(i, k, half)
        cols = [hp_v[:, pl.ds(128 * c, 128)] for c in tiles]
        if rl is not None:
            slot, t, lo2 = rl
            spots = [12 + 6 * q if half is None else 4 + 3 * q for q in range(8)]
            toks = {sp: relayout(slot, t, lo2 + 8 * q, 16) for q, sp in enumerate(spots)}
            if md is not None:
                for q, sp in enumerate(spots):
                    md[1] = mod_rows(md[0], 128 * k + 16 * q, 16, md[1])
                    toks[sp] = toks[sp] ^ token(md[1][:, :256] + md[1][:, 256:])
            for c in range(0, len(tiles), 4):
                cols[c] = jnp.concatenate(
                    [jnp.where(never, toks[8 * c + j], cols[c][8 * j:8 * j + 8])
                     if 8 * c + j in toks else cols[c][8 * j:8 * j + 8]
                     for j in range(32)], axis=0)
        hb = pltpu.bitcast(jnp.concatenate(cols, axis=1), BF)
        y = jnp.dot(hb, w, preferred_element_type=F32)
        if half == 0:
            part_v[i, k] = y
            return
        if half == 1:
            y = y + part_v[i, k]
        ring[k][i, pl.ds(RING - BULK, BULK), :] = y.astype(BF)

    def bulk_a(a, carry):
        never = jnp.full((8, 128), a, jnp.int32) < 0
        for k in range(4):
            bulk_dot(a, k, never, half=0)

        @pl.when(a == 0)
        def _():
            piece_copy(0, 5, 512, 512).start()

        @pl.when(a == 1)
        def _():
            piece_copy(1, 4, 512, 512).start()
        lo = pl.multiple_of(512 * a, 512)
        stage_wait(1 - a, 4 + a, lo, 512)
        w = bulk_w(a, 4, 0)
        for k in range(4, 8):
            w_next = bulk_w(a, k + 1, 0) if k < 7 else None
            bulk_dot(a, k, never, (1 - a, 1 - a, 256 * a + 64 * (k - 4)), half=0, w=w)
            w = w_next

        @pl.when(a == 0)
        def _():
            wmod_copy(3, 3).start()
        return carry
    lax.fori_loop(0, 2, bulk_a, 0)

    piece_copy(2, 0, 0, 512).start()
    wmod_copy(1, 2).wait()
    wmod_copy(3, 3).wait()
    mod_slab(1)
    mod_slab(3)
    modulate_half(1)

    def bulk_b(b, carry):
        never = jnp.full((8, 128), b, jnp.int32) < 0

        @pl.when(b == 1)
        def _():
            piece_copy(2, 0, 0, 512).wait()
        for k in range(4):
            bulk_dot(b, k, never, (1 - b, 1 + b, 64 * k), half=1)

        @pl.when(b == 0)
        def _():
            piece_copy(2, 1, 512, 512).start()
        stage_wait(1 - b, 4 - 3 * b, 512, 512)
        for k in range(4, 8):
            bulk_dot(b, k, never, (1 - b, 1 + b, 64 * k), half=1)

        @pl.when(b == 0)
        def _():
            piece_copy(3, 5).start()
        return carry
    lax.fori_loop(0, 2, bulk_b, 0)

    def bulk_qkv(i, carry):
        @pl.when(i < 11)
        def _():
            stage_wait((i + 1) & 1, 4 + ((i + 1) & 1))

        @pl.when((i >= 3) & (i < 11))
        def _():
            wmod_copy(i + 1, 2 + ((i + 1) & 1)).wait()

        for j in range(2, 10):
            @pl.when(i == j)
            def _():
                piece_copy(j + 2, 4 + j % 2).start()

        t = jnp.minimum(i + 1, 11)
        never = jnp.full((8, 128), i, jnp.int32) < 0
        md = [t, None]
        for k in range(8):
            bulk_dot(i, k, never, (t & 1, t, k * 64), md)
        macc_v[t] = md[1]

        for j in range(2, 10):
            @pl.when(i == j)
            def _():
                if j < 9:
                    wmod_copy(j + 3, 2 + (j + 3) % 2).start()
                    mid_copies[j - 2].start()
                else:
                    for cp in mid_copies[7:]:
                        cp.start()
        return carry
    wmod_copy(4, 2).start()
    lax.fori_loop(2, 12, bulk_qkv, 0)

    for k in range(4, 12):
        y = _rb(jnp.sum(macc_v[k], axis=0, keepdims=True))
        if k // 2 == 4:
            y = _rb(1.0 + y)
        mod_v[k // 2, :, pl.ds((k % 2) * 512, 512)] = jnp.broadcast_to(y, (8, 512))
    for cp in mid_copies:
        cp.wait()
    x2_copy.start()
    for cp in ffn_copies:
        cp.start()

    scale = DH ** -0.5
    kk = lax.broadcasted_iota(jnp.int32, (M + SEG, 80), 0)
    cc = lax.broadcasted_iota(jnp.int32, (M + SEG, 80), 1)
    second = ((cc >= 8) & (cc < 16)) | (cc >= 48)
    allowed = (cc < 16) | (kk <= jnp.where(second, cc - 40, cc - 8))

    def over_keys(f, fr, v):
        t = v[0:8]
        for j in range(8, M + SEG, 8):
            t = f(t, v[j:j + 8])
        return fr(t, axis=0, keepdims=True)

    def tied(u, never, toks):
        if not toks:
            return u
        parts, at = [], 0
        for j, tk in enumerate(toks):
            r = 64 * j
            if r > at:
                parts.append(u[at:r])
            w = tk.shape[1]
            sel = jnp.where(never[:, :w], tk, u[r:r + 8, :w])
            parts.append(sel if w == 128 else jnp.concatenate([sel, u[r:r + 8, w:]], axis=1))
            at = r + 8
        return jnp.concatenate(parts + [u[at:]], axis=0)

    def w_slab(t, g, lo=0, n=512, never=None, toks=()):
        return pltpu.bitcast(
            tied(wqkv_v[pl.ds((8 * t + g) * PITCH + lo, n), :], never, toks), BF)

    def step(s, mem, chained, left, att_prev):
        odd = left is not None
        wr = pl.multiple_of(lax.rem(RIDE * s, RING), 8)
        rd = pl.multiple_of(lax.rem(SEG * s + RING - BULK, RING), SEG)
        xin = jnp.concatenate(
            [mem, ho_v[0, pl.ds(pl.multiple_of(BULK + RIDE * s, 8), RIDE), :]], axis=0)

        prow = SEG * (s - 1) if odd else jnp.maximum(SEG * s - 40, 0)
        nrow = BULK + RIDE * jnp.minimum(s + 1, NSEG - 1)
        works = [post_work(pl.multiple_of(prow + 8 * q, 8), functools.partial(att_prev, q))
                 for q in range(3 if odd else 5)]
        works += [ln1_work(pl.multiple_of(nrow + 8 * q, 8)) for q in range(RIDE // 8)]
        never = jnp.full((8, 128), s, jnp.int32) < 0
        gap = (SIDE_END - SIDE0 - SIDE_LAT - SIDE_DUE) // len(works)
        sched = {}
        for q, wk in enumerate(works):
            sched.setdefault(SIDE0 + gap * q, []).append(wk[0])
            for c in range(1, len(wk)):
                sched.setdefault(SIDE0 + SIDE_LAT + gap * q + ((c - 1) * gap) // 4,
                                 []).append(wk[c])

        memqkv, probs, wl, new_left, toks = {}, {}, {}, {}, {}
        acc = []
        chain = []

        ndot = [0]

        def proj(g, t_lo, t_hi):
            part = {}
            if chained and ndot[0] == 0:
                for t in range(t_lo, t_lo + 6):
                    part[t] = jnp.dot(xin[:, :512], w_slab(t, g, 0, 256),
                                      preferred_element_type=F32)
            for t0 in range(t_lo, t_hi, 2):
                ys = []
                for t in (t0, t0 + 1):
                    n = ndot[0]
                    ndot[0] += 1
                    if t in part:
                        y = jnp.dot(xin[:, 512:], w_slab(t, g, 256, 256),
                                    preferred_element_type=F32) + part[t]
                    else:
                        y = jnp.dot(xin, w_slab(t, g, 0, 512, never, toks.get(n)),
                                    preferred_element_type=F32)
                    ring[g][t, pl.ds(wr, RIDE), :] = y[M:].astype(BF)
                    ys.append(y[:M])
                    for item in sched.get(n, ()):
                        tk = item((never, y[:M]))
                        if tk is not None:
                            toks.setdefault(n + SIDE_DUE, []).append(tk)
                memqkv[(t0, g)] = jnp.concatenate(ys, axis=0).astype(BF)

        def cat(t0, g):
            return jnp.concatenate([memqkv[(t0, g)], ring[g][t0, pl.ds(rd, SEG), :],
                                    ring[g][t0 + 1, pl.ds(rd, SEG), :]], axis=0)

        def scores(g):
            for p in (0, 2):
                st = lax.dot_general(cat(4 + p, g), cat(p, g), (((1,), (1,)), ((), ())),
                                     preferred_element_type=F32)
                st = jnp.where(second, jnp.concatenate([st[8:16], st[48:80]], axis=0),
                               jnp.concatenate([st[0:8], st[16:48]], axis=0))
                if chain:
                    st = jnp.concatenate(
                        [jnp.where(never[:, :80], chain[-1], st[0:8]), st[8:]], axis=0)
                st = jnp.where(allowed, st * scale, -1e9)
                e = jnp.exp(st - over_keys(jnp.maximum, jnp.max, st))
                l = over_keys(jnp.add, jnp.sum, e)
                chain.append(jnp.broadcast_to(l, (8, 80)))
                rc = pl.reciprocal(l, approx=True)
                e = e * (rc * (2.0 - l * rc))
                e0 = jnp.where(second, 0.0, e)
                e1 = jnp.where(second, e, 0.0)
                probs[(p, g)] = jnp.concatenate(
                    [e0[:M], e1[:M], e0[M:], e1[M:]], axis=0).astype(BF)

        def pv(g):
            for p in (0, 2):
                o = lax.dot_general(probs[(p, g)], cat(8 + p, g), (((0,), (0,)), ((), ())),
                                    preferred_element_type=F32)
                for j in range(2):
                    om, ot = o[8 * j:8 * j + 8], o[16 + 32 * j:48 + 32 * j]
                    if odd:
                        rows = [om, left[(p + j, g)], ot]
                    else:
                        rows = [om, ot[:RIDE]]
                        new_left[(p + j, g)] = ot[RIDE:]
                    wl[(p + j, g)] = jnp.concatenate(rows, axis=0).astype(BF)

        def wo(g):
            a = jnp.concatenate([wl[(o, g)] for o in range(4)], axis=1)
            w = jnp.concatenate(
                [jnp.concatenate([wo_v[n, pl.ds((8 * o + PERM[g]) * DH, DH), :]
                                  for o in range(4)], axis=0) for n in range(2)], axis=1)
            y = jnp.dot(a, w, preferred_element_type=F32)
            acc[:] = [y if not acc else y + acc[0]]

        for op in ORDER.split():
            g = int(op[1])
            if op[0] in "qkvux":
                proj(g, *{"q": (0, 12), "k": (0, 8), "v": (8, 12), "u": (0, 10), "x": (10, 12)}[op[0]])
            else:
                {"s": scores, "p": pv, "w": wo}[op[0]](g)
        y = acc[0].astype(BF)
        return y[:M], y[M:], (None if odd else new_left)

    def out_copy(row0, n, k):
        return pltpu.make_async_copy(ho_v.at[1, pl.ds(row0, n), :],
                                     out_hbm.at[0, pl.ds(row0, n), :], sems.at[3 + k])

    OB = SEG * UNROLL

    def carried(q):
        return att_v[pl.ds(8 * q, 8), :]

    def steps(i, carry):
        @pl.when(i == 16 // UNROLL)
        def _():
            x2_copy.wait()

        mem, left, att_prev = mem_v[...], None, carried
        for u in range(UNROLL):
            mem, att, left = step(i * UNROLL + u, mem, u > 0, left, att_prev)
            att_prev = (lambda a: lambda q: a[8 * q:8 * q + 8])(att)
        mem_v[...] = mem
        att_v[...] = att

        @pl.when(i >= 1)
        def _():
            out_copy(pl.multiple_of((i - 1) * OB, OB), OB, 0).start()
        return carry
    lax.fori_loop(0, NSEG // UNROLL, steps, 0)

    for cp in ffn_copies:
        cp.wait()
    last = []
    for q in range(5):
        for item in post_work(S - 40 + 8 * q, functools.partial(carried, q), last):
            item(None)
    out_copy(S - OB, OB, 0).start()

    def top2(val, idx, valid):
        def reduce(f, v):
            v = f(v, axis=0, keepdims=True)
            return v if v.shape[1] == 1 else f(v, axis=1, keepdims=True)

        def argtop(ok):
            v = jnp.where(ok, val, -jnp.inf)
            m = reduce(jnp.max, v)
            return m, reduce(jnp.min, jnp.where(ok & (v >= m), idx, float(S)))
        m1, i1 = argtop(valid)
        return (m1, i1), argtop(valid & (idx != i1))

    sub1 = lax.broadcasted_iota(jnp.int32, (16, 128), 0)
    lan1 = lax.broadcasted_iota(jnp.int32, (16, 128), 1)
    idx = (sub1 // 8) * 1024 + lan1 * 8 + sub1 % 8
    c_a, c_b = top2(_rb(r_v[...].reshape(16, 128)), idx.astype(F32), idx < S - 40)
    sub2 = lax.broadcasted_iota(jnp.int32, (48, 1), 0)
    val2 = jnp.concatenate([_rb(r) for r in last] + [jnp.where(sub2[:8] == 0, c_a[0], c_b[0])],
                           axis=0)
    idx2 = jnp.where(sub2 < 40, (sub2 + (S - 40)).astype(F32),
                     jnp.where(sub2 == 40, c_a[1], c_b[1]))
    (m_a, i_a), (m_b, i_b) = top2(val2, idx2, sub2 < 42)
    i_a = i_a.astype(jnp.int32)
    i_b = i_b.astype(jnp.int32)
    ia = jnp.clip(i_a[0, 0], 0, S - 1)
    ib = jnp.clip(i_b[0, 0], 0, S - 1)
    blk_a = pl.multiple_of((ia // 8) * 8, 8)
    blk_b = pl.multiple_of((ib // 8) * 8, 8)

    def two(ref):
        return jnp.concatenate([ref[pl.ds(blk_a, 8), :], ref[pl.ds(blk_b, 8), :]], axis=0)

    hs = two(ho_v.at[0])
    g = _rb(jnp.dot(hs, wg_v[...], preferred_element_type=F32))
    u = _rb(jnp.dot(hs, wu_v[...], preferred_element_type=F32))
    act = (_rb(g * jax.nn.sigmoid(g)) * u).astype(BF)
    y = jnp.concatenate(
        [jnp.dot(act, wd_v[k], preferred_element_type=F32) for k in range(2)], axis=1)
    sub = lax.broadcasted_iota(jnp.int32, (16, 1), 0)
    rows = jnp.where(sub < 8, blk_a + sub, blk_b + sub - 8)
    gate = jnp.where(rows == ia, jax.nn.sigmoid(m_a),
                     jnp.where(rows == ib, jax.nn.sigmoid(m_b), 0.0))
    upd = jnp.where((rows == ia) | (rows == ib), y * gate, 0.0).reshape(2, 8, D)
    fin = _b2(_f3(two(ho_v.at[1])) + mod_v[5] * upd)

    out_copy(0, S, 0).wait()
    ho_v[1, pl.ds(blk_a, 8), :] = fin[0:8]
    ho_v[1, pl.ds(blk_b, 8), :] = fin[8:16]
    out_copy(blk_a, 8, 0).start()

    @pl.when(blk_a != blk_b)
    def _():
        out_copy(blk_b, 8, 1).start()
        out_copy(blk_b, 8, 1).wait()
    out_copy(blk_a, 8, 0).wait()


@jax.jit
def pallas_adaLN_cond__memory_aug_recurrent_mem_tr__moe_arch_mod__prompt_kernel(
    A_x, A_mem0, A_Wq, A_Wk, A_Wv, A_Wo, A_seg_len, B_x, B_w_r, B_w_gate, B_w_up, B_w_down, c,
    w_mod,
):
    del B_x
    del A_seg_len
    assert A_x.shape == (1, S, D) and A_Wq.shape == (D, H, DH) and A_mem0.shape == (1, M, D)
    any_spec = pl.BlockSpec(memory_space=pl.ANY)
    scratch = [
        pltpu.VMEM((S, D), BF),
        pltpu.VMEM((X0, D), BF),
        pltpu.VMEM((BULK // 2, D), U32),
        pltpu.VMEM((40, D), BF),
        pltpu.VMEM((2, S, D), BF),
        pltpu.VMEM((96 * PITCH, 128), U32),
        pltpu.VMEM((2, H * DH, 512), BF),
        pltpu.VMEM((2, D, 8, 128), BF),
        pltpu.VMEM((12, D, 512), BF),
        pltpu.VMEM((D, FF), BF),
        pltpu.VMEM((D, FF), BF),
        pltpu.VMEM((2, FF, 512), BF),
        pltpu.VMEM((M, D), BF),
        pltpu.VMEM((1, D), BF),
        pltpu.VMEM((1, D), BF),
        pltpu.VMEM((7, 8, D), F32),
        pltpu.VMEM((2, 8, 128), F32),
        pltpu.VMEM((D, 128), F32),
        pltpu.VMEM((12, 8, 512), F32),
        pltpu.VMEM((2, 8, BULK, 128), F32),
        pltpu.SemaphoreType.DMA((6,)),
    ] + [pltpu.VMEM((12, RING, 128), BF)] * 8
    return pl.pallas_call(
        _kernel,
        out_shape=jax.ShapeDtypeStruct((1, S, D), BF),
        in_specs=[any_spec] * 12,
        out_specs=any_spec,
        scratch_shapes=scratch,
        compiler_params=pltpu.CompilerParams(vmem_limit_bytes=120 * 1024 * 1024),
    )(A_x, A_mem0, A_Wq, A_Wk, A_Wv, A_Wo.reshape(H * DH, D), B_w_r.reshape(1, D), B_w_gate,
      B_w_up, B_w_down, c, w_mod)
```

```python
import functools

import jax
import jax.numpy as jnp
from jax import lax
import jax.experimental.pallas as pl
import jax.experimental.pallas.tpu as pltpu

BF = jnp.bfloat16
F32 = jnp.float32
U32 = jnp.uint32

S = 2048
D = 1024
H = 32
DH = 128
M = 8
SEG = 32
NSEG = S // SEG
FF = 3584
RIDE = 24
BULK = S - RIDE * NSEG
X0 = BULK + 32
RING = 576
PITCH = 520
X1 = 1024
NP = 3
QK = D // 4
UNROLL = 4
EPS = 1e-5
SIDE0, SIDE_LAT, SIDE_DUE, SIDE_END = 2, 6, 6, 96
NEG = -3.0e38
ORDER = ("q0 q1 q2 q3 q4 q5 q6 s0 s1 s2 s3 s4 s5 q7 p0 p1 p2 p3 p4 p5 s6 s7 w0 w1 w2 p6 p7 w3 "
         "w4 w5 w6 w7")
PERM = (0, 2, 4, 6, 1, 3, 5, 7)


def _rb(v):
    return v.astype(BF).astype(F32)


def _layernorm(xf):
    mu = jnp.mean(xf, axis=-1, keepdims=True)
    dv = xf - mu
    var = jnp.mean(dv * dv, axis=-1, keepdims=True)
    sd = _rb(jnp.sqrt(_rb(_rb(var) + EPS)))
    return _rb(_rb(xf - _rb(mu)) * (1.0 / sd))


def _f3(v):
    return v.astype(F32).reshape(v.shape[0] // 8, 8, D)


def _b2(v):
    return v.reshape(v.shape[0] * 8, D).astype(BF)


def _kernel(x_hbm, mem0_hbm, wq_hbm, wk_hbm, wv_hbm, wo_hbm, wr_hbm, wg_hbm, wu_hbm, wd_hbm,
            c_hbm, wmod_hbm, out_hbm,
            x_v, h_v, hp_v, att_v, ho_v, wqkv_v, wo_v, stage, wmod_v,
            wg_v, wu_v, wd_v, mem_v, c_v, wr_v, mod_v, r_v, sb_v, macc_v,
            part_v, sems, *rings):
    w_hbm = (wq_hbm, wk_hbm, wv_hbm)
    ring = rings

    def piece_copy(t, sem, lo=0, n=D, dst=None):
        dst = (t % 2) * D + lo if dst is None else dst
        return pltpu.make_async_copy(
            w_hbm[t // 4].at[pl.ds(lo, n), pl.ds((t % 4) * 8, 8), :],
            stage.at[pl.ds(dst, n)], sems.at[sem])

    def unit_copy(j):
        return piece_copy(j % NP, 6 + min(j, 10) % 3, QK * (j // NP), QK, 2 * D + QK * j)

    def stage_wait(row, n, sem):
        dst = stage.at[pl.ds(row, n)]
        pltpu.make_async_copy(dst, dst, sems.at[sem]).wait()

    def mq_copy(q, part):
        return pltpu.make_async_copy(wmod_hbm.at[:, pl.ds(part * D + q * QK, QK)],
                                     wmod_v.at[q, :, pl.ds(part * QK, QK)], sems.at[2])

    def wmod_copy(k, sem):
        col = k * 512 if isinstance(k, int) else pl.multiple_of(k * 512, 512)
        return pltpu.make_async_copy(wmod_hbm.at[:, pl.ds(col, 512)], wmod_v.at[k], sems.at[sem])

    def x_copy(lo, hi, sem):
        return pltpu.make_async_copy(x_hbm.at[0, pl.ds(lo, hi - lo), :],
                                     x_v.at[pl.ds(lo, hi - lo), :], sems.at[sem])

    def wo_copy(n):
        lo, rows = ((n // 2) * 512, 512) if n < 6 else (1536, 2560)
        return pltpu.make_async_copy(wo_hbm.at[pl.ds(lo, rows), pl.ds((n % 2) * 512, 512)],
                                     wo_v.at[n % 2, pl.ds(lo, rows)], sems.at[0])

    small_copies = [pltpu.make_async_copy(c_hbm, c_v, sems.at[0]),
                    pltpu.make_async_copy(mem0_hbm.at[0], mem_v, sems.at[0]),
                    pltpu.make_async_copy(wr_hbm, wr_v, sems.at[0])]
    x0_copy = x_copy(0, X0, 1)
    mid_copies = ([x_copy(X0, (X0 + X1) // 2, 0), x_copy((X0 + X1) // 2, X1, 0)]
                  + [wo_copy(n) for n in range(8)])
    x2_copy = x_copy(X1, S, 1)
    ffn_copies = [pltpu.make_async_copy(wg_hbm, wg_v, sems.at[2]),
                  pltpu.make_async_copy(wu_hbm, wu_v, sems.at[2])] + [
        pltpu.make_async_copy(wd_hbm.at[:, pl.ds(k * 512, 512)], wd_v.at[k], sems.at[2])
        for k in range(2)]

    def relayout(src, base, n):
        u = pltpu.bitcast(stage[pl.ds(src, n)], U32)
        tok = None
        for i in range(n // 2):
            a = u[2 * i]
            b = u[2 * i + 1]
            even = (a & jnp.uint32(0xFFFF)) | (b << 16)
            odd = (a >> 16) | (b & jnp.uint32(0xFFFF0000))
            wqkv_v[pl.ds(base + i, 4, stride=PITCH), :] = even
            wqkv_v[pl.ds(base + 4 * PITCH + i, 4, stride=PITCH), :] = odd
            tok = even ^ odd if tok is None else tok ^ even ^ odd
        return jnp.concatenate([tok, tok], axis=0)

    CW = 256

    def ln_stats(xf):
        mu = jnp.mean(xf, axis=-1, keepdims=True)
        dv = xf - mu
        var = jnp.mean(dv * dv, axis=-1, keepdims=True)
        sd = _rb(jnp.sqrt(_rb(_rb(var) + EPS)))
        return _rb(mu), 1.0 / sd

    def mod_c(k, c):
        return mod_v[k, :, pl.ds(c * CW, CW)]

    def token(v):
        return pltpu.bitcast(v[:, :128] + v[:, 128:], U32)

    def after(v, trig):
        if trig is None:
            return v
        return jnp.concatenate([jnp.where(trig[0], trig[1], v[:, :128]), v[:, 128:]], axis=1)

    def post_work(row0, att, scores_out=None):
        st = {}

        def head(trig):
            a = after(att().astype(F32), trig)
            st["x2"] = _rb(x_v[pl.ds(row0, 8), :].astype(F32) + _rb(mod_v[2] * a))
            st["mu"], st["inv"] = ln_stats(st["x2"])

        def chunk(c, trig):
            xc = after(st["x2"][:, c * CW:(c + 1) * CW], trig)
            h2b = (_rb(_rb(_rb(xc - st["mu"]) * st["inv"]) * mod_c(4, c))
                   + mod_c(3, c)).astype(BF)
            h2 = h2b.astype(F32)
            ho_v[0, pl.ds(row0, 8), pl.ds(c * CW, CW)] = h2b
            o = xc + mod_c(5, c) * h2
            ho_v[1, pl.ds(row0, 8), pl.ds(c * CW, CW)] = o.astype(BF)
            rp = h2 * mod_c(6, c)
            st["r"] = rp if c == 0 else st["r"] + rp
            if c == D // CW - 1:
                r = jnp.sum(st["r"], axis=-1, keepdims=True)
                if scores_out is not None:
                    scores_out.append(r)
                    return None
                grp = row0 >> 3
                lanes = lax.broadcasted_iota(jnp.int32, (8, 128), 1)
                r_v[grp >> 7] = jnp.where(lanes == (grp & 127), r, r_v[grp >> 7])
            return token(o + st["r"])
        return [head] + [functools.partial(chunk, c) for c in range(D // CW)]

    def ln1_work(row0):
        st = {}

        def head(trig):
            st["x"] = after(x_v[pl.ds(row0, 8), :].astype(F32), trig)
            st["mu"], st["inv"] = ln_stats(st["x"])

        def chunk(c, trig):
            xc = after(st["x"][:, c * CW:(c + 1) * CW], trig)
            h = _rb(_rb(_rb(xc - st["mu"]) * st["inv"]) * mod_c(1, c)) + mod_c(0, c)
            ho_v[0, pl.ds(row0, 8), pl.ds(c * CW, CW)] = h.astype(BF)
            return token(h)
        return [head] + [functools.partial(chunk, c) for c in range(D // CW)]

    for cp in small_copies:
        cp.start()
    x0_copy.start()
    mq_copy(0, 0).start()

    r_v[...] = jnp.full(r_v.shape, NEG, F32)
    att_v[...] = jnp.zeros(att_v.shape, BF)

    for cp in small_copies:
        cp.wait()
    mod_v[6] = jnp.broadcast_to(wr_v[...].astype(F32), (8, D))
    cf = c_v[...].astype(F32)
    sil = (cf * jax.nn.sigmoid(cf)).astype(BF)
    sc = jnp.broadcast_to(sil, (16, D))
    for k in range(8):
        sb_v[pl.ds(128 * k, 128), :] = jnp.broadcast_to(
            sil[:, 128 * k:128 * k + 128].astype(F32), (128, 128)).T

    mq_copy(0, 1).start()
    x0_copy.wait()
    unit_copy(0).start()
    unit_copy(1).start()

    LNB = X0 // 4

    def ln0(i, carry):
        r0 = pl.multiple_of(i * LNB, 8)
        ln = _b2(_layernorm(_f3(x_v[pl.ds(r0, LNB), :])))
        for q in range(4):
            h_v[q, pl.ds(r0, LNB), :] = ln[:, q * QK:(q + 1) * QK]
        return carry
    lax.fori_loop(0, 4, ln0, 0)

    def shift_scale(acc):
        y = _rb(acc)
        return y[:, :QK], _rb(1.0 + y[:, QK:])

    def modulated(q, r0, n, sh, sca):
        ln = h_v[q, pl.ds(r0, n), :].astype(F32).reshape(n // 8, 8, QK)
        return (_rb(ln * sca) + sh).reshape(n, QK).astype(BF)

    for part in range(2):
        mq_copy(0, part).wait()
    acc0 = jnp.dot(sc, wmod_v[0], preferred_element_type=F32)[0:8]
    macc_v[0] = acc0
    hp_v[0] = pltpu.bitcast(modulated(0, 0, BULK, *shift_scale(acc0)), U32)
    unit_copy(0).wait()
    unit_copy(2).start()

    def relayout0(i, carry):
        relayout(2 * D + pl.multiple_of(i * 128, 128), i * 64, 128)
        return carry
    lax.fori_loop(0, QK // 128, relayout0, 0)
    mq_copy(1, 0).start()
    mq_copy(1, 1).start()
    unit_copy(3).start()

    def mod_rows(slab, r0, n, acc):
        for r in range(r0, r0 + n, 8):
            sv = sb_v[pl.ds(r, 8), :]
            t = wmod_v[slab, pl.ds(r, 8), :].astype(F32) * jnp.concatenate([sv] * 4, axis=1)
            acc = t if acc is None else acc + t
        return acc

    def tie_lhs(col, never, toks):
        return jnp.concatenate(
            [jnp.where(never, toks[j], col[8 * j:8 * j + 8]) if j in toks
             else col[8 * j:8 * j + 8] for j in range(32)], axis=0)

    def add_tok(toks, j, tk):
        toks[j] = tk if j not in toks else toks[j] ^ tk

    starts = {0: [unit_copy(4)], 1: [unit_copy(5), piece_copy(3, 5, 0, 256)],
              2: [unit_copy(6), mq_copy(2, 0), mq_copy(2, 1)],
              3: [unit_copy(7), piece_copy(3, 5, 256, 256)], 4: [unit_copy(8)],
              5: [unit_copy(9), mq_copy(3, 0), mq_copy(3, 1)],
              6: [unit_copy(10), unit_copy(11)], 7: [piece_copy(3, 3, 512, 512)],
              8: [piece_copy(4, 4)], 9: [], 10: [wmod_copy(4, 2)], 11: []}

    def quarter_block(b_lo, b_hi, b, carry):
        first, final = b_lo == 0, b_hi == 4 * NP
        q = b_lo // NP
        p = b - NP * q
        if final:
            src = jnp.where(p == 0, 2 * D + 10 * QK, D + 512 * (p - 1))
            sem = 7 - 2 * p
            stage_wait(pl.multiple_of(src, 512), 512, sem)
            b3 = 3 * 8 * PITCH + 256 * (p - 1)
            jobs = [(src, jnp.where(p == 0, 8 * PITCH + 384, b3)),
                    (src + QK, jnp.where(p == 0, 2 * 8 * PITCH + 384, b3 + 128))]
        else:
            src = 2 * D + QK * (b + 1)
            last = p == NP - 1
            stage_wait(pl.multiple_of(src, QK), QK, jnp.where(last, 6, 7 + p))
            jobs = [(src, jnp.where(last, 128 * (q + 1), (p + 1) * (8 * PITCH) + 128 * q))]

            @pl.when(last)
            def _():
                for part in range(2):
                    mq_copy(q + 1, part).wait()
            slab = jnp.where(last, q + 1, q)
        never = jnp.full((8, 128), b, jnp.int32) < 0

        def weights(k):
            return pltpu.bitcast(jnp.concatenate(
                [wqkv_v[pl.ds(pl.multiple_of((8 * p + kk) * PITCH + 128 * q, 8), 128), :]
                 for kk in (k, k + 1)], axis=1), BF)

        groups = [(s_ + 16 * g, d_ + 8 * g) for s_, d_ in jobs for g in range(QK // 16)]
        per = len(groups) // 4
        acc = None
        w = weights(0)
        for n, k in enumerate(range(0, 8, 2)):
            w_next = weights(k + 2) if k < 6 else None
            toks = {}
            for g in range(per):
                add_tok(toks, 4 + (g * 24) // per, relayout(*groups[n * per + g], 16))
            if not final and n < 2:
                for g in range(16):
                    acc = mod_rows(slab, 512 * n + 32 * g, 32, acc)
                    add_tok(toks, 2 * g + (n == 0), token(acc[:, :256] + acc[:, 256:]))
            if not final and n == 2:
                tot = jnp.broadcast_to(jnp.sum(acc, axis=0, keepdims=True), (8, 512))
                macc_v[q + 1] = tot
                sh, sca = shift_scale(tot)
            if not final and n >= 2:
                for g in range(16):
                    r0 = 256 * (n - 2) + 16 * g
                    hb = pltpu.bitcast(modulated(q + 1, r0, 16, sh, sca), U32)
                    hp_v[q + 1, pl.ds(r0 // 2, 8), :] = hb
                    add_tok(toks, (8 + (g * 3) // 2) if n == 2 else 2 * g,
                            hb[:, :128] ^ hb[:, 128:])
            lhs = jnp.concatenate([tie_lhs(hp_v[q, :, pl.ds(0, 128)], never, toks),
                                   hp_v[q, :, pl.ds(128, 128)]], axis=1)
            y = jnp.dot(pltpu.bitcast(lhs, BF), w, preferred_element_type=F32)
            if not first:
                y = y + part_v[p, n]
            if final:
                for j in range(2):
                    ring[k + j][p, pl.ds(RING - BULK, BULK), :] = (
                        y[:, 128 * j:128 * j + 128].astype(BF))
            else:
                part_v[p, n] = y
            w = w_next

        for j in range(b_lo, b_hi):
            if starts[j]:
                @pl.when(b == j)
                def _():
                    for cp in starts[j]:
                        cp.start()
        return carry

    for b_lo, b_hi in ((0, NP), (NP, 2 * NP), (2 * NP, 3 * NP), (3 * NP, 4 * NP)):
        quarters = functools.partial(quarter_block, b_lo, b_hi)
        lax.fori_loop(b_lo, b_hi, quarters, 0)

    def bulk_dot(i, k, never, t, md):
        w = pltpu.bitcast(wqkv_v[pl.ds(pl.multiple_of((8 * i + k) * PITCH, 8), 512), :], BF)
        cols = [hp_v[c // 2, :, pl.ds(128 * (c % 2), 128)] for c in range(8)]
        toks = {}
        for g in range(8):
            tk = relayout((t & 1) * D + 128 * k + 16 * g, t * (8 * PITCH) + 64 * k + 8 * g, 16)
            md[1] = mod_rows(md[0], 128 * k + 16 * g, 16, md[1])
            toks[12 + 6 * g] = tk ^ token(md[1][:, :256] + md[1][:, 256:])
        cols[0] = tie_lhs(cols[0], never, toks)
        cols[4] = tie_lhs(cols[4], never, {j - 32: tk for j, tk in toks.items()})
        hb = pltpu.bitcast(jnp.concatenate(cols, axis=1), BF)
        y = jnp.dot(hb, w, preferred_element_type=F32)
        ring[k][i, pl.ds(RING - BULK, BULK), :] = y.astype(BF)

    def bulk_qkv(i, carry):
        @pl.when(i < 11)
        def _():
            par = (i + 1) & 1
            stage_wait(pl.multiple_of(par * D, D), D, 4 + par)

        @pl.when(i > NP)
        def _():
            wmod_copy(i, 2 + (i & 1)).wait()

        for j in range(NP, 10):
            @pl.when(i == j)
            def _():
                piece_copy(j + 2, 4 + j % 2).start()

        t = jnp.minimum(i + 1, 11)
        never = jnp.full((8, 128), i, jnp.int32) < 0
        md = [i, None]
        for k in range(8):
            bulk_dot(i, k, never, t, md)
        macc_v[jnp.maximum(i, 4)] = md[1]

        for j in range(NP, 10):
            @pl.when(i == j)
            def _():
                wmod_copy(j + 2, 2 + j % 2).start()
                if j < 9:
                    mid_copies[j - NP + 1].start()
                else:
                    for cp in mid_copies[7:]:
                        cp.start()
        return carry
    mid_copies[0].start()
    lax.fori_loop(NP, 12, bulk_qkv, 0)

    for q in range(4):
        sh, sca = shift_scale(macc_v[q])
        mod_v[0, :, pl.ds(q * QK, QK)] = sh
        mod_v[1, :, pl.ds(q * QK, QK)] = sca
        ho_v[0, pl.ds(BULK, RIDE), pl.ds(q * QK, QK)] = modulated(q, BULK, RIDE, sh, sca)
    for k in range(4, 12):
        y = _rb(jnp.sum(macc_v[k], axis=0, keepdims=True))
        if k // 2 == 4:
            y = _rb(1.0 + y)
        mod_v[k // 2, :, pl.ds((k % 2) * 512, 512)] = jnp.broadcast_to(y, (8, 512))
    for cp in mid_copies:
        cp.wait()
    x2_copy.start()
    for cp in ffn_copies:
        cp.start()

    scale = DH ** -0.5
    kk = lax.broadcasted_iota(jnp.int32, (M + SEG, 80), 0)
    cc = lax.broadcasted_iota(jnp.int32, (M + SEG, 80), 1)
    second = ((cc >= 8) & (cc < 16)) | (cc >= 48)
    allowed = (cc < 16) | (kk <= jnp.where(second, cc - 40, cc - 8))

    def over_keys(f, fr, v):
        t = v[0:8]
        for j in range(8, M + SEG, 8):
            t = f(t, v[j:j + 8])
        return fr(t, axis=0, keepdims=True)

    def tied(u, never, toks):
        if not toks:
            return u
        parts, at = [], 0
        for j, tk in enumerate(toks):
            r = 64 * j
            if r > at:
                parts.append(u[at:r])
            w = tk.shape[1]
            sel = jnp.where(never[:, :w], tk, u[r:r + 8, :w])
            parts.append(sel if w == 128 else jnp.concatenate([sel, u[r:r + 8, w:]], axis=1))
            at = r + 8
        return jnp.concatenate(parts + [u[at:]], axis=0)

    def w_slab(t, g, lo=0, n=512, never=None, toks=()):
        return pltpu.bitcast(
            tied(wqkv_v[pl.ds((8 * t + g) * PITCH + lo, n), :], never, toks), BF)

    def step(s, mem, chained, left, att_prev):
        odd = left is not None
        wr = pl.multiple_of(lax.rem(RIDE * s, RING), 8)
        rd = pl.multiple_of(lax.rem(SEG * s + RING - BULK, RING), SEG)
        xin = jnp.concatenate(
            [mem, ho_v[0, pl.ds(pl.multiple_of(BULK + RIDE * s, 8), RIDE), :]], axis=0)

        prow = SEG * (s - 1) if odd else jnp.maximum(SEG * s - 40, 0)
        nrow = BULK + RIDE * jnp.minimum(s + 1, NSEG - 1)
        works = [post_work(pl.multiple_of(prow + 8 * q, 8), functools.partial(att_prev, q))
                 for q in range(3 if odd else 5)]
        works += [ln1_work(pl.multiple_of(nrow + 8 * q, 8)) for q in range(RIDE // 8)]
        never = jnp.full((8, 128), s, jnp.int32) < 0
        gap = (SIDE_END - SIDE0 - SIDE_LAT - SIDE_DUE) // len(works)
        sched = {}
        for q, wk in enumerate(works):
            sched.setdefault(SIDE0 + gap * q, []).append(wk[0])
            for c in range(1, len(wk)):
                sched.setdefault(SIDE0 + SIDE_LAT + gap * q + ((c - 1) * gap) // 4,
                                 []).append(wk[c])

        memqkv, probs, wl, new_left, toks = {}, {}, {}, {}, {}
        acc = []
        chain = []

        ndot = [0]

        def proj(g, t_lo, t_hi):
            part = {}
            if chained and ndot[0] == 0:
                for t in range(t_lo, t_lo + 6):
                    part[t] = jnp.dot(xin[:, :512], w_slab(t, g, 0, 256),
                                      preferred_element_type=F32)
            for t0 in range(t_lo, t_hi, 2):
                ys = []
                for t in (t0, t0 + 1):
                    n = ndot[0]
                    ndot[0] += 1
                    if t in part:
                        y = jnp.dot(xin[:, 512:], w_slab(t, g, 256, 256),
                                    preferred_element_type=F32) + part[t]
                    else:
                        y = jnp.dot(xin, w_slab(t, g, 0, 512, never, toks.get(n)),
                                    preferred_element_type=F32)
                    ring[g][t, pl.ds(wr, RIDE), :] = y[M:].astype(BF)
                    ys.append(y[:M])
                    for item in sched.get(n, ()):
                        tk = item((never, y[:M]))
                        if tk is not None:
                            toks.setdefault(n + SIDE_DUE, []).append(tk)
                memqkv[(t0, g)] = jnp.concatenate(ys, axis=0).astype(BF)

        def cat(t0, g):
            return jnp.concatenate([memqkv[(t0, g)], ring[g][t0, pl.ds(rd, SEG), :],
                                    ring[g][t0 + 1, pl.ds(rd, SEG), :]], axis=0)

        def scores(g):
            for p in (0, 2):
                st = lax.dot_general(cat(4 + p, g), cat(p, g), (((1,), (1,)), ((), ())),
                                     preferred_element_type=F32)
                st = jnp.where(second, jnp.concatenate([st[8:16], st[48:80]], axis=0),
                               jnp.concatenate([st[0:8], st[16:48]], axis=0))
                if chain:
                    st = jnp.concatenate(
                        [jnp.where(never[:, :80], chain[-1], st[0:8]), st[8:]], axis=0)
                st = jnp.where(allowed, st * scale, -1e9)
                e = jnp.exp(st - over_keys(jnp.maximum, jnp.max, st))
                l = over_keys(jnp.add, jnp.sum, e)
                chain.append(jnp.broadcast_to(l, (8, 80)))
                rc = pl.reciprocal(l, approx=True)
                e = e * (rc * (2.0 - l * rc))
                e0 = jnp.where(second, 0.0, e)
                e1 = jnp.where(second, e, 0.0)
                probs[(p, g)] = jnp.concatenate(
                    [e0[:M], e1[:M], e0[M:], e1[M:]], axis=0).astype(BF)

        def pv(g):
            for p in (0, 2):
                o = lax.dot_general(probs[(p, g)], cat(8 + p, g), (((0,), (0,)), ((), ())),
                                    preferred_element_type=F32)
                for j in range(2):
                    om, ot = o[8 * j:8 * j + 8], o[16 + 32 * j:48 + 32 * j]
                    if odd:
                        rows = [om, left[(p + j, g)], ot]
                    else:
                        rows = [om, ot[:RIDE]]
                        new_left[(p + j, g)] = ot[RIDE:]
                    wl[(p + j, g)] = jnp.concatenate(rows, axis=0).astype(BF)

        def wo(g):
            a = jnp.concatenate([wl[(o, g)] for o in range(4)], axis=1)
            w = jnp.concatenate(
                [jnp.concatenate([wo_v[n, pl.ds((8 * o + PERM[g]) * DH, DH), :]
                                  for o in range(4)], axis=0) for n in range(2)], axis=1)
            y = jnp.dot(a, w, preferred_element_type=F32)
            acc[:] = [y if not acc else y + acc[0]]

        for op in ORDER.split():
            g = int(op[1])
            if op[0] in "qkvux":
                proj(g, *{"q": (0, 12), "k": (0, 8), "v": (8, 12), "u": (0, 10), "x": (10, 12)}[op[0]])
            else:
                {"s": scores, "p": pv, "w": wo}[op[0]](g)
        y = acc[0].astype(BF)
        return y[:M], y[M:], (None if odd else new_left)

    def out_copy(row0, n, k):
        return pltpu.make_async_copy(ho_v.at[1, pl.ds(row0, n), :],
                                     out_hbm.at[0, pl.ds(row0, n), :], sems.at[3 + k])

    OB = SEG * UNROLL

    def carried(q):
        return att_v[pl.ds(8 * q, 8), :]

    def steps(i, carry):
        @pl.when(i == 16 // UNROLL)
        def _():
            x2_copy.wait()

        mem, left, att_prev = mem_v[...], None, carried
        for u in range(UNROLL):
            mem, att, left = step(i * UNROLL + u, mem, u > 0, left, att_prev)
            att_prev = (lambda a: lambda q: a[8 * q:8 * q + 8])(att)
        mem_v[...] = mem
        att_v[...] = att

        @pl.when(i >= 1)
        def _():
            out_copy(pl.multiple_of((i - 1) * OB, OB), OB, 0).start()
        return carry
    lax.fori_loop(0, NSEG // UNROLL, steps, 0)

    for cp in ffn_copies:
        cp.wait()
    last = []
    for q in range(5):
        for item in post_work(S - 40 + 8 * q, functools.partial(carried, q), last):
            item(None)
    out_copy(S - OB, OB, 0).start()

    def top2(val, idx, valid):
        def reduce(f, v):
            v = f(v, axis=0, keepdims=True)
            return v if v.shape[1] == 1 else f(v, axis=1, keepdims=True)

        def argtop(ok):
            v = jnp.where(ok, val, -jnp.inf)
            m = reduce(jnp.max, v)
            return m, reduce(jnp.min, jnp.where(ok & (v >= m), idx, float(S)))
        m1, i1 = argtop(valid)
        return (m1, i1), argtop(valid & (idx != i1))

    sub1 = lax.broadcasted_iota(jnp.int32, (16, 128), 0)
    lan1 = lax.broadcasted_iota(jnp.int32, (16, 128), 1)
    idx = (sub1 // 8) * 1024 + lan1 * 8 + sub1 % 8
    c_a, c_b = top2(_rb(r_v[...].reshape(16, 128)), idx.astype(F32), idx < S - 40)
    sub2 = lax.broadcasted_iota(jnp.int32, (48, 1), 0)
    val2 = jnp.concatenate([_rb(r) for r in last] + [jnp.where(sub2[:8] == 0, c_a[0], c_b[0])],
                           axis=0)
    idx2 = jnp.where(sub2 < 40, (sub2 + (S - 40)).astype(F32),
                     jnp.where(sub2 == 40, c_a[1], c_b[1]))
    (m_a, i_a), (m_b, i_b) = top2(val2, idx2, sub2 < 42)
    i_a = i_a.astype(jnp.int32)
    i_b = i_b.astype(jnp.int32)
    ia = jnp.clip(i_a[0, 0], 0, S - 1)
    ib = jnp.clip(i_b[0, 0], 0, S - 1)
    blk_a = pl.multiple_of((ia // 8) * 8, 8)
    blk_b = pl.multiple_of((ib // 8) * 8, 8)

    def two(ref):
        return jnp.concatenate([ref[pl.ds(blk_a, 8), :], ref[pl.ds(blk_b, 8), :]], axis=0)

    hs = two(ho_v.at[0])
    g = _rb(jnp.dot(hs, wg_v[...], preferred_element_type=F32))
    u = _rb(jnp.dot(hs, wu_v[...], preferred_element_type=F32))
    act = (_rb(g * jax.nn.sigmoid(g)) * u).astype(BF)
    y = jnp.concatenate(
        [jnp.dot(act, wd_v[k], preferred_element_type=F32) for k in range(2)], axis=1)
    sub = lax.broadcasted_iota(jnp.int32, (16, 1), 0)
    rows = jnp.where(sub < 8, blk_a + sub, blk_b + sub - 8)
    gate = jnp.where(rows == ia, jax.nn.sigmoid(m_a),
                     jnp.where(rows == ib, jax.nn.sigmoid(m_b), 0.0))
    upd = jnp.where((rows == ia) | (rows == ib), y * gate, 0.0).reshape(2, 8, D)
    fin = _b2(_f3(two(ho_v.at[1])) + mod_v[5] * upd)

    out_copy(0, S, 0).wait()
    ho_v[1, pl.ds(blk_a, 8), :] = fin[0:8]
    ho_v[1, pl.ds(blk_b, 8), :] = fin[8:16]
    out_copy(blk_a, 8, 0).start()

    @pl.when(blk_a != blk_b)
    def _():
        out_copy(blk_b, 8, 1).start()
        out_copy(blk_b, 8, 1).wait()
    out_copy(blk_a, 8, 0).wait()


@jax.jit
def pallas_adaLN_cond__memory_aug_recurrent_mem_tr__moe_arch_mod__prompt_kernel(
    A_x, A_mem0, A_Wq, A_Wk, A_Wv, A_Wo, A_seg_len, B_x, B_w_r, B_w_gate, B_w_up, B_w_down, c,
    w_mod,
):
    del B_x
    del A_seg_len
    assert A_x.shape == (1, S, D) and A_Wq.shape == (D, H, DH) and A_mem0.shape == (1, M, D)
    any_spec = pl.BlockSpec(memory_space=pl.ANY)
    scratch = [
        pltpu.VMEM((S, D), BF),
        pltpu.VMEM((4, X0, QK), BF),
        pltpu.VMEM((4, BULK // 2, QK), U32),
        pltpu.VMEM((40, D), BF),
        pltpu.VMEM((2, S, D), BF),
        pltpu.VMEM((96 * PITCH, 128), U32),
        pltpu.VMEM((2, H * DH, 512), BF),
        pltpu.VMEM((5 * D, 8, 128), BF),
        pltpu.VMEM((12, D, 512), BF),
        pltpu.VMEM((D, FF), BF),
        pltpu.VMEM((D, FF), BF),
        pltpu.VMEM((2, FF, 512), BF),
        pltpu.VMEM((M, D), BF),
        pltpu.VMEM((1, D), BF),
        pltpu.VMEM((1, D), BF),
        pltpu.VMEM((7, 8, D), F32),
        pltpu.VMEM((2, 8, 128), F32),
        pltpu.VMEM((D, 128), F32),
        pltpu.VMEM((12, 8, 512), F32),
        pltpu.VMEM((NP, 4, BULK, 256), F32),
        pltpu.SemaphoreType.DMA((9,)),
    ] + [pltpu.VMEM((12, RING, 128), BF)] * 8
    return pl.pallas_call(
        _kernel,
        out_shape=jax.ShapeDtypeStruct((1, S, D), BF),
        in_specs=[any_spec] * 12,
        out_specs=any_spec,
        scratch_shapes=scratch,
        compiler_params=pltpu.CompilerParams(vmem_limit_bytes=120 * 1024 * 1024),
    )(A_x, A_mem0, A_Wq, A_Wk, A_Wv, A_Wo.reshape(H * DH, D), B_w_r.reshape(1, D), B_w_gate,
      B_w_up, B_w_down, c, w_mod)
```

```python
import functools

import jax
import jax.numpy as jnp
from jax import lax
import jax.experimental.pallas as pl
import jax.experimental.pallas.tpu as pltpu

BF = jnp.bfloat16
F32 = jnp.float32
U32 = jnp.uint32

S = 2048
D = 1024
H = 32
DH = 128
M = 8
SEG = 32
NSEG = S // SEG
FF = 3584
RIDE = 24
BULK = S - RIDE * NSEG
X0 = BULK + 32
RING = 576
PITCH = 520
X1 = 1024
NP = 3
QK = D // 4
UNROLL = 4
EPS = 1e-5
SIDE0, SIDE_LAT, SIDE_DUE, SIDE_END = 2, 6, 6, 82
NEG = -3.0e38
ORDER = ("q0 q1 q2 q3 k4 k5 k6 k7 s0 s1 s2 s3 s4 s5 s6 s7 v4 v5 v6 v7 p0 p1 p2 p3 p4 p5 p6 p7 "
         "w0 w1 w2 w3 w4 w5 w6 w7")
PERM = (0, 2, 4, 6, 1, 3, 5, 7)


def _rb(v):
    return v.astype(BF).astype(F32)


def _layernorm(xf):
    mu = jnp.mean(xf, axis=-1, keepdims=True)
    dv = xf - mu
    var = jnp.mean(dv * dv, axis=-1, keepdims=True)
    sd = _rb(jnp.sqrt(_rb(_rb(var) + EPS)))
    return _rb(_rb(xf - _rb(mu)) * (1.0 / sd))


def _f3(v):
    return v.astype(F32).reshape(v.shape[0] // 8, 8, D)


def _b2(v):
    return v.reshape(v.shape[0] * 8, D).astype(BF)


def _kernel(x_hbm, mem0_hbm, wq_hbm, wk_hbm, wv_hbm, wo_hbm, wr_hbm, wg_hbm, wu_hbm, wd_hbm,
            c_hbm, wmod_hbm, out_hbm,
            x_v, h_v, hp_v, att_v, ho_v, wqkv_v, wo_v, stage, wmod_v,
            wg_v, wu_v, wd_v, mem_v, c_v, wr_v, mod_v, r_v, sb_v, macc_v,
            part_v, sems, *rings):
    w_hbm = (wq_hbm, wk_hbm, wv_hbm)
    ring = rings

    def piece_copy(t, sem, lo=0, n=D, dst=None):
        dst = (t % 2) * D + lo if dst is None else dst
        return pltpu.make_async_copy(
            w_hbm[t // 4].at[pl.ds(lo, n), pl.ds((t % 4) * 8, 8), :],
            stage.at[pl.ds(dst, n)], sems.at[sem])

    def unit_copy(j):
        return piece_copy(j % NP, 6 + min(j, 10) % 3, QK * (j // NP), QK, 2 * D + QK * j)

    def stage_wait(row, n, sem):
        dst = stage.at[pl.ds(row, n)]
        pltpu.make_async_copy(dst, dst, sems.at[sem]).wait()

    def mq_copy(q, part):
        return pltpu.make_async_copy(wmod_hbm.at[:, pl.ds(part * D + q * QK, QK)],
                                     wmod_v.at[q, :, pl.ds(part * QK, QK)], sems.at[2])

    def wmod_copy(k, sem):
        col = k * 512 if isinstance(k, int) else pl.multiple_of(k * 512, 512)
        return pltpu.make_async_copy(wmod_hbm.at[:, pl.ds(col, 512)], wmod_v.at[k], sems.at[sem])

    def x_copy(lo, hi, sem):
        return pltpu.make_async_copy(x_hbm.at[0, pl.ds(lo, hi - lo), :],
                                     x_v.at[pl.ds(lo, hi - lo), :], sems.at[sem])

    def wo_copy(n):
        lo, rows = ((n // 2) * 512, 512) if n < 6 else (1536, 2560)
        return pltpu.make_async_copy(wo_hbm.at[pl.ds(lo, rows), pl.ds((n % 2) * 512, 512)],
                                     wo_v.at[n % 2, pl.ds(lo, rows)], sems.at[0])

    small_copies = [pltpu.make_async_copy(c_hbm, c_v, sems.at[0]),
                    pltpu.make_async_copy(mem0_hbm.at[0], mem_v, sems.at[0]),
                    pltpu.make_async_copy(wr_hbm, wr_v, sems.at[0])]
    x0_copy = x_copy(0, X0, 1)
    mid_copies = ([x_copy(X0, (X0 + X1) // 2, 0), x_copy((X0 + X1) // 2, X1, 0)]
                  + [wo_copy(n) for n in range(8)])
    x2_copy = x_copy(X1, S, 1)
    ffn_copies = [pltpu.make_async_copy(wg_hbm, wg_v, sems.at[2]),
                  pltpu.make_async_copy(wu_hbm, wu_v, sems.at[2])] + [
        pltpu.make_async_copy(wd_hbm.at[:, pl.ds(k * 512, 512)], wd_v.at[k], sems.at[2])
        for k in range(2)]

    def relayout(src, base, n):
        u = pltpu.bitcast(stage[pl.ds(src, n)], U32)
        tok = None
        for i in range(n // 2):
            a = u[2 * i]
            b = u[2 * i + 1]
            even = (a & jnp.uint32(0xFFFF)) | (b << 16)
            odd = (a >> 16) | (b & jnp.uint32(0xFFFF0000))
            wqkv_v[pl.ds(base + i, 4, stride=PITCH), :] = even
            wqkv_v[pl.ds(base + 4 * PITCH + i, 4, stride=PITCH), :] = odd
            tok = even ^ odd if tok is None else tok ^ even ^ odd
        return jnp.concatenate([tok, tok], axis=0)

    CW = 256

    def ln_stats(xf):
        mu = jnp.mean(xf, axis=-1, keepdims=True)
        dv = xf - mu
        var = jnp.mean(dv * dv, axis=-1, keepdims=True)
        sd = _rb(jnp.sqrt(_rb(_rb(var) + EPS)))
        return _rb(mu), 1.0 / sd

    def mod_c(k, c):
        return mod_v[k, :, pl.ds(c * CW, CW)]

    def token(v):
        return pltpu.bitcast(v[:, :128] + v[:, 128:], U32)

    def after(v, trig):
        if trig is None:
            return v
        return jnp.concatenate([jnp.where(trig[0], trig[1], v[:, :128]), v[:, 128:]], axis=1)

    def post_work(row0, att, scores_out=None):
        st = {}

        def head(trig):
            a = after(att().astype(F32), trig)
            st["x2"] = _rb(x_v[pl.ds(row0, 8), :].astype(F32) + _rb(mod_v[2] * a))
            st["mu"], st["inv"] = ln_stats(st["x2"])

        def chunk(c, trig):
            xc = after(st["x2"][:, c * CW:(c + 1) * CW], trig)
            h2b = (_rb(_rb(_rb(xc - st["mu"]) * st["inv"]) * mod_c(4, c))
                   + mod_c(3, c)).astype(BF)
            h2 = h2b.astype(F32)
            ho_v[0, pl.ds(row0, 8), pl.ds(c * CW, CW)] = h2b
            o = xc + mod_c(5, c) * h2
            ho_v[1, pl.ds(row0, 8), pl.ds(c * CW, CW)] = o.astype(BF)
            rp = h2 * mod_c(6, c)
            st["r"] = rp if c == 0 else st["r"] + rp
            if c == D // CW - 1:
                r = jnp.sum(st["r"], axis=-1, keepdims=True)
                if scores_out is not None:
                    scores_out.append(r)
                    return None
                grp = row0 >> 3
                lanes = lax.broadcasted_iota(jnp.int32, (8, 128), 1)
                r_v[grp >> 7] = jnp.where(lanes == (grp & 127), r, r_v[grp >> 7])
            return token(o + st["r"])
        return [head] + [functools.partial(chunk, c) for c in range(D // CW)]

    def ln1_work(row0):
        st = {}

        def head(trig):
            st["x"] = after(x_v[pl.ds(row0, 8), :].astype(F32), trig)
            st["mu"], st["inv"] = ln_stats(st["x"])

        def chunk(c, trig):
            xc = after(st["x"][:, c * CW:(c + 1) * CW], trig)
            h = _rb(_rb(_rb(xc - st["mu"]) * st["inv"]) * mod_c(1, c)) + mod_c(0, c)
            ho_v[0, pl.ds(row0, 8), pl.ds(c * CW, CW)] = h.astype(BF)
            return token(h)
        return [head] + [functools.partial(chunk, c) for c in range(D // CW)]

    for cp in small_copies:
        cp.start()
    x0_copy.start()
    mq_copy(0, 0).start()

    r_v[...] = jnp.full(r_v.shape, NEG, F32)
    att_v[...] = jnp.zeros(att_v.shape, BF)

    for cp in small_copies:
        cp.wait()
    mod_v[6] = jnp.broadcast_to(wr_v[...].astype(F32), (8, D))
    cf = c_v[...].astype(F32)
    sil = (cf * jax.nn.sigmoid(cf)).astype(BF)
    sc = jnp.broadcast_to(sil, (16, D))
    for k in range(8):
        sb_v[pl.ds(128 * k, 128), :] = jnp.broadcast_to(
            sil[:, 128 * k:128 * k + 128].astype(F32), (128, 128)).T

    mq_copy(0, 1).start()
    x0_copy.wait()
    unit_copy(0).start()
    unit_copy(1).start()

    LNB = X0 // 4

    def ln0(i, carry):
        r0 = pl.multiple_of(i * LNB, 8)
        ln = _b2(_layernorm(_f3(x_v[pl.ds(r0, LNB), :])))
        for q in range(4):
            h_v[q, pl.ds(r0, LNB), :] = ln[:, q * QK:(q + 1) * QK]
        return carry
    lax.fori_loop(0, 4, ln0, 0)

    def shift_scale(acc):
        y = _rb(acc)
        return y[:, :QK], _rb(1.0 + y[:, QK:])

    def modulated(q, r0, n, sh, sca):
        ln = h_v[q, pl.ds(r0, n), :].astype(F32).reshape(n // 8, 8, QK)
        return (_rb(ln * sca) + sh).reshape(n, QK).astype(BF)

    for part in range(2):
        mq_copy(0, part).wait()
    acc0 = jnp.dot(sc, wmod_v[0], preferred_element_type=F32)[0:8]
    macc_v[0] = acc0
    hp_v[0] = pltpu.bitcast(modulated(0, 0, BULK, *shift_scale(acc0)), U32)
    unit_copy(0).wait()
    unit_copy(2).start()

    def relayout0(i, carry):
        relayout(2 * D + pl.multiple_of(i * 128, 128), i * 64, 128)
        return carry
    lax.fori_loop(0, QK // 128, relayout0, 0)
    mq_copy(1, 0).start()
    mq_copy(1, 1).start()
    unit_copy(3).start()

    def mod_rows(slab, r0, n, acc):
        for r in range(r0, r0 + n, 8):
            sv = sb_v[pl.ds(r, 8), :]
            t = wmod_v[slab, pl.ds(r, 8), :].astype(F32) * jnp.concatenate([sv] * 4, axis=1)
            acc = t if acc is None else acc + t
        return acc

    def tie_lhs(col, never, toks):
        return jnp.concatenate(
            [jnp.where(never, toks[j], col[8 * j:8 * j + 8]) if j in toks
             else col[8 * j:8 * j + 8] for j in range(32)], axis=0)

    def add_tok(toks, j, tk):
        toks[j] = tk if j not in toks else toks[j] ^ tk

    starts = {0: [unit_copy(4)], 1: [unit_copy(5), piece_copy(3, 5, 0, 256)],
              2: [unit_copy(6), mq_copy(2, 0), mq_copy(2, 1)],
              3: [unit_copy(7), piece_copy(3, 5, 256, 256)], 4: [unit_copy(8)],
              5: [unit_copy(9), mq_copy(3, 0), mq_copy(3, 1)],
              6: [unit_copy(10), unit_copy(11)], 7: [piece_copy(3, 3, 512, 512)],
              8: [piece_copy(4, 4)], 9: [], 10: [wmod_copy(4, 2)], 11: []}

    def quarter_block(b_lo, b_hi, b, carry):
        first, final = b_lo == 0, b_hi == 4 * NP
        q = b_lo // NP
        p = b - NP * q
        if final:
            src = jnp.where(p == 0, 2 * D + 10 * QK, D + 512 * (p - 1))
            sem = 7 - 2 * p
            stage_wait(pl.multiple_of(src, 512), 512, sem)
            b3 = 3 * 8 * PITCH + 256 * (p - 1)
            jobs = [(src, jnp.where(p == 0, 8 * PITCH + 384, b3)),
                    (src + QK, jnp.where(p == 0, 2 * 8 * PITCH + 384, b3 + 128))]
        else:
            src = 2 * D + QK * (b + 1)
            last = p == NP - 1
            stage_wait(pl.multiple_of(src, QK), QK, jnp.where(last, 6, 7 + p))
            jobs = [(src, jnp.where(last, 128 * (q + 1), (p + 1) * (8 * PITCH) + 128 * q))]

            @pl.when(last)
            def _():
                for part in range(2):
                    mq_copy(q + 1, part).wait()
            slab = jnp.where(last, q + 1, q)
        never = jnp.full((8, 128), b, jnp.int32) < 0

        def weights(k):
            return pltpu.bitcast(jnp.concatenate(
                [wqkv_v[pl.ds(pl.multiple_of((8 * p + kk) * PITCH + 128 * q, 8), 128), :]
                 for kk in (k, k + 1)], axis=1), BF)

        groups = [(s_ + 16 * g, d_ + 8 * g) for s_, d_ in jobs for g in range(QK // 16)]
        per = len(groups) // 4
        acc = None
        w = weights(0)
        for n, k in enumerate(range(0, 8, 2)):
            w_next = weights(k + 2) if k < 6 else None
            toks = {}
            for g in range(per):
                add_tok(toks, 4 + (g * 24) // per, relayout(*groups[n * per + g], 16))
            if not final and n < 2:
                for g in range(16):
                    acc = mod_rows(slab, 512 * n + 32 * g, 32, acc)
                    add_tok(toks, 2 * g + (n == 0), token(acc[:, :256] + acc[:, 256:]))
            if not final and n == 2:
                tot = jnp.broadcast_to(jnp.sum(acc, axis=0, keepdims=True), (8, 512))
                macc_v[q + 1] = tot
                sh, sca = shift_scale(tot)
            if not final and n >= 2:
                for g in range(16):
                    r0 = 256 * (n - 2) + 16 * g
                    hb = pltpu.bitcast(modulated(q + 1, r0, 16, sh, sca), U32)
                    hp_v[q + 1, pl.ds(r0 // 2, 8), :] = hb
                    add_tok(toks, (8 + (g * 3) // 2) if n == 2 else 2 * g,
                            hb[:, :128] ^ hb[:, 128:])
            lhs = jnp.concatenate([tie_lhs(hp_v[q, :, pl.ds(0, 128)], never, toks),
                                   hp_v[q, :, pl.ds(128, 128)]], axis=1)
            y = jnp.dot(pltpu.bitcast(lhs, BF), w, preferred_element_type=F32)
            if not first:
                y = y + part_v[p, n]
            if final:
                for j in range(2):
                    ring[k + j][p, pl.ds((RING - BULK) // 2, BULK // 2), :] = pltpu.bitcast(
                        y[:, 128 * j:128 * j + 128].astype(BF), U32)
            else:
                part_v[p, n] = y
            w = w_next

        for j in range(b_lo, b_hi):
            if starts[j]:
                @pl.when(b == j)
                def _():
                    for cp in starts[j]:
                        cp.start()
        return carry

    for b_lo, b_hi in ((0, NP), (NP, 2 * NP), (2 * NP, 3 * NP), (3 * NP, 4 * NP)):
        quarters = functools.partial(quarter_block, b_lo, b_hi)
        lax.fori_loop(b_lo, b_hi, quarters, 0)

    def bulk_dot(i, k, never, t, md):
        w = pltpu.bitcast(wqkv_v[pl.ds(pl.multiple_of((8 * i + k) * PITCH, 8), 512), :], BF)
        cols = [hp_v[c // 2, :, pl.ds(128 * (c % 2), 128)] for c in range(8)]
        toks = {}
        for g in range(8):
            tk = relayout((t & 1) * D + 128 * k + 16 * g, t * (8 * PITCH) + 64 * k + 8 * g, 16)
            md[1] = mod_rows(md[0], 128 * k + 16 * g, 16, md[1])
            toks[12 + 6 * g] = tk ^ token(md[1][:, :256] + md[1][:, 256:])
        cols[0] = tie_lhs(cols[0], never, toks)
        cols[4] = tie_lhs(cols[4], never, {j - 32: tk for j, tk in toks.items()})
        hb = pltpu.bitcast(jnp.concatenate(cols, axis=1), BF)
        y = jnp.dot(hb, w, preferred_element_type=F32)
        ring[k][i, pl.ds((RING - BULK) // 2, BULK // 2), :] = pltpu.bitcast(y.astype(BF), U32)

    def bulk_qkv(i, carry):
        @pl.when(i < 11)
        def _():
            par = (i + 1) & 1
            stage_wait(pl.multiple_of(par * D, D), D, 4 + par)

        @pl.when(i > NP)
        def _():
            wmod_copy(i, 2 + (i & 1)).wait()

        for j in range(NP, 10):
            @pl.when(i == j)
            def _():
                piece_copy(j + 2, 4 + j % 2).start()

        t = jnp.minimum(i + 1, 11)
        never = jnp.full((8, 128), i, jnp.int32) < 0
        md = [i, None]
        for k in range(8):
            bulk_dot(i, k, never, t, md)
        macc_v[jnp.maximum(i, 4)] = md[1]

        for j in range(NP, 10):
            @pl.when(i == j)
            def _():
                wmod_copy(j + 2, 2 + j % 2).start()
                if j < 9:
                    mid_copies[j - NP + 1].start()
                else:
                    for cp in mid_copies[7:]:
                        cp.start()
        return carry
    mid_copies[0].start()
    lax.fori_loop(NP, 12, bulk_qkv, 0)

    for q in range(4):
        sh, sca = shift_scale(macc_v[q])
        mod_v[0, :, pl.ds(q * QK, QK)] = sh
        mod_v[1, :, pl.ds(q * QK, QK)] = sca
        ho_v[0, pl.ds(BULK, RIDE), pl.ds(q * QK, QK)] = modulated(q, BULK, RIDE, sh, sca)
    for k in range(4, 12):
        y = _rb(jnp.sum(macc_v[k], axis=0, keepdims=True))
        if k // 2 == 4:
            y = _rb(1.0 + y)
        mod_v[k // 2, :, pl.ds((k % 2) * 512, 512)] = jnp.broadcast_to(y, (8, 512))
    for cp in mid_copies:
        cp.wait()
    x2_copy.start()
    for cp in ffn_copies:
        cp.start()

    scale = DH ** -0.5
    kk = lax.broadcasted_iota(jnp.int32, (M + SEG, 80), 0)
    cc = lax.broadcasted_iota(jnp.int32, (M + SEG, 80), 1)
    second = ((cc >= 8) & (cc < 16)) | (cc >= 48)
    allowed = (cc < 16) | (kk <= jnp.where(second, cc - 40, cc - 8))

    def over_keys(f, fr, v):
        t = v[0:8]
        for j in range(8, M + SEG, 8):
            t = f(t, v[j:j + 8])
        return fr(t, axis=0, keepdims=True)

    def tied(u, never, toks):
        if not toks:
            return u
        parts, at = [], 0
        for j, tk in enumerate(toks):
            r = 64 * j
            if r > at:
                parts.append(u[at:r])
            w = tk.shape[1]
            sel = jnp.where(never[:, :w], tk, u[r:r + 8, :w])
            parts.append(sel if w == 128 else jnp.concatenate([sel, u[r:r + 8, w:]], axis=1))
            at = r + 8
        return jnp.concatenate(parts + [u[at:]], axis=0)

    def w_slab(t, g, lo=0, n=512, never=None, toks=()):
        return pltpu.bitcast(
            tied(wqkv_v[pl.ds((8 * t + g) * PITCH + lo, n), :], never, toks), BF)

    def step(s, mem, chained, left, att_prev):
        odd = left is not None
        wr = pl.multiple_of(lax.rem(12 * s - 4 * odd, RING // 2), 8) + 4 * odd
        rd = pl.multiple_of(lax.rem(16 * s + (RING - BULK) // 2, RING // 2), 16)
        xin = jnp.concatenate(
            [mem, ho_v[0, pl.ds(pl.multiple_of(BULK + RIDE * s, 8), RIDE), :]], axis=0)

        prow = SEG * (s - 1) if odd else jnp.maximum(SEG * s - 40, 0)
        nrow = BULK + RIDE * jnp.minimum(s + 1, NSEG - 1)
        works = [post_work(pl.multiple_of(prow + 8 * q, 8), functools.partial(att_prev, q))
                 for q in range(3 if odd else 5)]
        works += [ln1_work(pl.multiple_of(nrow + 8 * q, 8)) for q in range(RIDE // 8)]
        never = jnp.full((8, 128), s, jnp.int32) < 0
        gap = (SIDE_END - SIDE0 - SIDE_LAT - SIDE_DUE) // len(works)
        sched = {}
        for q, wk in enumerate(works):
            sched.setdefault(SIDE0 + gap * q, []).append(wk[0])
            for c in range(1, len(wk)):
                sched.setdefault(SIDE0 + SIDE_LAT + gap * q + ((c - 1) * gap) // 4,
                                 []).append(wk[c])

        memqkv, probs, wl, new_left, toks = {}, {}, {}, {}, {}
        acc = []
        chain = []

        ndot = [0]

        def proj(g, t_lo, t_hi):
            part = {}
            if chained and ndot[0] == 0:
                for t in range(t_lo, t_lo + 6):
                    part[t] = jnp.dot(xin[:, :512], w_slab(t, g, 0, 256),
                                      preferred_element_type=F32)
            for t0 in range(t_lo, t_hi, 2):
                ys = []
                for t in (t0, t0 + 1):
                    n = ndot[0]
                    ndot[0] += 1
                    if t in part:
                        y = jnp.dot(xin[:, 512:], w_slab(t, g, 256, 256),
                                    preferred_element_type=F32) + part[t]
                    else:
                        y = jnp.dot(xin, w_slab(t, g, 0, 512, never, toks.get(n)),
                                    preferred_element_type=F32)
                    ring[g][t, pl.ds(wr, RIDE // 2), :] = (
                        pltpu.bitcast(y.astype(BF), U32)[M // 2:] if odd
                        else pltpu.bitcast(y[M:].astype(BF), U32))
                    ys.append(y[:M])
                    for item in sched.get(n, ()):
                        tk = item((never, y[:M]))
                        if tk is not None:
                            toks.setdefault(n + SIDE_DUE, []).append(tk)
                memqkv[(t0, g)] = jnp.concatenate(ys, axis=0).astype(BF)

        def cat(t0, g):
            return jnp.concatenate(
                [memqkv[(t0, g)]] + [pltpu.bitcast(ring[g][t, pl.ds(rd, SEG // 2), :], BF)
                                     for t in (t0, t0 + 1)], axis=0)

        def scores(g):
            for p in (0, 2):
                st = lax.dot_general(cat(4 + p, g), cat(p, g), (((1,), (1,)), ((), ())),
                                     preferred_element_type=F32)
                st = jnp.where(second, jnp.concatenate([st[8:16], st[48:80]], axis=0),
                               jnp.concatenate([st[0:8], st[16:48]], axis=0))
                if chain:
                    st = jnp.concatenate(
                        [jnp.where(never[:, :80], chain[-1], st[0:8]), st[8:]], axis=0)
                st = jnp.where(allowed, st * scale, -1e9)
                e = jnp.exp(st - over_keys(jnp.maximum, jnp.max, st))
                l = over_keys(jnp.add, jnp.sum, e)
                chain.append(jnp.broadcast_to(l, (8, 80)))
                rc = pl.reciprocal(l, approx=True)
                e = e * (rc * (2.0 - l * rc))
                e0 = jnp.where(second, 0.0, e)
                e1 = jnp.where(second, e, 0.0)
                probs[(p, g)] = jnp.concatenate(
                    [e0[:M], e1[:M], e0[M:], e1[M:]], axis=0).astype(BF)

        def pv(g):
            for p in (0, 2):
                o = lax.dot_general(probs[(p, g)], cat(8 + p, g), (((0,), (0,)), ((), ())),
                                    preferred_element_type=F32)
                for j in range(2):
                    om, ot = o[8 * j:8 * j + 8], o[16 + 32 * j:48 + 32 * j]
                    if odd:
                        rows = [om, left[(p + j, g)], ot]
                    else:
                        rows = [om, ot[:RIDE]]
                        new_left[(p + j, g)] = ot[RIDE:]
                    wl[(p + j, g)] = jnp.concatenate(rows, axis=0).astype(BF)

        def wo(g):
            a = jnp.concatenate([wl[(o, g)] for o in range(4)], axis=1)
            w = jnp.concatenate(
                [jnp.concatenate([wo_v[n, pl.ds((8 * o + PERM[g]) * DH, DH), :]
                                  for o in range(4)], axis=0) for n in range(2)], axis=1)
            y = jnp.dot(a, w, preferred_element_type=F32)
            acc[:] = [y if not acc else y + acc[0]]

        for op in ORDER.split():
            g = int(op[1])
            if op[0] in "qkvux":
                proj(g, *{"q": (0, 12), "k": (0, 8), "v": (8, 12), "u": (0, 10), "x": (10, 12)}[op[0]])
            else:
                {"s": scores, "p": pv, "w": wo}[op[0]](g)
        y = acc[0].astype(BF)
        return y[:M], y[M:], (None if odd else new_left)

    def out_copy(row0, n, k):
        return pltpu.make_async_copy(ho_v.at[1, pl.ds(row0, n), :],
                                     out_hbm.at[0, pl.ds(row0, n), :], sems.at[3 + k])

    OB = SEG * UNROLL

    def carried(q):
        return att_v[pl.ds(8 * q, 8), :]

    def steps(i, carry):
        @pl.when(i == 16 // UNROLL)
        def _():
            x2_copy.wait()

        mem, left, att_prev = mem_v[...], None, carried
        for u in range(UNROLL):
            mem, att, left = step(i * UNROLL + u, mem, u > 0, left, att_prev)
            att_prev = (lambda a: lambda q: a[8 * q:8 * q + 8])(att)
        mem_v[...] = mem
        att_v[...] = att

        @pl.when(i >= 1)
        def _():
            out_copy(pl.multiple_of((i - 1) * OB, OB), OB, 0).start()
        return carry
    lax.fori_loop(0, NSEG // UNROLL, steps, 0)

    for cp in ffn_copies:
        cp.wait()
    last = []
    for q in range(5):
        for item in post_work(S - 40 + 8 * q, functools.partial(carried, q), last):
            item(None)
    out_copy(S - OB, OB, 0).start()

    def top2(val, idx, valid):
        def reduce(f, v):
            v = f(v, axis=0, keepdims=True)
            return v if v.shape[1] == 1 else f(v, axis=1, keepdims=True)

        def argtop(ok):
            v = jnp.where(ok, val, -jnp.inf)
            m = reduce(jnp.max, v)
            return m, reduce(jnp.min, jnp.where(ok & (v >= m), idx, float(S)))
        m1, i1 = argtop(valid)
        return (m1, i1), argtop(valid & (idx != i1))

    sub1 = lax.broadcasted_iota(jnp.int32, (16, 128), 0)
    lan1 = lax.broadcasted_iota(jnp.int32, (16, 128), 1)
    idx = (sub1 // 8) * 1024 + lan1 * 8 + sub1 % 8
    c_a, c_b = top2(_rb(r_v[...].reshape(16, 128)), idx.astype(F32), idx < S - 40)
    sub2 = lax.broadcasted_iota(jnp.int32, (48, 1), 0)
    val2 = jnp.concatenate([_rb(r) for r in last] + [jnp.where(sub2[:8] == 0, c_a[0], c_b[0])],
                           axis=0)
    idx2 = jnp.where(sub2 < 40, (sub2 + (S - 40)).astype(F32),
                     jnp.where(sub2 == 40, c_a[1], c_b[1]))
    (m_a, i_a), (m_b, i_b) = top2(val2, idx2, sub2 < 42)
    i_a = i_a.astype(jnp.int32)
    i_b = i_b.astype(jnp.int32)
    ia = jnp.clip(i_a[0, 0], 0, S - 1)
    ib = jnp.clip(i_b[0, 0], 0, S - 1)
    blk_a = pl.multiple_of((ia // 8) * 8, 8)
    blk_b = pl.multiple_of((ib // 8) * 8, 8)

    def two(ref):
        return jnp.concatenate([ref[pl.ds(blk_a, 8), :], ref[pl.ds(blk_b, 8), :]], axis=0)

    hs = two(ho_v.at[0])
    g = _rb(jnp.dot(hs, wg_v[...], preferred_element_type=F32))
    u = _rb(jnp.dot(hs, wu_v[...], preferred_element_type=F32))
    act = (_rb(g * jax.nn.sigmoid(g)) * u).astype(BF)
    y = jnp.concatenate(
        [jnp.dot(act, wd_v[k], preferred_element_type=F32) for k in range(2)], axis=1)
    sub = lax.broadcasted_iota(jnp.int32, (16, 1), 0)
    rows = jnp.where(sub < 8, blk_a + sub, blk_b + sub - 8)
    gate = jnp.where(rows == ia, jax.nn.sigmoid(m_a),
                     jnp.where(rows == ib, jax.nn.sigmoid(m_b), 0.0))
    upd = jnp.where((rows == ia) | (rows == ib), y * gate, 0.0).reshape(2, 8, D)
    fin = _b2(_f3(two(ho_v.at[1])) + mod_v[5] * upd)

    out_copy(0, S, 0).wait()
    ho_v[1, pl.ds(blk_a, 8), :] = fin[0:8]
    ho_v[1, pl.ds(blk_b, 8), :] = fin[8:16]
    out_copy(blk_a, 8, 0).start()

    @pl.when(blk_a != blk_b)
    def _():
        out_copy(blk_b, 8, 1).start()
        out_copy(blk_b, 8, 1).wait()
    out_copy(blk_a, 8, 0).wait()


@jax.jit
def pallas_adaLN_cond__memory_aug_recurrent_mem_tr__moe_arch_mod__prompt_kernel(
    A_x, A_mem0, A_Wq, A_Wk, A_Wv, A_Wo, A_seg_len, B_x, B_w_r, B_w_gate, B_w_up, B_w_down, c,
    w_mod,
):
    del B_x
    del A_seg_len
    assert A_x.shape == (1, S, D) and A_Wq.shape == (D, H, DH) and A_mem0.shape == (1, M, D)
    any_spec = pl.BlockSpec(memory_space=pl.ANY)
    scratch = [
        pltpu.VMEM((S, D), BF),
        pltpu.VMEM((4, X0, QK), BF),
        pltpu.VMEM((4, BULK // 2, QK), U32),
        pltpu.VMEM((40, D), BF),
        pltpu.VMEM((2, S, D), BF),
        pltpu.VMEM((96 * PITCH, 128), U32),
        pltpu.VMEM((2, H * DH, 512), BF),
        pltpu.VMEM((5 * D, 8, 128), BF),
        pltpu.VMEM((12, D, 512), BF),
        pltpu.VMEM((D, FF), BF),
        pltpu.VMEM((D, FF), BF),
        pltpu.VMEM((2, FF, 512), BF),
        pltpu.VMEM((M, D), BF),
        pltpu.VMEM((1, D), BF),
        pltpu.VMEM((1, D), BF),
        pltpu.VMEM((7, 8, D), F32),
        pltpu.VMEM((2, 8, 128), F32),
        pltpu.VMEM((D, 128), F32),
        pltpu.VMEM((12, 8, 512), F32),
        pltpu.VMEM((NP, 4, BULK, 256), F32),
        pltpu.SemaphoreType.DMA((9,)),
    ] + [pltpu.VMEM((12, RING // 2, 128), U32)] * 8
    return pl.pallas_call(
        _kernel,
        out_shape=jax.ShapeDtypeStruct((1, S, D), BF),
        in_specs=[any_spec] * 12,
        out_specs=any_spec,
        scratch_shapes=scratch,
        compiler_params=pltpu.CompilerParams(vmem_limit_bytes=120 * 1024 * 1024),
    )(A_x, A_mem0, A_Wq, A_Wk, A_Wv, A_Wo.reshape(H * DH, D), B_w_r.reshape(1, D), B_w_gate,
      B_w_up, B_w_down, c, w_mod)
```

```python
import functools

import jax
import jax.numpy as jnp
from jax import lax
import jax.experimental.pallas as pl
import jax.experimental.pallas.tpu as pltpu

BF = jnp.bfloat16
F32 = jnp.float32
U32 = jnp.uint32

S = 2048
D = 1024
H = 32
DH = 128
M = 8
SEG = 32
NSEG = S // SEG
FF = 3584
RIDE = 24
BULK = S - RIDE * NSEG
X0 = BULK + 32
RING = 576
PITCH = 520
X1 = 1024
NP = 3
QK = D // 4
UNROLL = 4
EPS = 1e-5
SIDE0, SIDE_LAT, SIDE_DUE, SIDE_END = 2, 6, 6, 82
NEG = -3.0e38
ORDER = ("q0 q1 q2 q3 k4 k5 k6 k7 s0 s1 s2 s3 s4 s5 s6 s7 v4 v5 v6 v7 p0 p1 p2 p3 p4 p5 p6 p7 "
         "w0 w1 w2 w3 w4 w5 w6 w7")
PERM = (0, 2, 4, 6, 1, 3, 5, 7)


def _rb(v):
    return v.astype(BF).astype(F32)


def _layernorm(xf):
    mu = jnp.mean(xf, axis=-1, keepdims=True)
    dv = xf - mu
    var = jnp.mean(dv * dv, axis=-1, keepdims=True)
    sd = _rb(jnp.sqrt(_rb(_rb(var) + EPS)))
    return _rb(_rb(xf - _rb(mu)) * (1.0 / sd))


def _f3(v):
    return v.astype(F32).reshape(v.shape[0] // 8, 8, D)


def _b2(v):
    return v.reshape(v.shape[0] * 8, D).astype(BF)


def _kernel(x_hbm, mem0_hbm, wq_hbm, wk_hbm, wv_hbm, wo_hbm, wr_hbm, wg_hbm, wu_hbm, wd_hbm,
            c_hbm, wmod_hbm, out_hbm,
            x_v, h_v, hp_v, att_v, ho_v, wqkv_v, wo_v, stage, wmod_v,
            wg_v, wu_v, wd_v, mem_v, c_v, wr_v, mod_v, r_v, sb_v, macc_v,
            part_v, sems, *rings):
    w_hbm = (wq_hbm, wk_hbm, wv_hbm)
    ring = rings

    def piece_copy(t, sem, lo=0, n=D, dst=None):
        dst = (t % 2) * D + lo if dst is None else dst
        return pltpu.make_async_copy(
            w_hbm[t // 4].at[pl.ds(lo, n), pl.ds((t % 4) * 8, 8), :],
            stage.at[pl.ds(dst, n)], sems.at[sem])

    def unit_copy(j):
        return piece_copy(j % NP, 6 + min(j, 10) % 3, QK * (j // NP), QK, 2 * D + QK * j)

    def stage_wait(row, n, sem):
        dst = stage.at[pl.ds(row, n)]
        pltpu.make_async_copy(dst, dst, sems.at[sem]).wait()

    def mq_copy(q, part):
        return pltpu.make_async_copy(wmod_hbm.at[:, pl.ds(part * D + q * QK, QK)],
                                     wmod_v.at[q, :, pl.ds(part * QK, QK)], sems.at[2])

    def wmod_copy(k, sem):
        col = k * 512 if isinstance(k, int) else pl.multiple_of(k * 512, 512)
        return pltpu.make_async_copy(wmod_hbm.at[:, pl.ds(col, 512)], wmod_v.at[k], sems.at[sem])

    def x_copy(lo, hi, sem):
        return pltpu.make_async_copy(x_hbm.at[0, pl.ds(lo, hi - lo), :],
                                     x_v.at[pl.ds(lo, hi - lo), :], sems.at[sem])

    def wo_copy(n):
        lo, rows = ((n // 2) * 512, 512) if n < 6 else (1536, 2560)
        return pltpu.make_async_copy(wo_hbm.at[pl.ds(lo, rows), pl.ds((n % 2) * 512, 512)],
                                     wo_v.at[n % 2, pl.ds(lo, rows)], sems.at[0])

    small_copies = [pltpu.make_async_copy(c_hbm, c_v, sems.at[0]),
                    pltpu.make_async_copy(mem0_hbm.at[0], mem_v, sems.at[0]),
                    pltpu.make_async_copy(wr_hbm, wr_v, sems.at[0])]
    x0_copy = x_copy(0, X0, 1)
    mid_copies = ([x_copy(X0, (X0 + X1) // 2, 0), x_copy((X0 + X1) // 2, X1, 0)]
                  + [wo_copy(n) for n in range(8)])
    x2_copy = x_copy(X1, S, 1)
    ffn_copies = [pltpu.make_async_copy(wg_hbm, wg_v, sems.at[2]),
                  pltpu.make_async_copy(wu_hbm, wu_v, sems.at[2])] + [
        pltpu.make_async_copy(wd_hbm.at[:, pl.ds(k * 512, 512)], wd_v.at[k], sems.at[2])
        for k in range(2)]

    def relayout(src, base, n):
        u = pltpu.bitcast(stage[pl.ds(src, n)], U32)
        tok = None
        for i in range(n // 2):
            a = u[2 * i]
            b = u[2 * i + 1]
            even = (a & jnp.uint32(0xFFFF)) | (b << 16)
            odd = (a >> 16) | (b & jnp.uint32(0xFFFF0000))
            wqkv_v[pl.ds(base + i, 4, stride=PITCH), :] = even
            wqkv_v[pl.ds(base + 4 * PITCH + i, 4, stride=PITCH), :] = odd
            tok = even ^ odd if tok is None else tok ^ even ^ odd
        return jnp.concatenate([tok, tok], axis=0)

    CW = 256

    def ln_stats(xf):
        mu = jnp.mean(xf, axis=-1, keepdims=True)
        dv = xf - mu
        var = jnp.mean(dv * dv, axis=-1, keepdims=True)
        sd = _rb(jnp.sqrt(_rb(_rb(var) + EPS)))
        return _rb(mu), 1.0 / sd

    def mod_c(k, c):
        return mod_v[k, :, pl.ds(c * CW, CW)]

    def token(v):
        return pltpu.bitcast(v[:, :128] + v[:, 128:], U32)

    def after(v, trig):
        if trig is None:
            return v
        return jnp.concatenate([jnp.where(trig[0], trig[1], v[:, :128]), v[:, 128:]], axis=1)

    def post_work(row0, att, scores_out=None):
        st = {}

        def head(trig):
            a = after(att().astype(F32), trig)
            st["x2"] = _rb(x_v[pl.ds(row0, 8), :].astype(F32) + _rb(mod_v[2] * a))
            st["mu"], st["inv"] = ln_stats(st["x2"])

        def chunk(c, trig):
            xc = after(st["x2"][:, c * CW:(c + 1) * CW], trig)
            h2b = (_rb(_rb(_rb(xc - st["mu"]) * st["inv"]) * mod_c(4, c))
                   + mod_c(3, c)).astype(BF)
            h2 = h2b.astype(F32)
            ho_v[0, pl.ds(row0, 8), pl.ds(c * CW, CW)] = h2b
            o = xc + mod_c(5, c) * h2
            ho_v[1, pl.ds(row0, 8), pl.ds(c * CW, CW)] = o.astype(BF)
            rp = h2 * mod_c(6, c)
            st["r"] = rp if c == 0 else st["r"] + rp
            if c == D // CW - 1:
                r = jnp.sum(st["r"], axis=-1, keepdims=True)
                if scores_out is not None:
                    scores_out.append(r)
                    return None
                grp = row0 >> 3
                lanes = lax.broadcasted_iota(jnp.int32, (8, 128), 1)
                r_v[grp >> 7] = jnp.where(lanes == (grp & 127), r, r_v[grp >> 7])
            return token(o + st["r"])
        return [head] + [functools.partial(chunk, c) for c in range(D // CW)]

    def ln1_work(row0):
        st = {}

        def head(trig):
            st["x"] = after(x_v[pl.ds(row0, 8), :].astype(F32), trig)
            st["mu"], st["inv"] = ln_stats(st["x"])

        def chunk(c, trig):
            xc = after(st["x"][:, c * CW:(c + 1) * CW], trig)
            h = _rb(_rb(_rb(xc - st["mu"]) * st["inv"]) * mod_c(1, c)) + mod_c(0, c)
            ho_v[0, pl.ds(row0, 8), pl.ds(c * CW, CW)] = h.astype(BF)
            return token(h)
        return [head] + [functools.partial(chunk, c) for c in range(D // CW)]

    for cp in small_copies:
        cp.start()
    x0_copy.start()
    mq_copy(0, 0).start()

    r_v[...] = jnp.full(r_v.shape, NEG, F32)
    att_v[...] = jnp.zeros(att_v.shape, BF)

    for cp in small_copies:
        cp.wait()
    mod_v[6] = jnp.broadcast_to(wr_v[...].astype(F32), (8, D))
    cf = c_v[...].astype(F32)
    sil = (cf * jax.nn.sigmoid(cf)).astype(BF)
    sc = jnp.broadcast_to(sil, (16, D))
    for k in range(8):
        sb_v[pl.ds(128 * k, 128), :] = jnp.broadcast_to(
            sil[:, 128 * k:128 * k + 128].astype(F32), (128, 128)).T

    mq_copy(0, 1).start()
    x0_copy.wait()
    unit_copy(0).start()
    unit_copy(1).start()

    LNB = X0 // 4

    def ln0(i, carry):
        r0 = pl.multiple_of(i * LNB, 8)
        ln = _b2(_layernorm(_f3(x_v[pl.ds(r0, LNB), :])))
        for q in range(4):
            h_v[q, pl.ds(r0, LNB), :] = ln[:, q * QK:(q + 1) * QK]
        return carry
    lax.fori_loop(0, 4, ln0, 0)

    def shift_scale(acc):
        y = _rb(acc)
        return y[:, :QK], _rb(1.0 + y[:, QK:])

    def modulated(q, r0, n, sh, sca):
        ln = h_v[q, pl.ds(r0, n), :].astype(F32).reshape(n // 8, 8, QK)
        return (_rb(ln * sca) + sh).reshape(n, QK).astype(BF)

    for part in range(2):
        mq_copy(0, part).wait()
    acc0 = jnp.dot(sc, wmod_v[0], preferred_element_type=F32)[0:8]
    macc_v[0] = acc0
    hp_v[0] = pltpu.bitcast(modulated(0, 0, BULK, *shift_scale(acc0)), U32)
    unit_copy(0).wait()
    unit_copy(2).start()

    def relayout0(i, carry):
        relayout(2 * D + pl.multiple_of(i * 128, 128), i * 64, 128)
        return carry
    lax.fori_loop(0, QK // 128, relayout0, 0)
    mq_copy(1, 0).start()
    mq_copy(1, 1).start()
    unit_copy(3).start()

    def mod_rows(slab, r0, n, acc):
        for r in range(r0, r0 + n, 8):
            sv = sb_v[pl.ds(r, 8), :]
            t = wmod_v[slab, pl.ds(r, 8), :].astype(F32) * jnp.concatenate([sv] * 4, axis=1)
            acc = t if acc is None else acc + t
        return acc

    def tie_lhs(col, never, toks):
        return jnp.concatenate(
            [jnp.where(never, toks[j], col[8 * j:8 * j + 8]) if j in toks
             else col[8 * j:8 * j + 8] for j in range(32)], axis=0)

    def add_tok(toks, j, tk):
        toks[j] = tk if j not in toks else toks[j] ^ tk

    starts = {0: [unit_copy(4)], 1: [unit_copy(5), piece_copy(3, 5, 0, 256)],
              2: [unit_copy(6), mq_copy(2, 0), mq_copy(2, 1)],
              3: [unit_copy(7), piece_copy(3, 5, 256, 256)], 4: [unit_copy(8)],
              5: [unit_copy(9), mq_copy(3, 0), mq_copy(3, 1)],
              6: [unit_copy(10), unit_copy(11)], 7: [piece_copy(3, 3, 512, 512)],
              8: [piece_copy(4, 4)], 9: [], 10: [wmod_copy(4, 2)], 11: []}

    def quarter_block(b_lo, b_hi, b, carry):
        first, final = b_lo == 0, b_hi == 4 * NP
        q = b_lo // NP
        p = b - NP * q
        if final:
            src = jnp.where(p == 0, 2 * D + 10 * QK, D + 512 * (p - 1))
            sem = 7 - 2 * p
            stage_wait(pl.multiple_of(src, 512), 512, sem)
            b3 = 3 * 8 * PITCH + 256 * (p - 1)
            jobs = [(src, jnp.where(p == 0, 8 * PITCH + 384, b3)),
                    (src + QK, jnp.where(p == 0, 2 * 8 * PITCH + 384, b3 + 128))]
        else:
            src = 2 * D + QK * (b + 1)
            last = p == NP - 1
            stage_wait(pl.multiple_of(src, QK), QK, jnp.where(last, 6, 7 + p))
            jobs = [(src, jnp.where(last, 128 * (q + 1), (p + 1) * (8 * PITCH) + 128 * q))]

            @pl.when(last)
            def _():
                for part in range(2):
                    mq_copy(q + 1, part).wait()
            slab = jnp.where(last, q + 1, q)
        never = jnp.full((8, 128), b, jnp.int32) < 0

        def weights(k):
            return pltpu.bitcast(jnp.concatenate(
                [wqkv_v[pl.ds(pl.multiple_of((8 * p + kk) * PITCH + 128 * q, 8), 128), :]
                 for kk in (k, k + 1)], axis=1), BF)

        groups = [(s_ + 16 * g, d_ + 8 * g) for s_, d_ in jobs for g in range(QK // 16)]
        per = len(groups) // 4
        acc = None
        w = weights(0)
        for n, k in enumerate(range(0, 8, 2)):
            w_next = weights(k + 2) if k < 6 else None
            toks = {}
            for g in range(per):
                add_tok(toks, 4 + (g * 24) // per, relayout(*groups[n * per + g], 16))
            if not final and n < 2:
                for g in range(16):
                    acc = mod_rows(slab, 512 * n + 32 * g, 32, acc)
                    add_tok(toks, 2 * g + (n == 0), token(acc[:, :256] + acc[:, 256:]))
            if not final and n == 2:
                tot = jnp.broadcast_to(jnp.sum(acc, axis=0, keepdims=True), (8, 512))
                macc_v[q + 1] = tot
                sh, sca = shift_scale(tot)
            if not final and n >= 2:
                for g in range(16):
                    r0 = 256 * (n - 2) + 16 * g
                    hb = pltpu.bitcast(modulated(q + 1, r0, 16, sh, sca), U32)
                    hp_v[q + 1, pl.ds(r0 // 2, 8), :] = hb
                    add_tok(toks, (8 + (g * 3) // 2) if n == 2 else 2 * g,
                            hb[:, :128] ^ hb[:, 128:])
            lhs = jnp.concatenate([tie_lhs(hp_v[q, :, pl.ds(0, 128)], never, toks),
                                   hp_v[q, :, pl.ds(128, 128)]], axis=1)
            y = jnp.dot(pltpu.bitcast(lhs, BF), w, preferred_element_type=F32)
            if not first:
                y = y + part_v[p, n]
            if final:
                for j in range(2):
                    ring[k + j][p, pl.ds((RING - BULK) // 2, BULK // 2), :] = pltpu.bitcast(
                        y[:, 128 * j:128 * j + 128].astype(BF), U32)
            else:
                part_v[p, n] = y
            w = w_next

        for j in range(b_lo, b_hi):
            if starts[j]:
                @pl.when(b == j)
                def _():
                    for cp in starts[j]:
                        cp.start()
        return carry

    for b_lo, b_hi in ((0, NP), (NP, 2 * NP), (2 * NP, 3 * NP), (3 * NP, 4 * NP)):
        quarters = functools.partial(quarter_block, b_lo, b_hi)
        lax.fori_loop(b_lo, b_hi, quarters, 0)

    def bulk_dot(i, k, never, t, md):
        w = pltpu.bitcast(wqkv_v[pl.ds(pl.multiple_of((8 * i + k) * PITCH, 8), 512), :], BF)
        cols = [hp_v[c // 2, :, pl.ds(128 * (c % 2), 128)] for c in range(8)]
        toks = {}
        for g in range(8):
            tk = relayout((t & 1) * D + 128 * k + 16 * g, t * (8 * PITCH) + 64 * k + 8 * g, 16)
            md[1] = mod_rows(md[0], 128 * k + 16 * g, 16, md[1])
            toks[12 + 6 * g] = tk ^ token(md[1][:, :256] + md[1][:, 256:])
        cols[0] = tie_lhs(cols[0], never, toks)
        cols[4] = tie_lhs(cols[4], never, {j - 32: tk for j, tk in toks.items()})
        hb = pltpu.bitcast(jnp.concatenate(cols, axis=1), BF)
        y = jnp.dot(hb, w, preferred_element_type=F32)
        ring[k][i, pl.ds((RING - BULK) // 2, BULK // 2), :] = pltpu.bitcast(y.astype(BF), U32)

    def bulk_qkv(i, carry):
        @pl.when(i < 11)
        def _():
            par = (i + 1) & 1
            stage_wait(pl.multiple_of(par * D, D), D, 4 + par)

        @pl.when(i > NP)
        def _():
            wmod_copy(i, 2 + (i & 1)).wait()

        for j in range(NP, 10):
            @pl.when(i == j)
            def _():
                piece_copy(j + 2, 4 + j % 2).start()

        t = jnp.minimum(i + 1, 11)
        never = jnp.full((8, 128), i, jnp.int32) < 0
        md = [i, None]
        for k in range(8):
            bulk_dot(i, k, never, t, md)
        macc_v[jnp.maximum(i, 4)] = md[1]

        for j in range(NP, 10):
            @pl.when(i == j)
            def _():
                wmod_copy(j + 2, 2 + j % 2).start()
                if j < 9:
                    mid_copies[j - NP + 1].start()
                else:
                    for cp in mid_copies[7:]:
                        cp.start()
        return carry
    mid_copies[0].start()
    lax.fori_loop(NP, 12, bulk_qkv, 0)

    for q in range(4):
        sh, sca = shift_scale(macc_v[q])
        mod_v[0, :, pl.ds(q * QK, QK)] = sh
        mod_v[1, :, pl.ds(q * QK, QK)] = sca
        ho_v[0, pl.ds(BULK, RIDE), pl.ds(q * QK, QK)] = modulated(q, BULK, RIDE, sh, sca)
    for k in range(4, 12):
        y = _rb(jnp.sum(macc_v[k], axis=0, keepdims=True))
        if k // 2 == 4:
            y = _rb(1.0 + y)
        mod_v[k // 2, :, pl.ds((k % 2) * 512, 512)] = jnp.broadcast_to(y, (8, 512))
    for cp in mid_copies:
        cp.wait()
    x2_copy.start()
    for cp in ffn_copies:
        cp.start()

    scale = DH ** -0.5
    kk = lax.broadcasted_iota(jnp.int32, (M + SEG, 80), 0)
    cc = lax.broadcasted_iota(jnp.int32, (M + SEG, 80), 1)
    second = ((cc >= 8) & (cc < 16)) | (cc >= 48)
    allowed = (cc < 16) | (kk <= jnp.where(second, cc - 40, cc - 8))

    def over_keys(f, fr, v):
        t = v[0:8]
        for j in range(8, M + SEG, 8):
            t = f(t, v[j:j + 8])
        return fr(t, axis=0, keepdims=True)

    def tied(u, never, toks):
        if not toks:
            return u
        parts, at = [], 0
        for j, tk in enumerate(toks):
            r = 64 * j
            if r > at:
                parts.append(u[at:r])
            w = tk.shape[1]
            sel = jnp.where(never[:, :w], tk, u[r:r + 8, :w])
            parts.append(sel if w == 128 else jnp.concatenate([sel, u[r:r + 8, w:]], axis=1))
            at = r + 8
        return jnp.concatenate(parts + [u[at:]], axis=0)

    def w_slab(t, g, lo=0, n=512, never=None, toks=()):
        return pltpu.bitcast(
            tied(wqkv_v[pl.ds((8 * t + g) * PITCH + lo, n), :], never, toks), BF)

    def step(s, mem, chained, left, att_prev):
        odd = left is not None
        wr = pl.multiple_of(lax.rem(12 * s - 4 * odd, RING // 2), 8) + 4 * odd
        rd = pl.multiple_of(lax.rem(16 * s + (RING - BULK) // 2, RING // 2), 16)
        xin = jnp.concatenate(
            [mem, ho_v[0, pl.ds(pl.multiple_of(BULK + RIDE * s, 8), RIDE), :]], axis=0)

        prow = SEG * (s - 1) if odd else jnp.maximum(SEG * s - 40, 0)
        nrow = BULK + RIDE * jnp.minimum(s + 1, NSEG - 1)
        works = [post_work(pl.multiple_of(prow + 8 * q, 8), functools.partial(att_prev, q))
                 for q in range(3 if odd else 5)]
        works += [ln1_work(pl.multiple_of(nrow + 8 * q, 8)) for q in range(RIDE // 8)]
        never = jnp.full((8, 128), s, jnp.int32) < 0
        gap = (SIDE_END - SIDE0 - SIDE_LAT - SIDE_DUE) // len(works)
        sched = {}
        for q, wk in enumerate(works):
            sched.setdefault(SIDE0 + gap * q, []).append(wk[0])
            for c in range(1, len(wk)):
                sched.setdefault(SIDE0 + SIDE_LAT + gap * q + ((c - 1) * gap) // 4,
                                 []).append(wk[c])

        memqkv, probs, wl, new_left, toks = {}, {}, {}, {}, {}
        acc = []
        chain = []

        ndot = [0]

        def proj(g, t_lo, t_hi):
            part = {}
            if chained and ndot[0] == 0:
                for t in range(t_lo, t_lo + 6):
                    part[t] = jnp.dot(xin[:, :512], w_slab(t, g, 0, 256),
                                      preferred_element_type=F32)
            for t0 in range(t_lo, t_hi, 2):
                ys = []
                for t in (t0, t0 + 1):
                    n = ndot[0]
                    ndot[0] += 1
                    if t in part:
                        y = jnp.dot(xin[:, 512:], w_slab(t, g, 256, 256),
                                    preferred_element_type=F32) + part[t]
                    else:
                        y = jnp.dot(xin, w_slab(t, g, 0, 512, never, toks.get(n)),
                                    preferred_element_type=F32)
                    ring[g][t, pl.ds(wr, RIDE // 2), :] = (
                        pltpu.bitcast(y.astype(BF), U32)[M // 2:] if odd
                        else pltpu.bitcast(y[M:].astype(BF), U32))
                    ys.append(y[:M])
                    for item in sched.get(n, ()):
                        tk = item((never, y[:M]))
                        if tk is not None:
                            toks.setdefault(n + SIDE_DUE, []).append(tk)
                memqkv[(t0, g)] = jnp.concatenate(ys, axis=0).astype(BF)

        def cat(t0, g):
            return jnp.concatenate(
                [memqkv[(t0, g)]] + [pltpu.bitcast(ring[g][t, pl.ds(rd, SEG // 2), :], BF)
                                     for t in (t0, t0 + 1)], axis=0)

        def scores(g):
            for p in (0, 2):
                st = lax.dot_general(cat(4 + p, g), cat(p, g), (((1,), (1,)), ((), ())),
                                     preferred_element_type=F32)
                st = jnp.where(second, jnp.concatenate([st[8:16], st[48:80]], axis=0),
                               jnp.concatenate([st[0:8], st[16:48]], axis=0))
                if chain:
                    st = jnp.concatenate(
                        [jnp.where(never[:, :80], chain[-1], st[0:8]), st[8:]], axis=0)
                st = jnp.where(allowed, st * scale, -1e9)
                e = jnp.exp(st - over_keys(jnp.maximum, jnp.max, st))
                l = over_keys(jnp.add, jnp.sum, e)
                chain.append(jnp.broadcast_to(l, (8, 80)))
                rc = pl.reciprocal(l, approx=True)
                e = e * (rc * (2.0 - l * rc))
                e0 = jnp.where(second, 0.0, e)
                e1 = jnp.where(second, e, 0.0)
                probs[(p, g)] = jnp.concatenate(
                    [e0[:M], e1[:M], e0[M:], e1[M:]], axis=0).astype(BF)

        def pv(g):
            for p in (0, 2):
                o = lax.dot_general(probs[(p, g)], cat(8 + p, g), (((0,), (0,)), ((), ())),
                                    preferred_element_type=F32)
                for j in range(2):
                    om, ot = o[8 * j:8 * j + 8], o[16 + 32 * j:48 + 32 * j]
                    if odd:
                        rows = [om, left[(p + j, g)], ot]
                    else:
                        rows = [om, ot[:RIDE]]
                        new_left[(p + j, g)] = ot[RIDE:]
                    wl[(p + j, g)] = jnp.concatenate(rows, axis=0).astype(BF)

        def wo(g):
            a = jnp.concatenate([wl[(o, g)] for o in range(4)], axis=1)
            w = jnp.concatenate(
                [jnp.concatenate([wo_v[n, pl.ds((8 * o + PERM[g]) * DH, DH), :]
                                  for o in range(4)], axis=0) for n in range(2)], axis=1)
            y = jnp.dot(a, w, preferred_element_type=F32)
            acc[:] = [y if not acc else y + acc[0]]

        for op in ORDER.split():
            g = int(op[1])
            if op[0] in "qkvux":
                proj(g, *{"q": (0, 12), "k": (0, 8), "v": (8, 12), "u": (0, 10), "x": (10, 12)}[op[0]])
            else:
                {"s": scores, "p": pv, "w": wo}[op[0]](g)
        y = acc[0].astype(BF)
        return y[:M], y[M:], (None if odd else new_left)

    def out_copy(row0, n, k):
        return pltpu.make_async_copy(ho_v.at[1, pl.ds(row0, n), :],
                                     out_hbm.at[0, pl.ds(row0, n), :], sems.at[3 + k])

    OB = SEG * UNROLL

    def carried(q):
        return att_v[pl.ds(8 * q, 8), :]

    def steps(i, carry):
        @pl.when(i == 16 // UNROLL)
        def _():
            x2_copy.wait()

        mem, left, att_prev = mem_v[...], None, carried
        for u in range(UNROLL):
            mem, att, left = step(i * UNROLL + u, mem, u > 0, left, att_prev)
            att_prev = (lambda a: lambda q: a[8 * q:8 * q + 8])(att)
        mem_v[...] = mem
        att_v[...] = att

        @pl.when(i >= 1)
        def _():
            out_copy(pl.multiple_of((i - 1) * OB, OB), OB, 0).start()
        return carry
    lax.fori_loop(0, NSEG // UNROLL, steps, 0)

    for cp in ffn_copies:
        cp.wait()
    last = []
    for q in range(5):
        for item in post_work(S - 40 + 8 * q, functools.partial(carried, q), last):
            item(None)
    out_copy(S - OB, OB, 0).start()

    def top2(val, idx, valid):
        def reduce(f, v):
            v = f(v, axis=0, keepdims=True)
            return v if v.shape[1] == 1 else f(v, axis=1, keepdims=True)

        def argtop(ok):
            v = jnp.where(ok, val, -jnp.inf)
            m = reduce(jnp.max, v)
            return m, reduce(jnp.min, jnp.where(ok & (v >= m), idx, float(S)))
        m1, i1 = argtop(valid)
        return (m1, i1), argtop(valid & (idx != i1))

    sub1 = lax.broadcasted_iota(jnp.int32, (16, 128), 0)
    lan1 = lax.broadcasted_iota(jnp.int32, (16, 128), 1)
    idx = (sub1 // 8) * 1024 + lan1 * 8 + sub1 % 8
    c_a, c_b = top2(_rb(r_v[...].reshape(16, 128)), idx.astype(F32), idx < S - 40)
    sub2 = lax.broadcasted_iota(jnp.int32, (48, 1), 0)
    val2 = jnp.concatenate([_rb(r) for r in last] + [jnp.where(sub2[:8] == 0, c_a[0], c_b[0])],
                           axis=0)
    idx2 = jnp.where(sub2 < 40, (sub2 + (S - 40)).astype(F32),
                     jnp.where(sub2 == 40, c_a[1], c_b[1]))
    (m_a, i_a), (m_b, i_b) = top2(val2, idx2, sub2 < 42)
    i_a = i_a.astype(jnp.int32)
    i_b = i_b.astype(jnp.int32)
    ia = jnp.clip(i_a[0, 0], 0, S - 1)
    ib = jnp.clip(i_b[0, 0], 0, S - 1)
    blk_a = pl.multiple_of((ia // 8) * 8, 8)
    blk_b = pl.multiple_of((ib // 8) * 8, 8)

    def two(ref):
        return jnp.concatenate([ref[pl.ds(blk_a, 8), :], ref[pl.ds(blk_b, 8), :]], axis=0)

    hs = two(ho_v.at[0])
    acts, y = [], None
    for c in range(FF // 512 + 1):
        if c < FF // 512:
            g = _rb(jnp.dot(hs, wg_v[:, pl.ds(512 * c, 512)], preferred_element_type=F32))
            u = _rb(jnp.dot(hs, wu_v[:, pl.ds(512 * c, 512)], preferred_element_type=F32))
            acts.append((_rb(g * jax.nn.sigmoid(g)) * u).astype(BF))
        if c > 0:
            wd = jnp.concatenate([wd_v[k, pl.ds(512 * (c - 1), 512), :] for k in range(2)],
                                 axis=1)
            t = jnp.dot(acts[c - 1], wd, preferred_element_type=F32)
            y = t if y is None else t + y
    sub = lax.broadcasted_iota(jnp.int32, (16, 1), 0)
    rows = jnp.where(sub < 8, blk_a + sub, blk_b + sub - 8)
    gate = jnp.where(rows == ia, jax.nn.sigmoid(m_a),
                     jnp.where(rows == ib, jax.nn.sigmoid(m_b), 0.0))
    upd = jnp.where((rows == ia) | (rows == ib), y * gate, 0.0).reshape(2, 8, D)
    fin = _b2(_f3(two(ho_v.at[1])) + mod_v[5] * upd)

    out_copy(0, S, 0).wait()
    ho_v[1, pl.ds(blk_a, 8), :] = fin[0:8]
    ho_v[1, pl.ds(blk_b, 8), :] = fin[8:16]
    out_copy(blk_a, 8, 0).start()

    @pl.when(blk_a != blk_b)
    def _():
        out_copy(blk_b, 8, 1).start()
        out_copy(blk_b, 8, 1).wait()
    out_copy(blk_a, 8, 0).wait()


@jax.jit
def pallas_adaLN_cond__memory_aug_recurrent_mem_tr__moe_arch_mod__prompt_kernel(
    A_x, A_mem0, A_Wq, A_Wk, A_Wv, A_Wo, A_seg_len, B_x, B_w_r, B_w_gate, B_w_up, B_w_down, c,
    w_mod,
):
    del B_x
    del A_seg_len
    assert A_x.shape == (1, S, D) and A_Wq.shape == (D, H, DH) and A_mem0.shape == (1, M, D)
    any_spec = pl.BlockSpec(memory_space=pl.ANY)
    scratch = [
        pltpu.VMEM((S, D), BF),
        pltpu.VMEM((4, X0, QK), BF),
        pltpu.VMEM((4, BULK // 2, QK), U32),
        pltpu.VMEM((40, D), BF),
        pltpu.VMEM((2, S, D), BF),
        pltpu.VMEM((96 * PITCH, 128), U32),
        pltpu.VMEM((2, H * DH, 512), BF),
        pltpu.VMEM((5 * D, 8, 128), BF),
        pltpu.VMEM((12, D, 512), BF),
        pltpu.VMEM((D, FF), BF),
        pltpu.VMEM((D, FF), BF),
        pltpu.VMEM((2, FF, 512), BF),
        pltpu.VMEM((M, D), BF),
        pltpu.VMEM((1, D), BF),
        pltpu.VMEM((1, D), BF),
        pltpu.VMEM((7, 8, D), F32),
        pltpu.VMEM((2, 8, 128), F32),
        pltpu.VMEM((D, 128), F32),
        pltpu.VMEM((12, 8, 512), F32),
        pltpu.VMEM((NP, 4, BULK, 256), F32),
        pltpu.SemaphoreType.DMA((9,)),
    ] + [pltpu.VMEM((12, RING // 2, 128), U32)] * 8
    return pl.pallas_call(
        _kernel,
        out_shape=jax.ShapeDtypeStruct((1, S, D), BF),
        in_specs=[any_spec] * 12,
        out_specs=any_spec,
        scratch_shapes=scratch,
        compiler_params=pltpu.CompilerParams(vmem_limit_bytes=120 * 1024 * 1024),
    )(A_x, A_mem0, A_Wq, A_Wk, A_Wv, A_Wo.reshape(H * DH, D), B_w_r.reshape(1, D), B_w_gate,
      B_w_up, B_w_down, c, w_mod)
```

```python
import functools

import jax
import jax.numpy as jnp
from jax import lax
import jax.experimental.pallas as pl
import jax.experimental.pallas.tpu as pltpu

BF = jnp.bfloat16
F32 = jnp.float32
U32 = jnp.uint32

S = 2048
D = 1024
H = 32
DH = 128
M = 8
SEG = 32
NSEG = S // SEG
FF = 3584
RIDE = 24
BULK = S - RIDE * NSEG
X0 = BULK + 32
NRING = 18
PITCH = 520
X1 = 1024
NP = 3
QK = D // 4
UNROLL = 4
EPS = 1e-5
SIDE0, SIDE_LAT, SIDE_DUE, SIDE_END = 2, 6, 6, 82
NEG = -3.0e38
ORDER = ("q0 q1 q2 q3 k4 k5 k6 k7 s0 s1 s2 s3 s4 s5 s6 s7 v4 v5 v6 v7 p0 p1 p2 p3 p4 p5 p6 p7 "
         "w0 w1 w2 w3 w4 w5 w6 w7")
PERM = (0, 2, 4, 6, 1, 3, 5, 7)


def _rb(v):
    return v.astype(BF).astype(F32)


def _layernorm(xf):
    mu = jnp.mean(xf, axis=-1, keepdims=True)
    dv = xf - mu
    var = jnp.mean(dv * dv, axis=-1, keepdims=True)
    sd = _rb(jnp.sqrt(_rb(_rb(var) + EPS)))
    return _rb(_rb(xf - _rb(mu)) * (1.0 / sd))


def _f3(v):
    return v.astype(F32).reshape(v.shape[0] // 8, 8, D)


def _b2(v):
    return v.reshape(v.shape[0] * 8, D).astype(BF)


def _kernel(x_hbm, mem0_hbm, wq_hbm, wk_hbm, wv_hbm, wo_hbm, wr_hbm, wg_hbm, wu_hbm, wd_hbm,
            c_hbm, wmod_hbm, out_hbm,
            x_v, h_v, hp_v, att_v, ho_v, wqkv_v, wo_v, stage, wmod_v,
            wg_v, wu_v, wd_v, mem_v, c_v, wr_v, mod_v, r_v, sb_v, macc_v,
            part_v, sems, *rings):
    w_hbm = (wq_hbm, wk_hbm, wv_hbm)
    ring = rings

    def piece_copy(t, sem, lo=0, n=D, dst=None):
        dst = (t % 2) * D + lo if dst is None else dst
        return pltpu.make_async_copy(
            w_hbm[t // 4].at[pl.ds(lo, n), pl.ds((t % 4) * 8, 8), :],
            stage.at[pl.ds(dst, n)], sems.at[sem])

    def unit_copy(j):
        return piece_copy(j % NP, 6 + min(j, 10) % 3, QK * (j // NP), QK, 2 * D + QK * j)

    def stage_wait(row, n, sem):
        dst = stage.at[pl.ds(row, n)]
        pltpu.make_async_copy(dst, dst, sems.at[sem]).wait()

    def mq_copy(q, part):
        return pltpu.make_async_copy(wmod_hbm.at[:, pl.ds(part * D + q * QK, QK)],
                                     wmod_v.at[q, :, pl.ds(part * QK, QK)], sems.at[2])

    def wmod_copy(k, sem):
        col = k * 512 if isinstance(k, int) else pl.multiple_of(k * 512, 512)
        return pltpu.make_async_copy(wmod_hbm.at[:, pl.ds(col, 512)], wmod_v.at[k], sems.at[sem])

    def x_copy(lo, hi, sem):
        return pltpu.make_async_copy(x_hbm.at[0, pl.ds(lo, hi - lo), :],
                                     x_v.at[pl.ds(lo, hi - lo), :], sems.at[sem])

    def wo_copy(n):
        lo, rows = ((n // 2) * 512, 512) if n < 6 else (1536, 2560)
        return pltpu.make_async_copy(wo_hbm.at[pl.ds(lo, rows), pl.ds((n % 2) * 512, 512)],
                                     wo_v.at[n % 2, pl.ds(lo, rows)], sems.at[0])

    small_copies = [pltpu.make_async_copy(c_hbm, c_v, sems.at[0]),
                    pltpu.make_async_copy(mem0_hbm.at[0], mem_v, sems.at[0]),
                    pltpu.make_async_copy(wr_hbm, wr_v, sems.at[0])]
    x0_copy = x_copy(0, X0, 1)
    mid_copies = ([x_copy(X0, (X0 + X1) // 2, 0), x_copy((X0 + X1) // 2, X1, 0)]
                  + [wo_copy(n) for n in range(8)])
    x2_copy = x_copy(X1, S, 1)
    ffn_copies = [pltpu.make_async_copy(wg_hbm, wg_v, sems.at[2]),
                  pltpu.make_async_copy(wu_hbm, wu_v, sems.at[2])] + [
        pltpu.make_async_copy(wd_hbm.at[:, pl.ds(k * 512, 512)], wd_v.at[k], sems.at[2])
        for k in range(2)]

    def relayout(src, base, n):
        u = pltpu.bitcast(stage[pl.ds(src, n)], U32)
        tok = None
        for i in range(n // 2):
            a = u[2 * i]
            b = u[2 * i + 1]
            even = (a & jnp.uint32(0xFFFF)) | (b << 16)
            odd = (a >> 16) | (b & jnp.uint32(0xFFFF0000))
            wqkv_v[pl.ds(base + i, 4, stride=PITCH), :] = even
            wqkv_v[pl.ds(base + 4 * PITCH + i, 4, stride=PITCH), :] = odd
            tok = even ^ odd if tok is None else tok ^ even ^ odd
        return jnp.concatenate([tok, tok], axis=0)

    CW = 256

    def ln_stats(xf):
        mu = jnp.mean(xf, axis=-1, keepdims=True)
        dv = xf - mu
        var = jnp.mean(dv * dv, axis=-1, keepdims=True)
        sd = _rb(jnp.sqrt(_rb(_rb(var) + EPS)))
        return _rb(mu), 1.0 / sd

    def mod_c(k, c):
        return mod_v[k, :, pl.ds(c * CW, CW)]

    def token(v):
        return pltpu.bitcast(v[:, :128] + v[:, 128:], U32)

    def after(v, trig):
        if trig is None:
            return v
        return jnp.concatenate([jnp.where(trig[0], trig[1], v[:, :128]), v[:, 128:]], axis=1)

    def post_work(row0, att, scores_out=None):
        st = {}

        def head(trig):
            a = after(att().astype(F32), trig)
            st["x2"] = _rb(x_v[pl.ds(row0, 8), :].astype(F32) + _rb(mod_v[2] * a))
            st["mu"], st["inv"] = ln_stats(st["x2"])

        def chunk(c, trig):
            xc = after(st["x2"][:, c * CW:(c + 1) * CW], trig)
            h2b = (_rb(_rb(_rb(xc - st["mu"]) * st["inv"]) * mod_c(4, c))
                   + mod_c(3, c)).astype(BF)
            h2 = h2b.astype(F32)
            ho_v[0, pl.ds(row0, 8), pl.ds(c * CW, CW)] = h2b
            o = xc + mod_c(5, c) * h2
            ho_v[1, pl.ds(row0, 8), pl.ds(c * CW, CW)] = o.astype(BF)
            rp = h2 * mod_c(6, c)
            st["r"] = rp if c == 0 else st["r"] + rp
            if c == D // CW - 1:
                r = jnp.sum(st["r"], axis=-1, keepdims=True)
                if scores_out is not None:
                    scores_out.append(r)
                    return None
                grp = row0 >> 3
                lanes = lax.broadcasted_iota(jnp.int32, (8, 128), 1)
                r_v[grp >> 7] = jnp.where(lanes == (grp & 127), r, r_v[grp >> 7])
            return token(o + st["r"])
        return [head] + [functools.partial(chunk, c) for c in range(D // CW)]

    def ln1_work(row0):
        st = {}

        def head(trig):
            st["x"] = after(x_v[pl.ds(row0, 8), :].astype(F32), trig)
            st["mu"], st["inv"] = ln_stats(st["x"])

        def chunk(c, trig):
            xc = after(st["x"][:, c * CW:(c + 1) * CW], trig)
            h = _rb(_rb(_rb(xc - st["mu"]) * st["inv"]) * mod_c(1, c)) + mod_c(0, c)
            ho_v[0, pl.ds(row0, 8), pl.ds(c * CW, CW)] = h.astype(BF)
            return token(h)
        return [head] + [functools.partial(chunk, c) for c in range(D // CW)]

    for cp in small_copies:
        cp.start()
    x0_copy.start()
    mq_copy(0, 0).start()

    r_v[...] = jnp.full(r_v.shape, NEG, F32)
    att_v[...] = jnp.zeros(att_v.shape, BF)

    for cp in small_copies:
        cp.wait()
    mod_v[6] = jnp.broadcast_to(wr_v[...].astype(F32), (8, D))
    cf = c_v[...].astype(F32)
    sil = (cf * jax.nn.sigmoid(cf)).astype(BF)
    sc = jnp.broadcast_to(sil, (16, D))
    for k in range(8):
        sb_v[pl.ds(128 * k, 128), :] = jnp.broadcast_to(
            sil[:, 128 * k:128 * k + 128].astype(F32), (128, 128)).T

    mq_copy(0, 1).start()
    x0_copy.wait()
    unit_copy(0).start()
    unit_copy(1).start()

    LNB = X0 // 4

    def ln0(i, carry):
        r0 = pl.multiple_of(i * LNB, 8)
        ln = _b2(_layernorm(_f3(x_v[pl.ds(r0, LNB), :])))
        for q in range(4):
            h_v[q, pl.ds(r0, LNB), :] = ln[:, q * QK:(q + 1) * QK]
        return carry
    lax.fori_loop(0, 4, ln0, 0)

    def shift_scale(acc):
        y = _rb(acc)
        return y[:, :QK], _rb(1.0 + y[:, QK:])

    def modulated(q, r0, n, sh, sca):
        ln = h_v[q, pl.ds(r0, n), :].astype(F32).reshape(n // 8, 8, QK)
        return (_rb(ln * sca) + sh).reshape(n, QK).astype(BF)

    for part in range(2):
        mq_copy(0, part).wait()
    acc0 = jnp.dot(sc, wmod_v[0], preferred_element_type=F32)[0:8]
    macc_v[0] = acc0
    hp_v[0] = pltpu.bitcast(modulated(0, 0, BULK, *shift_scale(acc0)), U32)
    unit_copy(0).wait()
    unit_copy(2).start()

    def relayout0(i, carry):
        relayout(2 * D + pl.multiple_of(i * 128, 128), i * 64, 128)
        return carry
    lax.fori_loop(0, QK // 128, relayout0, 0)
    mq_copy(1, 0).start()
    mq_copy(1, 1).start()
    unit_copy(3).start()

    def mod_rows(slab, r0, n, acc):
        for r in range(r0, r0 + n, 8):
            sv = sb_v[pl.ds(r, 8), :]
            t = wmod_v[slab, pl.ds(r, 8), :].astype(F32) * jnp.concatenate([sv] * 4, axis=1)
            acc = t if acc is None else acc + t
        return acc

    def ring_fill(g, t, y):
        ring[g][t >> 1, pl.ds(NRING - BULK // SEG, BULK // SEG),
                pl.ds(pl.multiple_of(16 * (t & 1), 16), 16), :] = (
            pltpu.bitcast(y.astype(BF), U32).reshape(BULK // SEG, 16, 128))

    def tie_lhs(col, never, toks):
        return jnp.concatenate(
            [jnp.where(never, toks[j], col[8 * j:8 * j + 8]) if j in toks
             else col[8 * j:8 * j + 8] for j in range(32)], axis=0)

    def add_tok(toks, j, tk):
        toks[j] = tk if j not in toks else toks[j] ^ tk

    starts = {0: [unit_copy(4)], 1: [unit_copy(5), piece_copy(3, 5, 0, 256)],
              2: [unit_copy(6), mq_copy(2, 0), mq_copy(2, 1)],
              3: [unit_copy(7), piece_copy(3, 5, 256, 256)], 4: [unit_copy(8)],
              5: [unit_copy(9), mq_copy(3, 0), mq_copy(3, 1)],
              6: [unit_copy(10), unit_copy(11)], 7: [piece_copy(3, 3, 512, 512)],
              8: [piece_copy(4, 4)], 9: [], 10: [wmod_copy(4, 2)], 11: []}

    def quarter_block(b_lo, b_hi, b, carry):
        first, final = b_lo == 0, b_hi == 4 * NP
        q = b_lo // NP
        p = b - NP * q
        if final:
            src = jnp.where(p == 0, 2 * D + 10 * QK, D + 512 * (p - 1))
            sem = 7 - 2 * p
            stage_wait(pl.multiple_of(src, 512), 512, sem)
            b3 = 3 * 8 * PITCH + 256 * (p - 1)
            jobs = [(src, jnp.where(p == 0, 8 * PITCH + 384, b3)),
                    (src + QK, jnp.where(p == 0, 2 * 8 * PITCH + 384, b3 + 128))]
        else:
            src = 2 * D + QK * (b + 1)
            last = p == NP - 1
            stage_wait(pl.multiple_of(src, QK), QK, jnp.where(last, 6, 7 + p))
            jobs = [(src, jnp.where(last, 128 * (q + 1), (p + 1) * (8 * PITCH) + 128 * q))]

            @pl.when(last)
            def _():
                for part in range(2):
                    mq_copy(q + 1, part).wait()
            slab = jnp.where(last, q + 1, q)
        never = jnp.full((8, 128), b, jnp.int32) < 0

        def weights(k):
            return pltpu.bitcast(jnp.concatenate(
                [wqkv_v[pl.ds(pl.multiple_of((8 * p + kk) * PITCH + 128 * q, 8), 128), :]
                 for kk in (k, k + 1)], axis=1), BF)

        groups = [(s_ + 16 * g, d_ + 8 * g) for s_, d_ in jobs for g in range(QK // 16)]
        per = len(groups) // 4
        acc = None
        w = weights(0)
        for n, k in enumerate(range(0, 8, 2)):
            w_next = weights(k + 2) if k < 6 else None
            toks = {}
            for g in range(per):
                add_tok(toks, 4 + (g * 24) // per, relayout(*groups[n * per + g], 16))
            if not final and n < 2:
                for g in range(16):
                    acc = mod_rows(slab, 512 * n + 32 * g, 32, acc)
                    add_tok(toks, 2 * g + (n == 0), token(acc[:, :256] + acc[:, 256:]))
            if not final and n == 2:
                tot = jnp.broadcast_to(jnp.sum(acc, axis=0, keepdims=True), (8, 512))
                macc_v[q + 1] = tot
                sh, sca = shift_scale(tot)
            if not final and n >= 2:
                for g in range(16):
                    r0 = 256 * (n - 2) + 16 * g
                    hb = pltpu.bitcast(modulated(q + 1, r0, 16, sh, sca), U32)
                    hp_v[q + 1, pl.ds(r0 // 2, 8), :] = hb
                    add_tok(toks, (8 + (g * 3) // 2) if n == 2 else 2 * g,
                            hb[:, :128] ^ hb[:, 128:])
            lhs = jnp.concatenate([tie_lhs(hp_v[q, :, pl.ds(0, 128)], never, toks),
                                   hp_v[q, :, pl.ds(128, 128)]], axis=1)
            y = jnp.dot(pltpu.bitcast(lhs, BF), w, preferred_element_type=F32)
            if not first:
                y = y + part_v[p, n]
            if final:
                for j in range(2):
                    ring_fill(k + j, p, y[:, 128 * j:128 * j + 128])
            else:
                part_v[p, n] = y
            w = w_next

        for j in range(b_lo, b_hi):
            if starts[j]:
                @pl.when(b == j)
                def _():
                    for cp in starts[j]:
                        cp.start()
        return carry

    for b_lo, b_hi in ((0, NP), (NP, 2 * NP), (2 * NP, 3 * NP), (3 * NP, 4 * NP)):
        quarters = functools.partial(quarter_block, b_lo, b_hi)
        lax.fori_loop(b_lo, b_hi, quarters, 0)

    def bulk_dot(i, k, never, t, md):
        w = pltpu.bitcast(wqkv_v[pl.ds(pl.multiple_of((8 * i + k) * PITCH, 8), 512), :], BF)
        cols = [hp_v[c // 2, :, pl.ds(128 * (c % 2), 128)] for c in range(8)]
        toks = {}
        for g in range(8):
            tk = relayout((t & 1) * D + 128 * k + 16 * g, t * (8 * PITCH) + 64 * k + 8 * g, 16)
            md[1] = mod_rows(md[0], 128 * k + 16 * g, 16, md[1])
            toks[12 + 6 * g] = tk ^ token(md[1][:, :256] + md[1][:, 256:])
        cols[0] = tie_lhs(cols[0], never, toks)
        cols[4] = tie_lhs(cols[4], never, {j - 32: tk for j, tk in toks.items()})
        hb = pltpu.bitcast(jnp.concatenate(cols, axis=1), BF)
        y = jnp.dot(hb, w, preferred_element_type=F32)
        ring_fill(k, i, y)

    def bulk_qkv(i, carry):
        @pl.when(i < 11)
        def _():
            par = (i + 1) & 1
            stage_wait(pl.multiple_of(par * D, D), D, 4 + par)

        @pl.when(i > NP)
        def _():
            wmod_copy(i, 2 + (i & 1)).wait()

        for j in range(NP, 10):
            @pl.when(i == j)
            def _():
                piece_copy(j + 2, 4 + j % 2).start()

        t = jnp.minimum(i + 1, 11)
        never = jnp.full((8, 128), i, jnp.int32) < 0
        md = [i, None]
        for k in range(8):
            bulk_dot(i, k, never, t, md)
        macc_v[jnp.maximum(i, 4)] = md[1]

        for j in range(NP, 10):
            @pl.when(i == j)
            def _():
                wmod_copy(j + 2, 2 + j % 2).start()
                if j < 9:
                    mid_copies[j - NP + 1].start()
                else:
                    for cp in mid_copies[7:]:
                        cp.start()
        return carry
    mid_copies[0].start()
    lax.fori_loop(NP, 12, bulk_qkv, 0)

    for q in range(4):
        sh, sca = shift_scale(macc_v[q])
        mod_v[0, :, pl.ds(q * QK, QK)] = sh
        mod_v[1, :, pl.ds(q * QK, QK)] = sca
        ho_v[0, pl.ds(BULK, RIDE), pl.ds(q * QK, QK)] = modulated(q, BULK, RIDE, sh, sca)
    for k in range(4, 12):
        y = _rb(jnp.sum(macc_v[k], axis=0, keepdims=True))
        if k // 2 == 4:
            y = _rb(1.0 + y)
        mod_v[k // 2, :, pl.ds((k % 2) * 512, 512)] = jnp.broadcast_to(y, (8, 512))
    for cp in mid_copies:
        cp.wait()
    x2_copy.start()
    for cp in ffn_copies:
        cp.start()

    scale = DH ** -0.5
    kk = lax.broadcasted_iota(jnp.int32, (M + SEG, 80), 0)
    cc = lax.broadcasted_iota(jnp.int32, (M + SEG, 80), 1)
    second = ((cc >= 8) & (cc < 16)) | (cc >= 48)
    allowed = (cc < 16) | (kk <= jnp.where(second, cc - 40, cc - 8))

    def over_keys(f, fr, v):
        t = v[0:8]
        for j in range(8, M + SEG, 8):
            t = f(t, v[j:j + 8])
        return fr(t, axis=0, keepdims=True)

    def tied(u, never, toks):
        if not toks:
            return u
        parts, at = [], 0
        for j, tk in enumerate(toks):
            r = 64 * j
            if r > at:
                parts.append(u[at:r])
            w = tk.shape[1]
            sel = jnp.where(never[:, :w], tk, u[r:r + 8, :w])
            parts.append(sel if w == 128 else jnp.concatenate([sel, u[r:r + 8, w:]], axis=1))
            at = r + 8
        return jnp.concatenate(parts + [u[at:]], axis=0)

    def w_slab(t, g, lo=0, n=512, never=None, toks=()):
        return pltpu.bitcast(
            tied(wqkv_v[pl.ds((8 * t + g) * PITCH + lo, n), :], never, toks), BF)

    def step(s, u, mem, left, att_prev):
        odd = left is not None
        wr = 3 * lax.rem(s >> 2, NRING // 3)
        rd = lax.rem(s + NRING - BULK // SEG, NRING)

        def ring_put(g, t, y):
            if odd:
                u32 = pltpu.bitcast(y.astype(BF), U32)
                parts = [(3 * u, u32[4:8]), (3 * u + 1, u32[8:16])]
            else:
                u32 = pltpu.bitcast(y[M:].astype(BF), U32)
                parts = [(3 * u, u32[0:8]), (3 * u + 2, u32[8:12])]
            for grp, v in parts:
                ring[g][t // 2, wr + grp // 4,
                        pl.ds(16 * (t % 2) + 4 * (grp % 4), v.shape[0]), :] = v

        xin = jnp.concatenate(
            [mem, ho_v[0, pl.ds(pl.multiple_of(BULK + RIDE * s, 8), RIDE), :]], axis=0)

        prow = SEG * (s - 1) if odd else jnp.maximum(SEG * s - 40, 0)
        nrow = BULK + RIDE * jnp.minimum(s + 1, NSEG - 1)
        works = [post_work(pl.multiple_of(prow + 8 * q, 8), functools.partial(att_prev, q))
                 for q in range(3 if odd else 5)]
        works += [ln1_work(pl.multiple_of(nrow + 8 * q, 8)) for q in range(RIDE // 8)]
        never = jnp.full((8, 128), s, jnp.int32) < 0
        gap = (SIDE_END - SIDE0 - SIDE_LAT - SIDE_DUE) // len(works)
        sched = {}
        for q, wk in enumerate(works):
            sched.setdefault(SIDE0 + gap * q, []).append(wk[0])
            for c in range(1, len(wk)):
                sched.setdefault(SIDE0 + SIDE_LAT + gap * q + ((c - 1) * gap) // 4,
                                 []).append(wk[c])

        memqkv, probs, wl, new_left, toks = {}, {}, {}, {}, {}
        acc = []
        chain = []

        ndot = [0]

        def proj(g, t_lo, t_hi):
            part = {}
            if u > 0 and ndot[0] == 0:
                for t in range(t_lo, t_lo + 6):
                    part[t] = jnp.dot(xin[:, :512], w_slab(t, g, 0, 256),
                                      preferred_element_type=F32)
            for t0 in range(t_lo, t_hi, 2):
                ys = []
                for t in (t0, t0 + 1):
                    n = ndot[0]
                    ndot[0] += 1
                    if t in part:
                        y = jnp.dot(xin[:, 512:], w_slab(t, g, 256, 256),
                                    preferred_element_type=F32) + part[t]
                    else:
                        y = jnp.dot(xin, w_slab(t, g, 0, 512, never, toks.get(n)),
                                    preferred_element_type=F32)
                    ring_put(g, t, y)
                    ys.append(y[:M])
                    for item in sched.get(n, ()):
                        tk = item((never, y[:M]))
                        if tk is not None:
                            toks.setdefault(n + SIDE_DUE, []).append(tk)
                memqkv[(t0, g)] = jnp.concatenate(ys, axis=0).astype(BF)

        def cat(t0, g):
            return jnp.concatenate(
                [memqkv[(t0, g)], pltpu.bitcast(ring[g][t0 // 2, rd], BF)], axis=0)

        def scores(g):
            for p in (0, 2):
                st = lax.dot_general(cat(4 + p, g), cat(p, g), (((1,), (1,)), ((), ())),
                                     preferred_element_type=F32)
                st = jnp.where(second, jnp.concatenate([st[8:16], st[48:80]], axis=0),
                               jnp.concatenate([st[0:8], st[16:48]], axis=0))
                if chain:
                    st = jnp.concatenate(
                        [jnp.where(never[:, :80], chain[-1], st[0:8]), st[8:]], axis=0)
                st = jnp.where(allowed, st * scale, -1e9)
                e = jnp.exp(st - over_keys(jnp.maximum, jnp.max, st))
                l = over_keys(jnp.add, jnp.sum, e)
                chain.append(jnp.broadcast_to(l, (8, 80)))
                rc = pl.reciprocal(l, approx=True)
                e = e * (rc * (2.0 - l * rc))
                e0 = jnp.where(second, 0.0, e)
                e1 = jnp.where(second, e, 0.0)
                probs[(p, g)] = jnp.concatenate(
                    [e0[:M], e1[:M], e0[M:], e1[M:]], axis=0).astype(BF)

        def pv(g):
            for p in (0, 2):
                o = lax.dot_general(probs[(p, g)], cat(8 + p, g), (((0,), (0,)), ((), ())),
                                    preferred_element_type=F32)
                for j in range(2):
                    om, ot = o[8 * j:8 * j + 8], o[16 + 32 * j:48 + 32 * j]
                    if odd:
                        rows = [om, left[(p + j, g)], ot]
                    else:
                        rows = [om, ot[:RIDE]]
                        new_left[(p + j, g)] = ot[RIDE:]
                    wl[(p + j, g)] = jnp.concatenate(rows, axis=0).astype(BF)

        def wo(g):
            a = jnp.concatenate([wl[(o, g)] for o in range(4)], axis=1)
            w = jnp.concatenate(
                [jnp.concatenate([wo_v[n, pl.ds((8 * o + PERM[g]) * DH, DH), :]
                                  for o in range(4)], axis=0) for n in range(2)], axis=1)
            y = jnp.dot(a, w, preferred_element_type=F32)
            acc[:] = [y if not acc else y + acc[0]]

        for op in ORDER.split():
            g = int(op[1])
            if op[0] in "qkvux":
                proj(g, *{"q": (0, 12), "k": (0, 8), "v": (8, 12), "u": (0, 10), "x": (10, 12)}[op[0]])
            else:
                {"s": scores, "p": pv, "w": wo}[op[0]](g)
        y = acc[0].astype(BF)
        return y[:M], y[M:], (None if odd else new_left)

    def out_copy(row0, n, k):
        return pltpu.make_async_copy(ho_v.at[1, pl.ds(row0, n), :],
                                     out_hbm.at[0, pl.ds(row0, n), :], sems.at[3 + k])

    OB = SEG * UNROLL

    def carried(q):
        return att_v[pl.ds(8 * q, 8), :]

    def steps(i, carry):
        @pl.when(i == 16 // UNROLL)
        def _():
            x2_copy.wait()

        mem, left, att_prev = mem_v[...], None, carried
        for u in range(UNROLL):
            mem, att, left = step(i * UNROLL + u, u, mem, left, att_prev)
            att_prev = (lambda a: lambda q: a[8 * q:8 * q + 8])(att)
        mem_v[...] = mem
        att_v[...] = att

        @pl.when(i >= 1)
        def _():
            out_copy(pl.multiple_of((i - 1) * OB, OB), OB, 0).start()
        return carry
    lax.fori_loop(0, NSEG // UNROLL, steps, 0)

    for cp in ffn_copies:
        cp.wait()
    last = []
    for q in range(5):
        for item in post_work(S - 40 + 8 * q, functools.partial(carried, q), last):
            item(None)
    out_copy(S - OB, OB, 0).start()

    def top2(val, idx, valid):
        def reduce(f, v):
            v = f(v, axis=0, keepdims=True)
            return v if v.shape[1] == 1 else f(v, axis=1, keepdims=True)

        def argtop(ok):
            v = jnp.where(ok, val, -jnp.inf)
            m = reduce(jnp.max, v)
            return m, reduce(jnp.min, jnp.where(ok & (v >= m), idx, float(S)))
        m1, i1 = argtop(valid)
        return (m1, i1), argtop(valid & (idx != i1))

    sub1 = lax.broadcasted_iota(jnp.int32, (16, 128), 0)
    lan1 = lax.broadcasted_iota(jnp.int32, (16, 128), 1)
    idx = (sub1 // 8) * 1024 + lan1 * 8 + sub1 % 8
    c_a, c_b = top2(_rb(r_v[...].reshape(16, 128)), idx.astype(F32), idx < S - 40)
    sub2 = lax.broadcasted_iota(jnp.int32, (48, 1), 0)
    val2 = jnp.concatenate([_rb(r) for r in last] + [jnp.where(sub2[:8] == 0, c_a[0], c_b[0])],
                           axis=0)
    idx2 = jnp.where(sub2 < 40, (sub2 + (S - 40)).astype(F32),
                     jnp.where(sub2 == 40, c_a[1], c_b[1]))
    (m_a, i_a), (m_b, i_b) = top2(val2, idx2, sub2 < 42)
    i_a = i_a.astype(jnp.int32)
    i_b = i_b.astype(jnp.int32)
    ia = jnp.clip(i_a[0, 0], 0, S - 1)
    ib = jnp.clip(i_b[0, 0], 0, S - 1)
    blk_a = pl.multiple_of((ia // 8) * 8, 8)
    blk_b = pl.multiple_of((ib // 8) * 8, 8)

    def two(ref):
        return jnp.concatenate([ref[pl.ds(blk_a, 8), :], ref[pl.ds(blk_b, 8), :]], axis=0)

    hs = two(ho_v.at[0])
    acts, y = [], None
    for c in range(FF // 512 + 1):
        if c < FF // 512:
            g = _rb(jnp.dot(hs, wg_v[:, pl.ds(512 * c, 512)], preferred_element_type=F32))
            u = _rb(jnp.dot(hs, wu_v[:, pl.ds(512 * c, 512)], preferred_element_type=F32))
            acts.append((_rb(g * jax.nn.sigmoid(g)) * u).astype(BF))
        if c > 0:
            wd = jnp.concatenate([wd_v[k, pl.ds(512 * (c - 1), 512), :] for k in range(2)],
                                 axis=1)
            t = jnp.dot(acts[c - 1], wd, preferred_element_type=F32)
            y = t if y is None else t + y
    sub = lax.broadcasted_iota(jnp.int32, (16, 1), 0)
    rows = jnp.where(sub < 8, blk_a + sub, blk_b + sub - 8)
    gate = jnp.where(rows == ia, jax.nn.sigmoid(m_a),
                     jnp.where(rows == ib, jax.nn.sigmoid(m_b), 0.0))
    upd = jnp.where((rows == ia) | (rows == ib), y * gate, 0.0).reshape(2, 8, D)
    fin = _b2(_f3(two(ho_v.at[1])) + mod_v[5] * upd)

    out_copy(0, S, 0).wait()
    ho_v[1, pl.ds(blk_a, 8), :] = fin[0:8]
    ho_v[1, pl.ds(blk_b, 8), :] = fin[8:16]
    out_copy(blk_a, 8, 0).start()

    @pl.when(blk_a != blk_b)
    def _():
        out_copy(blk_b, 8, 1).start()
        out_copy(blk_b, 8, 1).wait()
    out_copy(blk_a, 8, 0).wait()


@jax.jit
def pallas_adaLN_cond__memory_aug_recurrent_mem_tr__moe_arch_mod__prompt_kernel(
    A_x, A_mem0, A_Wq, A_Wk, A_Wv, A_Wo, A_seg_len, B_x, B_w_r, B_w_gate, B_w_up, B_w_down, c,
    w_mod,
):
    del B_x
    del A_seg_len
    assert A_x.shape == (1, S, D) and A_Wq.shape == (D, H, DH) and A_mem0.shape == (1, M, D)
    any_spec = pl.BlockSpec(memory_space=pl.ANY)
    scratch = [
        pltpu.VMEM((S, D), BF),
        pltpu.VMEM((4, X0, QK), BF),
        pltpu.VMEM((4, BULK // 2, QK), U32),
        pltpu.VMEM((40, D), BF),
        pltpu.VMEM((2, S, D), BF),
        pltpu.VMEM((96 * PITCH, 128), U32),
        pltpu.VMEM((2, H * DH, 512), BF),
        pltpu.VMEM((5 * D, 8, 128), BF),
        pltpu.VMEM((12, D, 512), BF),
        pltpu.VMEM((D, FF), BF),
        pltpu.VMEM((D, FF), BF),
        pltpu.VMEM((2, FF, 512), BF),
        pltpu.VMEM((M, D), BF),
        pltpu.VMEM((1, D), BF),
        pltpu.VMEM((1, D), BF),
        pltpu.VMEM((7, 8, D), F32),
        pltpu.VMEM((2, 8, 128), F32),
        pltpu.VMEM((D, 128), F32),
        pltpu.VMEM((12, 8, 512), F32),
        pltpu.VMEM((NP, 4, BULK, 256), F32),
        pltpu.SemaphoreType.DMA((9,)),
    ] + [pltpu.VMEM((6, NRING, 32, 128), U32)] * 8
    return pl.pallas_call(
        _kernel,
        out_shape=jax.ShapeDtypeStruct((1, S, D), BF),
        in_specs=[any_spec] * 12,
        out_specs=any_spec,
        scratch_shapes=scratch,
        compiler_params=pltpu.CompilerParams(vmem_limit_bytes=120 * 1024 * 1024),
    )(A_x, A_mem0, A_Wq, A_Wk, A_Wv, A_Wo.reshape(H * DH, D), B_w_r.reshape(1, D), B_w_gate,
      B_w_up, B_w_down, c, w_mod)
```

```python
import functools

import jax
import jax.numpy as jnp
from jax import lax
import jax.experimental.pallas as pl
import jax.experimental.pallas.tpu as pltpu

BF = jnp.bfloat16
F32 = jnp.float32
U32 = jnp.uint32

S = 2048
D = 1024
H = 32
DH = 128
M = 8
SEG = 32
NSEG = S // SEG
FF = 3584
RIDE = 24
BULK = S - RIDE * NSEG
X0 = BULK + 32
NRING = 18
PITCH = 520
X1 = 1024
NP = 3
QK = D // 4
UNROLL = 4
EPS = 1e-5
SIDE0, SIDE_LAT, SIDE_DUE, SIDE_END = 0, 6, 6, 78
NEG = -3.0e38
ORDER = ("q0 q1 q2 q3 k4 k5 k6 k7 s0 s1 s2 s3 s4 s5 s6 s7 v4 v5 v6 v7 p0 p1 p2 p3 p4 p5 p6 p7 "
         "w0 w1 w2 w3 w4 w5 w6 w7")
PERM = (0, 2, 4, 6, 1, 3, 5, 7)


def _rb(v):
    return v.astype(BF).astype(F32)


def _layernorm(xf):
    mu = jnp.mean(xf, axis=-1, keepdims=True)
    dv = xf - mu
    var = jnp.mean(dv * dv, axis=-1, keepdims=True)
    sd = _rb(jnp.sqrt(_rb(_rb(var) + EPS)))
    return _rb(_rb(xf - _rb(mu)) * (1.0 / sd))


def _f3(v):
    return v.astype(F32).reshape(v.shape[0] // 8, 8, D)


def _b2(v):
    return v.reshape(v.shape[0] * 8, D).astype(BF)


def _kernel(x_hbm, mem0_hbm, wq_hbm, wk_hbm, wv_hbm, wo_hbm, wr_hbm, wg_hbm, wu_hbm, wd_hbm,
            c_hbm, wmod_hbm, out_hbm,
            x_v, h_v, hp_v, att_v, ho_v, wqkv_v, wo_v, stage, wmod_v,
            wg_v, wu_v, wd_v, mem_v, cw_v, mod_v, r_v, sb_v, macc_v,
            part_v, sems, *rings):
    w_hbm = (wq_hbm, wk_hbm, wv_hbm)
    ring = rings

    def piece_copy(t, sem, lo=0, n=D, dst=None):
        dst = (t % 2) * D + lo if dst is None else dst
        return pltpu.make_async_copy(
            w_hbm[t // 4].at[pl.ds(lo, n), pl.ds((t % 4) * 8, 8), :],
            stage.at[pl.ds(dst, n)], sems.at[sem])

    def unit_copy(j):
        return piece_copy(j % NP, 6 + min(j, 10) % 3, QK * (j // NP), QK, 2 * D + QK * j)

    def stage_wait(row, n, sem):
        dst = stage.at[pl.ds(row, n)]
        pltpu.make_async_copy(dst, dst, sems.at[sem]).wait()

    def mq_copy(q, part):
        return pltpu.make_async_copy(wmod_hbm.at[:, pl.ds(part * D + q * QK, QK)],
                                     wmod_v.at[q, :, pl.ds(part * QK, QK)], sems.at[2])

    def wmod_copy(k, sem):
        col = k * 512 if isinstance(k, int) else pl.multiple_of(k * 512, 512)
        return pltpu.make_async_copy(wmod_hbm.at[:, pl.ds(col, 512)], wmod_v.at[k], sems.at[sem])

    def x_copy(lo, hi, sem):
        return pltpu.make_async_copy(x_hbm.at[0, pl.ds(lo, hi - lo), :],
                                     x_v.at[pl.ds(lo, hi - lo), :], sems.at[sem])

    def wo_copy(n):
        lo, rows = ((n // 2) * 512, 512) if n < 6 else (1536, 2560)
        return pltpu.make_async_copy(wo_hbm.at[pl.ds(lo, rows), pl.ds((n % 2) * 512, 512)],
                                     wo_v.at[n % 2, pl.ds(lo, rows)], sems.at[0])

    small_copies = [pltpu.make_async_copy(c_hbm, cw_v.at[0], sems.at[0]),
                    pltpu.make_async_copy(mem0_hbm.at[0], mem_v, sems.at[0]),
                    pltpu.make_async_copy(wr_hbm, cw_v.at[1], sems.at[0])]
    x0_copy = x_copy(0, X0, 1)
    mid_copies = ([x_copy(X0, (X0 + X1) // 2, 0), x_copy((X0 + X1) // 2, X1, 0)]
                  + [wo_copy(n) for n in range(8)])
    x2_copy = x_copy(X1, S, 1)
    ffn_copies = [pltpu.make_async_copy(wg_hbm, wg_v, sems.at[2]),
                  pltpu.make_async_copy(wu_hbm, wu_v, sems.at[2])] + [
        pltpu.make_async_copy(wd_hbm.at[:, pl.ds(k * 512, 512)], wd_v.at[k], sems.at[2])
        for k in range(2)]

    def relayout(src, base, n):
        u = pltpu.bitcast(stage[pl.ds(src, n)], U32)
        tok = None
        for i in range(n // 2):
            a = u[2 * i]
            b = u[2 * i + 1]
            even = (a & jnp.uint32(0xFFFF)) | (b << 16)
            odd = (a >> 16) | (b & jnp.uint32(0xFFFF0000))
            wqkv_v[pl.ds(base + i, 4, stride=PITCH), :] = even
            wqkv_v[pl.ds(base + 4 * PITCH + i, 4, stride=PITCH), :] = odd
            tok = even ^ odd if tok is None else tok ^ even ^ odd
        return jnp.concatenate([tok, tok], axis=0)

    CW = 256

    def ln_stats(xf):
        mu = jnp.mean(xf, axis=-1, keepdims=True)
        dv = xf - mu
        var = jnp.mean(dv * dv, axis=-1, keepdims=True)
        sd = _rb(jnp.sqrt(_rb(_rb(var) + EPS)))
        return _rb(mu), 1.0 / sd

    def mod_c(k, c):
        return mod_v[k, :, pl.ds(c * CW, CW)]

    def token(v):
        return pltpu.bitcast(v[:, :128] + v[:, 128:], U32)

    def after(v, trig):
        if trig is None:
            return v
        return jnp.concatenate([jnp.where(trig[0], trig[1], v[:, :128]), v[:, 128:]], axis=1)

    def post_work(row0, att, scores_out=None):
        st = {}

        def head(trig):
            a = after(att().astype(F32), trig)
            st["x2"] = _rb(x_v[pl.ds(row0, 8), :].astype(F32) + _rb(mod_v[2] * a))
            st["mu"], st["inv"] = ln_stats(st["x2"])

        def chunk(c, trig):
            xc = after(st["x2"][:, c * CW:(c + 1) * CW], trig)
            h2b = (_rb(_rb(_rb(xc - st["mu"]) * st["inv"]) * mod_c(4, c))
                   + mod_c(3, c)).astype(BF)
            h2 = h2b.astype(F32)
            ho_v[0, pl.ds(row0, 8), pl.ds(c * CW, CW)] = h2b
            o = xc + mod_c(5, c) * h2
            ho_v[1, pl.ds(row0, 8), pl.ds(c * CW, CW)] = o.astype(BF)
            rp = h2 * mod_c(6, c)
            st["r"] = rp if c == 0 else st["r"] + rp
            if c == D // CW - 1:
                r = jnp.sum(st["r"], axis=-1, keepdims=True)
                if scores_out is not None:
                    scores_out.append(r)
                    return None
                grp = row0 >> 3
                lanes = lax.broadcasted_iota(jnp.int32, (8, 128), 1)
                r_v[grp >> 7] = jnp.where(lanes == (grp & 127), r, r_v[grp >> 7])
            return token(o + st["r"])
        return [head] + [functools.partial(chunk, c) for c in range(D // CW)]

    def ln1_work(row0):
        st = {}

        def head(trig):
            st["x"] = after(x_v[pl.ds(row0, 8), :].astype(F32), trig)
            st["mu"], st["inv"] = ln_stats(st["x"])

        def chunk(c, trig):
            xc = after(st["x"][:, c * CW:(c + 1) * CW], trig)
            h = _rb(_rb(_rb(xc - st["mu"]) * st["inv"]) * mod_c(1, c)) + mod_c(0, c)
            ho_v[0, pl.ds(row0, 8), pl.ds(c * CW, CW)] = h.astype(BF)
            return token(h)
        return [head] + [functools.partial(chunk, c) for c in range(D // CW)]

    for cp in small_copies:
        cp.start()
    x0_copy.start()
    mq_copy(0, 0).start()

    r_v[...] = jnp.full(r_v.shape, NEG, F32)
    att_v[...] = jnp.zeros(att_v.shape, BF)

    for cp in small_copies:
        cp.wait()
    mod_v[6] = jnp.broadcast_to(cw_v[1].astype(F32), (8, D))
    cf = cw_v[0].astype(F32)
    sil = (cf * jax.nn.sigmoid(cf)).astype(BF)
    sc = jnp.broadcast_to(sil, (16, D))
    for k in range(8):
        sb_v[pl.ds(128 * k, 128), :] = jnp.broadcast_to(
            sil[:, 128 * k:128 * k + 128].astype(F32), (128, 128)).T

    mq_copy(0, 1).start()
    x0_copy.wait()
    unit_copy(0).start()
    unit_copy(1).start()

    LNB = X0 // 4

    def ln0(i, carry):
        r0 = pl.multiple_of(i * LNB, 8)
        ln = _b2(_layernorm(_f3(x_v[pl.ds(r0, LNB), :])))
        for q in range(4):
            h_v[q, pl.ds(r0, LNB), :] = ln[:, q * QK:(q + 1) * QK]
        return carry
    lax.fori_loop(0, 4, ln0, 0)

    def shift_scale(acc):
        y = _rb(acc)
        return y[:, :QK], _rb(1.0 + y[:, QK:])

    def modulated(q, r0, n, sh, sca):
        ln = h_v[q, pl.ds(r0, n), :].astype(F32).reshape(n // 8, 8, QK)
        return (_rb(ln * sca) + sh).reshape(n, QK).astype(BF)

    for part in range(2):
        mq_copy(0, part).wait()
    acc0 = jnp.dot(sc, wmod_v[0], preferred_element_type=F32)[0:8]
    macc_v[0] = acc0
    hp_v[0] = pltpu.bitcast(modulated(0, 0, BULK, *shift_scale(acc0)), U32)
    unit_copy(0).wait()
    unit_copy(2).start()

    def relayout0(i, carry):
        relayout(2 * D + pl.multiple_of(i * 128, 128), i * 64, 128)
        return carry
    lax.fori_loop(0, QK // 128, relayout0, 0)
    mq_copy(1, 0).start()
    mq_copy(1, 1).start()
    unit_copy(3).start()

    def mod_rows(slab, r0, n, acc):
        for r in range(r0, r0 + n, 8):
            sv = sb_v[pl.ds(r, 8), :]
            t = wmod_v[slab, pl.ds(r, 8), :].astype(F32) * jnp.concatenate([sv] * 4, axis=1)
            acc = t if acc is None else acc + t
        return acc

    def ring_fill(g, t, y):
        ring[g][t >> 1, pl.ds(NRING - BULK // SEG, BULK // SEG),
                pl.ds(pl.multiple_of(16 * (t & 1), 16), 16), :] = (
            pltpu.bitcast(y.astype(BF), U32).reshape(BULK // SEG, 16, 128))

    def tie_lhs(col, never, toks):
        return jnp.concatenate(
            [jnp.where(never, toks[j], col[8 * j:8 * j + 8]) if j in toks
             else col[8 * j:8 * j + 8] for j in range(32)], axis=0)

    def add_tok(toks, j, tk):
        toks[j] = tk if j not in toks else toks[j] ^ tk

    starts = {0: [unit_copy(4)], 1: [unit_copy(5), piece_copy(3, 5, 0, 256)],
              2: [unit_copy(6), mq_copy(2, 0), mq_copy(2, 1)],
              3: [unit_copy(7), piece_copy(3, 5, 256, 256)], 4: [unit_copy(8)],
              5: [unit_copy(9), mq_copy(3, 0), mq_copy(3, 1)],
              6: [unit_copy(10), unit_copy(11)], 7: [piece_copy(3, 3, 512, 512)],
              8: [piece_copy(4, 4)], 9: [], 10: [wmod_copy(4, 2)], 11: []}

    def quarter_block(b_lo, b_hi, b, carry):
        first, final = b_lo == 0, b_hi == 4 * NP
        q = b_lo // NP
        p = b - NP * q
        if final:
            src = jnp.where(p == 0, 2 * D + 10 * QK, D + 512 * (p - 1))
            sem = 7 - 2 * p
            stage_wait(pl.multiple_of(src, 512), 512, sem)
            b3 = 3 * 8 * PITCH + 256 * (p - 1)
            jobs = [(src, jnp.where(p == 0, 8 * PITCH + 384, b3)),
                    (src + QK, jnp.where(p == 0, 2 * 8 * PITCH + 384, b3 + 128))]
        else:
            src = 2 * D + QK * (b + 1)
            last = p == NP - 1
            stage_wait(pl.multiple_of(src, QK), QK, jnp.where(last, 6, 7 + p))
            jobs = [(src, jnp.where(last, 128 * (q + 1), (p + 1) * (8 * PITCH) + 128 * q))]

            @pl.when(last)
            def _():
                for part in range(2):
                    mq_copy(q + 1, part).wait()
            slab = jnp.where(last, q + 1, q)
        never = jnp.full((8, 128), b, jnp.int32) < 0

        def weights(k):
            return pltpu.bitcast(jnp.concatenate(
                [wqkv_v[pl.ds(pl.multiple_of((8 * p + kk) * PITCH + 128 * q, 8), 128), :]
                 for kk in (k, k + 1)], axis=1), BF)

        groups = [(s_ + 16 * g, d_ + 8 * g) for s_, d_ in jobs for g in range(QK // 16)]
        per = len(groups) // 4
        acc = None
        w = weights(0)
        for n, k in enumerate(range(0, 8, 2)):
            w_next = weights(k + 2) if k < 6 else None
            toks = {}
            for g in range(per):
                add_tok(toks, 4 + (g * 24) // per, relayout(*groups[n * per + g], 16))
            if not final and n < 2:
                for g in range(16):
                    acc = mod_rows(slab, 512 * n + 32 * g, 32, acc)
                    add_tok(toks, 2 * g + (n == 0), token(acc[:, :256] + acc[:, 256:]))
            if not final and n == 2:
                tot = jnp.broadcast_to(jnp.sum(acc, axis=0, keepdims=True), (8, 512))
                macc_v[q + 1] = tot
                sh, sca = shift_scale(tot)
            if not final and n >= 2:
                for g in range(16):
                    r0 = 256 * (n - 2) + 16 * g
                    hb = pltpu.bitcast(modulated(q + 1, r0, 16, sh, sca), U32)
                    hp_v[q + 1, pl.ds(r0 // 2, 8), :] = hb
                    add_tok(toks, (8 + (g * 3) // 2) if n == 2 else 2 * g,
                            hb[:, :128] ^ hb[:, 128:])
            lhs = jnp.concatenate([tie_lhs(hp_v[q, :, pl.ds(0, 128)], never, toks),
                                   hp_v[q, :, pl.ds(128, 128)]], axis=1)
            y = jnp.dot(pltpu.bitcast(lhs, BF), w, preferred_element_type=F32)
            if not first:
                y = y + part_v[p, n]
            if final:
                for j in range(2):
                    ring_fill(k + j, p, y[:, 128 * j:128 * j + 128])
            else:
                part_v[p, n] = y
            w = w_next

        for j in range(b_lo, b_hi):
            if starts[j]:
                @pl.when(b == j)
                def _():
                    for cp in starts[j]:
                        cp.start()
        return carry

    for b_lo, b_hi in ((0, NP), (NP, 2 * NP), (2 * NP, 3 * NP), (3 * NP, 4 * NP)):
        quarters = functools.partial(quarter_block, b_lo, b_hi)
        lax.fori_loop(b_lo, b_hi, quarters, 0)

    def bulk_dot(i, k, never, t, md):
        w = pltpu.bitcast(wqkv_v[pl.ds(pl.multiple_of((8 * i + k) * PITCH, 8), 512), :], BF)
        cols = [hp_v[c // 2, :, pl.ds(128 * (c % 2), 128)] for c in range(8)]
        toks = {}
        for g in range(8):
            tk = relayout((t & 1) * D + 128 * k + 16 * g, t * (8 * PITCH) + 64 * k + 8 * g, 16)
            md[1] = mod_rows(md[0], 128 * k + 16 * g, 16, md[1])
            toks[12 + 6 * g] = tk ^ token(md[1][:, :256] + md[1][:, 256:])
        cols[0] = tie_lhs(cols[0], never, toks)
        cols[4] = tie_lhs(cols[4], never, {j - 32: tk for j, tk in toks.items()})
        hb = pltpu.bitcast(jnp.concatenate(cols, axis=1), BF)
        y = jnp.dot(hb, w, preferred_element_type=F32)
        ring_fill(k, i, y)

    def bulk_qkv(i, carry):
        @pl.when(i < 11)
        def _():
            par = (i + 1) & 1
            stage_wait(pl.multiple_of(par * D, D), D, 4 + par)

        @pl.when(i > NP)
        def _():
            wmod_copy(i, 2 + (i & 1)).wait()

        for j in range(NP, 10):
            @pl.when(i == j)
            def _():
                piece_copy(j + 2, 4 + j % 2).start()

        t = jnp.minimum(i + 1, 11)
        never = jnp.full((8, 128), i, jnp.int32) < 0
        md = [i, None]
        for k in range(8):
            bulk_dot(i, k, never, t, md)
        macc_v[jnp.maximum(i, 4)] = md[1]

        for j in range(NP, 10):
            @pl.when(i == j)
            def _():
                wmod_copy(j + 2, 2 + j % 2).start()
                if j < 9:
                    mid_copies[j - NP + 1].start()
                else:
                    for cp in mid_copies[7:]:
                        cp.start()
        return carry
    mid_copies[0].start()
    lax.fori_loop(NP, 12, bulk_qkv, 0)

    for q in range(4):
        sh, sca = shift_scale(macc_v[q])
        mod_v[0, :, pl.ds(q * QK, QK)] = sh
        mod_v[1, :, pl.ds(q * QK, QK)] = sca
        ho_v[0, pl.ds(BULK, RIDE), pl.ds(q * QK, QK)] = modulated(q, BULK, RIDE, sh, sca)
    for k in range(4, 12):
        y = _rb(jnp.sum(macc_v[k], axis=0, keepdims=True))
        if k // 2 == 4:
            y = _rb(1.0 + y)
        mod_v[k // 2, :, pl.ds((k % 2) * 512, 512)] = jnp.broadcast_to(y, (8, 512))
    for cp in mid_copies:
        cp.wait()
    x2_copy.start()
    for cp in ffn_copies:
        cp.start()

    scale = DH ** -0.5
    kk = lax.broadcasted_iota(jnp.int32, (M + SEG, 80), 0)
    cc = lax.broadcasted_iota(jnp.int32, (M + SEG, 80), 1)
    second = ((cc >= 8) & (cc < 16)) | (cc >= 48)
    allowed = (cc < 16) | (kk <= jnp.where(second, cc - 40, cc - 8))

    def over_keys(f, fr, v):
        t = v[0:8]
        for j in range(8, M + SEG, 8):
            t = f(t, v[j:j + 8])
        return fr(t, axis=0, keepdims=True)

    def tied(u, never, toks):
        if not toks:
            return u
        parts, at = [], 0
        for j, tk in enumerate(toks):
            r = 64 * j
            if r > at:
                parts.append(u[at:r])
            w = tk.shape[1]
            sel = jnp.where(never[:, :w], tk, u[r:r + 8, :w])
            parts.append(sel if w == 128 else jnp.concatenate([sel, u[r:r + 8, w:]], axis=1))
            at = r + 8
        return jnp.concatenate(parts + [u[at:]], axis=0)

    def w_slab(t, g, lo=0, n=512, never=None, toks=()):
        return pltpu.bitcast(
            tied(wqkv_v[pl.ds((8 * t + g) * PITCH + lo, n), :], never, toks), BF)

    def step(s, u, mem, left, att_prev):
        odd = left is not None
        wr = 3 * lax.rem(s >> 2, NRING // 3)
        rd = lax.rem(s + NRING - BULK // SEG, NRING)

        def ring_put(g, t, y):
            if odd:
                u32 = pltpu.bitcast(y.astype(BF), U32)
                parts = [(3 * u, u32[4:8]), (3 * u + 1, u32[8:16])]
            else:
                u32 = pltpu.bitcast(y[M:].astype(BF), U32)
                parts = [(3 * u, u32[0:8]), (3 * u + 2, u32[8:12])]
            for grp, v in parts:
                ring[g][t // 2, wr + grp // 4,
                        pl.ds(16 * (t % 2) + 4 * (grp % 4), v.shape[0]), :] = v

        xin = jnp.concatenate(
            [mem, ho_v[0, pl.ds(pl.multiple_of(BULK + RIDE * s, 8), RIDE), :]], axis=0)

        prow = SEG * (s - 1) if odd else jnp.maximum(SEG * s - 40, 0)
        nrow = BULK + RIDE * jnp.minimum(s + 1, NSEG - 1)
        works = [post_work(pl.multiple_of(prow + 8 * q, 8), functools.partial(att_prev, q))
                 for q in range(3 if odd else 5)]
        works += [ln1_work(pl.multiple_of(nrow + 8 * q, 8)) for q in range(RIDE // 8)]
        never = jnp.full((8, 128), s, jnp.int32) < 0
        gap = (SIDE_END - SIDE0 - SIDE_LAT - SIDE_DUE) // len(works)
        sched = {}
        for q, wk in enumerate(works):
            sched.setdefault(SIDE0 + gap * q, []).append(wk[0])
            for c in range(1, len(wk)):
                sched.setdefault(SIDE0 + SIDE_LAT + gap * q + ((c - 1) * gap) // 4,
                                 []).append(wk[c])

        memqkv, probs, wl, new_left, toks = {}, {}, {}, {}, {}
        acc = []
        chain = []

        ndot = [0]

        def proj(g, t_lo, t_hi):
            part = {}
            if u > 0 and ndot[0] == 0:
                for t in range(t_lo, t_lo + 6):
                    part[t] = jnp.dot(xin[:, :512], w_slab(t, g, 0, 256),
                                      preferred_element_type=F32)
            for t0 in range(t_lo, t_hi, 2):
                ys = []
                for t in (t0, t0 + 1):
                    n = ndot[0]
                    ndot[0] += 1
                    if t in part:
                        y = jnp.dot(xin[:, 512:], w_slab(t, g, 256, 256),
                                    preferred_element_type=F32) + part[t]
                    else:
                        y = jnp.dot(xin, w_slab(t, g, 0, 512, never, toks.get(n)),
                                    preferred_element_type=F32)
                    ring_put(g, t, y)
                    ys.append(y[:M])
                    for item in sched.get(n, ()):
                        tk = item((never, y[:M]))
                        if tk is not None:
                            toks.setdefault(n + SIDE_DUE, []).append(tk)
                memqkv[(t0, g)] = jnp.concatenate(ys, axis=0).astype(BF)

        def cat(t0, g):
            return jnp.concatenate(
                [memqkv[(t0, g)], pltpu.bitcast(ring[g][t0 // 2, rd], BF)], axis=0)

        def scores(g):
            for p in (0, 2):
                if len(chain) < 4:
                    qt = pltpu.bitcast(cat(p, g).T, U32)
                    qt = jnp.concatenate(
                        [jnp.where(never[:, :80], qt[8:16], qt[0:8]), qt[8:]], axis=0)
                    st = jnp.dot(cat(4 + p, g), pltpu.bitcast(qt, BF),
                                 preferred_element_type=F32)
                else:
                    st = lax.dot_general(cat(4 + p, g), cat(p, g), (((1,), (1,)), ((), ())),
                                         preferred_element_type=F32)
                st = jnp.where(second, jnp.concatenate([st[8:16], st[48:80]], axis=0),
                               jnp.concatenate([st[0:8], st[16:48]], axis=0))
                if chain:
                    st = jnp.concatenate(
                        [jnp.where(never[:, :80], chain[-1], st[0:8]), st[8:]], axis=0)
                st = jnp.where(allowed, st * scale, -1e9)
                e = jnp.exp(st - over_keys(jnp.maximum, jnp.max, st))
                l = over_keys(jnp.add, jnp.sum, e)
                chain.append(jnp.broadcast_to(l, (8, 80)))
                rc = pl.reciprocal(l, approx=True)
                e = e * (rc * (2.0 - l * rc))
                e0 = jnp.where(second, 0.0, e)
                e1 = jnp.where(second, e, 0.0)
                probs[(p, g)] = jnp.concatenate(
                    [e0[:M], e1[:M], e0[M:], e1[M:]], axis=0).astype(BF)

        def pv(g):
            for p in (0, 2):
                o = lax.dot_general(probs[(p, g)], cat(8 + p, g), (((0,), (0,)), ((), ())),
                                    preferred_element_type=F32)
                for j in range(2):
                    om, ot = o[8 * j:8 * j + 8], o[16 + 32 * j:48 + 32 * j]
                    if odd:
                        rows = [om, left[(p + j, g)], ot]
                    else:
                        rows = [om, ot[:RIDE]]
                        new_left[(p + j, g)] = ot[RIDE:]
                    wl[(p + j, g)] = jnp.concatenate(rows, axis=0).astype(BF)

        def wo(g):
            a = jnp.concatenate([wl[(o, g)] for o in range(4)], axis=1)
            w = jnp.concatenate(
                [jnp.concatenate([wo_v[n, pl.ds((8 * o + PERM[g]) * DH, DH), :]
                                  for o in range(4)], axis=0) for n in range(2)], axis=1)
            y = jnp.dot(a, w, preferred_element_type=F32)
            acc[:] = [y if not acc else y + acc[0]]

        for op in ORDER.split():
            g = int(op[1])
            if op[0] in "qkvux":
                proj(g, *{"q": (0, 12), "k": (0, 8), "v": (8, 12), "u": (0, 10), "x": (10, 12)}[op[0]])
            else:
                {"s": scores, "p": pv, "w": wo}[op[0]](g)
        y = acc[0].astype(BF)
        return y[:M], y[M:], (None if odd else new_left)

    def out_copy(row0, n, k):
        return pltpu.make_async_copy(ho_v.at[1, pl.ds(row0, n), :],
                                     out_hbm.at[0, pl.ds(row0, n), :], sems.at[3 + k])

    OB = SEG * UNROLL

    def carried(q):
        return att_v[pl.ds(8 * q, 8), :]

    def steps(i, carry):
        @pl.when(i == 16 // UNROLL)
        def _():
            x2_copy.wait()

        mem, left, att_prev = mem_v[...], None, carried
        for u in range(UNROLL):
            mem, att, left = step(i * UNROLL + u, u, mem, left, att_prev)
            att_prev = (lambda a: lambda q: a[8 * q:8 * q + 8])(att)
        mem_v[...] = mem
        att_v[...] = att

        @pl.when(i >= 1)
        def _():
            out_copy(pl.multiple_of((i - 1) * OB, OB), OB, 0).start()
        return carry
    lax.fori_loop(0, NSEG // UNROLL, steps, 0)

    for cp in ffn_copies:
        cp.wait()
    last = []
    for q in range(5):
        for item in post_work(S - 40 + 8 * q, functools.partial(carried, q), last):
            item(None)
    out_copy(S - OB, OB, 0).start()

    def top2(val, idx, valid):
        def reduce(f, v):
            v = f(v, axis=0, keepdims=True)
            return v if v.shape[1] == 1 else f(v, axis=1, keepdims=True)

        def argtop(ok):
            v = jnp.where(ok, val, -jnp.inf)
            m = reduce(jnp.max, v)
            return m, reduce(jnp.min, jnp.where(ok & (v >= m), idx, float(S)))
        m1, i1 = argtop(valid)
        return (m1, i1), argtop(valid & (idx != i1))

    sub1 = lax.broadcasted_iota(jnp.int32, (16, 128), 0)
    lan1 = lax.broadcasted_iota(jnp.int32, (16, 128), 1)
    idx = (sub1 // 8) * 1024 + lan1 * 8 + sub1 % 8
    c_a, c_b = top2(_rb(r_v[pl.ds(0, 2)].reshape(16, 128)), idx.astype(F32), idx < S - 40)
    sub2 = lax.broadcasted_iota(jnp.int32, (48, 1), 0)
    val2 = jnp.concatenate([_rb(r) for r in last] + [jnp.where(sub2[:8] == 0, c_a[0], c_b[0])],
                           axis=0)
    idx2 = jnp.where(sub2 < 40, (sub2 + (S - 40)).astype(F32),
                     jnp.where(sub2 == 40, c_a[1], c_b[1]))
    (m_a, i_a), (m_b, i_b) = top2(val2, idx2, sub2 < 42)
    i_a = i_a.astype(jnp.int32)
    i_b = i_b.astype(jnp.int32)
    ia = jnp.clip(i_a[0, 0], 0, S - 1)
    ib = jnp.clip(i_b[0, 0], 0, S - 1)
    blk_a = pl.multiple_of((ia // 8) * 8, 8)
    blk_b = pl.multiple_of((ib // 8) * 8, 8)

    def two(ref):
        return jnp.concatenate([ref[pl.ds(blk_a, 8), :], ref[pl.ds(blk_b, 8), :]], axis=0)

    hs = two(ho_v.at[0])
    acts, y = [], None
    for c in range(FF // 512 + 1):
        if c < FF // 512:
            g = _rb(jnp.dot(hs, wg_v[:, pl.ds(512 * c, 512)], preferred_element_type=F32))
            u = _rb(jnp.dot(hs, wu_v[:, pl.ds(512 * c, 512)], preferred_element_type=F32))
            acts.append((_rb(g * jax.nn.sigmoid(g)) * u).astype(BF))
        if c > 0:
            wd = jnp.concatenate([wd_v[k, pl.ds(512 * (c - 1), 512), :] for k in range(2)],
                                 axis=1)
            t = jnp.dot(acts[c - 1], wd, preferred_element_type=F32)
            y = t if y is None else t + y
    sub = lax.broadcasted_iota(jnp.int32, (16, 1), 0)
    rows = jnp.where(sub < 8, blk_a + sub, blk_b + sub - 8)
    gate = jnp.where(rows == ia, jax.nn.sigmoid(m_a),
                     jnp.where(rows == ib, jax.nn.sigmoid(m_b), 0.0))
    upd = jnp.where((rows == ia) | (rows == ib), y * gate, 0.0).reshape(2, 8, D)
    fin = _b2(_f3(two(ho_v.at[1])) + mod_v[5] * upd)

    out_copy(0, S, 0).wait()
    ho_v[1, pl.ds(blk_a, 8), :] = fin[0:8]
    ho_v[1, pl.ds(blk_b, 8), :] = fin[8:16]
    out_copy(blk_a, 8, 0).start()

    @pl.when(blk_a != blk_b)
    def _():
        out_copy(blk_b, 8, 1).start()
        out_copy(blk_b, 8, 1).wait()
    out_copy(blk_a, 8, 0).wait()


@jax.jit
def pallas_adaLN_cond__memory_aug_recurrent_mem_tr__moe_arch_mod__prompt_kernel(
    A_x, A_mem0, A_Wq, A_Wk, A_Wv, A_Wo, A_seg_len, B_x, B_w_r, B_w_gate, B_w_up, B_w_down, c,
    w_mod,
):
    del B_x
    del A_seg_len
    assert A_x.shape == (1, S, D) and A_Wq.shape == (D, H, DH) and A_mem0.shape == (1, M, D)
    any_spec = pl.BlockSpec(memory_space=pl.ANY)
    scratch = [
        pltpu.VMEM((S, D), BF),
        pltpu.VMEM((4, X0, QK), BF),
        pltpu.VMEM((4, BULK // 2, QK), U32),
        pltpu.VMEM((40, D), BF),
        pltpu.VMEM((2, S, D), BF),
        pltpu.VMEM((100 * PITCH, 128), U32),
        pltpu.VMEM((2, H * DH, 512), BF),
        pltpu.VMEM((5 * D, 8, 128), BF),
        pltpu.VMEM((12, D, 512), BF),
        pltpu.VMEM((D, FF), BF),
        pltpu.VMEM((D, FF), BF),
        pltpu.VMEM((2, FF, 512), BF),
        pltpu.VMEM((M, D), BF),
        pltpu.VMEM((4, 1, D), BF),
        pltpu.VMEM((7, 8, D), F32),
        pltpu.VMEM((4, 8, 128), F32),
        pltpu.VMEM((D, 128), F32),
        pltpu.VMEM((12, 8, 512), F32),
        pltpu.VMEM((NP, 4, BULK, 256), F32),
        pltpu.SemaphoreType.DMA((9,)),
    ] + [pltpu.VMEM((6, NRING, 32, 128), U32)] * 8
    return pl.pallas_call(
        _kernel,
        out_shape=jax.ShapeDtypeStruct((1, S, D), BF),
        in_specs=[any_spec] * 12,
        out_specs=any_spec,
        scratch_shapes=scratch,
        compiler_params=pltpu.CompilerParams(vmem_limit_bytes=120 * 1024 * 1024),
    )(A_x, A_mem0, A_Wq, A_Wk, A_Wv, A_Wo.reshape(H * DH, D), B_w_r.reshape(1, D), B_w_gate,
      B_w_up, B_w_down, c, w_mod)
```

```python
import functools

import jax
import jax.numpy as jnp
from jax import lax
import jax.experimental.pallas as pl
import jax.experimental.pallas.tpu as pltpu

BF = jnp.bfloat16
F32 = jnp.float32
U32 = jnp.uint32

S = 2048
D = 1024
H = 32
DH = 128
M = 8
SEG = 32
NSEG = S // SEG
FF = 3584
RIDE = 24
BULK = S - RIDE * NSEG
X0 = BULK + 32
NRING = 18
PITCH = 520
X1 = 1024
NP = 3
QK = D // 4
UNROLL = 4
EPS = 1e-5
SIDE0, SIDE_LAT, SIDE_DUE, SIDE_END = 0, 6, 6, 78
NEG = -3.0e38
ORDER = ("q0 q1 q2 q3 k4 k5 k6 k7 s0 s1 s2 s3 s4 s5 s6 s7 v4 v5 v6 v7 p0 p1 p2 p3 p4 p5 p6 p7 "
         "w0 w1 w2 w3 w4 w5 w6 w7")
PERM = (0, 2, 4, 6, 1, 3, 5, 7)


def _rb(v):
    return v.astype(BF).astype(F32)


def _layernorm(xf):
    mu = jnp.mean(xf, axis=-1, keepdims=True)
    dv = xf - mu
    var = jnp.mean(dv * dv, axis=-1, keepdims=True)
    sd = _rb(jnp.sqrt(_rb(_rb(var) + EPS)))
    return _rb(_rb(xf - _rb(mu)) * (1.0 / sd))


def _f3(v):
    return v.astype(F32).reshape(v.shape[0] // 8, 8, D)


def _b2(v):
    return v.reshape(v.shape[0] * 8, D).astype(BF)


def _kernel(x_hbm, mem0_hbm, wq_hbm, wk_hbm, wv_hbm, wo_hbm, wr_hbm, wg_hbm, wu_hbm, wd_hbm,
            c_hbm, wmod_hbm, out_hbm,
            x_v, h_v, hp_v, att_v, ho_v, wqkv_v, wo_v, stage, wmod_v,
            wg_v, wu_v, wd_v, mem_v, cw_v, mod_v, r_v, sb_v, macc_v,
            part_v, sems, *rings):
    w_hbm = (wq_hbm, wk_hbm, wv_hbm)
    ring = rings

    def piece_copy(t, sem, lo=0, n=D, dst=None):
        dst = (t % 2) * D + lo if dst is None else dst
        return pltpu.make_async_copy(
            w_hbm[t // 4].at[pl.ds(lo, n), pl.ds((t % 4) * 8, 8), :],
            stage.at[pl.ds(dst, n)], sems.at[sem])

    def unit_copy(j):
        sem = 1 if j == 1 else 6 + min(j, 10) % 3
        return piece_copy(j % NP, sem, QK * (j // NP), QK, 2 * D + QK * j)

    def stage_wait(row, n, sem):
        dst = stage.at[pl.ds(row, n)]
        pltpu.make_async_copy(dst, dst, sems.at[sem]).wait()

    def mq_copy(q, part):
        return pltpu.make_async_copy(wmod_hbm.at[:, pl.ds(part * D + q * QK, QK)],
                                     wmod_v.at[q, :, pl.ds(part * QK, QK)], sems.at[2])

    def wmod_copy(k, sem):
        col = k * 512 if isinstance(k, int) else pl.multiple_of(k * 512, 512)
        return pltpu.make_async_copy(wmod_hbm.at[:, pl.ds(col, 512)], wmod_v.at[k], sems.at[sem])

    def x_copy(lo, hi, sem):
        return pltpu.make_async_copy(x_hbm.at[0, pl.ds(lo, hi - lo), :],
                                     x_v.at[pl.ds(lo, hi - lo), :], sems.at[sem])

    def wo_copy(n):
        lo, rows = ((n // 2) * 512, 512) if n < 6 else (1536, 2560)
        return pltpu.make_async_copy(wo_hbm.at[pl.ds(lo, rows), pl.ds((n % 2) * 512, 512)],
                                     wo_v.at[n % 2, pl.ds(lo, rows)], sems.at[0])

    small_copies = [pltpu.make_async_copy(c_hbm, cw_v.at[0], sems.at[0]),
                    pltpu.make_async_copy(mem0_hbm.at[0], mem_v, sems.at[0]),
                    pltpu.make_async_copy(wr_hbm, cw_v.at[1], sems.at[0])]
    x0_copy = x_copy(0, X0, 1)
    mid_copies = ([x_copy(X0, (X0 + X1) // 2, 0), x_copy((X0 + X1) // 2, X1, 0)]
                  + [wo_copy(n) for n in range(8)])
    x2_copy = x_copy(X1, S, 1)
    ffn_copies = [pltpu.make_async_copy(wg_hbm, wg_v, sems.at[2]),
                  pltpu.make_async_copy(wu_hbm, wu_v, sems.at[2])] + [
        pltpu.make_async_copy(wd_hbm.at[:, pl.ds(k * 512, 512)], wd_v.at[k], sems.at[2])
        for k in range(2)]

    def relayout(src, base, n):
        u = pltpu.bitcast(stage[pl.ds(src, n)], U32)
        tok = None
        for i in range(n // 2):
            a = u[2 * i]
            b = u[2 * i + 1]
            even = (a & jnp.uint32(0xFFFF)) | (b << 16)
            odd = (a >> 16) | (b & jnp.uint32(0xFFFF0000))
            wqkv_v[pl.ds(base + i, 4, stride=PITCH), :] = even
            wqkv_v[pl.ds(base + 4 * PITCH + i, 4, stride=PITCH), :] = odd
            tok = even ^ odd if tok is None else tok ^ even ^ odd
        return jnp.concatenate([tok, tok], axis=0)

    CW = 256

    def ln_stats(xf):
        mu = jnp.mean(xf, axis=-1, keepdims=True)
        dv = xf - mu
        var = jnp.mean(dv * dv, axis=-1, keepdims=True)
        sd = _rb(jnp.sqrt(_rb(_rb(var) + EPS)))
        return _rb(mu), 1.0 / sd

    def mod_c(k, c):
        return mod_v[k, :, pl.ds(c * CW, CW)]

    def token(v):
        return pltpu.bitcast(v[:, :128] + v[:, 128:], U32)

    def after(v, trig):
        if trig is None:
            return v
        return jnp.concatenate([jnp.where(trig[0], trig[1], v[:, :128]), v[:, 128:]], axis=1)

    def post_work(row0, att, scores_out=None):
        st = {}

        def head(trig):
            a = after(att().astype(F32), trig)
            st["x2"] = _rb(x_v[pl.ds(row0, 8), :].astype(F32) + _rb(mod_v[2] * a))
            st["mu"], st["inv"] = ln_stats(st["x2"])

        def chunk(c, trig):
            xc = after(st["x2"][:, c * CW:(c + 1) * CW], trig)
            h2b = (_rb(_rb(_rb(xc - st["mu"]) * st["inv"]) * mod_c(4, c))
                   + mod_c(3, c)).astype(BF)
            h2 = h2b.astype(F32)
            ho_v[0, pl.ds(row0, 8), pl.ds(c * CW, CW)] = h2b
            o = xc + mod_c(5, c) * h2
            ho_v[1, pl.ds(row0, 8), pl.ds(c * CW, CW)] = o.astype(BF)
            rp = h2 * mod_c(6, c)
            st["r"] = rp if c == 0 else st["r"] + rp
            if c == D // CW - 1:
                r = jnp.sum(st["r"], axis=-1, keepdims=True)
                if scores_out is not None:
                    scores_out.append(r)
                    return None
                grp = row0 >> 3
                lanes = lax.broadcasted_iota(jnp.int32, (8, 128), 1)
                r_v[grp >> 7] = jnp.where(lanes == (grp & 127), r, r_v[grp >> 7])
            return token(o + st["r"])
        return [head] + [functools.partial(chunk, c) for c in range(D // CW)]

    def ln1_work(row0):
        st = {}

        def head(trig):
            st["x"] = after(x_v[pl.ds(row0, 8), :].astype(F32), trig)
            st["mu"], st["inv"] = ln_stats(st["x"])

        def chunk(c, trig):
            xc = after(st["x"][:, c * CW:(c + 1) * CW], trig)
            h = _rb(_rb(_rb(xc - st["mu"]) * st["inv"]) * mod_c(1, c)) + mod_c(0, c)
            ho_v[0, pl.ds(row0, 8), pl.ds(c * CW, CW)] = h.astype(BF)
            return token(h)
        return [head] + [functools.partial(chunk, c) for c in range(D // CW)]

    for cp in small_copies:
        cp.start()
    x0_copy.start()
    mq_copy(0, 0).start()

    r_v[...] = jnp.full(r_v.shape, NEG, F32)
    att_v[...] = jnp.zeros(att_v.shape, BF)

    for cp in small_copies:
        cp.wait()
    mod_v[6] = jnp.broadcast_to(cw_v[1].astype(F32), (8, D))
    cf = cw_v[0].astype(F32)
    sil = (cf * jax.nn.sigmoid(cf)).astype(BF)
    sc = jnp.broadcast_to(sil, (16, D))
    for k in range(8):
        sb_v[pl.ds(128 * k, 128), :] = jnp.broadcast_to(
            sil[:, 128 * k:128 * k + 128].astype(F32), (128, 128)).T

    mq_copy(0, 1).start()
    x0_copy.wait()

    LNB = X0 // 4

    def ln0(i, carry):
        r0 = pl.multiple_of(i * LNB, 8)
        ln = _b2(_layernorm(_f3(x_v[pl.ds(r0, LNB), :])))
        for q in range(4):
            h_v[q, pl.ds(r0, LNB), :] = ln[:, q * QK:(q + 1) * QK]

        @pl.when(i == 1)
        def _():
            unit_copy(0).start()
        return carry
    lax.fori_loop(0, 4, ln0, 0)

    def shift_scale(acc):
        y = _rb(acc)
        return y[:, :QK], _rb(1.0 + y[:, QK:])

    def modulated(q, r0, n, sh, sca):
        ln = h_v[q, pl.ds(r0, n), :].astype(F32).reshape(n // 8, 8, QK)
        return (_rb(ln * sca) + sh).reshape(n, QK).astype(BF)

    unit_copy(1).start()
    for part in range(2):
        mq_copy(0, part).wait()
    acc0 = jnp.dot(sc, wmod_v[0], preferred_element_type=F32)[0:8]
    macc_v[0] = acc0
    hp_v[0] = pltpu.bitcast(modulated(0, 0, BULK, *shift_scale(acc0)), U32)
    unit_copy(2).start()

    def first_unit(j):
        def relayout0(i, carry):
            relayout(2 * D + QK * j + pl.multiple_of(i * 128, 128), j * 8 * PITCH + i * 64, 128)
            return carry
        unit_copy(j).wait()
        lax.fori_loop(0, QK // 128, relayout0, 0)

    first_unit(0)
    mq_copy(1, 0).start()
    mq_copy(1, 1).start()
    unit_copy(3).start()

    def mod_rows(slab, r0, n, acc):
        for r in range(r0, r0 + n, 8):
            sv = sb_v[pl.ds(r, 8), :]
            t = wmod_v[slab, pl.ds(r, 8), :].astype(F32) * jnp.concatenate([sv] * 4, axis=1)
            acc = t if acc is None else acc + t
        return acc

    def ring_fill(g, t, y):
        ring[g][t >> 1, pl.ds(NRING - BULK // SEG, BULK // SEG),
                pl.ds(pl.multiple_of(16 * (t & 1), 16), 16), :] = (
            pltpu.bitcast(y.astype(BF), U32).reshape(BULK // SEG, 16, 128))

    def tie_lhs(col, never, toks):
        return jnp.concatenate(
            [jnp.where(never, toks[j], col[8 * j:8 * j + 8]) if j in toks
             else col[8 * j:8 * j + 8] for j in range(32)], axis=0)

    def add_tok(toks, j, tk):
        toks[j] = tk if j not in toks else toks[j] ^ tk

    starts = {0: [unit_copy(4)], 1: [unit_copy(5), piece_copy(3, 5, 0, 256)],
              2: [unit_copy(6), mq_copy(2, 0), mq_copy(2, 1)],
              3: [unit_copy(7), piece_copy(3, 5, 256, 256)], 4: [unit_copy(8)],
              5: [unit_copy(9), mq_copy(3, 0), mq_copy(3, 1)],
              6: [unit_copy(10), unit_copy(11)], 7: [piece_copy(3, 3, 512, 512)],
              8: [piece_copy(4, 4)], 9: [], 10: [wmod_copy(4, 2)], 11: []}

    def quarter_block(b_lo, b_hi, b, carry):
        first, final = b_lo == 0, b_hi == 4 * NP
        q = b_lo // NP
        p = b - NP * q
        if final:
            src = jnp.where(p == 0, 2 * D + 10 * QK, D + 512 * (p - 1))
            sem = 7 - 2 * p
            stage_wait(pl.multiple_of(src, 512), 512, sem)
            b3 = 3 * 8 * PITCH + 256 * (p - 1)
            jobs = [(src, jnp.where(p == 0, 8 * PITCH + 384, b3)),
                    (src + QK, jnp.where(p == 0, 2 * 8 * PITCH + 384, b3 + 128))]
        else:
            src = 2 * D + QK * (b + 1)
            last = p == NP - 1
            dst = jnp.where(last, 128 * (q + 1), (p + 1) * (8 * PITCH) + 128 * q)

            def unit_wait():
                stage_wait(pl.multiple_of(src, QK), QK, jnp.where(last, 6, 7 + p))
            if first:
                pl.when(b == 1)(functools.partial(first_unit, 1))
                pl.when(b > 0)(unit_wait)
                jobs = [(jnp.where(b == 0, 2 * D, src), jnp.where(b == 0, 0, dst))]
            else:
                unit_wait()
                jobs = [(src, dst)]

            @pl.when(last)
            def _():
                for part in range(2):
                    mq_copy(q + 1, part).wait()
            slab = jnp.where(last, q + 1, q)
        never = jnp.full((8, 128), b, jnp.int32) < 0

        def weights(k):
            return pltpu.bitcast(jnp.concatenate(
                [wqkv_v[pl.ds(pl.multiple_of((8 * p + kk) * PITCH + 128 * q, 8), 128), :]
                 for kk in (k, k + 1)], axis=1), BF)

        groups = [(s_ + 16 * g, d_ + 8 * g) for s_, d_ in jobs for g in range(QK // 16)]
        per = len(groups) // 4
        acc = None
        w = weights(0)
        for n, k in enumerate(range(0, 8, 2)):
            w_next = weights(k + 2) if k < 6 else None
            toks = {}
            for g in range(per):
                add_tok(toks, 4 + (g * 24) // per, relayout(*groups[n * per + g], 16))
            if not final and n < 2:
                for g in range(16):
                    acc = mod_rows(slab, 512 * n + 32 * g, 32, acc)
                    add_tok(toks, 2 * g + (n == 0), token(acc[:, :256] + acc[:, 256:]))
            if not final and n == 2:
                tot = jnp.broadcast_to(jnp.sum(acc, axis=0, keepdims=True), (8, 512))
                macc_v[q + 1] = tot
                sh, sca = shift_scale(tot)
            if not final and n >= 2:
                for g in range(16):
                    r0 = 256 * (n - 2) + 16 * g
                    hb = pltpu.bitcast(modulated(q + 1, r0, 16, sh, sca), U32)
                    hp_v[q + 1, pl.ds(r0 // 2, 8), :] = hb
                    add_tok(toks, (8 + (g * 3) // 2) if n == 2 else 2 * g,
                            hb[:, :128] ^ hb[:, 128:])
            lhs = jnp.concatenate([tie_lhs(hp_v[q, :, pl.ds(0, 128)], never, toks),
                                   hp_v[q, :, pl.ds(128, 128)]], axis=1)
            y = jnp.dot(pltpu.bitcast(lhs, BF), w, preferred_element_type=F32)
            if not first:
                y = y + part_v[p, n]
            if final:
                for j in range(2):
                    ring_fill(k + j, p, y[:, 128 * j:128 * j + 128])
            else:
                part_v[p, n] = y
            w = w_next

        for j in range(b_lo, b_hi):
            if starts[j]:
                @pl.when(b == j)
                def _():
                    for cp in starts[j]:
                        cp.start()
        return carry

    for b_lo, b_hi in ((0, NP), (NP, 2 * NP), (2 * NP, 3 * NP), (3 * NP, 4 * NP)):
        quarters = functools.partial(quarter_block, b_lo, b_hi)
        lax.fori_loop(b_lo, b_hi, quarters, 0)

    def bulk_dot(i, k, never, t, md):
        w = pltpu.bitcast(wqkv_v[pl.ds(pl.multiple_of((8 * i + k) * PITCH, 8), 512), :], BF)
        cols = [hp_v[c // 2, :, pl.ds(128 * (c % 2), 128)] for c in range(8)]
        toks = {}
        for g in range(8):
            tk = relayout((t & 1) * D + 128 * k + 16 * g, t * (8 * PITCH) + 64 * k + 8 * g, 16)
            md[1] = mod_rows(md[0], 128 * k + 16 * g, 16, md[1])
            toks[12 + 6 * g] = tk ^ token(md[1][:, :256] + md[1][:, 256:])
        cols[0] = tie_lhs(cols[0], never, toks)
        cols[4] = tie_lhs(cols[4], never, {j - 32: tk for j, tk in toks.items()})
        hb = pltpu.bitcast(jnp.concatenate(cols, axis=1), BF)
        y = jnp.dot(hb, w, preferred_element_type=F32)
        ring_fill(k, i, y)

    def bulk_qkv(i, carry):
        @pl.when(i < 11)
        def _():
            par = (i + 1) & 1
            stage_wait(pl.multiple_of(par * D, D), D, 4 + par)

        @pl.when(i > NP)
        def _():
            wmod_copy(i, 2 + (i & 1)).wait()

        for j in range(NP, 10):
            @pl.when(i == j)
            def _():
                piece_copy(j + 2, 4 + j % 2).start()

        t = jnp.minimum(i + 1, 11)
        never = jnp.full((8, 128), i, jnp.int32) < 0
        md = [i, None]
        for k in range(8):
            bulk_dot(i, k, never, t, md)
        macc_v[jnp.maximum(i, 4)] = md[1]

        for j in range(NP, 10):
            @pl.when(i == j)
            def _():
                wmod_copy(j + 2, 2 + j % 2).start()
                if j < 9:
                    mid_copies[j - NP + 1].start()
                else:
                    for cp in mid_copies[7:]:
                        cp.start()
        return carry
    mid_copies[0].start()
    lax.fori_loop(NP, 12, bulk_qkv, 0)

    for q in range(4):
        sh, sca = shift_scale(macc_v[q])
        mod_v[0, :, pl.ds(q * QK, QK)] = sh
        mod_v[1, :, pl.ds(q * QK, QK)] = sca
        ho_v[0, pl.ds(BULK, RIDE), pl.ds(q * QK, QK)] = modulated(q, BULK, RIDE, sh, sca)
    for k in range(4, 12):
        y = _rb(jnp.sum(macc_v[k], axis=0, keepdims=True))
        if k // 2 == 4:
            y = _rb(1.0 + y)
        mod_v[k // 2, :, pl.ds((k % 2) * 512, 512)] = jnp.broadcast_to(y, (8, 512))
    for cp in mid_copies:
        cp.wait()
    x2_copy.start()
    for cp in ffn_copies:
        cp.start()

    scale = DH ** -0.5
    kk = lax.broadcasted_iota(jnp.int32, (M + SEG, 80), 0)
    cc = lax.broadcasted_iota(jnp.int32, (M + SEG, 80), 1)
    second = ((cc >= 8) & (cc < 16)) | (cc >= 48)
    allowed = (cc < 16) | (kk <= jnp.where(second, cc - 40, cc - 8))

    def over_keys(f, fr, v):
        t = v[0:8]
        for j in range(8, M + SEG, 8):
            t = f(t, v[j:j + 8])
        return fr(t, axis=0, keepdims=True)

    def tied(u, never, toks):
        if not toks:
            return u
        parts, at = [], 0
        for j, tk in enumerate(toks):
            r = 64 * j
            if r > at:
                parts.append(u[at:r])
            w = tk.shape[1]
            sel = jnp.where(never[:, :w], tk, u[r:r + 8, :w])
            parts.append(sel if w == 128 else jnp.concatenate([sel, u[r:r + 8, w:]], axis=1))
            at = r + 8
        return jnp.concatenate(parts + [u[at:]], axis=0)

    def w_slab(t, g, lo=0, n=512, never=None, toks=()):
        return pltpu.bitcast(
            tied(wqkv_v[pl.ds((8 * t + g) * PITCH + lo, n), :], never, toks), BF)

    def step(s, u, mem, left, att_prev):
        odd = left is not None
        wr = 3 * lax.rem(s >> 2, NRING // 3)
        rd = lax.rem(s + NRING - BULK // SEG, NRING)

        def ring_put(g, t, y):
            if odd:
                u32 = pltpu.bitcast(y.astype(BF), U32)
                parts = [(3 * u, u32[4:8]), (3 * u + 1, u32[8:16])]
            else:
                u32 = pltpu.bitcast(y[M:].astype(BF), U32)
                parts = [(3 * u, u32[0:8]), (3 * u + 2, u32[8:12])]
            for grp, v in parts:
                ring[g][t // 2, wr + grp // 4,
                        pl.ds(16 * (t % 2) + 4 * (grp % 4), v.shape[0]), :] = v

        xin = jnp.concatenate(
            [mem, ho_v[0, pl.ds(pl.multiple_of(BULK + RIDE * s, 8), RIDE), :]], axis=0)

        prow = SEG * (s - 1) if odd else jnp.maximum(SEG * s - 40, 0)
        nrow = BULK + RIDE * jnp.minimum(s + 1, NSEG - 1)
        works = [post_work(pl.multiple_of(prow + 8 * q, 8), functools.partial(att_prev, q))
                 for q in range(3 if odd else 5)]
        works += [ln1_work(pl.multiple_of(nrow + 8 * q, 8)) for q in range(RIDE // 8)]
        never = jnp.full((8, 128), s, jnp.int32) < 0
        gap = (SIDE_END - SIDE0 - SIDE_LAT - SIDE_DUE) // len(works)
        sched = {}
        for q, wk in enumerate(works):
            sched.setdefault(SIDE0 + gap * q, []).append(wk[0])
            for c in range(1, len(wk)):
                sched.setdefault(SIDE0 + SIDE_LAT + gap * q + ((c - 1) * gap) // 4,
                                 []).append(wk[c])

        memqkv, probs, wl, new_left, toks = {}, {}, {}, {}, {}
        acc = []
        chain = []

        ndot = [0]

        def proj(g, t_lo, t_hi):
            part = {}
            if u > 0 and ndot[0] == 0:
                for t in range(t_lo, t_lo + 6):
                    part[t] = jnp.dot(xin[:, :512], w_slab(t, g, 0, 256),
                                      preferred_element_type=F32)
            for t0 in range(t_lo, t_hi, 2):
                ys = []
                for t in (t0, t0 + 1):
                    n = ndot[0]
                    ndot[0] += 1
                    if t in part:
                        y = jnp.dot(xin[:, 512:], w_slab(t, g, 256, 256),
                                    preferred_element_type=F32) + part[t]
                    else:
                        y = jnp.dot(xin, w_slab(t, g, 0, 512, never, toks.get(n)),
                                    preferred_element_type=F32)
                    ring_put(g, t, y)
                    ys.append(y[:M])
                    for item in sched.get(n, ()):
                        tk = item((never, y[:M]))
                        if tk is not None:
                            toks.setdefault(n + SIDE_DUE, []).append(tk)
                memqkv[(t0, g)] = jnp.concatenate(ys, axis=0).astype(BF)

        def cat(t0, g):
            return jnp.concatenate(
                [memqkv[(t0, g)], pltpu.bitcast(ring[g][t0 // 2, rd], BF)], axis=0)

        def scores(g):
            for p in (0, 2):
                if len(chain) < 4:
                    qt = pltpu.bitcast(cat(p, g).T, U32)
                    qt = jnp.concatenate(
                        [jnp.where(never[:, :80], qt[8:16], qt[0:8]), qt[8:]], axis=0)
                    st = jnp.dot(cat(4 + p, g), pltpu.bitcast(qt, BF),
                                 preferred_element_type=F32)
                else:
                    st = lax.dot_general(cat(4 + p, g), cat(p, g), (((1,), (1,)), ((), ())),
                                         preferred_element_type=F32)
                st = jnp.where(second, jnp.concatenate([st[8:16], st[48:80]], axis=0),
                               jnp.concatenate([st[0:8], st[16:48]], axis=0))
                if chain:
                    st = jnp.concatenate(
                        [jnp.where(never[:, :80], chain[-1], st[0:8]), st[8:]], axis=0)
                st = jnp.where(allowed, st * scale, -1e9)
                e = jnp.exp(st - over_keys(jnp.maximum, jnp.max, st))
                l = over_keys(jnp.add, jnp.sum, e)
                chain.append(jnp.broadcast_to(l, (8, 80)))
                rc = pl.reciprocal(l, approx=True)
                e = e * (rc * (2.0 - l * rc))
                e0 = jnp.where(second, 0.0, e)
                e1 = jnp.where(second, e, 0.0)
                probs[(p, g)] = jnp.concatenate(
                    [e0[:M], e1[:M], e0[M:], e1[M:]], axis=0).astype(BF)

        def pv(g):
            for p in (0, 2):
                o = lax.dot_general(probs[(p, g)], cat(8 + p, g), (((0,), (0,)), ((), ())),
                                    preferred_element_type=F32)
                for j in range(2):
                    om, ot = o[8 * j:8 * j + 8], o[16 + 32 * j:48 + 32 * j]
                    if odd:
                        rows = [om, left[(p + j, g)], ot]
                    else:
                        rows = [om, ot[:RIDE]]
                        new_left[(p + j, g)] = ot[RIDE:]
                    wl[(p + j, g)] = jnp.concatenate(rows, axis=0).astype(BF)

        def wo(g):
            a = jnp.concatenate([wl[(o, g)] for o in range(4)], axis=1)
            w = jnp.concatenate(
                [jnp.concatenate([wo_v[n, pl.ds((8 * o + PERM[g]) * DH, DH), :]
                                  for o in range(4)], axis=0) for n in range(2)], axis=1)
            y = jnp.dot(a, w, preferred_element_type=F32)
            acc[:] = [y if not acc else y + acc[0]]

        for op in ORDER.split():
            g = int(op[1])
            if op[0] in "qkvux":
                proj(g, *{"q": (0, 12), "k": (0, 8), "v": (8, 12), "u": (0, 10), "x": (10, 12)}[op[0]])
            else:
                {"s": scores, "p": pv, "w": wo}[op[0]](g)
        y = acc[0].astype(BF)
        return y[:M], y[M:], (None if odd else new_left)

    def out_copy(row0, n, k):
        return pltpu.make_async_copy(ho_v.at[1, pl.ds(row0, n), :],
                                     out_hbm.at[0, pl.ds(row0, n), :], sems.at[3 + k])

    OB = SEG * UNROLL

    def carried(q):
        return att_v[pl.ds(8 * q, 8), :]

    def steps(i, carry):
        @pl.when(i == 16 // UNROLL)
        def _():
            x2_copy.wait()

        mem, left, att_prev = mem_v[...], None, carried
        for u in range(UNROLL):
            mem, att, left = step(i * UNROLL + u, u, mem, left, att_prev)
            att_prev = (lambda a: lambda q: a[8 * q:8 * q + 8])(att)
        mem_v[...] = mem
        att_v[...] = att

        @pl.when(i >= 1)
        def _():
            out_copy(pl.multiple_of((i - 1) * OB, OB), OB, 0).start()
        return carry
    lax.fori_loop(0, NSEG // UNROLL, steps, 0)

    for cp in ffn_copies:
        cp.wait()
    last = []
    for q in range(5):
        for item in post_work(S - 40 + 8 * q, functools.partial(carried, q), last):
            item(None)
    out_copy(S - OB, OB, 0).start()

    def top2(val, idx, valid):
        def reduce(f, v):
            v = f(v, axis=0, keepdims=True)
            return v if v.shape[1] == 1 else f(v, axis=1, keepdims=True)

        def argtop(ok):
            v = jnp.where(ok, val, -jnp.inf)
            m = reduce(jnp.max, v)
            return m, reduce(jnp.min, jnp.where(ok & (v >= m), idx, float(S)))
        m1, i1 = argtop(valid)
        return (m1, i1), argtop(valid & (idx != i1))

    sub1 = lax.broadcasted_iota(jnp.int32, (16, 128), 0)
    lan1 = lax.broadcasted_iota(jnp.int32, (16, 128), 1)
    idx = (sub1 // 8) * 1024 + lan1 * 8 + sub1 % 8
    c_a, c_b = top2(_rb(r_v[pl.ds(0, 2)].reshape(16, 128)), idx.astype(F32), idx < S - 40)
    sub2 = lax.broadcasted_iota(jnp.int32, (48, 1), 0)
    val2 = jnp.concatenate([_rb(r) for r in last] + [jnp.where(sub2[:8] == 0, c_a[0], c_b[0])],
                           axis=0)
    idx2 = jnp.where(sub2 < 40, (sub2 + (S - 40)).astype(F32),
                     jnp.where(sub2 == 40, c_a[1], c_b[1]))
    (m_a, i_a), (m_b, i_b) = top2(val2, idx2, sub2 < 42)
    i_a = i_a.astype(jnp.int32)
    i_b = i_b.astype(jnp.int32)
    ia = jnp.clip(i_a[0, 0], 0, S - 1)
    ib = jnp.clip(i_b[0, 0], 0, S - 1)
    blk_a = pl.multiple_of((ia // 8) * 8, 8)
    blk_b = pl.multiple_of((ib // 8) * 8, 8)

    def two(ref):
        return jnp.concatenate([ref[pl.ds(blk_a, 8), :], ref[pl.ds(blk_b, 8), :]], axis=0)

    hs = two(ho_v.at[0])
    acts, y = [], None
    for c in range(FF // 512 + 1):
        if c < FF // 512:
            g = _rb(jnp.dot(hs, wg_v[:, pl.ds(512 * c, 512)], preferred_element_type=F32))
            u = _rb(jnp.dot(hs, wu_v[:, pl.ds(512 * c, 512)], preferred_element_type=F32))
            acts.append((_rb(g * jax.nn.sigmoid(g)) * u).astype(BF))
        if c > 0:
            wd = jnp.concatenate([wd_v[k, pl.ds(512 * (c - 1), 512), :] for k in range(2)],
                                 axis=1)
            t = jnp.dot(acts[c - 1], wd, preferred_element_type=F32)
            y = t if y is None else t + y
    sub = lax.broadcasted_iota(jnp.int32, (16, 1), 0)
    rows = jnp.where(sub < 8, blk_a + sub, blk_b + sub - 8)
    gate = jnp.where(rows == ia, jax.nn.sigmoid(m_a),
                     jnp.where(rows == ib, jax.nn.sigmoid(m_b), 0.0))
    upd = jnp.where((rows == ia) | (rows == ib), y * gate, 0.0).reshape(2, 8, D)
    fin = _b2(_f3(two(ho_v.at[1])) + mod_v[5] * upd)

    out_copy(0, S, 0).wait()
    ho_v[1, pl.ds(blk_a, 8), :] = fin[0:8]
    ho_v[1, pl.ds(blk_b, 8), :] = fin[8:16]
    out_copy(blk_a, 8, 0).start()

    @pl.when(blk_a != blk_b)
    def _():
        out_copy(blk_b, 8, 1).start()
        out_copy(blk_b, 8, 1).wait()
    out_copy(blk_a, 8, 0).wait()


@jax.jit
def pallas_adaLN_cond__memory_aug_recurrent_mem_tr__moe_arch_mod__prompt_kernel(
    A_x, A_mem0, A_Wq, A_Wk, A_Wv, A_Wo, A_seg_len, B_x, B_w_r, B_w_gate, B_w_up, B_w_down, c,
    w_mod,
):
    del B_x
    del A_seg_len
    assert A_x.shape == (1, S, D) and A_Wq.shape == (D, H, DH) and A_mem0.shape == (1, M, D)
    any_spec = pl.BlockSpec(memory_space=pl.ANY)
    scratch = [
        pltpu.VMEM((S, D), BF),
        pltpu.VMEM((4, X0, QK), BF),
        pltpu.VMEM((4, BULK // 2, QK), U32),
        pltpu.VMEM((40, D), BF),
        pltpu.VMEM((2, S, D), BF),
        pltpu.VMEM((100 * PITCH, 128), U32),
        pltpu.VMEM((2, H * DH, 512), BF),
        pltpu.VMEM((5 * D, 8, 128), BF),
        pltpu.VMEM((12, D, 512), BF),
        pltpu.VMEM((D, FF), BF),
        pltpu.VMEM((D, FF), BF),
        pltpu.VMEM((2, FF, 512), BF),
        pltpu.VMEM((M, D), BF),
        pltpu.VMEM((4, 1, D), BF),
        pltpu.VMEM((7, 8, D), F32),
        pltpu.VMEM((4, 8, 128), F32),
        pltpu.VMEM((D, 128), F32),
        pltpu.VMEM((12, 8, 512), F32),
        pltpu.VMEM((NP, 4, BULK, 256), F32),
        pltpu.SemaphoreType.DMA((9,)),
    ] + [pltpu.VMEM((6, NRING, 32, 128), U32)] * 8
    return pl.pallas_call(
        _kernel,
        out_shape=jax.ShapeDtypeStruct((1, S, D), BF),
        in_specs=[any_spec] * 12,
        out_specs=any_spec,
        scratch_shapes=scratch,
        compiler_params=pltpu.CompilerParams(vmem_limit_bytes=120 * 1024 * 1024),
    )(A_x, A_mem0, A_Wq, A_Wk, A_Wv, A_Wo.reshape(H * DH, D), B_w_r.reshape(1, D), B_w_gate,
      B_w_up, B_w_down, c, w_mod)
```

```python
import functools

import jax
import jax.numpy as jnp
from jax import lax
import jax.experimental.pallas as pl
import jax.experimental.pallas.tpu as pltpu

BF = jnp.bfloat16
F32 = jnp.float32
U32 = jnp.uint32

S = 2048
D = 1024
H = 32
DH = 128
M = 8
SEG = 32
NSEG = S // SEG
FF = 3584
RIDE = 24
BULK = S - RIDE * NSEG
X0 = BULK + 32
NRING = 18
PITCH = 520
X1 = 1024
NP = 3
QK = D // 4
UNROLL = 4
EPS = 1e-5
SIDE0, SIDE_LAT, SIDE_DUE, SIDE_END = 0, 6, 6, 78
NEG = -3.0e38
ORDER = ("q0 q1 q2 q3 k4 k5 k6 k7 s0 s1 s2 s3 s4 s5 s6 s7 v4 v5 v6 v7 p0 p1 p2 p3 p4 p5 p6 p7 "
         "w0 w1 w2 w3 w4 w5 w6 w7")
PERM = (0, 2, 4, 6, 1, 3, 5, 7)


def _rb(v):
    return v.astype(BF).astype(F32)


def _layernorm(xf):
    mu = jnp.mean(xf, axis=-1, keepdims=True)
    dv = xf - mu
    var = jnp.mean(dv * dv, axis=-1, keepdims=True)
    sd = _rb(jnp.sqrt(_rb(_rb(var) + EPS)))
    return _rb(_rb(xf - _rb(mu)) * (1.0 / sd))


def _f3(v):
    return v.astype(F32).reshape(v.shape[0] // 8, 8, D)


def _b2(v):
    return v.reshape(v.shape[0] * 8, D).astype(BF)


def _kernel(x_hbm, mem0_hbm, wq_hbm, wk_hbm, wv_hbm, wo_hbm, wr_hbm, wg_hbm, wu_hbm, wd_hbm,
            c_hbm, wmod_hbm, out_hbm,
            x_v, h_v, hp_v, att_v, ho_v, wqkv_v, wo_v, stage, wmod_v,
            wg_v, wu_v, wd_v, mem_v, cw_v, mod_v, r_v, sb_v, macc_v,
            part_v, sems, *rings):
    w_hbm = (wq_hbm, wk_hbm, wv_hbm)
    ring = rings

    def piece_copy(t, sem, lo=0, n=D, dst=None):
        dst = (t % 2) * D + lo if dst is None else dst
        return pltpu.make_async_copy(
            w_hbm[t // 4].at[pl.ds(lo, n), pl.ds((t % 4) * 8, 8), :],
            stage.at[pl.ds(dst, n)], sems.at[sem])

    def unit_copy(j):
        sem = 1 if j == 1 else 6 + min(j, 10) % 3
        return piece_copy(j % NP, sem, QK * (j // NP), QK, 2 * D + QK * j)

    def stage_wait(row, n, sem):
        dst = stage.at[pl.ds(row, n)]
        pltpu.make_async_copy(dst, dst, sems.at[sem]).wait()

    def mq_copy(q, part):
        return pltpu.make_async_copy(wmod_hbm.at[:, pl.ds(part * D + q * QK, QK)],
                                     wmod_v.at[q, :, pl.ds(part * QK, QK)], sems.at[2])

    def wmod_copy(k, sem):
        col = k * 512 if isinstance(k, int) else pl.multiple_of(k * 512, 512)
        return pltpu.make_async_copy(wmod_hbm.at[:, pl.ds(col, 512)], wmod_v.at[k], sems.at[sem])

    def x_copy(lo, hi, sem):
        return pltpu.make_async_copy(x_hbm.at[0, pl.ds(lo, hi - lo), :],
                                     x_v.at[pl.ds(lo, hi - lo), :], sems.at[sem])

    def wo_copy(n):
        lo, rows = ((n // 2) * 512, 512) if n < 6 else (1536, 2560)
        return pltpu.make_async_copy(wo_hbm.at[pl.ds(lo, rows), pl.ds((n % 2) * 512, 512)],
                                     wo_v.at[n % 2, pl.ds(lo, rows)], sems.at[0])

    small_copies = [pltpu.make_async_copy(c_hbm, cw_v.at[0], sems.at[0]),
                    pltpu.make_async_copy(mem0_hbm.at[0], mem_v, sems.at[0]),
                    pltpu.make_async_copy(wr_hbm, cw_v.at[1], sems.at[0])]
    x0_copy = x_copy(0, X0, 1)
    mid_copies = ([x_copy(X0, (X0 + X1) // 2, 0), x_copy((X0 + X1) // 2, X1, 0)]
                  + [wo_copy(n) for n in range(8)])
    x2_copy = x_copy(X1, S, 1)
    ffn_copies = [pltpu.make_async_copy(wg_hbm, wg_v, sems.at[2]),
                  pltpu.make_async_copy(wu_hbm, wu_v, sems.at[2])] + [
        pltpu.make_async_copy(wd_hbm.at[:, pl.ds(k * 512, 512)], wd_v.at[k], sems.at[2])
        for k in range(2)]

    def relayout(src, base, n):
        u = pltpu.bitcast(stage[pl.ds(src, n)], U32)
        tok = None
        for i in range(n // 2):
            a = u[2 * i]
            b = u[2 * i + 1]
            even = (a & jnp.uint32(0xFFFF)) | (b << 16)
            odd = (a >> 16) | (b & jnp.uint32(0xFFFF0000))
            wqkv_v[pl.ds(base + i, 4, stride=PITCH), :] = even
            wqkv_v[pl.ds(base + 4 * PITCH + i, 4, stride=PITCH), :] = odd
            tok = even ^ odd if tok is None else tok ^ even ^ odd
        return jnp.concatenate([tok, tok], axis=0)

    CW = 256

    def ln_stats(xf):
        mu = jnp.mean(xf, axis=-1, keepdims=True)
        dv = xf - mu
        var = jnp.mean(dv * dv, axis=-1, keepdims=True)
        sd = _rb(jnp.sqrt(_rb(_rb(var) + EPS)))
        return _rb(mu), 1.0 / sd

    def mod_c(k, c):
        return mod_v[k, :, pl.ds(c * CW, CW)]

    def token(v):
        return pltpu.bitcast(v[:, :128] + v[:, 128:], U32)

    def after(v, trig):
        if trig is None:
            return v
        return jnp.concatenate([jnp.where(trig[0], trig[1], v[:, :128]), v[:, 128:]], axis=1)

    def post_work(row0, att, scores_out=None):
        st = {}

        def head(trig):
            a = after(att().astype(F32), trig)
            st["x2"] = _rb(x_v[pl.ds(row0, 8), :].astype(F32) + _rb(mod_v[2] * a))
            st["mu"], st["inv"] = ln_stats(st["x2"])

        def chunk(c, trig):
            xc = after(st["x2"][:, c * CW:(c + 1) * CW], trig)
            h2b = (_rb(_rb(_rb(xc - st["mu"]) * st["inv"]) * mod_c(4, c))
                   + mod_c(3, c)).astype(BF)
            h2 = h2b.astype(F32)
            ho_v[0, pl.ds(row0, 8), pl.ds(c * CW, CW)] = h2b
            o = xc + mod_c(5, c) * h2
            ho_v[1, pl.ds(row0, 8), pl.ds(c * CW, CW)] = o.astype(BF)
            rp = h2 * mod_c(6, c)
            st["r"] = rp if c == 0 else st["r"] + rp
            if c == D // CW - 1:
                r = jnp.sum(st["r"], axis=-1, keepdims=True)
                if scores_out is not None:
                    scores_out.append(r)
                    return None
                grp = row0 >> 3
                lanes = lax.broadcasted_iota(jnp.int32, (8, 128), 1)
                r_v[grp >> 7] = jnp.where(lanes == (grp & 127), r, r_v[grp >> 7])
            return token(o + st["r"])
        return [head] + [functools.partial(chunk, c) for c in range(D // CW)]

    def ln1_work(row0):
        st = {}

        def head(trig):
            st["x"] = after(x_v[pl.ds(row0, 8), :].astype(F32), trig)
            st["mu"], st["inv"] = ln_stats(st["x"])

        def chunk(c, trig):
            xc = after(st["x"][:, c * CW:(c + 1) * CW], trig)
            h = _rb(_rb(_rb(xc - st["mu"]) * st["inv"]) * mod_c(1, c)) + mod_c(0, c)
            ho_v[0, pl.ds(row0, 8), pl.ds(c * CW, CW)] = h.astype(BF)
            return token(h)
        return [head] + [functools.partial(chunk, c) for c in range(D // CW)]

    for cp in small_copies:
        cp.start()
    x0_copy.start()
    mq_copy(0, 0).start()

    r_v[...] = jnp.full(r_v.shape, NEG, F32)
    att_v[...] = jnp.zeros(att_v.shape, BF)

    for cp in small_copies:
        cp.wait()
    mod_v[6] = jnp.broadcast_to(cw_v[1].astype(F32), (8, D))
    cf = cw_v[0].astype(F32)
    sil = (cf * jax.nn.sigmoid(cf)).astype(BF)
    sc = jnp.broadcast_to(sil, (16, D))
    for k in range(8):
        sb_v[pl.ds(128 * k, 128), :] = jnp.broadcast_to(
            sil[:, 128 * k:128 * k + 128].astype(F32), (128, 128)).T

    mq_copy(0, 1).start()
    x0_copy.wait()

    LNB = X0 // 4

    def ln0(i, carry):
        r0 = pl.multiple_of(i * LNB, 8)
        ln = _b2(_layernorm(_f3(x_v[pl.ds(r0, LNB), :])))
        for q in range(4):
            h_v[q, pl.ds(r0, LNB), :] = ln[:, q * QK:(q + 1) * QK]

        @pl.when(i == 1)
        def _():
            unit_copy(0).start()
        return carry
    lax.fori_loop(0, 4, ln0, 0)

    def shift_scale(acc):
        y = _rb(acc)
        return y[:, :QK], _rb(1.0 + y[:, QK:])

    def modulated(q, r0, n, sh, sca):
        ln = h_v[q, pl.ds(r0, n), :].astype(F32).reshape(n // 8, 8, QK)
        return (_rb(ln * sca) + sh).reshape(n, QK).astype(BF)

    unit_copy(1).start()
    for part in range(2):
        mq_copy(0, part).wait()
    acc0 = jnp.dot(sc, wmod_v[0], preferred_element_type=F32)[0:8]
    macc_v[0] = acc0
    hp_v[0] = pltpu.bitcast(modulated(0, 0, BULK, *shift_scale(acc0)), U32)
    unit_copy(2).start()

    def first_unit(j):
        def relayout0(i, carry):
            relayout(2 * D + QK * j + pl.multiple_of(i * 128, 128), j * 8 * PITCH + i * 64, 128)
            return carry
        unit_copy(j).wait()
        lax.fori_loop(0, QK // 128, relayout0, 0)

    first_unit(0)
    mq_copy(1, 0).start()
    mq_copy(1, 1).start()
    unit_copy(3).start()

    def mod_rows(slab, r0, n, acc):
        for r in range(r0, r0 + n, 8):
            sv = sb_v[pl.ds(r, 8), :]
            t = wmod_v[slab, pl.ds(r, 8), :].astype(F32) * jnp.concatenate([sv] * 4, axis=1)
            acc = t if acc is None else acc + t
        return acc

    def ring_fill(g, t, y):
        ring[g][t >> 1, pl.ds(NRING - BULK // SEG, BULK // SEG),
                pl.ds(pl.multiple_of(16 * (t & 1), 16), 16), :] = (
            pltpu.bitcast(y.astype(BF), U32).reshape(BULK // SEG, 16, 128))

    def tie_lhs(col, never, toks):
        return jnp.concatenate(
            [jnp.where(never, toks[j], col[8 * j:8 * j + 8]) if j in toks
             else col[8 * j:8 * j + 8] for j in range(32)], axis=0)

    def add_tok(toks, j, tk):
        toks[j] = tk if j not in toks else toks[j] ^ tk

    starts = {0: [unit_copy(4)], 1: [unit_copy(5), piece_copy(3, 5, 0, 256)],
              2: [unit_copy(6), mq_copy(2, 0), mq_copy(2, 1)],
              3: [unit_copy(7), piece_copy(3, 5, 256, 256)], 4: [unit_copy(8)],
              5: [unit_copy(9), mq_copy(3, 0), mq_copy(3, 1)],
              6: [unit_copy(10), unit_copy(11)], 7: [piece_copy(3, 3, 512, 512)],
              8: [piece_copy(4, 4)], 9: [], 10: [wmod_copy(4, 2)], 11: []}

    def quarter_block(b_lo, b_hi, b, carry):
        first, final = b_lo == 0, b_hi == 4 * NP
        q = b_lo // NP
        p = b - NP * q
        if final:
            src = jnp.where(p == 0, 2 * D + 10 * QK, D + 512 * (p - 1))
            sem = 7 - 2 * p
            stage_wait(pl.multiple_of(src, 512), 512, sem)
            b3 = 3 * 8 * PITCH + 256 * (p - 1)
            jobs = [(src, jnp.where(p == 0, 8 * PITCH + 384, b3)),
                    (src + QK, jnp.where(p == 0, 2 * 8 * PITCH + 384, b3 + 128))]
        else:
            src = 2 * D + QK * (b + 1)
            last = p == NP - 1
            dst = jnp.where(last, 128 * (q + 1), (p + 1) * (8 * PITCH) + 128 * q)

            def unit_wait():
                stage_wait(pl.multiple_of(src, QK), QK, jnp.where(last, 6, 7 + p))
            if first:
                pl.when(b == 1)(functools.partial(first_unit, 1))
                pl.when(b > 0)(unit_wait)
                jobs = [(jnp.where(b == 0, 2 * D, src), jnp.where(b == 0, 0, dst))]
            else:
                unit_wait()
                jobs = [(src, dst)]

            @pl.when(last)
            def _():
                for part in range(2):
                    mq_copy(q + 1, part).wait()
            slab = jnp.where(last, q + 1, q)
        never = jnp.full((8, 128), b, jnp.int32) < 0

        def weights(k):
            return pltpu.bitcast(jnp.concatenate(
                [wqkv_v[pl.ds(pl.multiple_of((8 * p + kk) * PITCH + 128 * q, 8), 128), :]
                 for kk in (k, k + 1)], axis=1), BF)

        groups = [(s_ + 16 * g, d_ + 8 * g) for s_, d_ in jobs for g in range(QK // 16)]
        per = len(groups) // 4
        acc = None
        w = weights(0)
        for n, k in enumerate(range(0, 8, 2)):
            w_next = weights(k + 2) if k < 6 else None
            toks = {}
            if final and n == 2:
                wu = pltpu.bitcast(w_next, U32)
                wu = wu[:, :128] ^ wu[:, 128:]
                add_tok(toks, 3, functools.reduce(
                    jnp.bitwise_xor, [wu[8 * j:8 * j + 8] for j in range(16)]))
            for g in range(per):
                add_tok(toks, 4 + (g * 24) // per, relayout(*groups[n * per + g], 16))
            if not final and n < 2:
                for g in range(16):
                    acc = mod_rows(slab, 512 * n + 32 * g, 32, acc)
                    add_tok(toks, 2 * g + (n == 0), token(acc[:, :256] + acc[:, 256:]))
            if not final and n == 2:
                tot = jnp.broadcast_to(jnp.sum(acc, axis=0, keepdims=True), (8, 512))
                macc_v[q + 1] = tot
                sh, sca = shift_scale(tot)
            if not final and n >= 2:
                for g in range(16):
                    r0 = 256 * (n - 2) + 16 * g
                    hb = pltpu.bitcast(modulated(q + 1, r0, 16, sh, sca), U32)
                    hp_v[q + 1, pl.ds(r0 // 2, 8), :] = hb
                    add_tok(toks, (8 + (g * 3) // 2) if n == 2 else 2 * g,
                            hb[:, :128] ^ hb[:, 128:])
            lhs = jnp.concatenate([tie_lhs(hp_v[q, :, pl.ds(0, 128)], never, toks),
                                   hp_v[q, :, pl.ds(128, 128)]], axis=1)
            y = jnp.dot(pltpu.bitcast(lhs, BF), w, preferred_element_type=F32)
            if not first:
                y = y + part_v[p, n]
            if final:
                for j in range(2):
                    ring_fill(k + j, p, y[:, 128 * j:128 * j + 128])
            else:
                part_v[p, n] = y
            w = w_next

        for j in range(b_lo, b_hi):
            if starts[j]:
                @pl.when(b == j)
                def _():
                    for cp in starts[j]:
                        cp.start()
        return carry

    for b_lo, b_hi in ((0, NP), (NP, 2 * NP), (2 * NP, 3 * NP), (3 * NP, 4 * NP)):
        quarters = functools.partial(quarter_block, b_lo, b_hi)
        lax.fori_loop(b_lo, b_hi, quarters, 0)

    def bulk_dot(i, k, never, t, md):
        w = pltpu.bitcast(wqkv_v[pl.ds(pl.multiple_of((8 * i + k) * PITCH, 8), 512), :], BF)
        cols = [hp_v[c // 2, :, pl.ds(128 * (c % 2), 128)] for c in range(8)]
        toks = {}
        for g in range(8):
            tk = relayout((t & 1) * D + 128 * k + 16 * g, t * (8 * PITCH) + 64 * k + 8 * g, 16)
            md[1] = mod_rows(md[0], 128 * k + 16 * g, 16, md[1])
            toks[10 + 6 * (g + g // 4)] = tk ^ token(md[1][:, :256] + md[1][:, 256:])
        cols[0] = tie_lhs(cols[0], never, toks)
        cols[4] = tie_lhs(cols[4], never, {j - 32: tk for j, tk in toks.items()})
        hb = pltpu.bitcast(jnp.concatenate(cols, axis=1), BF)
        y = jnp.dot(hb, w, preferred_element_type=F32)
        ring_fill(k, i, y)

    def bulk_qkv(i, carry):
        @pl.when(i < 11)
        def _():
            par = (i + 1) & 1
            stage_wait(pl.multiple_of(par * D, D), D, 4 + par)

        @pl.when(i > NP)
        def _():
            wmod_copy(i, 2 + (i & 1)).wait()

        for j in range(NP, 10):
            @pl.when(i == j)
            def _():
                piece_copy(j + 2, 4 + j % 2).start()

        t = jnp.minimum(i + 1, 11)
        never = jnp.full((8, 128), i, jnp.int32) < 0
        md = [i, None]
        for k in range(8):
            bulk_dot(i, k, never, t, md)
        macc_v[jnp.maximum(i, 4)] = md[1]

        for j in range(NP, 10):
            @pl.when(i == j)
            def _():
                wmod_copy(j + 2, 2 + j % 2).start()
                if j < 9:
                    mid_copies[j - NP + 1].start()
                else:
                    for cp in mid_copies[7:]:
                        cp.start()
        return carry
    mid_copies[0].start()
    lax.fori_loop(NP, 12, bulk_qkv, 0)

    for q in range(4):
        sh, sca = shift_scale(macc_v[q])
        mod_v[0, :, pl.ds(q * QK, QK)] = sh
        mod_v[1, :, pl.ds(q * QK, QK)] = sca
        ho_v[0, pl.ds(BULK, RIDE), pl.ds(q * QK, QK)] = modulated(q, BULK, RIDE, sh, sca)
    for k in range(4, 12):
        y = _rb(jnp.sum(macc_v[k], axis=0, keepdims=True))
        if k // 2 == 4:
            y = _rb(1.0 + y)
        mod_v[k // 2, :, pl.ds((k % 2) * 512, 512)] = jnp.broadcast_to(y, (8, 512))
    for cp in mid_copies:
        cp.wait()
    x2_copy.start()
    for cp in ffn_copies:
        cp.start()

    scale = DH ** -0.5
    kk = lax.broadcasted_iota(jnp.int32, (M + SEG, 80), 0)
    cc = lax.broadcasted_iota(jnp.int32, (M + SEG, 80), 1)
    second = ((cc >= 8) & (cc < 16)) | (cc >= 48)
    allowed = (cc < 16) | (kk <= jnp.where(second, cc - 40, cc - 8))

    def over_keys(f, fr, v):
        t = v[0:8]
        for j in range(8, M + SEG, 8):
            t = f(t, v[j:j + 8])
        return fr(t, axis=0, keepdims=True)

    def tied(u, never, toks):
        if not toks:
            return u
        parts, at = [], 0
        for j, tk in enumerate(toks):
            r = 64 * j
            if r > at:
                parts.append(u[at:r])
            w = tk.shape[1]
            sel = jnp.where(never[:, :w], tk, u[r:r + 8, :w])
            parts.append(sel if w == 128 else jnp.concatenate([sel, u[r:r + 8, w:]], axis=1))
            at = r + 8
        return jnp.concatenate(parts + [u[at:]], axis=0)

    def w_slab(t, g, lo=0, n=512, never=None, toks=()):
        return pltpu.bitcast(
            tied(wqkv_v[pl.ds((8 * t + g) * PITCH + lo, n), :], never, toks), BF)

    def step(s, u, mem, left, att_prev):
        odd = left is not None
        wr = 3 * lax.rem(s >> 2, NRING // 3)
        rd = lax.rem(s + NRING - BULK // SEG, NRING)

        def ring_put(g, t, y):
            if odd:
                u32 = pltpu.bitcast(y.astype(BF), U32)
                parts = [(3 * u, u32[4:8]), (3 * u + 1, u32[8:16])]
            else:
                u32 = pltpu.bitcast(y[M:].astype(BF), U32)
                parts = [(3 * u, u32[0:8]), (3 * u + 2, u32[8:12])]
            for grp, v in parts:
                ring[g][t // 2, wr + grp // 4,
                        pl.ds(16 * (t % 2) + 4 * (grp % 4), v.shape[0]), :] = v

        xin = jnp.concatenate(
            [mem, ho_v[0, pl.ds(pl.multiple_of(BULK + RIDE * s, 8), RIDE), :]], axis=0)

        prow = SEG * (s - 1) if odd else jnp.maximum(SEG * s - 40, 0)
        nrow = BULK + RIDE * jnp.minimum(s + 1, NSEG - 1)
        works = [post_work(pl.multiple_of(prow + 8 * q, 8), functools.partial(att_prev, q))
                 for q in range(3 if odd else 5)]
        works += [ln1_work(pl.multiple_of(nrow + 8 * q, 8)) for q in range(RIDE // 8)]
        never = jnp.full((8, 128), s, jnp.int32) < 0
        gap = (SIDE_END - SIDE0 - SIDE_LAT - SIDE_DUE) // len(works)
        sched = {}
        for q, wk in enumerate(works):
            sched.setdefault(SIDE0 + gap * q, []).append(wk[0])
            for c in range(1, len(wk)):
                sched.setdefault(SIDE0 + SIDE_LAT + gap * q + ((c - 1) * gap) // 4,
                                 []).append(wk[c])

        memqkv, probs, wl, new_left, toks = {}, {}, {}, {}, {}
        acc = []
        chain = []

        ndot = [0]

        def proj(g, t_lo, t_hi):
            part = {}
            if u > 0 and ndot[0] == 0:
                for t in range(t_lo, t_lo + 6):
                    part[t] = jnp.dot(xin[:, :512], w_slab(t, g, 0, 256),
                                      preferred_element_type=F32)
            for t0 in range(t_lo, t_hi, 2):
                ys = []
                for t in (t0, t0 + 1):
                    n = ndot[0]
                    ndot[0] += 1
                    if t in part:
                        y = jnp.dot(xin[:, 512:], w_slab(t, g, 256, 256),
                                    preferred_element_type=F32) + part[t]
                    else:
                        y = jnp.dot(xin, w_slab(t, g, 0, 512, never, toks.get(n)),
                                    preferred_element_type=F32)
                    ring_put(g, t, y)
                    ys.append(y[:M])
                    for item in sched.get(n, ()):
                        tk = item((never, y[:M]))
                        if tk is not None:
                            toks.setdefault(n + SIDE_DUE, []).append(tk)
                memqkv[(t0, g)] = jnp.concatenate(ys, axis=0).astype(BF)

        def cat(t0, g):
            return jnp.concatenate(
                [memqkv[(t0, g)], pltpu.bitcast(ring[g][t0 // 2, rd], BF)], axis=0)

        def scores(g):
            for p in (0, 2):
                if len(chain) < 4:
                    qt = pltpu.bitcast(cat(p, g).T, U32)
                    qt = jnp.concatenate(
                        [jnp.where(never[:, :80], qt[8:16], qt[0:8]), qt[8:]], axis=0)
                    st = jnp.dot(cat(4 + p, g), pltpu.bitcast(qt, BF),
                                 preferred_element_type=F32)
                else:
                    st = lax.dot_general(cat(4 + p, g), cat(p, g), (((1,), (1,)), ((), ())),
                                         preferred_element_type=F32)
                st = jnp.where(second, jnp.concatenate([st[8:16], st[48:80]], axis=0),
                               jnp.concatenate([st[0:8], st[16:48]], axis=0))
                if chain:
                    st = jnp.concatenate(
                        [jnp.where(never[:, :80], chain[-1], st[0:8]), st[8:]], axis=0)
                st = jnp.where(allowed, st * scale, -1e9)
                e = jnp.exp(st - over_keys(jnp.maximum, jnp.max, st))
                l = over_keys(jnp.add, jnp.sum, e)
                chain.append(jnp.broadcast_to(l, (8, 80)))
                rc = pl.reciprocal(l, approx=True)
                e = e * (rc * (2.0 - l * rc))
                e0 = jnp.where(second, 0.0, e)
                e1 = jnp.where(second, e, 0.0)
                probs[(p, g)] = jnp.concatenate(
                    [e0[:M], e1[:M], e0[M:], e1[M:]], axis=0).astype(BF)

        def pv(g):
            for p in (0, 2):
                o = lax.dot_general(probs[(p, g)], cat(8 + p, g), (((0,), (0,)), ((), ())),
                                    preferred_element_type=F32)
                for j in range(2):
                    om, ot = o[8 * j:8 * j + 8], o[16 + 32 * j:48 + 32 * j]
                    if odd:
                        rows = [om, left[(p + j, g)], ot]
                    else:
                        rows = [om, ot[:RIDE]]
                        new_left[(p + j, g)] = ot[RIDE:]
                    wl[(p + j, g)] = jnp.concatenate(rows, axis=0).astype(BF)

        def wo(g):
            a = jnp.concatenate([wl[(o, g)] for o in range(4)], axis=1)
            w = jnp.concatenate(
                [jnp.concatenate([wo_v[n, pl.ds((8 * o + PERM[g]) * DH, DH), :]
                                  for o in range(4)], axis=0) for n in range(2)], axis=1)
            y = jnp.dot(a, w, preferred_element_type=F32)
            acc[:] = [y if not acc else y + acc[0]]

        for op in ORDER.split():
            g = int(op[1])
            if op[0] in "qkvux":
                proj(g, *{"q": (0, 12), "k": (0, 8), "v": (8, 12), "u": (0, 10), "x": (10, 12)}[op[0]])
            else:
                {"s": scores, "p": pv, "w": wo}[op[0]](g)
        y = acc[0].astype(BF)
        return y[:M], y[M:], (None if odd else new_left)

    def out_copy(row0, n, k):
        return pltpu.make_async_copy(ho_v.at[1, pl.ds(row0, n), :],
                                     out_hbm.at[0, pl.ds(row0, n), :], sems.at[3 + k])

    OB = SEG * UNROLL

    def carried(q):
        return att_v[pl.ds(8 * q, 8), :]

    def steps(i, carry):
        @pl.when(i == 16 // UNROLL)
        def _():
            x2_copy.wait()

        mem, left, att_prev = mem_v[...], None, carried
        for u in range(UNROLL):
            mem, att, left = step(i * UNROLL + u, u, mem, left, att_prev)
            att_prev = (lambda a: lambda q: a[8 * q:8 * q + 8])(att)
        mem_v[...] = mem
        att_v[...] = att

        @pl.when(i >= 1)
        def _():
            out_copy(pl.multiple_of((i - 1) * OB, OB), OB, 0).start()
        return carry
    lax.fori_loop(0, NSEG // UNROLL, steps, 0)

    for cp in ffn_copies:
        cp.wait()
    last = []
    for q in range(5):
        for item in post_work(S - 40 + 8 * q, functools.partial(carried, q), last):
            item(None)
    out_copy(S - OB, OB, 0).start()

    def top2(val, idx, valid):
        def reduce(f, v):
            v = f(v, axis=0, keepdims=True)
            return v if v.shape[1] == 1 else f(v, axis=1, keepdims=True)

        def argtop(ok):
            v = jnp.where(ok, val, -jnp.inf)
            m = reduce(jnp.max, v)
            return m, reduce(jnp.min, jnp.where(ok & (v >= m), idx, float(S)))
        m1, i1 = argtop(valid)
        return (m1, i1), argtop(valid & (idx != i1))

    sub1 = lax.broadcasted_iota(jnp.int32, (16, 128), 0)
    lan1 = lax.broadcasted_iota(jnp.int32, (16, 128), 1)
    idx = (sub1 // 8) * 1024 + lan1 * 8 + sub1 % 8
    c_a, c_b = top2(_rb(r_v[pl.ds(0, 2)].reshape(16, 128)), idx.astype(F32), idx < S - 40)
    sub2 = lax.broadcasted_iota(jnp.int32, (48, 1), 0)
    val2 = jnp.concatenate([_rb(r) for r in last] + [jnp.where(sub2[:8] == 0, c_a[0], c_b[0])],
                           axis=0)
    idx2 = jnp.where(sub2 < 40, (sub2 + (S - 40)).astype(F32),
                     jnp.where(sub2 == 40, c_a[1], c_b[1]))
    (m_a, i_a), (m_b, i_b) = top2(val2, idx2, sub2 < 42)
    i_a = i_a.astype(jnp.int32)
    i_b = i_b.astype(jnp.int32)
    ia = jnp.clip(i_a[0, 0], 0, S - 1)
    ib = jnp.clip(i_b[0, 0], 0, S - 1)
    blk_a = pl.multiple_of((ia // 8) * 8, 8)
    blk_b = pl.multiple_of((ib // 8) * 8, 8)

    def two(ref):
        return jnp.concatenate([ref[pl.ds(blk_a, 8), :], ref[pl.ds(blk_b, 8), :]], axis=0)

    hs = two(ho_v.at[0])
    acts, y = [], None
    for c in range(FF // 512 + 1):
        if c < FF // 512:
            g = _rb(jnp.dot(hs, wg_v[:, pl.ds(512 * c, 512)], preferred_element_type=F32))
            u = _rb(jnp.dot(hs, wu_v[:, pl.ds(512 * c, 512)], preferred_element_type=F32))
            acts.append((_rb(g * jax.nn.sigmoid(g)) * u).astype(BF))
        if c > 0:
            wd = jnp.concatenate([wd_v[k, pl.ds(512 * (c - 1), 512), :] for k in range(2)],
                                 axis=1)
            t = jnp.dot(acts[c - 1], wd, preferred_element_type=F32)
            y = t if y is None else t + y
    sub = lax.broadcasted_iota(jnp.int32, (16, 1), 0)
    rows = jnp.where(sub < 8, blk_a + sub, blk_b + sub - 8)
    gate = jnp.where(rows == ia, jax.nn.sigmoid(m_a),
                     jnp.where(rows == ib, jax.nn.sigmoid(m_b), 0.0))
    upd = jnp.where((rows == ia) | (rows == ib), y * gate, 0.0).reshape(2, 8, D)
    fin = _b2(_f3(two(ho_v.at[1])) + mod_v[5] * upd)

    out_copy(0, S, 0).wait()
    ho_v[1, pl.ds(blk_a, 8), :] = fin[0:8]
    ho_v[1, pl.ds(blk_b, 8), :] = fin[8:16]
    out_copy(blk_a, 8, 0).start()

    @pl.when(blk_a != blk_b)
    def _():
        out_copy(blk_b, 8, 1).start()
        out_copy(blk_b, 8, 1).wait()
    out_copy(blk_a, 8, 0).wait()


@jax.jit
def pallas_adaLN_cond__memory_aug_recurrent_mem_tr__moe_arch_mod__prompt_kernel(
    A_x, A_mem0, A_Wq, A_Wk, A_Wv, A_Wo, A_seg_len, B_x, B_w_r, B_w_gate, B_w_up, B_w_down, c,
    w_mod,
):
    del B_x
    del A_seg_len
    assert A_x.shape == (1, S, D) and A_Wq.shape == (D, H, DH) and A_mem0.shape == (1, M, D)
    any_spec = pl.BlockSpec(memory_space=pl.ANY)
    scratch = [
        pltpu.VMEM((S, D), BF),
        pltpu.VMEM((4, X0, QK), BF),
        pltpu.VMEM((4, BULK // 2, QK), U32),
        pltpu.VMEM((40, D), BF),
        pltpu.VMEM((2, S, D), BF),
        pltpu.VMEM((100 * PITCH, 128), U32),
        pltpu.VMEM((2, H * DH, 512), BF),
        pltpu.VMEM((5 * D, 8, 128), BF),
        pltpu.VMEM((12, D, 512), BF),
        pltpu.VMEM((D, FF), BF),
        pltpu.VMEM((D, FF), BF),
        pltpu.VMEM((2, FF, 512), BF),
        pltpu.VMEM((M, D), BF),
        pltpu.VMEM((4, 1, D), BF),
        pltpu.VMEM((7, 8, D), F32),
        pltpu.VMEM((4, 8, 128), F32),
        pltpu.VMEM((D, 128), F32),
        pltpu.VMEM((12, 8, 512), F32),
        pltpu.VMEM((NP, 4, BULK, 256), F32),
        pltpu.SemaphoreType.DMA((9,)),
    ] + [pltpu.VMEM((6, NRING, 32, 128), U32)] * 8
    return pl.pallas_call(
        _kernel,
        out_shape=jax.ShapeDtypeStruct((1, S, D), BF),
        in_specs=[any_spec] * 12,
        out_specs=any_spec,
        scratch_shapes=scratch,
        compiler_params=pltpu.CompilerParams(vmem_limit_bytes=120 * 1024 * 1024),
    )(A_x, A_mem0, A_Wq, A_Wk, A_Wv, A_Wo.reshape(H * DH, D), B_w_r.reshape(1, D), B_w_gate,
      B_w_up, B_w_down, c, w_mod)
```

```python
import functools

import jax
import jax.numpy as jnp
from jax import lax
import jax.experimental.pallas as pl
import jax.experimental.pallas.tpu as pltpu

BF = jnp.bfloat16
F32 = jnp.float32
U32 = jnp.uint32

S = 2048
D = 1024
H = 32
DH = 128
M = 8
SEG = 32
NSEG = S // SEG
FF = 3584
RIDE = 24
BULK = S - RIDE * NSEG
X0 = BULK + 32
NRING = 18
PITCH = 520
X1 = 1024
NP = 3
QK = D // 4
UNROLL = 4
EPS = 1e-5
SIDE0, SIDE_LAT, SIDE_DUE, SIDE_END = 0, 6, 6, 78
NEG = -3.0e38
ORDER = ("q0 q1 q2 q3 k4 k5 k6 k7 s0 s1 s2 s3 s4 s5 s6 s7 v4 v5 v6 v7 p0 p1 p2 p3 p4 p5 p6 p7 "
         "w0 w1 w2 w3 w4 w5 w6 w7")
PERM = (0, 2, 4, 6, 1, 3, 5, 7)


def _rb(v):
    return v.astype(BF).astype(F32)


def _layernorm(xf):
    mu = jnp.mean(xf, axis=-1, keepdims=True)
    dv = xf - mu
    var = jnp.mean(dv * dv, axis=-1, keepdims=True)
    sd = _rb(jnp.sqrt(_rb(_rb(var) + EPS)))
    return _rb(_rb(xf - _rb(mu)) * (1.0 / sd))


def _f3(v):
    return v.astype(F32).reshape(v.shape[0] // 8, 8, D)


def _b2(v):
    return v.reshape(v.shape[0] * 8, D).astype(BF)


def _kernel(x_hbm, mem0_hbm, wq_hbm, wk_hbm, wv_hbm, wo_hbm, wr_hbm, wg_hbm, wu_hbm, wd_hbm,
            c_hbm, wmod_hbm, out_hbm,
            x_v, h_v, hp_v, att_v, ho_v, wqkv_v, wo_v, stage, wmod_v,
            wg_v, wu_v, wd_v, mem_v, cw_v, mod_v, r_v, sb_v, macc_v,
            part_v, sems, *rings):
    w_hbm = (wq_hbm, wk_hbm, wv_hbm)
    ring = rings

    def piece_copy(t, sem, lo=0, n=D, dst=None):
        dst = (t % 2) * D + lo if dst is None else dst
        return pltpu.make_async_copy(
            w_hbm[t // 4].at[pl.ds(lo, n), pl.ds((t % 4) * 8, 8), :],
            stage.at[pl.ds(dst, n)], sems.at[sem])

    def unit_copy(j):
        sem = 1 if j == 1 else 6 + min(j, 10) % 3
        return piece_copy(j % NP, sem, QK * (j // NP), QK, 2 * D + QK * j)

    def stage_wait(row, n, sem):
        dst = stage.at[pl.ds(row, n)]
        pltpu.make_async_copy(dst, dst, sems.at[sem]).wait()

    def mq_copy(q, part):
        return pltpu.make_async_copy(wmod_hbm.at[:, pl.ds(part * D + q * QK, QK)],
                                     wmod_v.at[q, :, pl.ds(part * QK, QK)], sems.at[2])

    def wmod_copy(k, sem):
        col = k * 512 if isinstance(k, int) else pl.multiple_of(k * 512, 512)
        return pltpu.make_async_copy(wmod_hbm.at[:, pl.ds(col, 512)], wmod_v.at[k], sems.at[sem])

    def x_copy(lo, hi, sem):
        return pltpu.make_async_copy(x_hbm.at[0, pl.ds(lo, hi - lo), :],
                                     x_v.at[pl.ds(lo, hi - lo), :], sems.at[sem])

    def wo_copy(n):
        lo, rows = ((n // 2) * 512, 512) if n < 6 else (1536, 2560)
        return pltpu.make_async_copy(wo_hbm.at[pl.ds(lo, rows), pl.ds((n % 2) * 512, 512)],
                                     wo_v.at[n % 2, pl.ds(lo, rows)], sems.at[0])

    small_copies = [pltpu.make_async_copy(c_hbm, cw_v.at[0], sems.at[0]),
                    pltpu.make_async_copy(mem0_hbm.at[0], mem_v, sems.at[0]),
                    pltpu.make_async_copy(wr_hbm, cw_v.at[1], sems.at[0])]
    x0_copy = x_copy(0, X0, 1)
    mid_copies = ([x_copy(X0, (X0 + X1) // 2, 0), x_copy((X0 + X1) // 2, X1, 0)]
                  + [wo_copy(n) for n in range(8)])
    x2_copy = x_copy(X1, S, 1)
    ffn_copies = [pltpu.make_async_copy(wg_hbm, wg_v, sems.at[2]),
                  pltpu.make_async_copy(wu_hbm, wu_v, sems.at[2])] + [
        pltpu.make_async_copy(wd_hbm.at[:, pl.ds(k * 512, 512)], wd_v.at[k], sems.at[2])
        for k in range(2)]

    def relayout(src, base, n):
        u = pltpu.bitcast(stage[pl.ds(src, n)], U32)
        tok = None
        for i in range(n // 2):
            a = u[2 * i]
            b = u[2 * i + 1]
            even = (a & jnp.uint32(0xFFFF)) | (b << 16)
            odd = (a >> 16) | (b & jnp.uint32(0xFFFF0000))
            wqkv_v[pl.ds(base + i, 4, stride=PITCH), :] = even
            wqkv_v[pl.ds(base + 4 * PITCH + i, 4, stride=PITCH), :] = odd
            tok = even ^ odd if tok is None else tok ^ even ^ odd
        return jnp.concatenate([tok, tok], axis=0)

    CW = 256

    def ln_stats(xf):
        mu = jnp.mean(xf, axis=-1, keepdims=True)
        dv = xf - mu
        var = jnp.mean(dv * dv, axis=-1, keepdims=True)
        sd = _rb(jnp.sqrt(_rb(_rb(var) + EPS)))
        return _rb(mu), 1.0 / sd

    def mod_c(k, c):
        return mod_v[k, :, pl.ds(c * CW, CW)]

    def token(v):
        return pltpu.bitcast(v[:, :128] + v[:, 128:], U32)

    def after(v, trig):
        if trig is None:
            return v
        return jnp.concatenate([jnp.where(trig[0], trig[1], v[:, :128]), v[:, 128:]], axis=1)

    def post_work(row0, att, scores_out=None):
        st = {}

        def head(trig):
            a = after(att().astype(F32), trig)
            st["x2"] = _rb(x_v[pl.ds(row0, 8), :].astype(F32) + _rb(mod_v[2] * a))
            st["mu"], st["inv"] = ln_stats(st["x2"])

        def chunk(c, trig):
            xc = after(st["x2"][:, c * CW:(c + 1) * CW], trig)
            h2b = (_rb(_rb(_rb(xc - st["mu"]) * st["inv"]) * mod_c(4, c))
                   + mod_c(3, c)).astype(BF)
            h2 = h2b.astype(F32)
            ho_v[0, pl.ds(row0, 8), pl.ds(c * CW, CW)] = h2b
            o = xc + mod_c(5, c) * h2
            ho_v[1, pl.ds(row0, 8), pl.ds(c * CW, CW)] = o.astype(BF)
            rp = h2 * mod_c(6, c)
            st["r"] = rp if c == 0 else st["r"] + rp
            if c == D // CW - 1:
                r = jnp.sum(st["r"], axis=-1, keepdims=True)
                if scores_out is not None:
                    scores_out.append(r)
                    return None
                grp = row0 >> 3
                lanes = lax.broadcasted_iota(jnp.int32, (8, 128), 1)
                r_v[grp >> 7] = jnp.where(lanes == (grp & 127), r, r_v[grp >> 7])
            return token(o + st["r"])
        return [head] + [functools.partial(chunk, c) for c in range(D // CW)]

    def ln1_work(row0):
        st = {}

        def head(trig):
            st["x"] = after(x_v[pl.ds(row0, 8), :].astype(F32), trig)
            st["mu"], st["inv"] = ln_stats(st["x"])

        def chunk(c, trig):
            xc = after(st["x"][:, c * CW:(c + 1) * CW], trig)
            h = _rb(_rb(_rb(xc - st["mu"]) * st["inv"]) * mod_c(1, c)) + mod_c(0, c)
            ho_v[0, pl.ds(row0, 8), pl.ds(c * CW, CW)] = h.astype(BF)
            return token(h)
        return [head] + [functools.partial(chunk, c) for c in range(D // CW)]

    for cp in small_copies:
        cp.start()
    x0_copy.start()
    mq_copy(0, 0).start()

    r_v[...] = jnp.full(r_v.shape, NEG, F32)
    att_v[...] = jnp.zeros(att_v.shape, BF)

    for cp in small_copies:
        cp.wait()
    mod_v[6] = jnp.broadcast_to(cw_v[1].astype(F32), (8, D))
    cf = cw_v[0].astype(F32)
    sil = (cf * jax.nn.sigmoid(cf)).astype(BF)
    sc = jnp.broadcast_to(sil, (16, D))
    for k in range(8):
        sb_v[pl.ds(128 * k, 128), :] = jnp.broadcast_to(
            sil[:, 128 * k:128 * k + 128].astype(F32), (128, 128)).T

    mq_copy(0, 1).start()
    x0_copy.wait()

    LNB = X0 // 4

    def ln0(i, carry):
        r0 = pl.multiple_of(i * LNB, 8)
        ln = _b2(_layernorm(_f3(x_v[pl.ds(r0, LNB), :])))
        for q in range(4):
            h_v[q, pl.ds(r0, LNB), :] = ln[:, q * QK:(q + 1) * QK]

        @pl.when(i == 1)
        def _():
            unit_copy(0).start()
        return carry
    lax.fori_loop(0, 4, ln0, 0)

    def shift_scale(acc):
        y = _rb(acc)
        return y[:, :QK], _rb(1.0 + y[:, QK:])

    def modulated(q, r0, n, sh, sca):
        ln = h_v[q, pl.ds(r0, n), :].astype(F32).reshape(n // 8, 8, QK)
        return (_rb(ln * sca) + sh).reshape(n, QK).astype(BF)

    unit_copy(1).start()
    for part in range(2):
        mq_copy(0, part).wait()
    acc0 = jnp.dot(sc, wmod_v[0], preferred_element_type=F32)[0:8]
    macc_v[0] = acc0
    hp_v[0] = pltpu.bitcast(modulated(0, 0, BULK, *shift_scale(acc0)), U32)
    unit_copy(2).start()

    def first_unit(j):
        def relayout0(i, carry):
            relayout(2 * D + QK * j + pl.multiple_of(i * 128, 128), j * 8 * PITCH + i * 64, 128)
            return carry
        unit_copy(j).wait()
        lax.fori_loop(0, QK // 128, relayout0, 0)

    first_unit(0)
    mq_copy(1, 0).start()
    mq_copy(1, 1).start()
    unit_copy(3).start()

    def mod_rows(slab, r0, n, acc):
        for r in range(r0, r0 + n, 8):
            sv = sb_v[pl.ds(r, 8), :]
            t = wmod_v[slab, pl.ds(r, 8), :].astype(F32) * jnp.concatenate([sv] * 4, axis=1)
            acc = t if acc is None else acc + t
        return acc

    def ring_fill(g, t, y):
        ring[g][t >> 1, pl.ds(NRING - BULK // SEG, BULK // SEG),
                pl.ds(pl.multiple_of(16 * (t & 1), 16), 16), :] = (
            pltpu.bitcast(y.astype(BF), U32).reshape(BULK // SEG, 16, 128))

    def tie_lhs(col, never, toks):
        return jnp.concatenate(
            [jnp.where(never, toks[j], col[8 * j:8 * j + 8]) if j in toks
             else col[8 * j:8 * j + 8] for j in range(32)], axis=0)

    def add_tok(toks, j, tk):
        toks[j] = tk if j not in toks else toks[j] ^ tk

    starts = {0: [unit_copy(4)], 1: [unit_copy(5), piece_copy(3, 5, 0, 256)],
              2: [unit_copy(6), mq_copy(2, 0), mq_copy(2, 1)],
              3: [unit_copy(7), piece_copy(3, 5, 256, 256)], 4: [unit_copy(8)],
              5: [unit_copy(9), mq_copy(3, 0), mq_copy(3, 1)],
              6: [unit_copy(10), unit_copy(11)], 7: [piece_copy(3, 3, 512, 512)],
              8: [piece_copy(4, 4)], 9: [], 10: [wmod_copy(4, 2)], 11: []}

    def quarter_block(b_lo, b_hi, b, carry):
        first, final = b_lo == 0, b_hi == 4 * NP
        q = b_lo // NP
        p = b - NP * q
        if final:
            src = jnp.where(p == 0, 2 * D + 10 * QK, D + 512 * (p - 1))
            sem = 7 - 2 * p
            stage_wait(pl.multiple_of(src, 512), 512, sem)
            b3 = 3 * 8 * PITCH + 256 * (p - 1)
            jobs = [(src, jnp.where(p == 0, 8 * PITCH + 384, b3)),
                    (src + QK, jnp.where(p == 0, 2 * 8 * PITCH + 384, b3 + 128))]
        else:
            src = 2 * D + QK * (b + 1)
            last = p == NP - 1
            dst = jnp.where(last, 128 * (q + 1), (p + 1) * (8 * PITCH) + 128 * q)

            def unit_wait():
                stage_wait(pl.multiple_of(src, QK), QK, jnp.where(last, 6, 7 + p))
            if first:
                pl.when(b == 1)(functools.partial(first_unit, 1))
                pl.when(b > 0)(unit_wait)
                jobs = [(jnp.where(b == 0, 2 * D, src), jnp.where(b == 0, 0, dst))]
            else:
                unit_wait()
                jobs = [(src, dst)]

            @pl.when(last)
            def _():
                for part in range(2):
                    mq_copy(q + 1, part).wait()
            slab = jnp.where(last, q + 1, q)
        never = jnp.full((8, 128), b, jnp.int32) < 0

        def weights(k):
            return pltpu.bitcast(jnp.concatenate(
                [wqkv_v[pl.ds(pl.multiple_of((8 * p + kk) * PITCH + 128 * q, 8), 128), :]
                 for kk in (k, k + 1)], axis=1), BF)

        groups = [(s_ + 16 * g, d_ + 8 * g) for s_, d_ in jobs for g in range(QK // 16)]
        per = len(groups) // 4
        acc = None
        w = weights(0)
        for n, k in enumerate(range(0, 8, 2)):
            w_next = weights(k + 2) if k < 6 else None
            toks = {}
            if final and n == 2:
                wu = pltpu.bitcast(w_next, U32)
                wu = wu[:, :128] ^ wu[:, 128:]
                add_tok(toks, 3, functools.reduce(
                    jnp.bitwise_xor, [wu[8 * j:8 * j + 8] for j in range(16)]))
            for g in range(per):
                add_tok(toks, 4 + (g * 24) // per, relayout(*groups[n * per + g], 16))
            if not final and n < 2:
                for g in range(16):
                    acc = mod_rows(slab, 512 * n + 32 * g, 32, acc)
                    add_tok(toks, 2 * g + (n == 0), token(acc[:, :256] + acc[:, 256:]))
            if not final and n == 2:
                tot = jnp.broadcast_to(jnp.sum(acc, axis=0, keepdims=True), (8, 512))
                macc_v[q + 1] = tot
                sh, sca = shift_scale(tot)
            if not final and n >= 2:
                for g in range(16):
                    r0 = 256 * (n - 2) + 16 * g
                    hb = pltpu.bitcast(modulated(q + 1, r0, 16, sh, sca), U32)
                    hp_v[q + 1, pl.ds(r0 // 2, 8), :] = hb
                    add_tok(toks, (8 + (g * 3) // 2) if n == 2 else 2 * g,
                            hb[:, :128] ^ hb[:, 128:])
            lhs = jnp.concatenate([tie_lhs(hp_v[q, :, pl.ds(0, 128)], never, toks),
                                   hp_v[q, :, pl.ds(128, 128)]], axis=1)
            y = jnp.dot(pltpu.bitcast(lhs, BF), w, preferred_element_type=F32)
            if not first:
                y = y + part_v[p, n]
            if final:
                for j in range(2):
                    ring_fill(k + j, p, y[:, 128 * j:128 * j + 128])
            else:
                part_v[p, n] = y
            w = w_next

        for j in range(b_lo, b_hi):
            if starts[j]:
                @pl.when(b == j)
                def _():
                    for cp in starts[j]:
                        cp.start()
        return carry

    for b_lo, b_hi in ((0, NP), (NP, 2 * NP), (2 * NP, 3 * NP), (3 * NP, 4 * NP)):
        quarters = functools.partial(quarter_block, b_lo, b_hi)
        lax.fori_loop(b_lo, b_hi, quarters, 0)

    def bulk_dot(i, k, never, t, md):
        w = pltpu.bitcast(wqkv_v[pl.ds(pl.multiple_of((8 * i + k) * PITCH, 8), 512), :], BF)
        cols = [hp_v[c // 2, :, pl.ds(128 * (c % 2), 128)] for c in range(8)]
        toks = {}
        for g in range(8):
            tk = relayout((t & 1) * D + 128 * k + 16 * g, t * (8 * PITCH) + 64 * k + 8 * g, 16)
            md[1] = mod_rows(md[0], 128 * k + 16 * g, 16, md[1])
            toks[10 + 6 * (g + g // 4)] = tk ^ token(md[1][:, :256] + md[1][:, 256:])
        cols[0] = tie_lhs(cols[0], never, toks)
        cols[4] = tie_lhs(cols[4], never, {j - 32: tk for j, tk in toks.items()})
        hb = pltpu.bitcast(jnp.concatenate(cols, axis=1), BF)
        y = jnp.dot(hb, w, preferred_element_type=F32)
        ring_fill(k, i, y)

    def bulk_qkv(i, carry):
        @pl.when(i < 11)
        def _():
            par = (i + 1) & 1
            stage_wait(pl.multiple_of(par * D, D), D, 4 + par)

        @pl.when(i > NP)
        def _():
            wmod_copy(i, 2 + (i & 1)).wait()

        for j in range(NP, 10):
            @pl.when(i == j)
            def _():
                piece_copy(j + 2, 4 + j % 2).start()

        t = jnp.minimum(i + 1, 11)
        never = jnp.full((8, 128), i, jnp.int32) < 0
        md = [i, None]
        for k in range(8):
            bulk_dot(i, k, never, t, md)
        macc_v[jnp.maximum(i, 4)] = md[1]

        for j in range(NP, 10):
            @pl.when(i == j)
            def _():
                wmod_copy(j + 2, 2 + j % 2).start()
                if j < 9:
                    mid_copies[j - NP + 1].start()
                else:
                    for cp in mid_copies[7:]:
                        cp.start()
        return carry
    mid_copies[0].start()
    lax.fori_loop(NP, 12, bulk_qkv, 0)

    for q in range(4):
        sh, sca = shift_scale(macc_v[q])
        mod_v[0, :, pl.ds(q * QK, QK)] = sh
        mod_v[1, :, pl.ds(q * QK, QK)] = sca
        ho_v[0, pl.ds(BULK, RIDE), pl.ds(q * QK, QK)] = modulated(q, BULK, RIDE, sh, sca)
    for k in range(4, 12):
        y = _rb(jnp.sum(macc_v[k], axis=0, keepdims=True))
        if k // 2 == 4:
            y = _rb(1.0 + y)
        mod_v[k // 2, :, pl.ds((k % 2) * 512, 512)] = jnp.broadcast_to(y, (8, 512))
    for cp in mid_copies:
        cp.wait()
    x2_copy.start()
    for cp in ffn_copies:
        cp.start()

    scale = DH ** -0.5
    kk = lax.broadcasted_iota(jnp.int32, (M + SEG, 80), 0)
    cc = lax.broadcasted_iota(jnp.int32, (M + SEG, 80), 1)
    second = ((cc >= 8) & (cc < 16)) | (cc >= 48)
    allowed = (cc < 16) | (kk <= jnp.where(second, cc - 40, cc - 8))

    def over_keys(f, fr, v):
        t = v[0:8]
        for j in range(8, M + SEG, 8):
            t = f(t, v[j:j + 8])
        return fr(t, axis=0, keepdims=True)

    def tied(u, never, toks):
        if not toks:
            return u
        parts, at = [], 0
        for j, tk in enumerate(toks):
            r = 64 * j
            if r > at:
                parts.append(u[at:r])
            parts.append(jnp.where(never, tk, u[r:r + 8]))
            at = r + 8
        return jnp.concatenate(parts + [u[at:]], axis=0)

    def w_slab(t, g, lo=0, n=512, never=None, toks=()):
        return pltpu.bitcast(
            tied(wqkv_v[pl.ds((8 * t + g) * PITCH + lo, n), :], never, toks), BF)

    def step(s, u, mem, left, att_prev):
        odd = left is not None
        wr = 3 * lax.rem(s >> 2, NRING // 3)
        rd = lax.rem(s + NRING - BULK // SEG, NRING)

        def ring_put(g, t, y):
            if odd:
                u32 = pltpu.bitcast(y.astype(BF), U32)
                parts = [(3 * u, u32[4:8]), (3 * u + 1, u32[8:16])]
            else:
                u32 = pltpu.bitcast(y[M:].astype(BF), U32)
                parts = [(3 * u, u32[0:8]), (3 * u + 2, u32[8:12])]
            for grp, v in parts:
                ring[g][t // 2, wr + grp // 4,
                        pl.ds(16 * (t % 2) + 4 * (grp % 4), v.shape[0]), :] = v

        xin = jnp.concatenate(
            [mem, ho_v[0, pl.ds(pl.multiple_of(BULK + RIDE * s, 8), RIDE), :]], axis=0)

        prow = SEG * (s - 1) if odd else jnp.maximum(SEG * s - 40, 0)
        nrow = BULK + RIDE * jnp.minimum(s + 1, NSEG - 1)
        works = [post_work(pl.multiple_of(prow + 8 * q, 8), functools.partial(att_prev, q))
                 for q in range(3 if odd else 5)]
        works += [ln1_work(pl.multiple_of(nrow + 8 * q, 8)) for q in range(RIDE // 8)]
        never = jnp.full((8, 128), s, jnp.int32) < 0
        gap = (SIDE_END - SIDE0 - SIDE_LAT - SIDE_DUE) // len(works)
        sched = {}
        for q, wk in enumerate(works):
            sched.setdefault(SIDE0 + gap * q, []).append(wk[0])
            for c in range(1, len(wk)):
                sched.setdefault(SIDE0 + SIDE_LAT + gap * q + ((c - 1) * gap) // 4,
                                 []).append(wk[c])

        memqkv, probs, wl, new_left, toks = {}, {}, {}, {}, {}
        acc = []
        chain = []

        ndot = [0]

        def proj(g, t_lo, t_hi):
            part = {}
            if u > 0 and ndot[0] == 0:
                for t in range(t_lo, t_lo + 6):
                    part[t] = jnp.dot(xin[:, :512], w_slab(t, g, 0, 256),
                                      preferred_element_type=F32)
            for t0 in range(t_lo, t_hi, 2):
                ys = []
                for t in (t0, t0 + 1):
                    n = ndot[0]
                    ndot[0] += 1
                    if t in part:
                        y = jnp.dot(xin[:, 512:], w_slab(t, g, 256, 256),
                                    preferred_element_type=F32) + part[t]
                    else:
                        y = jnp.dot(xin, w_slab(t, g, 0, 512, never, toks.get(n)),
                                    preferred_element_type=F32)
                    ring_put(g, t, y)
                    ys.append(y[:M])
                    for item in sched.get(n, ()):
                        tk = item((never, y[:M]))
                        if tk is not None:
                            toks.setdefault(n + SIDE_DUE, []).append(tk)
                memqkv[(t0, g)] = jnp.concatenate(ys, axis=0).astype(BF)

        def cat(t0, g):
            return jnp.concatenate(
                [memqkv[(t0, g)], pltpu.bitcast(ring[g][t0 // 2, rd], BF)], axis=0)

        def scores(g):
            for p in (0, 2):
                if len(chain) < 4:
                    qt = pltpu.bitcast(cat(p, g).T, U32)
                    qt = jnp.concatenate(
                        [jnp.where(never[:, :80], qt[8:16], qt[0:8]), qt[8:]], axis=0)
                    st = jnp.dot(cat(4 + p, g), pltpu.bitcast(qt, BF),
                                 preferred_element_type=F32)
                else:
                    st = lax.dot_general(cat(4 + p, g), cat(p, g), (((1,), (1,)), ((), ())),
                                         preferred_element_type=F32)
                st = jnp.where(second, jnp.concatenate([st[8:16], st[48:80]], axis=0),
                               jnp.concatenate([st[0:8], st[16:48]], axis=0))
                if chain:
                    st = jnp.concatenate(
                        [jnp.where(never[:, :80], chain[-1], st[0:8]), st[8:]], axis=0)
                st = jnp.where(allowed, st * scale, -1e9)
                e = jnp.exp(st - over_keys(jnp.maximum, jnp.max, st))
                l = over_keys(jnp.add, jnp.sum, e)
                chain.append(jnp.broadcast_to(l, (8, 80)))
                rc = pl.reciprocal(l, approx=True)
                e = e * (rc * (2.0 - l * rc))
                e0 = jnp.where(second, 0.0, e)
                e1 = jnp.where(second, e, 0.0)
                probs[(p, g)] = jnp.concatenate(
                    [e0[:M], e1[:M], e0[M:], e1[M:]], axis=0).astype(BF)

        def pv(g):
            for p in (0, 2):
                o = lax.dot_general(probs[(p, g)], cat(8 + p, g), (((0,), (0,)), ((), ())),
                                    preferred_element_type=F32)
                for j in range(2):
                    om, ot = o[8 * j:8 * j + 8], o[16 + 32 * j:48 + 32 * j]
                    if odd:
                        rows = [om, left[(p + j, g)], ot]
                    else:
                        rows = [om, ot[:RIDE]]
                        new_left[(p + j, g)] = ot[RIDE:]
                    wl[(p + j, g)] = jnp.concatenate(rows, axis=0).astype(BF)

        def wo(g):
            a = jnp.concatenate([wl[(o, g)] for o in range(4)], axis=1)
            w = jnp.concatenate(
                [jnp.concatenate([wo_v[n, pl.ds((8 * o + PERM[g]) * DH, DH), :]
                                  for o in range(4)], axis=0) for n in range(2)], axis=1)
            y = jnp.dot(a, w, preferred_element_type=F32)
            acc[:] = [y if not acc else y + acc[0]]

        for op in ORDER.split():
            g = int(op[1])
            if op[0] in "qkv":
                proj(g, *{"q": (0, 12), "k": (0, 8), "v": (8, 12)}[op[0]])
            else:
                {"s": scores, "p": pv, "w": wo}[op[0]](g)
        y = acc[0].astype(BF)
        return y[:M], y[M:], (None if odd else new_left)

    def out_copy(row0, n, k):
        return pltpu.make_async_copy(ho_v.at[1, pl.ds(row0, n), :],
                                     out_hbm.at[0, pl.ds(row0, n), :], sems.at[3 + k])

    OB = SEG * UNROLL

    def carried(q):
        return att_v[pl.ds(8 * q, 8), :]

    def steps(i, carry):
        @pl.when(i == 16 // UNROLL)
        def _():
            x2_copy.wait()

        mem, left, att_prev = mem_v[...], None, carried
        for u in range(UNROLL):
            mem, att, left = step(i * UNROLL + u, u, mem, left, att_prev)
            att_prev = (lambda a: lambda q: a[8 * q:8 * q + 8])(att)
        mem_v[...] = mem
        att_v[...] = att

        @pl.when(i >= 1)
        def _():
            out_copy(pl.multiple_of((i - 1) * OB, OB), OB, 0).start()
        return carry
    lax.fori_loop(0, NSEG // UNROLL, steps, 0)

    for cp in ffn_copies:
        cp.wait()
    last = []
    for q in range(5):
        for item in post_work(S - 40 + 8 * q, functools.partial(carried, q), last):
            item(None)
    out_copy(S - OB, OB, 0).start()

    def top2(val, idx, valid):
        def reduce(f, v):
            v = f(v, axis=0, keepdims=True)
            return v if v.shape[1] == 1 else f(v, axis=1, keepdims=True)

        def argtop(ok):
            v = jnp.where(ok, val, -jnp.inf)
            m = reduce(jnp.max, v)
            return m, reduce(jnp.min, jnp.where(ok & (v >= m), idx, float(S)))
        m1, i1 = argtop(valid)
        return (m1, i1), argtop(valid & (idx != i1))

    sub1 = lax.broadcasted_iota(jnp.int32, (16, 128), 0)
    lan1 = lax.broadcasted_iota(jnp.int32, (16, 128), 1)
    idx = (sub1 // 8) * 1024 + lan1 * 8 + sub1 % 8
    c_a, c_b = top2(_rb(r_v[pl.ds(0, 2)].reshape(16, 128)), idx.astype(F32), idx < S - 40)
    sub2 = lax.broadcasted_iota(jnp.int32, (48, 1), 0)
    val2 = jnp.concatenate([_rb(r) for r in last] + [jnp.where(sub2[:8] == 0, c_a[0], c_b[0])],
                           axis=0)
    idx2 = jnp.where(sub2 < 40, (sub2 + (S - 40)).astype(F32),
                     jnp.where(sub2 == 40, c_a[1], c_b[1]))
    (m_a, i_a), (m_b, i_b) = top2(val2, idx2, sub2 < 42)
    i_a = i_a.astype(jnp.int32)
    i_b = i_b.astype(jnp.int32)
    ia = jnp.clip(i_a[0, 0], 0, S - 1)
    ib = jnp.clip(i_b[0, 0], 0, S - 1)
    blk_a = pl.multiple_of((ia // 8) * 8, 8)
    blk_b = pl.multiple_of((ib // 8) * 8, 8)

    def two(ref):
        return jnp.concatenate([ref[pl.ds(blk_a, 8), :], ref[pl.ds(blk_b, 8), :]], axis=0)

    hs = two(ho_v.at[0])
    acts, y = [], None
    for c in range(FF // 512 + 1):
        if c < FF // 512:
            g = _rb(jnp.dot(hs, wg_v[:, pl.ds(512 * c, 512)], preferred_element_type=F32))
            u = _rb(jnp.dot(hs, wu_v[:, pl.ds(512 * c, 512)], preferred_element_type=F32))
            acts.append((_rb(g * jax.nn.sigmoid(g)) * u).astype(BF))
        if c > 0:
            wd = jnp.concatenate([wd_v[k, pl.ds(512 * (c - 1), 512), :] for k in range(2)],
                                 axis=1)
            t = jnp.dot(acts[c - 1], wd, preferred_element_type=F32)
            y = t if y is None else t + y
    sub = lax.broadcasted_iota(jnp.int32, (16, 1), 0)
    rows = jnp.where(sub < 8, blk_a + sub, blk_b + sub - 8)
    gate = jnp.where(rows == ia, jax.nn.sigmoid(m_a),
                     jnp.where(rows == ib, jax.nn.sigmoid(m_b), 0.0))
    upd = jnp.where((rows == ia) | (rows == ib), y * gate, 0.0).reshape(2, 8, D)
    fin = _b2(_f3(two(ho_v.at[1])) + mod_v[5] * upd)

    out_copy(0, S, 0).wait()
    ho_v[1, pl.ds(blk_a, 8), :] = fin[0:8]
    ho_v[1, pl.ds(blk_b, 8), :] = fin[8:16]
    out_copy(blk_a, 8, 0).start()

    @pl.when(blk_a != blk_b)
    def _():
        out_copy(blk_b, 8, 1).start()
        out_copy(blk_b, 8, 1).wait()
    out_copy(blk_a, 8, 0).wait()


@jax.jit
def pallas_adaLN_cond__memory_aug_recurrent_mem_tr__moe_arch_mod__prompt_kernel(
    A_x, A_mem0, A_Wq, A_Wk, A_Wv, A_Wo, A_seg_len, B_x, B_w_r, B_w_gate, B_w_up, B_w_down, c,
    w_mod,
):
    del B_x
    del A_seg_len
    assert A_x.shape == (1, S, D) and A_Wq.shape == (D, H, DH) and A_mem0.shape == (1, M, D)
    any_spec = pl.BlockSpec(memory_space=pl.ANY)
    scratch = [
        pltpu.VMEM((S, D), BF),
        pltpu.VMEM((4, X0, QK), BF),
        pltpu.VMEM((4, BULK // 2, QK), U32),
        pltpu.VMEM((40, D), BF),
        pltpu.VMEM((2, S, D), BF),
        pltpu.VMEM((100 * PITCH, 128), U32),
        pltpu.VMEM((2, H * DH, 512), BF),
        pltpu.VMEM((5 * D, 8, 128), BF),
        pltpu.VMEM((12, D, 512), BF),
        pltpu.VMEM((D, FF), BF),
        pltpu.VMEM((D, FF), BF),
        pltpu.VMEM((2, FF, 512), BF),
        pltpu.VMEM((M, D), BF),
        pltpu.VMEM((4, 1, D), BF),
        pltpu.VMEM((7, 8, D), F32),
        pltpu.VMEM((4, 8, 128), F32),
        pltpu.VMEM((D, 128), F32),
        pltpu.VMEM((12, 8, 512), F32),
        pltpu.VMEM((NP, 4, BULK, 256), F32),
        pltpu.SemaphoreType.DMA((9,)),
    ] + [pltpu.VMEM((6, NRING, 32, 128), U32)] * 8
    return pl.pallas_call(
        _kernel,
        out_shape=jax.ShapeDtypeStruct((1, S, D), BF),
        in_specs=[any_spec] * 12,
        out_specs=any_spec,
        scratch_shapes=scratch,
        compiler_params=pltpu.CompilerParams(vmem_limit_bytes=120 * 1024 * 1024),
    )(A_x, A_mem0, A_Wq, A_Wk, A_Wv, A_Wo.reshape(H * DH, D), B_w_r.reshape(1, D), B_w_gate,
      B_w_up, B_w_down, c, w_mod)
```

```python
import functools

import jax
import jax.numpy as jnp
from jax import lax
import jax.experimental.pallas as pl
import jax.experimental.pallas.tpu as pltpu

BF = jnp.bfloat16
F32 = jnp.float32
U32 = jnp.uint32

S = 2048
D = 1024
H = 32
DH = 128
M = 8
SEG = 32
NSEG = S // SEG
FF = 3584
RIDE = 24
BULK = S - RIDE * NSEG
X0 = BULK + 32
NRING = 18
PITCH = 520
X1 = 1024
NP = 3
QK = D // 4
UNROLL = 4
EPS = 1e-5
SIDE0, SIDE_LAT, SIDE_DUE, SIDE_END = 0, 6, 6, 78
NEG = -3.0e38
ORDER = ("q0 q1 q2 q3 k4 k5 k6 k7 s0 s1 s2 s3 s4 s5 s6 s7 v4 v5 v6 v7 p0 p1 p2 p3 p4 p5 p6 p7 "
         "w0 w1 w2 w3 w4 w5 w6 w7")
PERM = (0, 2, 4, 6, 1, 3, 5, 7)


def _rb(v):
    return v.astype(BF).astype(F32)


def _layernorm(xf):
    mu = jnp.mean(xf, axis=-1, keepdims=True)
    dv = xf - mu
    var = jnp.mean(dv * dv, axis=-1, keepdims=True)
    sd = _rb(jnp.sqrt(_rb(_rb(var) + EPS)))
    return _rb(_rb(xf - _rb(mu)) * (1.0 / sd))


def _f3(v):
    return v.astype(F32).reshape(v.shape[0] // 8, 8, D)


def _b2(v):
    return v.reshape(v.shape[0] * 8, D).astype(BF)


def _kernel(x_hbm, mem0_hbm, wq_hbm, wk_hbm, wv_hbm, wo_hbm, wr_hbm, wg_hbm, wu_hbm, wd_hbm,
            c_hbm, wmod_hbm, out_hbm,
            x_v, h_v, hp_v, att_v, ho_v, wqkv_v, wo_v, stage, wmod_v,
            wg_v, wu_v, wd_v, mem_v, cw_v, mod_v, r_v, sb_v, macc_v,
            part_v, fin_v, sems, *rings):
    w_hbm = (wq_hbm, wk_hbm, wv_hbm)
    ring = rings

    def piece_copy(t, sem, lo=0, n=D, dst=None):
        dst = (t % 2) * D + lo if dst is None else dst
        return pltpu.make_async_copy(
            w_hbm[t // 4].at[pl.ds(lo, n), pl.ds((t % 4) * 8, 8), :],
            stage.at[pl.ds(dst, n)], sems.at[sem])

    def unit_copy(j):
        sem = 1 if j == 1 else 6 + min(j, 10) % 3
        return piece_copy(j % NP, sem, QK * (j // NP), QK, 2 * D + QK * j)

    def stage_wait(row, n, sem):
        dst = stage.at[pl.ds(row, n)]
        pltpu.make_async_copy(dst, dst, sems.at[sem]).wait()

    def mq_copy(q, part):
        return pltpu.make_async_copy(wmod_hbm.at[:, pl.ds(part * D + q * QK, QK)],
                                     wmod_v.at[q, :, pl.ds(part * QK, QK)], sems.at[2])

    def wmod_copy(k, sem):
        col = k * 512 if isinstance(k, int) else pl.multiple_of(k * 512, 512)
        return pltpu.make_async_copy(wmod_hbm.at[:, pl.ds(col, 512)], wmod_v.at[k], sems.at[sem])

    def x_copy(lo, hi, sem):
        return pltpu.make_async_copy(x_hbm.at[0, pl.ds(lo, hi - lo), :],
                                     x_v.at[pl.ds(lo, hi - lo), :], sems.at[sem])

    def wo_copy(n):
        lo, rows = ((n // 2) * 512, 512) if n < 6 else (1536, 2560)
        return pltpu.make_async_copy(wo_hbm.at[pl.ds(lo, rows), pl.ds((n % 2) * 512, 512)],
                                     wo_v.at[n % 2, pl.ds(lo, rows)], sems.at[0])

    small_copies = [pltpu.make_async_copy(c_hbm, cw_v.at[0], sems.at[0]),
                    pltpu.make_async_copy(mem0_hbm.at[0], mem_v, sems.at[0]),
                    pltpu.make_async_copy(wr_hbm, cw_v.at[1], sems.at[0])]
    x0_copy = x_copy(0, X0, 1)
    mid_copies = ([x_copy(X0, (X0 + X1) // 2, 0), x_copy((X0 + X1) // 2, X1, 0)]
                  + [wo_copy(n) for n in range(8)])
    x2_copy = x_copy(X1, S, 1)
    ffn_copies = [pltpu.make_async_copy(wg_hbm, wg_v, sems.at[2]),
                  pltpu.make_async_copy(wu_hbm, wu_v, sems.at[2])] + [
        pltpu.make_async_copy(wd_hbm.at[:, pl.ds(k * 512, 512)], wd_v.at[k], sems.at[2])
        for k in range(2)]

    def relayout(src, base, n):
        u = pltpu.bitcast(stage[pl.ds(src, n)], U32)
        tok = None
        for i in range(n // 2):
            a = u[2 * i]
            b = u[2 * i + 1]
            even = (a & jnp.uint32(0xFFFF)) | (b << 16)
            odd = (a >> 16) | (b & jnp.uint32(0xFFFF0000))
            wqkv_v[pl.ds(base + i, 4, stride=PITCH), :] = even
            wqkv_v[pl.ds(base + 4 * PITCH + i, 4, stride=PITCH), :] = odd
            tok = even ^ odd if tok is None else tok ^ even ^ odd
        return jnp.concatenate([tok, tok], axis=0)

    CW = 256

    def ln_stats(xf):
        mu = jnp.mean(xf, axis=-1, keepdims=True)
        dv = xf - mu
        var = jnp.mean(dv * dv, axis=-1, keepdims=True)
        sd = _rb(jnp.sqrt(_rb(_rb(var) + EPS)))
        return _rb(mu), 1.0 / sd

    def mod_c(k, c):
        return mod_v[k, :, pl.ds(c * CW, CW)]

    def token(v):
        return pltpu.bitcast(v[:, :128] + v[:, 128:], U32)

    def after(v, trig):
        if trig is None:
            return v
        return jnp.concatenate([jnp.where(trig[0], trig[1], v[:, :128]), v[:, 128:]], axis=1)

    def post_work(row0, att, scores_out=None):
        st = {}

        def head(trig):
            a = after(att().astype(F32), trig)
            st["x2"] = _rb(x_v[pl.ds(row0, 8), :].astype(F32) + _rb(mod_v[2] * a))
            st["mu"], st["inv"] = ln_stats(st["x2"])

        def chunk(c, trig):
            xc = after(st["x2"][:, c * CW:(c + 1) * CW], trig)
            h2b = (_rb(_rb(_rb(xc - st["mu"]) * st["inv"]) * mod_c(4, c))
                   + mod_c(3, c)).astype(BF)
            h2 = h2b.astype(F32)
            ho_v[0, pl.ds(row0, 8), pl.ds(c * CW, CW)] = h2b
            o = xc + mod_c(5, c) * h2
            ho_v[1, pl.ds(row0, 8), pl.ds(c * CW, CW)] = o.astype(BF)
            rp = h2 * mod_c(6, c)
            st["r"] = rp if c == 0 else st["r"] + rp
            if c == D // CW - 1:
                r = jnp.sum(st["r"], axis=-1, keepdims=True)
                if scores_out is not None:
                    scores_out.append(r)
                    return None
                grp = row0 >> 3
                lanes = lax.broadcasted_iota(jnp.int32, (8, 128), 1)
                r_v[grp >> 7] = jnp.where(lanes == (grp & 127), r, r_v[grp >> 7])
            return token(o + st["r"])
        return [head] + [functools.partial(chunk, c) for c in range(D // CW)]

    def ln1_work(row0):
        st = {}

        def head(trig):
            st["x"] = after(x_v[pl.ds(row0, 8), :].astype(F32), trig)
            st["mu"], st["inv"] = ln_stats(st["x"])

        def chunk(c, trig):
            xc = after(st["x"][:, c * CW:(c + 1) * CW], trig)
            h = _rb(_rb(_rb(xc - st["mu"]) * st["inv"]) * mod_c(1, c)) + mod_c(0, c)
            ho_v[0, pl.ds(row0, 8), pl.ds(c * CW, CW)] = h.astype(BF)
            return token(h)
        return [head] + [functools.partial(chunk, c) for c in range(D // CW)]

    for cp in small_copies:
        cp.start()
    x0_copy.start()
    mq_copy(0, 0).start()

    r_v[...] = jnp.full(r_v.shape, NEG, F32)
    att_v[...] = jnp.zeros(att_v.shape, BF)

    for cp in small_copies:
        cp.wait()
    mod_v[6] = jnp.broadcast_to(cw_v[1].astype(F32), (8, D))
    cf = cw_v[0].astype(F32)
    sil = (cf * jax.nn.sigmoid(cf)).astype(BF)
    sc = jnp.broadcast_to(sil, (16, D))
    for k in range(8):
        sb_v[pl.ds(128 * k, 128), :] = jnp.broadcast_to(
            sil[:, 128 * k:128 * k + 128].astype(F32), (128, 128)).T

    mq_copy(0, 1).start()
    x0_copy.wait()

    LNB = X0 // 4

    def ln0(i, carry):
        r0 = pl.multiple_of(i * LNB, 8)
        ln = _b2(_layernorm(_f3(x_v[pl.ds(r0, LNB), :])))
        for q in range(4):
            h_v[q, pl.ds(r0, LNB), :] = ln[:, q * QK:(q + 1) * QK]

        @pl.when(i == 1)
        def _():
            unit_copy(0).start()
        return carry
    lax.fori_loop(0, 4, ln0, 0)

    def shift_scale(acc):
        y = _rb(acc)
        return y[:, :QK], _rb(1.0 + y[:, QK:])

    def modulated(q, r0, n, sh, sca):
        ln = h_v[q, pl.ds(r0, n), :].astype(F32).reshape(n // 8, 8, QK)
        return (_rb(ln * sca) + sh).reshape(n, QK).astype(BF)

    unit_copy(1).start()
    for part in range(2):
        mq_copy(0, part).wait()
    acc0 = jnp.dot(sc, wmod_v[0], preferred_element_type=F32)[0:8]
    macc_v[0] = acc0
    hp_v[0] = pltpu.bitcast(modulated(0, 0, BULK, *shift_scale(acc0)), U32)
    unit_copy(2).start()

    def first_unit(j):
        def relayout0(i, carry):
            relayout(2 * D + QK * j + pl.multiple_of(i * 128, 128), j * 8 * PITCH + i * 64, 128)
            return carry
        unit_copy(j).wait()
        lax.fori_loop(0, QK // 128, relayout0, 0)

    first_unit(0)
    mq_copy(1, 0).start()
    mq_copy(1, 1).start()
    unit_copy(3).start()

    def mod_rows(slab, r0, n, acc):
        for r in range(r0, r0 + n, 8):
            sv = sb_v[pl.ds(r, 8), :]
            t = wmod_v[slab, pl.ds(r, 8), :].astype(F32) * jnp.concatenate([sv] * 4, axis=1)
            acc = t if acc is None else acc + t
        return acc

    def ring_fill(g, t, y):
        ring[g][t >> 1, pl.ds(NRING - BULK // SEG, BULK // SEG),
                pl.ds(pl.multiple_of(16 * (t & 1), 16), 16), :] = (
            pltpu.bitcast(y.astype(BF), U32).reshape(BULK // SEG, 16, 128))

    def tie_lhs(col, never, toks):
        return jnp.concatenate(
            [jnp.where(never, toks[j], col[8 * j:8 * j + 8]) if j in toks
             else col[8 * j:8 * j + 8] for j in range(32)], axis=0)

    def add_tok(toks, j, tk):
        toks[j] = tk if j not in toks else toks[j] ^ tk

    starts = {0: [unit_copy(4)], 1: [unit_copy(5), piece_copy(3, 5, 0, 256)],
              2: [unit_copy(6), mq_copy(2, 0), mq_copy(2, 1)],
              3: [unit_copy(7), piece_copy(3, 5, 256, 256)], 4: [unit_copy(8)],
              5: [unit_copy(9), mq_copy(3, 0), mq_copy(3, 1)],
              6: [unit_copy(10), unit_copy(11)], 7: [piece_copy(3, 3, 512, 512)],
              8: [piece_copy(4, 4)], 9: [], 10: [wmod_copy(4, 2)], 11: []}

    def quarter_block(b_lo, b_hi, b, carry):
        first, final = b_lo == 0, b_hi == 4 * NP
        q = b_lo // NP
        p = b - NP * q
        if final:
            src = jnp.where(p == 0, 2 * D + 10 * QK, D + 512 * (p - 1))
            sem = 7 - 2 * p
            stage_wait(pl.multiple_of(src, 512), 512, sem)
            b3 = 3 * 8 * PITCH + 256 * (p - 1)
            jobs = [(src, jnp.where(p == 0, 8 * PITCH + 384, b3)),
                    (src + QK, jnp.where(p == 0, 2 * 8 * PITCH + 384, b3 + 128))]
        else:
            src = 2 * D + QK * (b + 1)
            last = p == NP - 1
            dst = jnp.where(last, 128 * (q + 1), (p + 1) * (8 * PITCH) + 128 * q)

            def unit_wait():
                stage_wait(pl.multiple_of(src, QK), QK, jnp.where(last, 6, 7 + p))
            if first:
                pl.when(b == 1)(functools.partial(first_unit, 1))
                pl.when(b > 0)(unit_wait)
                jobs = [(jnp.where(b == 0, 2 * D, src), jnp.where(b == 0, 0, dst))]
            else:
                unit_wait()
                jobs = [(src, dst)]

            @pl.when(last)
            def _():
                for part in range(2):
                    mq_copy(q + 1, part).wait()
            slab = jnp.where(last, q + 1, q)
        never = jnp.full((8, 128), b, jnp.int32) < 0

        def weights(k):
            return pltpu.bitcast(jnp.concatenate(
                [wqkv_v[pl.ds(pl.multiple_of((8 * p + kk) * PITCH + 128 * q, 8), 128), :]
                 for kk in (k, k + 1)], axis=1), BF)

        groups = [(s_ + 16 * g, d_ + 8 * g) for s_, d_ in jobs for g in range(QK // 16)]
        per = len(groups) // 4
        acc = None
        w = weights(0)
        for n, k in enumerate(range(0, 8, 2)):
            w_next = weights(k + 2) if k < 6 else None
            toks = {}
            if final and n == 2:
                wu = pltpu.bitcast(w_next, U32)
                wu = wu[:, :128] ^ wu[:, 128:]
                add_tok(toks, 3, functools.reduce(
                    jnp.bitwise_xor, [wu[8 * j:8 * j + 8] for j in range(16)]))
            for g in range(per):
                add_tok(toks, 4 + (g * 24) // per, relayout(*groups[n * per + g], 16))
            if not final and n < 2:
                for g in range(16):
                    acc = mod_rows(slab, 512 * n + 32 * g, 32, acc)
                    add_tok(toks, 2 * g + (n == 0), token(acc[:, :256] + acc[:, 256:]))
            if not final and n == 2:
                tot = jnp.broadcast_to(jnp.sum(acc, axis=0, keepdims=True), (8, 512))
                macc_v[q + 1] = tot
                sh, sca = shift_scale(tot)
            if not final and n >= 2:
                for g in range(16):
                    r0 = 256 * (n - 2) + 16 * g
                    hb = pltpu.bitcast(modulated(q + 1, r0, 16, sh, sca), U32)
                    hp_v[q + 1, pl.ds(r0 // 2, 8), :] = hb
                    add_tok(toks, (8 + (g * 3) // 2) if n == 2 else 2 * g,
                            hb[:, :128] ^ hb[:, 128:])
            lhs = jnp.concatenate([tie_lhs(hp_v[q, :, pl.ds(0, 128)], never, toks),
                                   hp_v[q, :, pl.ds(128, 128)]], axis=1)
            y = jnp.dot(pltpu.bitcast(lhs, BF), w, preferred_element_type=F32)
            if not first:
                y = y + part_v[p, n]
            if final:
                for j in range(2):
                    ring_fill(k + j, p, y[:, 128 * j:128 * j + 128])
            else:
                part_v[p, n] = y
            w = w_next

        for j in range(b_lo, b_hi):
            if starts[j]:
                @pl.when(b == j)
                def _():
                    for cp in starts[j]:
                        cp.start()
        return carry

    for b_lo, b_hi in ((0, NP), (NP, 2 * NP), (2 * NP, 3 * NP), (3 * NP, 4 * NP)):
        quarters = functools.partial(quarter_block, b_lo, b_hi)
        lax.fori_loop(b_lo, b_hi, quarters, 0)

    def bulk_dot(i, k, never, t, md):
        w = pltpu.bitcast(wqkv_v[pl.ds(pl.multiple_of((8 * i + k) * PITCH, 8), 512), :], BF)
        cols = [hp_v[c // 2, :, pl.ds(128 * (c % 2), 128)] for c in range(8)]
        toks = {}
        for g in range(8):
            tk = relayout((t & 1) * D + 128 * k + 16 * g, t * (8 * PITCH) + 64 * k + 8 * g, 16)
            md[1] = mod_rows(md[0], 128 * k + 16 * g, 16, md[1])
            toks[10 + 6 * (g + g // 4)] = tk ^ token(md[1][:, :256] + md[1][:, 256:])
        cols[0] = tie_lhs(cols[0], never, toks)
        cols[4] = tie_lhs(cols[4], never, {j - 32: tk for j, tk in toks.items()})
        hb = pltpu.bitcast(jnp.concatenate(cols, axis=1), BF)
        y = jnp.dot(hb, w, preferred_element_type=F32)
        ring_fill(k, i, y)

    def bulk_qkv(i, carry):
        @pl.when(i < 11)
        def _():
            par = (i + 1) & 1
            stage_wait(pl.multiple_of(par * D, D), D, 4 + par)

        @pl.when(i > NP)
        def _():
            wmod_copy(i, 2 + (i & 1)).wait()

        for j in range(NP, 10):
            @pl.when(i == j)
            def _():
                piece_copy(j + 2, 4 + j % 2).start()

        t = jnp.minimum(i + 1, 11)
        never = jnp.full((8, 128), i, jnp.int32) < 0
        md = [i, None]
        for k in range(8):
            bulk_dot(i, k, never, t, md)
        macc_v[jnp.maximum(i, 4)] = md[1]

        for j in range(NP, 10):
            @pl.when(i == j)
            def _():
                wmod_copy(j + 2, 2 + j % 2).start()
                if j < 9:
                    mid_copies[j - NP + 1].start()
                else:
                    for cp in mid_copies[7:]:
                        cp.start()
        return carry
    mid_copies[0].start()
    lax.fori_loop(NP, 12, bulk_qkv, 0)

    for q in range(4):
        sh, sca = shift_scale(macc_v[q])
        mod_v[0, :, pl.ds(q * QK, QK)] = sh
        mod_v[1, :, pl.ds(q * QK, QK)] = sca
        ho_v[0, pl.ds(BULK, RIDE), pl.ds(q * QK, QK)] = modulated(q, BULK, RIDE, sh, sca)
    for k in range(4, 12):
        y = _rb(jnp.sum(macc_v[k], axis=0, keepdims=True))
        if k // 2 == 4:
            y = _rb(1.0 + y)
        mod_v[k // 2, :, pl.ds((k % 2) * 512, 512)] = jnp.broadcast_to(y, (8, 512))
    for cp in mid_copies:
        cp.wait()
    x2_copy.start()
    for cp in ffn_copies:
        cp.start()

    scale = DH ** -0.5
    kk = lax.broadcasted_iota(jnp.int32, (M + SEG, 80), 0)
    cc = lax.broadcasted_iota(jnp.int32, (M + SEG, 80), 1)
    second = ((cc >= 8) & (cc < 16)) | (cc >= 48)
    allowed = (cc < 16) | (kk <= jnp.where(second, cc - 40, cc - 8))

    def over_keys(f, fr, v):
        t = v[0:8]
        for j in range(8, M + SEG, 8):
            t = f(t, v[j:j + 8])
        return fr(t, axis=0, keepdims=True)

    def tied(u, never, toks):
        if not toks:
            return u
        parts, at = [], 0
        for j, tk in enumerate(toks):
            r = 64 * j
            if r > at:
                parts.append(u[at:r])
            parts.append(jnp.where(never, tk, u[r:r + 8]))
            at = r + 8
        return jnp.concatenate(parts + [u[at:]], axis=0)

    def w_slab(t, g, lo=0, n=512, never=None, toks=()):
        return pltpu.bitcast(
            tied(wqkv_v[pl.ds((8 * t + g) * PITCH + lo, n), :], never, toks), BF)

    def step(s, u, mem, left, att_prev):
        odd = left is not None
        wr = 3 * lax.rem(s >> 2, NRING // 3)
        rd = lax.rem(s + NRING - BULK // SEG, NRING)

        def ring_put(g, t, y):
            if odd:
                u32 = pltpu.bitcast(y.astype(BF), U32)
                parts = [(3 * u, u32[4:8]), (3 * u + 1, u32[8:16])]
            else:
                u32 = pltpu.bitcast(y[M:].astype(BF), U32)
                parts = [(3 * u, u32[0:8]), (3 * u + 2, u32[8:12])]
            for grp, v in parts:
                ring[g][t // 2, wr + grp // 4,
                        pl.ds(16 * (t % 2) + 4 * (grp % 4), v.shape[0]), :] = v

        xin = jnp.concatenate(
            [mem, ho_v[0, pl.ds(pl.multiple_of(BULK + RIDE * s, 8), RIDE), :]], axis=0)

        prow = SEG * (s - 1) if odd else jnp.maximum(SEG * s - 40, 0)
        nrow = BULK + RIDE * jnp.minimum(s + 1, NSEG - 1)
        works = [post_work(pl.multiple_of(prow + 8 * q, 8), functools.partial(att_prev, q))
                 for q in range(3 if odd else 5)]
        works += [ln1_work(pl.multiple_of(nrow + 8 * q, 8)) for q in range(RIDE // 8)]
        never = jnp.full((8, 128), s, jnp.int32) < 0
        gap = (SIDE_END - SIDE0 - SIDE_LAT - SIDE_DUE) // len(works)
        sched = {}
        for q, wk in enumerate(works):
            sched.setdefault(SIDE0 + gap * q, []).append(wk[0])
            for c in range(1, len(wk)):
                sched.setdefault(SIDE0 + SIDE_LAT + gap * q + ((c - 1) * gap) // 4,
                                 []).append(wk[c])

        memqkv, probs, wl, new_left, toks = {}, {}, {}, {}, {}
        acc = []
        chain = []

        ndot = [0]

        def proj(g, t_lo, t_hi):
            part = {}
            if u > 0 and ndot[0] == 0:
                for t in range(t_lo, t_lo + 6):
                    part[t] = jnp.dot(xin[:, :512], w_slab(t, g, 0, 256),
                                      preferred_element_type=F32)
            for t0 in range(t_lo, t_hi, 2):
                ys = []
                for t in (t0, t0 + 1):
                    n = ndot[0]
                    ndot[0] += 1
                    if t in part:
                        y = jnp.dot(xin[:, 512:], w_slab(t, g, 256, 256),
                                    preferred_element_type=F32) + part[t]
                    else:
                        y = jnp.dot(xin, w_slab(t, g, 0, 512, never, toks.get(n)),
                                    preferred_element_type=F32)
                    ring_put(g, t, y)
                    ys.append(y[:M])
                    for item in sched.get(n, ()):
                        tk = item((never, y[:M]))
                        if tk is not None:
                            toks.setdefault(n + SIDE_DUE, []).append(tk)
                memqkv[(t0, g)] = jnp.concatenate(ys, axis=0).astype(BF)

        def cat(t0, g):
            return jnp.concatenate(
                [memqkv[(t0, g)], pltpu.bitcast(ring[g][t0 // 2, rd], BF)], axis=0)

        def scores(g):
            for p in (0, 2):
                if len(chain) < 4:
                    qt = pltpu.bitcast(cat(p, g).T, U32)
                    qt = jnp.concatenate(
                        [jnp.where(never[:, :80], qt[8:16], qt[0:8]), qt[8:]], axis=0)
                    st = jnp.dot(cat(4 + p, g), pltpu.bitcast(qt, BF),
                                 preferred_element_type=F32)
                else:
                    st = lax.dot_general(cat(4 + p, g), cat(p, g), (((1,), (1,)), ((), ())),
                                         preferred_element_type=F32)
                st = jnp.where(second, jnp.concatenate([st[8:16], st[48:80]], axis=0),
                               jnp.concatenate([st[0:8], st[16:48]], axis=0))
                if chain:
                    st = jnp.concatenate(
                        [jnp.where(never[:, :80], chain[-1], st[0:8]), st[8:]], axis=0)
                st = jnp.where(allowed, st * scale, -1e9)
                e = jnp.exp(st - over_keys(jnp.maximum, jnp.max, st))
                l = over_keys(jnp.add, jnp.sum, e)
                chain.append(jnp.broadcast_to(l, (8, 80)))
                rc = pl.reciprocal(l, approx=True)
                e = e * (rc * (2.0 - l * rc))
                e0 = jnp.where(second, 0.0, e)
                e1 = jnp.where(second, e, 0.0)
                probs[(p, g)] = jnp.concatenate(
                    [e0[:M], e1[:M], e0[M:], e1[M:]], axis=0).astype(BF)

        def pv(g):
            for p in (0, 2):
                o = lax.dot_general(probs[(p, g)], cat(8 + p, g), (((0,), (0,)), ((), ())),
                                    preferred_element_type=F32)
                for j in range(2):
                    om, ot = o[8 * j:8 * j + 8], o[16 + 32 * j:48 + 32 * j]
                    if odd:
                        rows = [om, left[(p + j, g)], ot]
                    else:
                        rows = [om, ot[:RIDE]]
                        new_left[(p + j, g)] = ot[RIDE:]
                    wl[(p + j, g)] = jnp.concatenate(rows, axis=0).astype(BF)

        def wo(g):
            a = jnp.concatenate([wl[(o, g)] for o in range(4)], axis=1)
            w = jnp.concatenate(
                [jnp.concatenate([wo_v[n, pl.ds((8 * o + PERM[g]) * DH, DH), :]
                                  for o in range(4)], axis=0) for n in range(2)], axis=1)
            y = jnp.dot(a, w, preferred_element_type=F32)
            acc[:] = [y if not acc else y + acc[0]]

        for op in ORDER.split():
            g = int(op[1])
            if op[0] in "qkv":
                proj(g, *{"q": (0, 12), "k": (0, 8), "v": (8, 12)}[op[0]])
            else:
                {"s": scores, "p": pv, "w": wo}[op[0]](g)
        y = acc[0].astype(BF)
        return y[:M], y[M:], (None if odd else new_left)

    def out_copy(row0, n, k):
        return pltpu.make_async_copy(ho_v.at[1, pl.ds(row0, n), :],
                                     out_hbm.at[0, pl.ds(row0, n), :], sems.at[3 + k])

    OB = SEG * UNROLL

    def carried(q):
        return att_v[pl.ds(8 * q, 8), :]

    def steps(i, carry):
        @pl.when(i == 16 // UNROLL)
        def _():
            x2_copy.wait()

        mem, left, att_prev = mem_v[...], None, carried
        for u in range(UNROLL):
            mem, att, left = step(i * UNROLL + u, u, mem, left, att_prev)
            att_prev = (lambda a: lambda q: a[8 * q:8 * q + 8])(att)
        mem_v[...] = mem
        att_v[...] = att

        @pl.when(i >= 1)
        def _():
            out_copy(pl.multiple_of((i - 1) * OB, OB), OB, 0).start()
        return carry
    lax.fori_loop(0, NSEG // UNROLL, steps, 0)

    for cp in ffn_copies:
        cp.wait()

    def two(ref, a, b):
        return jnp.concatenate([ref[pl.ds(a, 8), :], ref[pl.ds(b, 8), :]], axis=0)

    def ffn_act(h, c):
        g = _rb(jnp.dot(h, wg_v[:, pl.ds(512 * c, 512)], preferred_element_type=F32))
        u = _rb(jnp.dot(h, wu_v[:, pl.ds(512 * c, 512)], preferred_element_type=F32))
        return (_rb(g * jax.nn.sigmoid(g)) * u).astype(BF)

    def ffn_down(a, c):
        wd = jnp.concatenate([wd_v[k, pl.ds(512 * c, 512), :] for k in range(2)], axis=1)
        return jnp.dot(a, wd, preferred_element_type=F32)

    sub1 = lax.broadcasted_iota(jnp.int32, (16, 128), 0)
    lan1 = lax.broadcasted_iota(jnp.int32, (16, 128), 1)
    idx = (sub1 // 8) * 1024 + lan1 * 8 + sub1 % 8
    early = _rb(r_v[pl.ds(0, 2)].reshape(16, 128))

    key = jnp.where(idx < S - 40,
                    pltpu.bitcast(pltpu.bitcast(early, jnp.int32) | (S - 1 - idx), F32), -jnp.inf)

    def guess(k):
        m = jnp.max(jnp.max(k, axis=0, keepdims=True), axis=1, keepdims=True)
        i = S - 1 - (pltpu.bitcast(jnp.broadcast_to(m, (8, 128)), jnp.int32) & (S - 1))
        return m, pl.multiple_of(jnp.minimum(i[0, 0] >> 3, (S - 48) // 8) * 8, 8)
    k_a, gs_a = guess(key)
    _, gs_b = guess(jnp.where(key >= k_a, -jnp.inf, key))
    acts = [ffn_act(two(ho_v.at[0], gs_a, gs_b), 0)]

    last = []
    for q in range(5):
        for item in post_work(S - 40 + 8 * q, functools.partial(carried, q), last):
            item(None)
    out_copy(S - OB, OB, 0).start()

    def top2(val, idx, valid):
        def reduce(f, v):
            v = f(v, axis=0, keepdims=True)
            return v if v.shape[1] == 1 else f(v, axis=1, keepdims=True)

        def argtop(ok):
            v = jnp.where(ok, val, -jnp.inf)
            m = reduce(jnp.max, v)
            return m, reduce(jnp.min, jnp.where(ok & (v >= m), idx, float(S)))
        m1, i1 = argtop(valid)
        return (m1, i1), argtop(valid & (idx != i1))

    c_a, c_b = top2(early, idx.astype(F32), idx < S - 40)
    sub2 = lax.broadcasted_iota(jnp.int32, (48, 1), 0)
    val2 = jnp.concatenate([_rb(r) for r in last] + [jnp.where(sub2[:8] == 0, c_a[0], c_b[0])],
                           axis=0)
    idx2 = jnp.where(sub2 < 40, (sub2 + (S - 40)).astype(F32),
                     jnp.where(sub2 == 40, c_a[1], c_b[1]))
    (m_a, i_a), (m_b, i_b) = top2(val2, idx2, sub2 < 42)
    i_a = i_a.astype(jnp.int32)
    i_b = i_b.astype(jnp.int32)
    ia = jnp.clip(i_a[0, 0], 0, S - 1)
    ib = jnp.clip(i_b[0, 0], 0, S - 1)
    blk_a = pl.multiple_of((ia // 8) * 8, 8)
    blk_b = pl.multiple_of((ib // 8) * 8, 8)

    hs = two(ho_v.at[0], blk_a, blk_b)
    y0 = y = None
    for c in range(1, FF // 512 + 1):
        if c < FF // 512:
            acts.append(ffn_act(hs, c))
        t = ffn_down(acts[c - 1], c - 1)
        if c == 1:
            y0 = t
        else:
            y = t if y is None else t + y
    sub = lax.broadcasted_iota(jnp.int32, (16, 1), 0)
    rows = jnp.where(sub < 8, blk_a + sub, blk_b + sub - 8)
    gate = jnp.where(rows == ia, jax.nn.sigmoid(m_a),
                     jnp.where(rows == ib, jax.nn.sigmoid(m_b), 0.0))

    def finish(ffn):
        upd = jnp.where((rows == ia) | (rows == ib), ffn * gate, 0.0).reshape(2, 8, D)
        fin_v[...] = _b2(_f3(two(ho_v.at[1], blk_a, blk_b)) + mod_v[5] * upd)

    finish(y + y0)

    @pl.when((gs_a != blk_a) | (gs_b != blk_b))
    def _():
        finish(y + ffn_down(ffn_act(hs, 0), 0))

    def patch(k, blk):
        return pltpu.make_async_copy(fin_v.at[pl.ds(8 * k, 8), :],
                                     out_hbm.at[0, pl.ds(blk, 8), :], sems.at[3 + k])

    out_copy(0, S, 0).wait()
    patch(0, blk_a).start()

    @pl.when(blk_a != blk_b)
    def _():
        patch(1, blk_b).start()
        patch(1, blk_b).wait()
    patch(0, blk_a).wait()


@jax.jit
def pallas_adaLN_cond__memory_aug_recurrent_mem_tr__moe_arch_mod__prompt_kernel(
    A_x, A_mem0, A_Wq, A_Wk, A_Wv, A_Wo, A_seg_len, B_x, B_w_r, B_w_gate, B_w_up, B_w_down, c,
    w_mod,
):
    del B_x
    del A_seg_len
    assert A_x.shape == (1, S, D) and A_Wq.shape == (D, H, DH) and A_mem0.shape == (1, M, D)
    any_spec = pl.BlockSpec(memory_space=pl.ANY)
    scratch = [
        pltpu.VMEM((S, D), BF),
        pltpu.VMEM((4, X0, QK), BF),
        pltpu.VMEM((4, BULK // 2, QK), U32),
        pltpu.VMEM((40, D), BF),
        pltpu.VMEM((2, S, D), BF),
        pltpu.VMEM((100 * PITCH, 128), U32),
        pltpu.VMEM((2, H * DH, 512), BF),
        pltpu.VMEM((5 * D, 8, 128), BF),
        pltpu.VMEM((12, D, 512), BF),
        pltpu.VMEM((D, FF), BF),
        pltpu.VMEM((D, FF), BF),
        pltpu.VMEM((2, FF, 512), BF),
        pltpu.VMEM((M, D), BF),
        pltpu.VMEM((4, 1, D), BF),
        pltpu.VMEM((7, 8, D), F32),
        pltpu.VMEM((4, 8, 128), F32),
        pltpu.VMEM((D, 128), F32),
        pltpu.VMEM((12, 8, 512), F32),
        pltpu.VMEM((NP, 4, BULK, 256), F32),
        pltpu.VMEM((16, D), BF),
        pltpu.SemaphoreType.DMA((9,)),
    ] + [pltpu.VMEM((6, NRING, 32, 128), U32)] * 8
    return pl.pallas_call(
        _kernel,
        out_shape=jax.ShapeDtypeStruct((1, S, D), BF),
        in_specs=[any_spec] * 12,
        out_specs=any_spec,
        scratch_shapes=scratch,
        compiler_params=pltpu.CompilerParams(vmem_limit_bytes=120 * 1024 * 1024),
    )(A_x, A_mem0, A_Wq, A_Wk, A_Wv, A_Wo.reshape(H * DH, D), B_w_r.reshape(1, D), B_w_gate,
      B_w_up, B_w_down, c, w_mod)
```

```python
import functools

import jax
import jax.numpy as jnp
from jax import lax
import jax.experimental.pallas as pl
import jax.experimental.pallas.tpu as pltpu

BF = jnp.bfloat16
F32 = jnp.float32
U32 = jnp.uint32

S = 2048
D = 1024
H = 32
DH = 128
M = 8
SEG = 32
NSEG = S // SEG
FF = 3584
RIDE = 24
BULK = S - RIDE * NSEG
X0 = BULK + 32
NRING = 18
PITCH = 520
X1 = 1024
NP = 3
QK = D // 4
UNROLL = 4
NSPEC = 2
EPS = 1e-5
SIDE0, SIDE_LAT, SIDE_DUE, SIDE_END = 0, 6, 6, 78
NEG = -3.0e38
ORDER = ("q0 q1 q2 q3 k4 k5 k6 k7 s0 s1 s2 s3 s4 s5 s6 s7 v4 v5 v6 v7 p0 p1 p2 p3 p4 p5 p6 p7 "
         "w0 w1 w2 w3 w4 w5 w6 w7")
PERM = (0, 2, 4, 6, 1, 3, 5, 7)


def _rb(v):
    return v.astype(BF).astype(F32)


def _layernorm(xf):
    mu = jnp.mean(xf, axis=-1, keepdims=True)
    dv = xf - mu
    var = jnp.mean(dv * dv, axis=-1, keepdims=True)
    sd = _rb(jnp.sqrt(_rb(_rb(var) + EPS)))
    return _rb(_rb(xf - _rb(mu)) * (1.0 / sd))


def _f3(v):
    return v.astype(F32).reshape(v.shape[0] // 8, 8, D)


def _b2(v):
    return v.reshape(v.shape[0] * 8, D).astype(BF)


def _kernel(x_hbm, mem0_hbm, wq_hbm, wk_hbm, wv_hbm, wo_hbm, wr_hbm, wg_hbm, wu_hbm, wd_hbm,
            c_hbm, wmod_hbm, out_hbm,
            x_v, h_v, hp_v, att_v, ho_v, wqkv_v, wo_v, stage, wmod_v,
            wg_v, wu_v, wd_v, mem_v, cw_v, mod_v, r_v, sb_v, macc_v,
            part_v, fin_v, sems, *rings):
    w_hbm = (wq_hbm, wk_hbm, wv_hbm)
    ring = rings

    def piece_copy(t, sem, lo=0, n=D, dst=None):
        dst = (t % 2) * D + lo if dst is None else dst
        return pltpu.make_async_copy(
            w_hbm[t // 4].at[pl.ds(lo, n), pl.ds((t % 4) * 8, 8), :],
            stage.at[pl.ds(dst, n)], sems.at[sem])

    def unit_copy(j):
        sem = 1 if j == 1 else 6 + min(j, 10) % 3
        return piece_copy(j % NP, sem, QK * (j // NP), QK, 2 * D + QK * j)

    def stage_wait(row, n, sem):
        dst = stage.at[pl.ds(row, n)]
        pltpu.make_async_copy(dst, dst, sems.at[sem]).wait()

    def mq_copy(q, part):
        return pltpu.make_async_copy(wmod_hbm.at[:, pl.ds(part * D + q * QK, QK)],
                                     wmod_v.at[q, :, pl.ds(part * QK, QK)], sems.at[2])

    def wmod_copy(k, sem):
        col = k * 512 if isinstance(k, int) else pl.multiple_of(k * 512, 512)
        return pltpu.make_async_copy(wmod_hbm.at[:, pl.ds(col, 512)], wmod_v.at[k], sems.at[sem])

    def x_copy(lo, hi, sem):
        return pltpu.make_async_copy(x_hbm.at[0, pl.ds(lo, hi - lo), :],
                                     x_v.at[pl.ds(lo, hi - lo), :], sems.at[sem])

    def wo_copy(n):
        lo, rows = ((n // 2) * 512, 512) if n < 6 else (1536, 2560)
        return pltpu.make_async_copy(wo_hbm.at[pl.ds(lo, rows), pl.ds((n % 2) * 512, 512)],
                                     wo_v.at[n % 2, pl.ds(lo, rows)], sems.at[0])

    small_copies = [pltpu.make_async_copy(c_hbm, cw_v.at[0], sems.at[0]),
                    pltpu.make_async_copy(mem0_hbm.at[0], mem_v, sems.at[0]),
                    pltpu.make_async_copy(wr_hbm, cw_v.at[1], sems.at[0])]
    x0_copy = x_copy(0, X0, 1)
    mid_copies = ([x_copy(X0, (X0 + X1) // 2, 0), x_copy((X0 + X1) // 2, X1, 0)]
                  + [wo_copy(n) for n in range(8)])
    x2_copy = x_copy(X1, S, 1)
    ffn_copies = [pltpu.make_async_copy(wg_hbm, wg_v, sems.at[2]),
                  pltpu.make_async_copy(wu_hbm, wu_v, sems.at[2])] + [
        pltpu.make_async_copy(wd_hbm.at[:, pl.ds(k * 512, 512)], wd_v.at[k], sems.at[2])
        for k in range(2)]

    def relayout(src, base, n):
        u = pltpu.bitcast(stage[pl.ds(src, n)], U32)
        tok = None
        for i in range(n // 2):
            a = u[2 * i]
            b = u[2 * i + 1]
            even = (a & jnp.uint32(0xFFFF)) | (b << 16)
            odd = (a >> 16) | (b & jnp.uint32(0xFFFF0000))
            wqkv_v[pl.ds(base + i, 4, stride=PITCH), :] = even
            wqkv_v[pl.ds(base + 4 * PITCH + i, 4, stride=PITCH), :] = odd
            tok = even ^ odd if tok is None else tok ^ even ^ odd
        return jnp.concatenate([tok, tok], axis=0)

    CW = 256

    def ln_stats(xf):
        mu = jnp.mean(xf, axis=-1, keepdims=True)
        dv = xf - mu
        var = jnp.mean(dv * dv, axis=-1, keepdims=True)
        sd = _rb(jnp.sqrt(_rb(_rb(var) + EPS)))
        return _rb(mu), 1.0 / sd

    def mod_c(k, c):
        return mod_v[k, :, pl.ds(c * CW, CW)]

    def token(v):
        return pltpu.bitcast(v[:, :128] + v[:, 128:], U32)

    def after(v, trig):
        if trig is None:
            return v
        return jnp.concatenate([jnp.where(trig[0], trig[1], v[:, :128]), v[:, 128:]], axis=1)

    def post_work(row0, att, scores_out=None):
        st = {}

        def head(trig):
            a = after(att().astype(F32), trig)
            st["x2"] = _rb(x_v[pl.ds(row0, 8), :].astype(F32) + _rb(mod_v[2] * a))
            st["mu"], st["inv"] = ln_stats(st["x2"])

        def chunk(c, trig):
            xc = after(st["x2"][:, c * CW:(c + 1) * CW], trig)
            h2b = (_rb(_rb(_rb(xc - st["mu"]) * st["inv"]) * mod_c(4, c))
                   + mod_c(3, c)).astype(BF)
            h2 = h2b.astype(F32)
            ho_v[0, pl.ds(row0, 8), pl.ds(c * CW, CW)] = h2b
            o = xc + mod_c(5, c) * h2
            ho_v[1, pl.ds(row0, 8), pl.ds(c * CW, CW)] = o.astype(BF)
            rp = h2 * mod_c(6, c)
            st["r"] = rp if c == 0 else st["r"] + rp
            if c == D // CW - 1:
                r = jnp.sum(st["r"], axis=-1, keepdims=True)
                if scores_out is not None:
                    scores_out.append(r)
                    return None
                grp = row0 >> 3
                lanes = lax.broadcasted_iota(jnp.int32, (8, 128), 1)
                r_v[grp >> 7] = jnp.where(lanes == (grp & 127), r, r_v[grp >> 7])
            return token(o + st["r"])
        return [head] + [functools.partial(chunk, c) for c in range(D // CW)]

    def ln1_work(row0):
        st = {}

        def head(trig):
            st["x"] = after(x_v[pl.ds(row0, 8), :].astype(F32), trig)
            st["mu"], st["inv"] = ln_stats(st["x"])

        def chunk(c, trig):
            xc = after(st["x"][:, c * CW:(c + 1) * CW], trig)
            h = _rb(_rb(_rb(xc - st["mu"]) * st["inv"]) * mod_c(1, c)) + mod_c(0, c)
            ho_v[0, pl.ds(row0, 8), pl.ds(c * CW, CW)] = h.astype(BF)
            return token(h)
        return [head] + [functools.partial(chunk, c) for c in range(D // CW)]

    for cp in small_copies:
        cp.start()
    x0_copy.start()
    mq_copy(0, 0).start()

    r_v[...] = jnp.full(r_v.shape, NEG, F32)
    att_v[...] = jnp.zeros(att_v.shape, BF)

    for cp in small_copies:
        cp.wait()
    mod_v[6] = jnp.broadcast_to(cw_v[1].astype(F32), (8, D))
    cf = cw_v[0].astype(F32)
    sil = (cf * jax.nn.sigmoid(cf)).astype(BF)
    sc = jnp.broadcast_to(sil, (16, D))
    for k in range(8):
        sb_v[pl.ds(128 * k, 128), :] = jnp.broadcast_to(
            sil[:, 128 * k:128 * k + 128].astype(F32), (128, 128)).T

    mq_copy(0, 1).start()
    x0_copy.wait()

    LNB = X0 // 4

    def ln0(i, carry):
        r0 = pl.multiple_of(i * LNB, 8)
        ln = _b2(_layernorm(_f3(x_v[pl.ds(r0, LNB), :])))
        for q in range(4):
            h_v[q, pl.ds(r0, LNB), :] = ln[:, q * QK:(q + 1) * QK]

        @pl.when(i == 1)
        def _():
            unit_copy(0).start()
        return carry
    lax.fori_loop(0, 4, ln0, 0)

    def shift_scale(acc):
        y = _rb(acc)
        return y[:, :QK], _rb(1.0 + y[:, QK:])

    def modulated(q, r0, n, sh, sca):
        ln = h_v[q, pl.ds(r0, n), :].astype(F32).reshape(n // 8, 8, QK)
        return (_rb(ln * sca) + sh).reshape(n, QK).astype(BF)

    unit_copy(1).start()
    for part in range(2):
        mq_copy(0, part).wait()
    acc0 = jnp.dot(sc, wmod_v[0], preferred_element_type=F32)[0:8]
    macc_v[0] = acc0
    hp_v[0] = pltpu.bitcast(modulated(0, 0, BULK, *shift_scale(acc0)), U32)
    unit_copy(2).start()

    def first_unit(j):
        def relayout0(i, carry):
            relayout(2 * D + QK * j + pl.multiple_of(i * 128, 128), j * 8 * PITCH + i * 64, 128)
            return carry
        unit_copy(j).wait()
        lax.fori_loop(0, QK // 128, relayout0, 0)

    first_unit(0)
    mq_copy(1, 0).start()
    mq_copy(1, 1).start()
    unit_copy(3).start()

    def mod_rows(slab, r0, n, acc):
        for r in range(r0, r0 + n, 8):
            sv = sb_v[pl.ds(r, 8), :]
            t = wmod_v[slab, pl.ds(r, 8), :].astype(F32) * jnp.concatenate([sv] * 4, axis=1)
            acc = t if acc is None else acc + t
        return acc

    def ring_fill(g, t, y):
        ring[g][t >> 1, pl.ds(NRING - BULK // SEG, BULK // SEG),
                pl.ds(pl.multiple_of(16 * (t & 1), 16), 16), :] = (
            pltpu.bitcast(y.astype(BF), U32).reshape(BULK // SEG, 16, 128))

    def tie_lhs(col, never, toks):
        return jnp.concatenate(
            [jnp.where(never, toks[j], col[8 * j:8 * j + 8]) if j in toks
             else col[8 * j:8 * j + 8] for j in range(32)], axis=0)

    def add_tok(toks, j, tk):
        toks[j] = tk if j not in toks else toks[j] ^ tk

    starts = {0: [unit_copy(4)], 1: [unit_copy(5), piece_copy(3, 5, 0, 256)],
              2: [unit_copy(6), mq_copy(2, 0), mq_copy(2, 1)],
              3: [unit_copy(7), piece_copy(3, 5, 256, 256)], 4: [unit_copy(8)],
              5: [unit_copy(9), mq_copy(3, 0), mq_copy(3, 1)],
              6: [unit_copy(10), unit_copy(11)], 7: [piece_copy(3, 3, 512, 512)],
              8: [piece_copy(4, 4)], 9: [], 10: [wmod_copy(4, 2)], 11: []}

    def quarter_block(b_lo, b_hi, b, carry):
        first, final = b_lo == 0, b_hi == 4 * NP
        q = b_lo // NP
        p = b - NP * q
        if final:
            src = jnp.where(p == 0, 2 * D + 10 * QK, D + 512 * (p - 1))
            sem = 7 - 2 * p
            stage_wait(pl.multiple_of(src, 512), 512, sem)
            b3 = 3 * 8 * PITCH + 256 * (p - 1)
            jobs = [(src, jnp.where(p == 0, 8 * PITCH + 384, b3)),
                    (src + QK, jnp.where(p == 0, 2 * 8 * PITCH + 384, b3 + 128))]
        else:
            src = 2 * D + QK * (b + 1)
            last = p == NP - 1
            dst = jnp.where(last, 128 * (q + 1), (p + 1) * (8 * PITCH) + 128 * q)

            def unit_wait():
                stage_wait(pl.multiple_of(src, QK), QK, jnp.where(last, 6, 7 + p))
            if first:
                pl.when(b == 1)(functools.partial(first_unit, 1))
                pl.when(b > 0)(unit_wait)
                jobs = [(jnp.where(b == 0, 2 * D, src), jnp.where(b == 0, 0, dst))]
            else:
                unit_wait()
                jobs = [(src, dst)]

            @pl.when(last)
            def _():
                for part in range(2):
                    mq_copy(q + 1, part).wait()
            slab = jnp.where(last, q + 1, q)
        never = jnp.full((8, 128), b, jnp.int32) < 0

        def weights(k):
            return pltpu.bitcast(jnp.concatenate(
                [wqkv_v[pl.ds(pl.multiple_of((8 * p + kk) * PITCH + 128 * q, 8), 128), :]
                 for kk in (k, k + 1)], axis=1), BF)

        groups = [(s_ + 16 * g, d_ + 8 * g) for s_, d_ in jobs for g in range(QK // 16)]
        per = len(groups) // 4
        acc = None
        w = weights(0)
        for n, k in enumerate(range(0, 8, 2)):
            w_next = weights(k + 2) if k < 6 else None
            toks = {}
            if final and n == 2:
                wu = pltpu.bitcast(w_next, U32)
                wu = wu[:, :128] ^ wu[:, 128:]
                add_tok(toks, 3, functools.reduce(
                    jnp.bitwise_xor, [wu[8 * j:8 * j + 8] for j in range(16)]))
            for g in range(per):
                add_tok(toks, 4 + (g * 24) // per, relayout(*groups[n * per + g], 16))
            if not final and n < 2:
                for g in range(16):
                    acc = mod_rows(slab, 512 * n + 32 * g, 32, acc)
                    add_tok(toks, 2 * g + (n == 0), token(acc[:, :256] + acc[:, 256:]))
            if not final and n == 2:
                tot = jnp.broadcast_to(jnp.sum(acc, axis=0, keepdims=True), (8, 512))
                macc_v[q + 1] = tot
                sh, sca = shift_scale(tot)
            if not final and n >= 2:
                for g in range(16):
                    r0 = 256 * (n - 2) + 16 * g
                    hb = pltpu.bitcast(modulated(q + 1, r0, 16, sh, sca), U32)
                    hp_v[q + 1, pl.ds(r0 // 2, 8), :] = hb
                    add_tok(toks, (8 + (g * 3) // 2) if n == 2 else 2 * g,
                            hb[:, :128] ^ hb[:, 128:])
            lhs = jnp.concatenate([tie_lhs(hp_v[q, :, pl.ds(0, 128)], never, toks),
                                   hp_v[q, :, pl.ds(128, 128)]], axis=1)
            y = jnp.dot(pltpu.bitcast(lhs, BF), w, preferred_element_type=F32)
            if not first:
                y = y + part_v[p, n]
            if final:
                for j in range(2):
                    ring_fill(k + j, p, y[:, 128 * j:128 * j + 128])
            else:
                part_v[p, n] = y
            w = w_next

        for j in range(b_lo, b_hi):
            if starts[j]:
                @pl.when(b == j)
                def _():
                    for cp in starts[j]:
                        cp.start()
        return carry

    for b_lo, b_hi in ((0, NP), (NP, 2 * NP), (2 * NP, 3 * NP), (3 * NP, 4 * NP)):
        quarters = functools.partial(quarter_block, b_lo, b_hi)
        lax.fori_loop(b_lo, b_hi, quarters, 0)

    def bulk_dot(i, k, never, t, md):
        w = pltpu.bitcast(wqkv_v[pl.ds(pl.multiple_of((8 * i + k) * PITCH, 8), 512), :], BF)
        cols = [hp_v[c // 2, :, pl.ds(128 * (c % 2), 128)] for c in range(8)]
        toks = {}
        for g in range(8):
            tk = relayout((t & 1) * D + 128 * k + 16 * g, t * (8 * PITCH) + 64 * k + 8 * g, 16)
            md[1] = mod_rows(md[0], 128 * k + 16 * g, 16, md[1])
            toks[10 + 6 * (g + g // 4)] = tk ^ token(md[1][:, :256] + md[1][:, 256:])
        cols[0] = tie_lhs(cols[0], never, toks)
        cols[4] = tie_lhs(cols[4], never, {j - 32: tk for j, tk in toks.items()})
        hb = pltpu.bitcast(jnp.concatenate(cols, axis=1), BF)
        y = jnp.dot(hb, w, preferred_element_type=F32)
        ring_fill(k, i, y)

    def bulk_qkv(i, carry):
        @pl.when(i < 11)
        def _():
            par = (i + 1) & 1
            stage_wait(pl.multiple_of(par * D, D), D, 4 + par)

        @pl.when(i > NP)
        def _():
            wmod_copy(i, 2 + (i & 1)).wait()

        for j in range(NP, 10):
            @pl.when(i == j)
            def _():
                piece_copy(j + 2, 4 + j % 2).start()

        t = jnp.minimum(i + 1, 11)
        never = jnp.full((8, 128), i, jnp.int32) < 0
        md = [i, None]
        for k in range(8):
            bulk_dot(i, k, never, t, md)
        macc_v[jnp.maximum(i, 4)] = md[1]

        for j in range(NP, 10):
            @pl.when(i == j)
            def _():
                wmod_copy(j + 2, 2 + j % 2).start()
                if j < 9:
                    mid_copies[j - NP + 1].start()
                else:
                    for cp in mid_copies[7:]:
                        cp.start()
        return carry
    mid_copies[0].start()
    lax.fori_loop(NP, 12, bulk_qkv, 0)

    for q in range(4):
        sh, sca = shift_scale(macc_v[q])
        mod_v[0, :, pl.ds(q * QK, QK)] = sh
        mod_v[1, :, pl.ds(q * QK, QK)] = sca
        ho_v[0, pl.ds(BULK, RIDE), pl.ds(q * QK, QK)] = modulated(q, BULK, RIDE, sh, sca)
    for k in range(4, 12):
        y = _rb(jnp.sum(macc_v[k], axis=0, keepdims=True))
        if k // 2 == 4:
            y = _rb(1.0 + y)
        mod_v[k // 2, :, pl.ds((k % 2) * 512, 512)] = jnp.broadcast_to(y, (8, 512))
    for cp in mid_copies:
        cp.wait()
    x2_copy.start()
    for cp in ffn_copies:
        cp.start()

    scale = DH ** -0.5
    kk = lax.broadcasted_iota(jnp.int32, (M + SEG, 80), 0)
    cc = lax.broadcasted_iota(jnp.int32, (M + SEG, 80), 1)
    second = ((cc >= 8) & (cc < 16)) | (cc >= 48)
    allowed = (cc < 16) | (kk <= jnp.where(second, cc - 40, cc - 8))

    def over_keys(f, fr, v):
        t = v[0:8]
        for j in range(8, M + SEG, 8):
            t = f(t, v[j:j + 8])
        return fr(t, axis=0, keepdims=True)

    def tied(u, never, toks):
        if not toks:
            return u
        parts, at = [], 0
        for j, tk in enumerate(toks):
            r = 64 * j
            if r > at:
                parts.append(u[at:r])
            parts.append(jnp.where(never, tk, u[r:r + 8]))
            at = r + 8
        return jnp.concatenate(parts + [u[at:]], axis=0)

    def w_slab(t, g, lo=0, n=512, never=None, toks=()):
        return pltpu.bitcast(
            tied(wqkv_v[pl.ds((8 * t + g) * PITCH + lo, n), :], never, toks), BF)

    def step(s, u, mem, left, att_prev):
        odd = left is not None
        wr = 3 * lax.rem(s >> 2, NRING // 3)
        rd = lax.rem(s + NRING - BULK // SEG, NRING)

        def ring_put(g, t, y):
            if odd:
                u32 = pltpu.bitcast(y.astype(BF), U32)
                parts = [(3 * u, u32[4:8]), (3 * u + 1, u32[8:16])]
            else:
                u32 = pltpu.bitcast(y[M:].astype(BF), U32)
                parts = [(3 * u, u32[0:8]), (3 * u + 2, u32[8:12])]
            for grp, v in parts:
                ring[g][t // 2, wr + grp // 4,
                        pl.ds(16 * (t % 2) + 4 * (grp % 4), v.shape[0]), :] = v

        xin = jnp.concatenate(
            [mem, ho_v[0, pl.ds(pl.multiple_of(BULK + RIDE * s, 8), RIDE), :]], axis=0)

        prow = SEG * (s - 1) if odd else jnp.maximum(SEG * s - 40, 0)
        nrow = BULK + RIDE * jnp.minimum(s + 1, NSEG - 1)
        works = [post_work(pl.multiple_of(prow + 8 * q, 8), functools.partial(att_prev, q))
                 for q in range(3 if odd else 5)]
        works += [ln1_work(pl.multiple_of(nrow + 8 * q, 8)) for q in range(RIDE // 8)]
        never = jnp.full((8, 128), s, jnp.int32) < 0
        gap = (SIDE_END - SIDE0 - SIDE_LAT - SIDE_DUE) // len(works)
        sched = {}
        for q, wk in enumerate(works):
            sched.setdefault(SIDE0 + gap * q, []).append(wk[0])
            for c in range(1, len(wk)):
                sched.setdefault(SIDE0 + SIDE_LAT + gap * q + ((c - 1) * gap) // 4,
                                 []).append(wk[c])

        memqkv, probs, wl, new_left, toks = {}, {}, {}, {}, {}
        acc = []
        chain = []

        ndot = [0]

        def proj(g, t_lo, t_hi):
            part = {}
            if u > 0 and ndot[0] == 0:
                for t in range(t_lo, t_lo + 6):
                    part[t] = jnp.dot(xin[:, :512], w_slab(t, g, 0, 256),
                                      preferred_element_type=F32)
            for t0 in range(t_lo, t_hi, 2):
                ys = []
                for t in (t0, t0 + 1):
                    n = ndot[0]
                    ndot[0] += 1
                    if t in part:
                        y = jnp.dot(xin[:, 512:], w_slab(t, g, 256, 256),
                                    preferred_element_type=F32) + part[t]
                    else:
                        y = jnp.dot(xin, w_slab(t, g, 0, 512, never, toks.get(n)),
                                    preferred_element_type=F32)
                    ring_put(g, t, y)
                    ys.append(y[:M])
                    for item in sched.get(n, ()):
                        tk = item((never, y[:M]))
                        if tk is not None:
                            toks.setdefault(n + SIDE_DUE, []).append(tk)
                memqkv[(t0, g)] = jnp.concatenate(ys, axis=0).astype(BF)

        def cat(t0, g):
            return jnp.concatenate(
                [memqkv[(t0, g)], pltpu.bitcast(ring[g][t0 // 2, rd], BF)], axis=0)

        def scores(g):
            for p in (0, 2):
                if len(chain) < 4:
                    qt = pltpu.bitcast(cat(p, g).T, U32)
                    qt = jnp.concatenate(
                        [jnp.where(never[:, :80], qt[8:16], qt[0:8]), qt[8:]], axis=0)
                    st = jnp.dot(cat(4 + p, g), pltpu.bitcast(qt, BF),
                                 preferred_element_type=F32)
                else:
                    st = lax.dot_general(cat(4 + p, g), cat(p, g), (((1,), (1,)), ((), ())),
                                         preferred_element_type=F32)
                st = jnp.where(second, jnp.concatenate([st[8:16], st[48:80]], axis=0),
                               jnp.concatenate([st[0:8], st[16:48]], axis=0))
                if chain:
                    st = jnp.concatenate(
                        [jnp.where(never[:, :80], chain[-1], st[0:8]), st[8:]], axis=0)
                st = jnp.where(allowed, st * scale, -1e9)
                e = jnp.exp(st - over_keys(jnp.maximum, jnp.max, st))
                l = over_keys(jnp.add, jnp.sum, e)
                chain.append(jnp.broadcast_to(l, (8, 80)))
                rc = pl.reciprocal(l, approx=True)
                e = e * (rc * (2.0 - l * rc))
                e0 = jnp.where(second, 0.0, e)
                e1 = jnp.where(second, e, 0.0)
                probs[(p, g)] = jnp.concatenate(
                    [e0[:M], e1[:M], e0[M:], e1[M:]], axis=0).astype(BF)

        def pv(g):
            for p in (0, 2):
                o = lax.dot_general(probs[(p, g)], cat(8 + p, g), (((0,), (0,)), ((), ())),
                                    preferred_element_type=F32)
                for j in range(2):
                    om, ot = o[8 * j:8 * j + 8], o[16 + 32 * j:48 + 32 * j]
                    if odd:
                        rows = [om, left[(p + j, g)], ot]
                    else:
                        rows = [om, ot[:RIDE]]
                        new_left[(p + j, g)] = ot[RIDE:]
                    wl[(p + j, g)] = jnp.concatenate(rows, axis=0).astype(BF)

        def wo(g):
            a = jnp.concatenate([wl[(o, g)] for o in range(4)], axis=1)
            w = jnp.concatenate(
                [jnp.concatenate([wo_v[n, pl.ds((8 * o + PERM[g]) * DH, DH), :]
                                  for o in range(4)], axis=0) for n in range(2)], axis=1)
            y = jnp.dot(a, w, preferred_element_type=F32)
            acc[:] = [y if not acc else y + acc[0]]

        for op in ORDER.split():
            g = int(op[1])
            if op[0] in "qkv":
                proj(g, *{"q": (0, 12), "k": (0, 8), "v": (8, 12)}[op[0]])
            else:
                {"s": scores, "p": pv, "w": wo}[op[0]](g)
        y = acc[0].astype(BF)
        return y[:M], y[M:], (None if odd else new_left)

    def out_copy(row0, n, k):
        return pltpu.make_async_copy(ho_v.at[1, pl.ds(row0, n), :],
                                     out_hbm.at[0, pl.ds(row0, n), :], sems.at[3 + k])

    OB = SEG * UNROLL

    def carried(q):
        return att_v[pl.ds(8 * q, 8), :]

    sub1 = lax.broadcasted_iota(jnp.int32, (16, 128), 0)
    lan1 = lax.broadcasted_iota(jnp.int32, (16, 128), 1)
    idx = (sub1 // 8) * 1024 + lan1 * 8 + sub1 % 8

    def guess_blocks():
        r = pltpu.bitcast(_rb(r_v[pl.ds(0, 2)].reshape(16, 128)), jnp.int32)
        key = pltpu.bitcast(r | (S - 1 - idx), F32)
        for k in range(2):
            m = jnp.max(jnp.max(key, axis=0, keepdims=True), axis=1, keepdims=True)
            r_v[2 + k] = jnp.broadcast_to(m, (8, 128))
            key = jnp.where(key >= m, -jnp.inf, key)

    def steps(i, carry):
        @pl.when(i == 16 // UNROLL)
        def _():
            x2_copy.wait()

        mem, left, att_prev = mem_v[...], None, carried
        for u in range(UNROLL):
            mem, att, left = step(i * UNROLL + u, u, mem, left, att_prev)
            att_prev = (lambda a: lambda q: a[8 * q:8 * q + 8])(att)
        mem_v[...] = mem
        att_v[...] = att
        guess_blocks()

        @pl.when(i >= 1)
        def _():
            out_copy(pl.multiple_of((i - 1) * OB, OB), OB, 0).start()
        return carry
    lax.fori_loop(0, NSEG // UNROLL, steps, 0)

    for cp in ffn_copies:
        cp.wait()

    def two(ref, a, b):
        return jnp.concatenate([ref[pl.ds(a, 8), :], ref[pl.ds(b, 8), :]], axis=0)

    def ffn_act(h, c):
        g = _rb(jnp.dot(h, wg_v[:, pl.ds(512 * c, 512)], preferred_element_type=F32))
        u = _rb(jnp.dot(h, wu_v[:, pl.ds(512 * c, 512)], preferred_element_type=F32))
        return (_rb(g * jax.nn.sigmoid(g)) * u).astype(BF)

    def ffn_down(a, c):
        wd = jnp.concatenate([wd_v[k, pl.ds(512 * c, 512), :] for k in range(2)], axis=1)
        return jnp.dot(a, wd, preferred_element_type=F32)

    early = _rb(r_v[pl.ds(0, 2)].reshape(16, 128))


    def guessed(k):
        j = S - 1 - (pltpu.bitcast(r_v[2 + k], jnp.int32) & (S - 1))
        return pl.multiple_of(jnp.minimum(j[0, 0] >> 3, (S - 48) // 8) * 8, 8)
    gs_a, gs_b = guessed(0), guessed(1)
    h_gs = two(ho_v.at[0], gs_a, gs_b)
    acts = [ffn_act(h_gs, c) for c in range(NSPEC)]

    last = []
    for q in range(5):
        for item in post_work(S - 40 + 8 * q, functools.partial(carried, q), last):
            item(None)
    out_copy(S - OB, OB, 0).start()

    def top2(val, idx, valid):
        def reduce(f, v):
            v = f(v, axis=0, keepdims=True)
            return v if v.shape[1] == 1 else f(v, axis=1, keepdims=True)

        def argtop(ok):
            v = jnp.where(ok, val, -jnp.inf)
            m = reduce(jnp.max, v)
            return m, reduce(jnp.min, jnp.where(ok & (v >= m), idx, float(S)))
        m1, i1 = argtop(valid)
        return (m1, i1), argtop(valid & (idx != i1))

    c_a, c_b = top2(early, idx.astype(F32), idx < S - 40)
    sub2 = lax.broadcasted_iota(jnp.int32, (48, 1), 0)
    val2 = jnp.concatenate([_rb(r) for r in last] + [jnp.where(sub2[:8] == 0, c_a[0], c_b[0])],
                           axis=0)
    idx2 = jnp.where(sub2 < 40, (sub2 + (S - 40)).astype(F32),
                     jnp.where(sub2 == 40, c_a[1], c_b[1]))
    (m_a, i_a), (m_b, i_b) = top2(val2, idx2, sub2 < 42)
    i_a = i_a.astype(jnp.int32)
    i_b = i_b.astype(jnp.int32)
    ia = jnp.clip(i_a[0, 0], 0, S - 1)
    ib = jnp.clip(i_b[0, 0], 0, S - 1)
    blk_a = pl.multiple_of((ia // 8) * 8, 8)
    blk_b = pl.multiple_of((ib // 8) * 8, 8)

    hs = two(ho_v.at[0], blk_a, blk_b)
    y0 = y = None
    for c in range(1, FF // 512 + 1):
        if NSPEC <= c < FF // 512:
            acts.append(ffn_act(hs, c))
        t = ffn_down(acts[c - 1], c - 1)
        if c <= NSPEC:
            y0 = t if y0 is None else t + y0
        else:
            y = t if y is None else t + y
    sub = lax.broadcasted_iota(jnp.int32, (16, 1), 0)
    rows = jnp.where(sub < 8, blk_a + sub, blk_b + sub - 8)
    gate = jnp.where(rows == ia, jax.nn.sigmoid(m_a),
                     jnp.where(rows == ib, jax.nn.sigmoid(m_b), 0.0))

    def finish(ffn):
        upd = jnp.where((rows == ia) | (rows == ib), ffn * gate, 0.0).reshape(2, 8, D)
        fin_v[...] = _b2(_f3(two(ho_v.at[1], blk_a, blk_b)) + mod_v[5] * upd)

    finish(y + y0)

    @pl.when((gs_a != blk_a) | (gs_b != blk_b))
    def _():
        redo = [ffn_act(hs, c) for c in range(NSPEC)]
        finish(functools.reduce(lambda a, c: ffn_down(redo[c], c) + a, range(NSPEC), y))

    def patch(k, blk):
        return pltpu.make_async_copy(fin_v.at[pl.ds(8 * k, 8), :],
                                     out_hbm.at[0, pl.ds(blk, 8), :], sems.at[3 + k])

    out_copy(0, S, 0).wait()
    patch(0, blk_a).start()

    @pl.when(blk_a != blk_b)
    def _():
        patch(1, blk_b).start()
        patch(1, blk_b).wait()
    patch(0, blk_a).wait()


@jax.jit
def pallas_adaLN_cond__memory_aug_recurrent_mem_tr__moe_arch_mod__prompt_kernel(
    A_x, A_mem0, A_Wq, A_Wk, A_Wv, A_Wo, A_seg_len, B_x, B_w_r, B_w_gate, B_w_up, B_w_down, c,
    w_mod,
):
    del B_x
    del A_seg_len
    assert A_x.shape == (1, S, D) and A_Wq.shape == (D, H, DH) and A_mem0.shape == (1, M, D)
    any_spec = pl.BlockSpec(memory_space=pl.ANY)
    scratch = [
        pltpu.VMEM((S, D), BF),
        pltpu.VMEM((4, X0, QK), BF),
        pltpu.VMEM((4, BULK // 2, QK), U32),
        pltpu.VMEM((40, D), BF),
        pltpu.VMEM((2, S, D), BF),
        pltpu.VMEM((100 * PITCH, 128), U32),
        pltpu.VMEM((2, H * DH, 512), BF),
        pltpu.VMEM((5 * D, 8, 128), BF),
        pltpu.VMEM((12, D, 512), BF),
        pltpu.VMEM((D, FF), BF),
        pltpu.VMEM((D, FF), BF),
        pltpu.VMEM((2, FF, 512), BF),
        pltpu.VMEM((M, D), BF),
        pltpu.VMEM((4, 1, D), BF),
        pltpu.VMEM((7, 8, D), F32),
        pltpu.VMEM((4, 8, 128), F32),
        pltpu.VMEM((D, 128), F32),
        pltpu.VMEM((12, 8, 512), F32),
        pltpu.VMEM((NP, 4, BULK, 256), F32),
        pltpu.VMEM((16, D), BF),
        pltpu.SemaphoreType.DMA((9,)),
    ] + [pltpu.VMEM((6, NRING, 32, 128), U32)] * 8
    return pl.pallas_call(
        _kernel,
        out_shape=jax.ShapeDtypeStruct((1, S, D), BF),
        in_specs=[any_spec] * 12,
        out_specs=any_spec,
        scratch_shapes=scratch,
        compiler_params=pltpu.CompilerParams(vmem_limit_bytes=120 * 1024 * 1024),
    )(A_x, A_mem0, A_Wq, A_Wk, A_Wv, A_Wo.reshape(H * DH, D), B_w_r.reshape(1, D), B_w_gate,
      B_w_up, B_w_down, c, w_mod)
```

```python
import functools

import jax
import jax.numpy as jnp
from jax import lax
import jax.experimental.pallas as pl
import jax.experimental.pallas.tpu as pltpu

BF = jnp.bfloat16
F32 = jnp.float32
U32 = jnp.uint32

S = 2048
D = 1024
H = 32
DH = 128
M = 8
SEG = 32
NSEG = S // SEG
FF = 3584
RIDE = 24
BULK = S - RIDE * NSEG
X0 = BULK + 32
NRING = 18
PITCH = 520
X1 = 1024
NP = 3
QK = D // 4
UNROLL = 4
NSPEC = 2
EPS = 1e-5
SIDE0, SIDE_LAT, SIDE_DUE, SIDE_END = 0, 6, 6, 78
NEG = -3.0e38
ORDER = ("q0 q1 q2 q3 k4 k5 k6 k7 s0 s1 s2 s3 s4 s5 s6 s7 v4 v5 v6 v7 p0 p1 p2 p3 p4 p5 p6 p7 "
         "w0 w1 w2 w3 w4 w5 w6 w7")
PERM = (0, 2, 4, 6, 1, 3, 5, 7)


def _rb(v):
    return v.astype(BF).astype(F32)


def _layernorm(xf):
    mu = jnp.mean(xf, axis=-1, keepdims=True)
    dv = xf - mu
    var = jnp.mean(dv * dv, axis=-1, keepdims=True)
    sd = _rb(jnp.sqrt(_rb(_rb(var) + EPS)))
    return _rb(_rb(xf - _rb(mu)) * (1.0 / sd))


def _f3(v):
    return v.astype(F32).reshape(v.shape[0] // 8, 8, D)


def _b2(v):
    return v.reshape(v.shape[0] * 8, D).astype(BF)


def _kernel(x_hbm, mem0_hbm, wq_hbm, wk_hbm, wv_hbm, wo_hbm, wr_hbm, wg_hbm, wu_hbm, wd_hbm,
            c_hbm, wmod_hbm, out_hbm,
            x_v, h_v, hp_v, att_v, ho_v, wqkv_v, wo_v, stage, wmod_v,
            wg_v, wu_v, wd_v, mem_v, cw_v, mod_v, r_v, sb_v, macc_v,
            part_v, fin_v, sems, *rings):
    w_hbm = (wq_hbm, wk_hbm, wv_hbm)
    ring = rings

    def piece_copy(t, sem, lo=0, n=D, dst=None):
        dst = (t % 2) * D + lo if dst is None else dst
        return pltpu.make_async_copy(
            w_hbm[t // 4].at[pl.ds(lo, n), pl.ds((t % 4) * 8, 8), :],
            stage.at[pl.ds(dst, n)], sems.at[sem])

    def unit_copy(j):
        sem = 1 if j == 1 else 6 + min(j, 10) % 3
        return piece_copy(j % NP, sem, QK * (j // NP), QK, 2 * D + QK * j)

    def stage_wait(row, n, sem):
        dst = stage.at[pl.ds(row, n)]
        pltpu.make_async_copy(dst, dst, sems.at[sem]).wait()

    def mq_copy(q, part):
        return pltpu.make_async_copy(wmod_hbm.at[:, pl.ds(part * D + q * QK, QK)],
                                     wmod_v.at[q, :, pl.ds(part * QK, QK)], sems.at[2])

    def wmod_copy(k, sem):
        col = k * 512 if isinstance(k, int) else pl.multiple_of(k * 512, 512)
        return pltpu.make_async_copy(wmod_hbm.at[:, pl.ds(col, 512)], wmod_v.at[k], sems.at[sem])

    def x_copy(lo, hi, sem):
        return pltpu.make_async_copy(x_hbm.at[0, pl.ds(lo, hi - lo), :],
                                     x_v.at[pl.ds(lo, hi - lo), :], sems.at[sem])

    def wo_copy(n):
        lo, rows = ((n // 2) * 512, 512) if n < 6 else (1536, 2560)
        return pltpu.make_async_copy(wo_hbm.at[pl.ds(lo, rows), pl.ds((n % 2) * 512, 512)],
                                     wo_v.at[n % 2, pl.ds(lo, rows)], sems.at[0])

    small_copies = [pltpu.make_async_copy(c_hbm, cw_v.at[0], sems.at[0]),
                    pltpu.make_async_copy(mem0_hbm.at[0], mem_v, sems.at[0]),
                    pltpu.make_async_copy(wr_hbm, cw_v.at[1], sems.at[0])]
    x0_copy = x_copy(0, X0, 1)
    mid_copies = ([x_copy(X0, (X0 + X1) // 2, 0), x_copy((X0 + X1) // 2, X1, 0)]
                  + [wo_copy(n) for n in range(8)])
    x2_copy = x_copy(X1, S, 1)
    ffn_copies = [pltpu.make_async_copy(wg_hbm, wg_v, sems.at[2]),
                  pltpu.make_async_copy(wu_hbm, wu_v, sems.at[2])] + [
        pltpu.make_async_copy(wd_hbm.at[:, pl.ds(k * 512, 512)], wd_v.at[k], sems.at[2])
        for k in range(2)]

    def relayout(src, base, n):
        u = pltpu.bitcast(stage[pl.ds(src, n)], U32)
        tok = None
        for i in range(n // 2):
            a = u[2 * i]
            b = u[2 * i + 1]
            even = (a & jnp.uint32(0xFFFF)) | (b << 16)
            odd = (a >> 16) | (b & jnp.uint32(0xFFFF0000))
            wqkv_v[pl.ds(base + i, 4, stride=PITCH), :] = even
            wqkv_v[pl.ds(base + 4 * PITCH + i, 4, stride=PITCH), :] = odd
            tok = even ^ odd if tok is None else tok ^ even ^ odd
        return jnp.concatenate([tok, tok], axis=0)

    CW = 256

    def ln_stats(xf):
        mu = jnp.mean(xf, axis=-1, keepdims=True)
        dv = xf - mu
        var = jnp.mean(dv * dv, axis=-1, keepdims=True)
        sd = _rb(jnp.sqrt(_rb(_rb(var) + EPS)))
        return _rb(mu), 1.0 / sd

    def mod_c(k, c):
        return mod_v[k, :, pl.ds(c * CW, CW)]

    def token(v):
        return pltpu.bitcast(v[:, :128] + v[:, 128:], U32)

    def after(v, trig):
        if trig is None:
            return v
        return jnp.concatenate([jnp.where(trig[0], trig[1], v[:, :128]), v[:, 128:]], axis=1)

    def post_work(row0, att, scores_out=None):
        st = {}

        def head(trig):
            a = after(att().astype(F32), trig)
            st["x2"] = _rb(x_v[pl.ds(row0, 8), :].astype(F32) + _rb(mod_v[2] * a))
            st["mu"], st["inv"] = ln_stats(st["x2"])

        def chunk(c, trig):
            xc = after(st["x2"][:, c * CW:(c + 1) * CW], trig)
            h2b = (_rb(_rb(_rb(xc - st["mu"]) * st["inv"]) * mod_c(4, c))
                   + mod_c(3, c)).astype(BF)
            h2 = h2b.astype(F32)
            ho_v[0, pl.ds(row0, 8), pl.ds(c * CW, CW)] = h2b
            o = xc + mod_c(5, c) * h2
            ho_v[1, pl.ds(row0, 8), pl.ds(c * CW, CW)] = o.astype(BF)
            rp = h2 * mod_c(6, c)
            st["r"] = rp if c == 0 else st["r"] + rp
            if c == D // CW - 1:
                r = jnp.sum(st["r"], axis=-1, keepdims=True)
                if scores_out is not None:
                    scores_out.append(r)
                else:
                    grp = row0 >> 3
                    lanes = lax.broadcasted_iota(jnp.int32, (8, 128), 1)
                    r_v[grp >> 7] = jnp.where(lanes == (grp & 127), r, r_v[grp >> 7])
            return token(o + st["r"])
        return [head] + [functools.partial(chunk, c) for c in range(D // CW)]

    def ln1_work(row0):
        st = {}

        def head(trig):
            st["x"] = after(x_v[pl.ds(row0, 8), :].astype(F32), trig)
            st["mu"], st["inv"] = ln_stats(st["x"])

        def chunk(c, trig):
            xc = after(st["x"][:, c * CW:(c + 1) * CW], trig)
            h = _rb(_rb(_rb(xc - st["mu"]) * st["inv"]) * mod_c(1, c)) + mod_c(0, c)
            ho_v[0, pl.ds(row0, 8), pl.ds(c * CW, CW)] = h.astype(BF)
            return token(h)
        return [head] + [functools.partial(chunk, c) for c in range(D // CW)]

    for cp in small_copies:
        cp.start()
    x0_copy.start()
    mq_copy(0, 0).start()

    r_v[...] = jnp.full(r_v.shape, NEG, F32)
    att_v[...] = jnp.zeros(att_v.shape, BF)

    for cp in small_copies:
        cp.wait()
    mod_v[6] = jnp.broadcast_to(cw_v[1].astype(F32), (8, D))
    cf = cw_v[0].astype(F32)
    sil = (cf * jax.nn.sigmoid(cf)).astype(BF)
    sc = jnp.broadcast_to(sil, (16, D))
    for k in range(8):
        sb_v[pl.ds(128 * k, 128), :] = jnp.broadcast_to(
            sil[:, 128 * k:128 * k + 128].astype(F32), (128, 128)).T

    mq_copy(0, 1).start()
    x0_copy.wait()

    LNB = X0 // 4

    def ln0(i, carry):
        r0 = pl.multiple_of(i * LNB, 8)
        ln = _b2(_layernorm(_f3(x_v[pl.ds(r0, LNB), :])))
        for q in range(4):
            h_v[q, pl.ds(r0, LNB), :] = ln[:, q * QK:(q + 1) * QK]

        @pl.when(i == 1)
        def _():
            unit_copy(0).start()
        return carry
    lax.fori_loop(0, 4, ln0, 0)

    def shift_scale(acc):
        y = _rb(acc)
        return y[:, :QK], _rb(1.0 + y[:, QK:])

    def modulated(q, r0, n, sh, sca):
        ln = h_v[q, pl.ds(r0, n), :].astype(F32).reshape(n // 8, 8, QK)
        return (_rb(ln * sca) + sh).reshape(n, QK).astype(BF)

    unit_copy(1).start()
    for part in range(2):
        mq_copy(0, part).wait()
    acc0 = jnp.dot(sc, wmod_v[0], preferred_element_type=F32)[0:8]
    macc_v[0] = acc0
    hp_v[0] = pltpu.bitcast(modulated(0, 0, BULK, *shift_scale(acc0)), U32)
    unit_copy(2).start()

    def first_unit(j):
        def relayout0(i, carry):
            relayout(2 * D + QK * j + pl.multiple_of(i * 128, 128), j * 8 * PITCH + i * 64, 128)
            return carry
        unit_copy(j).wait()
        lax.fori_loop(0, QK // 128, relayout0, 0)

    first_unit(0)
    mq_copy(1, 0).start()
    mq_copy(1, 1).start()
    unit_copy(3).start()

    def mod_rows(slab, r0, n, acc):
        for r in range(r0, r0 + n, 8):
            sv = sb_v[pl.ds(r, 8), :]
            t = wmod_v[slab, pl.ds(r, 8), :].astype(F32) * jnp.concatenate([sv] * 4, axis=1)
            acc = t if acc is None else acc + t
        return acc

    def ring_fill(g, t, y):
        ring[g][t >> 1, pl.ds(NRING - BULK // SEG, BULK // SEG),
                pl.ds(pl.multiple_of(16 * (t & 1), 16), 16), :] = (
            pltpu.bitcast(y.astype(BF), U32).reshape(BULK // SEG, 16, 128))

    def tie_lhs(col, never, toks):
        return jnp.concatenate(
            [jnp.where(never, toks[j], col[8 * j:8 * j + 8]) if j in toks
             else col[8 * j:8 * j + 8] for j in range(32)], axis=0)

    def add_tok(toks, j, tk):
        toks[j] = tk if j not in toks else toks[j] ^ tk

    starts = {0: [unit_copy(4)], 1: [unit_copy(5), piece_copy(3, 5, 0, 256)],
              2: [unit_copy(6), mq_copy(2, 0), mq_copy(2, 1)],
              3: [unit_copy(7), piece_copy(3, 5, 256, 256)], 4: [unit_copy(8)],
              5: [unit_copy(9), mq_copy(3, 0), mq_copy(3, 1)],
              6: [unit_copy(10), unit_copy(11)], 7: [piece_copy(3, 3, 512, 512)],
              8: [piece_copy(4, 4)], 9: [], 10: [wmod_copy(4, 2)], 11: []}

    def quarter_block(b_lo, b_hi, b, carry):
        first, final = b_lo == 0, b_hi == 4 * NP
        q = b_lo // NP
        p = b - NP * q
        if final:
            src = jnp.where(p == 0, 2 * D + 10 * QK, D + 512 * (p - 1))
            sem = 7 - 2 * p
            stage_wait(pl.multiple_of(src, 512), 512, sem)
            b3 = 3 * 8 * PITCH + 256 * (p - 1)
            jobs = [(src, jnp.where(p == 0, 8 * PITCH + 384, b3)),
                    (src + QK, jnp.where(p == 0, 2 * 8 * PITCH + 384, b3 + 128))]
        else:
            src = 2 * D + QK * (b + 1)
            last = p == NP - 1
            dst = jnp.where(last, 128 * (q + 1), (p + 1) * (8 * PITCH) + 128 * q)

            def unit_wait():
                stage_wait(pl.multiple_of(src, QK), QK, jnp.where(last, 6, 7 + p))
            if first:
                pl.when(b == 1)(functools.partial(first_unit, 1))
                pl.when(b > 0)(unit_wait)
                jobs = [(jnp.where(b == 0, 2 * D, src), jnp.where(b == 0, 0, dst))]
            else:
                unit_wait()
                jobs = [(src, dst)]

            @pl.when(last)
            def _():
                for part in range(2):
                    mq_copy(q + 1, part).wait()
            slab = jnp.where(last, q + 1, q)
        never = jnp.full((8, 128), b, jnp.int32) < 0

        def weights(k):
            return pltpu.bitcast(jnp.concatenate(
                [wqkv_v[pl.ds(pl.multiple_of((8 * p + kk) * PITCH + 128 * q, 8), 128), :]
                 for kk in (k, k + 1)], axis=1), BF)

        groups = [(s_ + 16 * g, d_ + 8 * g) for s_, d_ in jobs for g in range(QK // 16)]
        per = len(groups) // 4
        acc = None
        w = weights(0)
        for n, k in enumerate(range(0, 8, 2)):
            w_next = weights(k + 2) if k < 6 else None
            toks = {}
            if final and n == 2:
                wu = pltpu.bitcast(w_next, U32)
                wu = wu[:, :128] ^ wu[:, 128:]
                add_tok(toks, 3, functools.reduce(
                    jnp.bitwise_xor, [wu[8 * j:8 * j + 8] for j in range(16)]))
            for g in range(per):
                add_tok(toks, 4 + (g * 24) // per, relayout(*groups[n * per + g], 16))
            if not final and n < 2:
                for g in range(16):
                    acc = mod_rows(slab, 512 * n + 32 * g, 32, acc)
                    add_tok(toks, 2 * g + (n == 0), token(acc[:, :256] + acc[:, 256:]))
            if not final and n == 2:
                tot = jnp.broadcast_to(jnp.sum(acc, axis=0, keepdims=True), (8, 512))
                macc_v[q + 1] = tot
                sh, sca = shift_scale(tot)
            if not final and n >= 2:
                for g in range(16):
                    r0 = 256 * (n - 2) + 16 * g
                    hb = pltpu.bitcast(modulated(q + 1, r0, 16, sh, sca), U32)
                    hp_v[q + 1, pl.ds(r0 // 2, 8), :] = hb
                    add_tok(toks, (8 + (g * 3) // 2) if n == 2 else 2 * g,
                            hb[:, :128] ^ hb[:, 128:])
            lhs = jnp.concatenate([tie_lhs(hp_v[q, :, pl.ds(0, 128)], never, toks),
                                   hp_v[q, :, pl.ds(128, 128)]], axis=1)
            y = jnp.dot(pltpu.bitcast(lhs, BF), w, preferred_element_type=F32)
            if not first:
                y = y + part_v[p, n]
            if final:
                for j in range(2):
                    ring_fill(k + j, p, y[:, 128 * j:128 * j + 128])
            else:
                part_v[p, n] = y
            w = w_next

        for j in range(b_lo, b_hi):
            if starts[j]:
                @pl.when(b == j)
                def _():
                    for cp in starts[j]:
                        cp.start()
        return carry

    for b_lo, b_hi in ((0, NP), (NP, 2 * NP), (2 * NP, 3 * NP), (3 * NP, 4 * NP)):
        quarters = functools.partial(quarter_block, b_lo, b_hi)
        lax.fori_loop(b_lo, b_hi, quarters, 0)

    def bulk_dot(i, k, never, t, md):
        w = pltpu.bitcast(wqkv_v[pl.ds(pl.multiple_of((8 * i + k) * PITCH, 8), 512), :], BF)
        cols = [hp_v[c // 2, :, pl.ds(128 * (c % 2), 128)] for c in range(8)]
        toks = {}
        for g in range(8):
            tk = relayout((t & 1) * D + 128 * k + 16 * g, t * (8 * PITCH) + 64 * k + 8 * g, 16)
            md[1] = mod_rows(md[0], 128 * k + 16 * g, 16, md[1])
            toks[10 + 6 * (g + g // 4)] = tk ^ token(md[1][:, :256] + md[1][:, 256:])
        cols[0] = tie_lhs(cols[0], never, toks)
        cols[4] = tie_lhs(cols[4], never, {j - 32: tk for j, tk in toks.items()})
        hb = pltpu.bitcast(jnp.concatenate(cols, axis=1), BF)
        y = jnp.dot(hb, w, preferred_element_type=F32)
        ring_fill(k, i, y)

    def bulk_qkv(i, carry):
        @pl.when(i < 11)
        def _():
            par = (i + 1) & 1
            stage_wait(pl.multiple_of(par * D, D), D, 4 + par)

        @pl.when(i > NP)
        def _():
            wmod_copy(i, 2 + (i & 1)).wait()

        for j in range(NP, 10):
            @pl.when(i == j)
            def _():
                piece_copy(j + 2, 4 + j % 2).start()

        t = jnp.minimum(i + 1, 11)
        never = jnp.full((8, 128), i, jnp.int32) < 0
        md = [i, None]
        for k in range(8):
            bulk_dot(i, k, never, t, md)
        macc_v[jnp.maximum(i, 4)] = md[1]

        for j in range(NP, 10):
            @pl.when(i == j)
            def _():
                wmod_copy(j + 2, 2 + j % 2).start()
                if j < 9:
                    mid_copies[j - NP + 1].start()
                else:
                    for cp in mid_copies[7:]:
                        cp.start()
        return carry
    mid_copies[0].start()
    lax.fori_loop(NP, 12, bulk_qkv, 0)

    for q in range(4):
        sh, sca = shift_scale(macc_v[q])
        mod_v[0, :, pl.ds(q * QK, QK)] = sh
        mod_v[1, :, pl.ds(q * QK, QK)] = sca
        ho_v[0, pl.ds(BULK, RIDE), pl.ds(q * QK, QK)] = modulated(q, BULK, RIDE, sh, sca)
    for k in range(4, 12):
        y = _rb(jnp.sum(macc_v[k], axis=0, keepdims=True))
        if k // 2 == 4:
            y = _rb(1.0 + y)
        mod_v[k // 2, :, pl.ds((k % 2) * 512, 512)] = jnp.broadcast_to(y, (8, 512))
    for cp in mid_copies:
        cp.wait()
    x2_copy.start()
    for cp in ffn_copies:
        cp.start()

    scale = DH ** -0.5
    kk = lax.broadcasted_iota(jnp.int32, (M + SEG, 80), 0)
    cc = lax.broadcasted_iota(jnp.int32, (M + SEG, 80), 1)
    second = ((cc >= 8) & (cc < 16)) | (cc >= 48)
    allowed = (cc < 16) | (kk <= jnp.where(second, cc - 40, cc - 8))

    def over_keys(f, fr, v):
        t = v[0:8]
        for j in range(8, M + SEG, 8):
            t = f(t, v[j:j + 8])
        return fr(t, axis=0, keepdims=True)

    def tied(u, never, toks):
        if not toks:
            return u
        parts, at = [], 0
        for j, tk in enumerate(toks):
            r = 64 * j
            if r > at:
                parts.append(u[at:r])
            parts.append(jnp.where(never, tk, u[r:r + 8]))
            at = r + 8
        return jnp.concatenate(parts + [u[at:]], axis=0)

    def w_slab(t, g, lo=0, n=512, never=None, toks=()):
        return pltpu.bitcast(
            tied(wqkv_v[pl.ds((8 * t + g) * PITCH + lo, n), :], never, toks), BF)

    def step(s, u, mem, left, att_prev):
        odd = left is not None
        wr = 3 * lax.rem(s >> 2, NRING // 3)
        rd = lax.rem(s + NRING - BULK // SEG, NRING)

        def ring_put(g, t, y):
            if odd:
                u32 = pltpu.bitcast(y.astype(BF), U32)
                parts = [(3 * u, u32[4:8]), (3 * u + 1, u32[8:16])]
            else:
                u32 = pltpu.bitcast(y[M:].astype(BF), U32)
                parts = [(3 * u, u32[0:8]), (3 * u + 2, u32[8:12])]
            for grp, v in parts:
                ring[g][t // 2, wr + grp // 4,
                        pl.ds(16 * (t % 2) + 4 * (grp % 4), v.shape[0]), :] = v

        xin = jnp.concatenate(
            [mem, ho_v[0, pl.ds(pl.multiple_of(BULK + RIDE * s, 8), RIDE), :]], axis=0)

        prow = SEG * (s - 1) if odd else jnp.maximum(SEG * s - 40, 0)
        nrow = BULK + RIDE * jnp.minimum(s + 1, NSEG - 1)
        works = [post_work(pl.multiple_of(prow + 8 * q, 8), functools.partial(att_prev, q))
                 for q in range(3 if odd else 5)]
        works += [ln1_work(pl.multiple_of(nrow + 8 * q, 8)) for q in range(RIDE // 8)]
        never = jnp.full((8, 128), s, jnp.int32) < 0
        gap = (SIDE_END - SIDE0 - SIDE_LAT - SIDE_DUE) // len(works)
        sched = {}
        for q, wk in enumerate(works):
            sched.setdefault(SIDE0 + gap * q, []).append(wk[0])
            for c in range(1, len(wk)):
                sched.setdefault(SIDE0 + SIDE_LAT + gap * q + ((c - 1) * gap) // 4,
                                 []).append(wk[c])

        memqkv, probs, wl, new_left, toks = {}, {}, {}, {}, {}
        acc = []
        chain = []

        ndot = [0]

        def proj(g, t_lo, t_hi):
            part = {}
            if u > 0 and ndot[0] == 0:
                for t in range(t_lo, t_lo + 6):
                    part[t] = jnp.dot(xin[:, :512], w_slab(t, g, 0, 256),
                                      preferred_element_type=F32)
            for t0 in range(t_lo, t_hi, 2):
                ys = []
                for t in (t0, t0 + 1):
                    n = ndot[0]
                    ndot[0] += 1
                    if t in part:
                        y = jnp.dot(xin[:, 512:], w_slab(t, g, 256, 256),
                                    preferred_element_type=F32) + part[t]
                    else:
                        y = jnp.dot(xin, w_slab(t, g, 0, 512, never, toks.get(n)),
                                    preferred_element_type=F32)
                    ring_put(g, t, y)
                    ys.append(y[:M])
                    for item in sched.get(n, ()):
                        tk = item((never, y[:M]))
                        if tk is not None:
                            toks.setdefault(n + SIDE_DUE, []).append(tk)
                memqkv[(t0, g)] = jnp.concatenate(ys, axis=0).astype(BF)

        def cat(t0, g):
            return jnp.concatenate(
                [memqkv[(t0, g)], pltpu.bitcast(ring[g][t0 // 2, rd], BF)], axis=0)

        def scores(g):
            for p in (0, 2):
                if len(chain) < 4:
                    qt = pltpu.bitcast(cat(p, g).T, U32)
                    qt = jnp.concatenate(
                        [jnp.where(never[:, :80], qt[8:16], qt[0:8]), qt[8:]], axis=0)
                    st = jnp.dot(cat(4 + p, g), pltpu.bitcast(qt, BF),
                                 preferred_element_type=F32)
                else:
                    st = lax.dot_general(cat(4 + p, g), cat(p, g), (((1,), (1,)), ((), ())),
                                         preferred_element_type=F32)
                st = jnp.where(second, jnp.concatenate([st[8:16], st[48:80]], axis=0),
                               jnp.concatenate([st[0:8], st[16:48]], axis=0))
                if chain:
                    st = jnp.concatenate(
                        [jnp.where(never[:, :80], chain[-1], st[0:8]), st[8:]], axis=0)
                st = jnp.where(allowed, st * scale, -1e9)
                e = jnp.exp(st - over_keys(jnp.maximum, jnp.max, st))
                l = over_keys(jnp.add, jnp.sum, e)
                chain.append(jnp.broadcast_to(l, (8, 80)))
                rc = pl.reciprocal(l, approx=True)
                e = e * (rc * (2.0 - l * rc))
                e0 = jnp.where(second, 0.0, e)
                e1 = jnp.where(second, e, 0.0)
                probs[(p, g)] = jnp.concatenate(
                    [e0[:M], e1[:M], e0[M:], e1[M:]], axis=0).astype(BF)

        def pv(g):
            for p in (0, 2):
                o = lax.dot_general(probs[(p, g)], cat(8 + p, g), (((0,), (0,)), ((), ())),
                                    preferred_element_type=F32)
                for j in range(2):
                    om, ot = o[8 * j:8 * j + 8], o[16 + 32 * j:48 + 32 * j]
                    if odd:
                        rows = [om, left[(p + j, g)], ot]
                    else:
                        rows = [om, ot[:RIDE]]
                        new_left[(p + j, g)] = ot[RIDE:]
                    wl[(p + j, g)] = jnp.concatenate(rows, axis=0).astype(BF)

        def wo(g):
            a = jnp.concatenate([wl[(o, g)] for o in range(4)], axis=1)
            w = jnp.concatenate(
                [jnp.concatenate([wo_v[n, pl.ds((8 * o + PERM[g]) * DH, DH), :]
                                  for o in range(4)], axis=0) for n in range(2)], axis=1)
            y = jnp.dot(a, w, preferred_element_type=F32)
            acc[:] = [y if not acc else y + acc[0]]

        for op in ORDER.split():
            g = int(op[1])
            if op[0] in "qkv":
                proj(g, *{"q": (0, 12), "k": (0, 8), "v": (8, 12)}[op[0]])
            else:
                {"s": scores, "p": pv, "w": wo}[op[0]](g)
        y = acc[0].astype(BF)
        return y[:M], y[M:], (None if odd else new_left)

    def out_copy(row0, n, k):
        return pltpu.make_async_copy(ho_v.at[1, pl.ds(row0, n), :],
                                     out_hbm.at[0, pl.ds(row0, n), :], sems.at[3 + k])

    OB = SEG * UNROLL

    def carried(q):
        return att_v[pl.ds(8 * q, 8), :]

    sub1 = lax.broadcasted_iota(jnp.int32, (16, 128), 0)
    lan1 = lax.broadcasted_iota(jnp.int32, (16, 128), 1)
    idx = (sub1 // 8) * 1024 + lan1 * 8 + sub1 % 8

    def guess_blocks():
        r = pltpu.bitcast(_rb(r_v[pl.ds(0, 2)].reshape(16, 128)), jnp.int32)
        key = pltpu.bitcast(r | (S - 1 - idx), F32)
        for k in range(2):
            m = jnp.max(jnp.max(key, axis=0, keepdims=True), axis=1, keepdims=True)
            r_v[2 + k] = jnp.broadcast_to(m, (8, 128))
            key = jnp.where(key >= m, -jnp.inf, key)

    def steps(i, carry):
        @pl.when(i == 16 // UNROLL)
        def _():
            x2_copy.wait()

        mem, left, att_prev = mem_v[...], None, carried
        for u in range(UNROLL):
            mem, att, left = step(i * UNROLL + u, u, mem, left, att_prev)
            att_prev = (lambda a: lambda q: a[8 * q:8 * q + 8])(att)
        mem_v[...] = mem
        att_v[...] = att
        guess_blocks()

        @pl.when(i >= 1)
        def _():
            out_copy(pl.multiple_of((i - 1) * OB, OB), OB, 0).start()
        return carry
    lax.fori_loop(0, NSEG // UNROLL, steps, 0)

    for cp in ffn_copies:
        cp.wait()

    def two(ref, a, b):
        return jnp.concatenate([ref[pl.ds(a, 8), :], ref[pl.ds(b, 8), :]], axis=0)

    def ffn_act(h, c):
        g = _rb(jnp.dot(h, wg_v[:, pl.ds(512 * c, 512)], preferred_element_type=F32))
        u = _rb(jnp.dot(h, wu_v[:, pl.ds(512 * c, 512)], preferred_element_type=F32))
        return (_rb(g * jax.nn.sigmoid(g)) * u).astype(BF)

    def ffn_down(a, c):
        wd = jnp.concatenate([wd_v[k, pl.ds(512 * c, 512), :] for k in range(2)], axis=1)
        return jnp.dot(a, wd, preferred_element_type=F32)

    early = _rb(r_v[pl.ds(0, 2)].reshape(16, 128))


    def guessed(k):
        j = S - 1 - (pltpu.bitcast(r_v[2 + k], jnp.int32) & (S - 1))
        return pl.multiple_of(jnp.minimum(j[0, 0] >> 3, (S - 48) // 8) * 8, 8)
    gs_a, gs_b = guessed(0), guessed(1)
    h_gs = two(ho_v.at[0], gs_a, gs_b)
    acts = [ffn_act(h_gs, c) for c in range(NSPEC)]

    last, done = [], []
    never = jnp.full((8, 128), gs_a, jnp.int32) < 0
    for q in range(5):
        items = post_work(S - 40 + 8 * q, functools.partial(carried, q), last)
        items[0](None)
        for item in items[1:]:
            done.append(item((never, pltpu.bitcast(done[-2], F32)) if len(done) >= 2 else None))
    out_copy(S - OB, OB, 0).start()

    def top2(val, idx, valid):
        def reduce(f, v):
            v = f(v, axis=0, keepdims=True)
            return v if v.shape[1] == 1 else f(v, axis=1, keepdims=True)

        def argtop(ok):
            v = jnp.where(ok, val, -jnp.inf)
            m = reduce(jnp.max, v)
            return m, reduce(jnp.min, jnp.where(ok & (v >= m), idx, float(S)))
        m1, i1 = argtop(valid)
        return (m1, i1), argtop(valid & (idx != i1))

    c_a, c_b = top2(early, idx.astype(F32), idx < S - 40)
    sub2 = lax.broadcasted_iota(jnp.int32, (48, 1), 0)
    val2 = jnp.concatenate([_rb(r) for r in last] + [jnp.where(sub2[:8] == 0, c_a[0], c_b[0])],
                           axis=0)
    idx2 = jnp.where(sub2 < 40, (sub2 + (S - 40)).astype(F32),
                     jnp.where(sub2 == 40, c_a[1], c_b[1]))
    (m_a, i_a), (m_b, i_b) = top2(val2, idx2, sub2 < 42)
    i_a = i_a.astype(jnp.int32)
    i_b = i_b.astype(jnp.int32)
    ia = jnp.clip(i_a[0, 0], 0, S - 1)
    ib = jnp.clip(i_b[0, 0], 0, S - 1)
    blk_a = pl.multiple_of((ia // 8) * 8, 8)
    blk_b = pl.multiple_of((ib // 8) * 8, 8)

    hs = two(ho_v.at[0], blk_a, blk_b)
    y0 = y = None
    for c in range(1, FF // 512 + 1):
        if NSPEC <= c < FF // 512:
            acts.append(ffn_act(hs, c))
        t = ffn_down(acts[c - 1], c - 1)
        if c <= NSPEC:
            y0 = t if y0 is None else t + y0
        else:
            y = t if y is None else t + y
    sub = lax.broadcasted_iota(jnp.int32, (16, 1), 0)
    rows = jnp.where(sub < 8, blk_a + sub, blk_b + sub - 8)
    gate = jnp.where(rows == ia, jax.nn.sigmoid(m_a),
                     jnp.where(rows == ib, jax.nn.sigmoid(m_b), 0.0))

    def finish(ffn):
        upd = jnp.where((rows == ia) | (rows == ib), ffn * gate, 0.0).reshape(2, 8, D)
        fin_v[...] = _b2(_f3(two(ho_v.at[1], blk_a, blk_b)) + mod_v[5] * upd)

    finish(y + y0)

    @pl.when((gs_a != blk_a) | (gs_b != blk_b))
    def _():
        redo = [ffn_act(hs, c) for c in range(NSPEC)]
        finish(functools.reduce(lambda a, c: ffn_down(redo[c], c) + a, range(NSPEC), y))

    def patch(k, blk):
        return pltpu.make_async_copy(fin_v.at[pl.ds(8 * k, 8), :],
                                     out_hbm.at[0, pl.ds(blk, 8), :], sems.at[3 + k])

    out_copy(0, S, 0).wait()
    patch(0, blk_a).start()

    @pl.when(blk_a != blk_b)
    def _():
        patch(1, blk_b).start()
        patch(1, blk_b).wait()
    patch(0, blk_a).wait()


@jax.jit
def pallas_adaLN_cond__memory_aug_recurrent_mem_tr__moe_arch_mod__prompt_kernel(
    A_x, A_mem0, A_Wq, A_Wk, A_Wv, A_Wo, A_seg_len, B_x, B_w_r, B_w_gate, B_w_up, B_w_down, c,
    w_mod,
):
    del B_x
    del A_seg_len
    assert A_x.shape == (1, S, D) and A_Wq.shape == (D, H, DH) and A_mem0.shape == (1, M, D)
    any_spec = pl.BlockSpec(memory_space=pl.ANY)
    scratch = [
        pltpu.VMEM((S, D), BF),
        pltpu.VMEM((4, X0, QK), BF),
        pltpu.VMEM((4, BULK // 2, QK), U32),
        pltpu.VMEM((40, D), BF),
        pltpu.VMEM((2, S, D), BF),
        pltpu.VMEM((100 * PITCH, 128), U32),
        pltpu.VMEM((2, H * DH, 512), BF),
        pltpu.VMEM((5 * D, 8, 128), BF),
        pltpu.VMEM((12, D, 512), BF),
        pltpu.VMEM((D, FF), BF),
        pltpu.VMEM((D, FF), BF),
        pltpu.VMEM((2, FF, 512), BF),
        pltpu.VMEM((M, D), BF),
        pltpu.VMEM((4, 1, D), BF),
        pltpu.VMEM((7, 8, D), F32),
        pltpu.VMEM((4, 8, 128), F32),
        pltpu.VMEM((D, 128), F32),
        pltpu.VMEM((12, 8, 512), F32),
        pltpu.VMEM((NP, 4, BULK, 256), F32),
        pltpu.VMEM((16, D), BF),
        pltpu.SemaphoreType.DMA((9,)),
    ] + [pltpu.VMEM((6, NRING, 32, 128), U32)] * 8
    return pl.pallas_call(
        _kernel,
        out_shape=jax.ShapeDtypeStruct((1, S, D), BF),
        in_specs=[any_spec] * 12,
        out_specs=any_spec,
        scratch_shapes=scratch,
        compiler_params=pltpu.CompilerParams(vmem_limit_bytes=120 * 1024 * 1024),
    )(A_x, A_mem0, A_Wq, A_Wk, A_Wv, A_Wo.reshape(H * DH, D), B_w_r.reshape(1, D), B_w_gate,
      B_w_up, B_w_down, c, w_mod)
```

```python
import functools

import jax
import jax.numpy as jnp
from jax import lax
import jax.experimental.pallas as pl
import jax.experimental.pallas.tpu as pltpu

BF = jnp.bfloat16
F32 = jnp.float32
U32 = jnp.uint32

S = 2048
D = 1024
H = 32
DH = 128
M = 8
SEG = 32
NSEG = S // SEG
FF = 3584
RIDE = 24
BULK = S - RIDE * NSEG
X0 = BULK + 32
NRING = 18
PITCH = 520
X1 = 1024
NP = 3
QK = D // 4
UNROLL = 4
NSPEC = 2
EPS = 1e-5
SIDE0, SIDE_LAT, SIDE_DUE, SIDE_END = 0, 6, 6, 78
NEG = -3.0e38
ORDER = ("q0 q1 q2 q3 k4 k5 k6 k7 s0 s1 s2 s3 s4 s5 s6 s7 v4 v5 v6 v7 p0 p1 p2 p3 p4 p5 p6 p7 "
         "w0 w1 w2 w3 w4 w5 w6 w7")
PERM = (0, 2, 4, 6, 1, 3, 5, 7)


def _rb(v):
    return v.astype(BF).astype(F32)


def _layernorm(xf):
    mu = jnp.mean(xf, axis=-1, keepdims=True)
    dv = xf - mu
    var = jnp.mean(dv * dv, axis=-1, keepdims=True)
    sd = _rb(jnp.sqrt(_rb(_rb(var) + EPS)))
    return _rb(_rb(xf - _rb(mu)) * (1.0 / sd))


def _f3(v):
    return v.astype(F32).reshape(v.shape[0] // 8, 8, D)


def _b2(v):
    return v.reshape(v.shape[0] * 8, D).astype(BF)


def _kernel(x_hbm, mem0_hbm, wq_hbm, wk_hbm, wv_hbm, wo_hbm, wr_hbm, wg_hbm, wu_hbm, wd_hbm,
            c_hbm, wmod_hbm, out_hbm,
            x_v, h_v, hp_v, att_v, ho_v, wqkv_v, wo_v, stage, wmod_v,
            wg_v, wu_v, wd_v, mem_v, cw_v, mod_v, r_v, sb_v, macc_v,
            part_v, fin_v, sems, *rings):
    w_hbm = (wq_hbm, wk_hbm, wv_hbm)
    ring = rings

    def piece_copy(t, sem, lo=0, n=D, dst=None):
        dst = (t % 2) * D + lo if dst is None else dst
        return pltpu.make_async_copy(
            w_hbm[t // 4].at[pl.ds(lo, n), pl.ds((t % 4) * 8, 8), :],
            stage.at[pl.ds(dst, n)], sems.at[sem])

    def unit_copy(j):
        sem = 1 if j == 1 else 6 + min(j, 10) % 3
        return piece_copy(j % NP, sem, QK * (j // NP), QK, 2 * D + QK * j)

    def stage_wait(row, n, sem):
        dst = stage.at[pl.ds(row, n)]
        pltpu.make_async_copy(dst, dst, sems.at[sem]).wait()

    def mq_copy(q, part):
        return pltpu.make_async_copy(wmod_hbm.at[:, pl.ds(part * D + q * QK, QK)],
                                     wmod_v.at[q, :, pl.ds(part * QK, QK)], sems.at[2])

    def wmod_copy(k, sem):
        col = k * 512 if isinstance(k, int) else pl.multiple_of(k * 512, 512)
        return pltpu.make_async_copy(wmod_hbm.at[:, pl.ds(col, 512)], wmod_v.at[k], sems.at[sem])

    def x_copy(lo, hi, sem):
        return pltpu.make_async_copy(x_hbm.at[0, pl.ds(lo, hi - lo), :],
                                     x_v.at[pl.ds(lo, hi - lo), :], sems.at[sem])

    def wo_copy(n):
        lo, rows = ((n // 2) * 512, 512) if n < 6 else (1536, 2560)
        return pltpu.make_async_copy(wo_hbm.at[pl.ds(lo, rows), pl.ds((n % 2) * 512, 512)],
                                     wo_v.at[n % 2, pl.ds(lo, rows)], sems.at[0])

    small_copies = [pltpu.make_async_copy(c_hbm, cw_v.at[0], sems.at[0]),
                    pltpu.make_async_copy(mem0_hbm.at[0], mem_v, sems.at[0]),
                    pltpu.make_async_copy(wr_hbm, cw_v.at[1], sems.at[0])]
    x0_copy = x_copy(0, X0, 1)
    mid_copies = ([x_copy(X0, (X0 + X1) // 2, 0), x_copy((X0 + X1) // 2, X1, 0)]
                  + [wo_copy(n) for n in range(8)])
    x2_copy = x_copy(X1, S, 1)
    ffn_copies = [pltpu.make_async_copy(wg_hbm, wg_v, sems.at[2]),
                  pltpu.make_async_copy(wu_hbm, wu_v, sems.at[2])] + [
        pltpu.make_async_copy(wd_hbm.at[:, pl.ds(k * 512, 512)], wd_v.at[k], sems.at[2])
        for k in range(2)]

    def relayout(src, base, n):
        u = pltpu.bitcast(stage[pl.ds(src, n)], U32)
        tok = None
        for i in range(n // 2):
            a = u[2 * i]
            b = u[2 * i + 1]
            even = (a & jnp.uint32(0xFFFF)) | (b << 16)
            odd = (a >> 16) | (b & jnp.uint32(0xFFFF0000))
            wqkv_v[pl.ds(base + i, 4, stride=PITCH), :] = even
            wqkv_v[pl.ds(base + 4 * PITCH + i, 4, stride=PITCH), :] = odd
            tok = even ^ odd if tok is None else tok ^ even ^ odd
        return jnp.concatenate([tok, tok], axis=0)

    CW = 256

    def ln_stats(xf):
        mu = jnp.mean(xf, axis=-1, keepdims=True)
        dv = xf - mu
        var = jnp.mean(dv * dv, axis=-1, keepdims=True)
        sd = _rb(jnp.sqrt(_rb(_rb(var) + EPS)))
        return _rb(mu), 1.0 / sd

    def mod_c(k, c):
        return mod_v[k, :, pl.ds(c * CW, CW)]

    def token(v):
        return pltpu.bitcast(v[:, :128] + v[:, 128:], U32)

    def after(v, trig):
        if trig is None:
            return v
        return jnp.concatenate([jnp.where(trig[0], trig[1], v[:, :128]), v[:, 128:]], axis=1)

    def post_work(row0, att, scores_out):
        st = {}

        def head(trig):
            a = after(att().astype(F32), trig)
            st["x2"] = _rb(x_v[pl.ds(row0, 8), :].astype(F32) + _rb(mod_v[2] * a))
            st["mu"], st["inv"] = ln_stats(st["x2"])

        def chunk(c, trig):
            xc = after(st["x2"][:, c * CW:(c + 1) * CW], trig)
            h2b = (_rb(_rb(_rb(xc - st["mu"]) * st["inv"]) * mod_c(4, c))
                   + mod_c(3, c)).astype(BF)
            h2 = h2b.astype(F32)
            ho_v[0, pl.ds(row0, 8), pl.ds(c * CW, CW)] = h2b
            o = xc + mod_c(5, c) * h2
            ho_v[1, pl.ds(row0, 8), pl.ds(c * CW, CW)] = o.astype(BF)
            rp = h2 * mod_c(6, c)
            st["r"] = rp if c == 0 else st["r"] + rp
            if c == D // CW - 1:
                scores_out.append(jnp.sum(st["r"], axis=-1, keepdims=True))
            return token(o + st["r"])
        return [head] + [functools.partial(chunk, c) for c in range(D // CW)]

    def ln1_work(row0):
        st = {}

        def head(trig):
            st["x"] = after(x_v[pl.ds(row0, 8), :].astype(F32), trig)
            st["mu"], st["inv"] = ln_stats(st["x"])

        def chunk(c, trig):
            xc = after(st["x"][:, c * CW:(c + 1) * CW], trig)
            h = _rb(_rb(_rb(xc - st["mu"]) * st["inv"]) * mod_c(1, c)) + mod_c(0, c)
            ho_v[0, pl.ds(row0, 8), pl.ds(c * CW, CW)] = h.astype(BF)
            return token(h)
        return [head] + [functools.partial(chunk, c) for c in range(D // CW)]

    for cp in small_copies:
        cp.start()
    x0_copy.start()
    mq_copy(0, 0).start()

    r_v[...] = jnp.full(r_v.shape, NEG, F32)
    att_v[...] = jnp.zeros(att_v.shape, BF)

    for cp in small_copies:
        cp.wait()
    mod_v[6] = jnp.broadcast_to(cw_v[1].astype(F32), (8, D))
    cf = cw_v[0].astype(F32)
    sil = (cf * jax.nn.sigmoid(cf)).astype(BF)
    sc = jnp.broadcast_to(sil, (16, D))
    for k in range(8):
        sb_v[pl.ds(128 * k, 128), :] = jnp.broadcast_to(
            sil[:, 128 * k:128 * k + 128].astype(F32), (128, 128)).T

    mq_copy(0, 1).start()
    x0_copy.wait()

    LNB = X0 // 4

    def ln0(i, carry):
        r0 = pl.multiple_of(i * LNB, 8)
        ln = _b2(_layernorm(_f3(x_v[pl.ds(r0, LNB), :])))
        for q in range(4):
            h_v[q, pl.ds(r0, LNB), :] = ln[:, q * QK:(q + 1) * QK]

        @pl.when(i == 1)
        def _():
            unit_copy(0).start()
        return carry
    lax.fori_loop(0, 4, ln0, 0)

    def shift_scale(acc):
        y = _rb(acc)
        return y[:, :QK], _rb(1.0 + y[:, QK:])

    def modulated(q, r0, n, sh, sca):
        ln = h_v[q, pl.ds(r0, n), :].astype(F32).reshape(n // 8, 8, QK)
        return (_rb(ln * sca) + sh).reshape(n, QK).astype(BF)

    unit_copy(1).start()
    for part in range(2):
        mq_copy(0, part).wait()
    acc0 = jnp.dot(sc, wmod_v[0], preferred_element_type=F32)[0:8]
    macc_v[0] = acc0
    hp_v[0] = pltpu.bitcast(modulated(0, 0, BULK, *shift_scale(acc0)), U32)
    unit_copy(2).start()

    def first_unit(j):
        def relayout0(i, carry):
            relayout(2 * D + QK * j + pl.multiple_of(i * 128, 128), j * 8 * PITCH + i * 64, 128)
            return carry
        unit_copy(j).wait()
        lax.fori_loop(0, QK // 128, relayout0, 0)

    first_unit(0)
    mq_copy(1, 0).start()
    mq_copy(1, 1).start()
    unit_copy(3).start()

    def mod_rows(slab, r0, n, acc):
        for r in range(r0, r0 + n, 8):
            sv = sb_v[pl.ds(r, 8), :]
            t = wmod_v[slab, pl.ds(r, 8), :].astype(F32) * jnp.concatenate([sv] * 4, axis=1)
            acc = t if acc is None else acc + t
        return acc

    def ring_fill(g, t, y):
        ring[g][t >> 1, pl.ds(NRING - BULK // SEG, BULK // SEG),
                pl.ds(pl.multiple_of(16 * (t & 1), 16), 16), :] = (
            pltpu.bitcast(y.astype(BF), U32).reshape(BULK // SEG, 16, 128))

    def tie_lhs(col, never, toks):
        return jnp.concatenate(
            [jnp.where(never, toks[j], col[8 * j:8 * j + 8]) if j in toks
             else col[8 * j:8 * j + 8] for j in range(32)], axis=0)

    def add_tok(toks, j, tk):
        toks[j] = tk if j not in toks else toks[j] ^ tk

    starts = {0: [unit_copy(4)], 1: [unit_copy(5), piece_copy(3, 5, 0, 256)],
              2: [unit_copy(6), mq_copy(2, 0), mq_copy(2, 1)],
              3: [unit_copy(7), piece_copy(3, 5, 256, 256)], 4: [unit_copy(8)],
              5: [unit_copy(9), mq_copy(3, 0), mq_copy(3, 1)],
              6: [unit_copy(10), unit_copy(11)], 7: [piece_copy(3, 3, 512, 512)],
              8: [piece_copy(4, 4)], 9: [], 10: [wmod_copy(4, 2)], 11: []}

    def quarter_block(b_lo, b_hi, b, carry):
        first, final = b_lo == 0, b_hi == 4 * NP
        q = b_lo // NP
        p = b - NP * q
        if final:
            src = jnp.where(p == 0, 2 * D + 10 * QK, D + 512 * (p - 1))
            sem = 7 - 2 * p
            stage_wait(pl.multiple_of(src, 512), 512, sem)
            b3 = 3 * 8 * PITCH + 256 * (p - 1)
            jobs = [(src, jnp.where(p == 0, 8 * PITCH + 384, b3)),
                    (src + QK, jnp.where(p == 0, 2 * 8 * PITCH + 384, b3 + 128))]
        else:
            src = 2 * D + QK * (b + 1)
            last = p == NP - 1
            dst = jnp.where(last, 128 * (q + 1), (p + 1) * (8 * PITCH) + 128 * q)

            def unit_wait():
                stage_wait(pl.multiple_of(src, QK), QK, jnp.where(last, 6, 7 + p))
            if first:
                pl.when(b == 1)(functools.partial(first_unit, 1))
                pl.when(b > 0)(unit_wait)
                jobs = [(jnp.where(b == 0, 2 * D, src), jnp.where(b == 0, 0, dst))]
            else:
                unit_wait()
                jobs = [(src, dst)]

            @pl.when(last)
            def _():
                for part in range(2):
                    mq_copy(q + 1, part).wait()
            slab = jnp.where(last, q + 1, q)
        never = jnp.full((8, 128), b, jnp.int32) < 0

        def weights(k):
            return pltpu.bitcast(jnp.concatenate(
                [wqkv_v[pl.ds(pl.multiple_of((8 * p + kk) * PITCH + 128 * q, 8), 128), :]
                 for kk in (k, k + 1)], axis=1), BF)

        groups = [(s_ + 16 * g, d_ + 8 * g) for s_, d_ in jobs for g in range(QK // 16)]
        per = len(groups) // 4
        acc = None
        w = weights(0)
        for n, k in enumerate(range(0, 8, 2)):
            w_next = weights(k + 2) if k < 6 else None
            toks = {}
            if final and n == 2:
                wu = pltpu.bitcast(w_next, U32)
                wu = wu[:, :128] ^ wu[:, 128:]
                add_tok(toks, 3, functools.reduce(
                    jnp.bitwise_xor, [wu[8 * j:8 * j + 8] for j in range(16)]))
            for g in range(per):
                add_tok(toks, 4 + (g * 24) // per, relayout(*groups[n * per + g], 16))
            if not final and n < 2:
                for g in range(16):
                    acc = mod_rows(slab, 512 * n + 32 * g, 32, acc)
                    add_tok(toks, 2 * g + (n == 0), token(acc[:, :256] + acc[:, 256:]))
            if not final and n == 2:
                tot = jnp.broadcast_to(jnp.sum(acc, axis=0, keepdims=True), (8, 512))
                macc_v[q + 1] = tot
                sh, sca = shift_scale(tot)
            if not final and n >= 2:
                for g in range(16):
                    r0 = 256 * (n - 2) + 16 * g
                    hb = pltpu.bitcast(modulated(q + 1, r0, 16, sh, sca), U32)
                    hp_v[q + 1, pl.ds(r0 // 2, 8), :] = hb
                    add_tok(toks, (8 + (g * 3) // 2) if n == 2 else 2 * g,
                            hb[:, :128] ^ hb[:, 128:])
            lhs = jnp.concatenate([tie_lhs(hp_v[q, :, pl.ds(0, 128)], never, toks),
                                   hp_v[q, :, pl.ds(128, 128)]], axis=1)
            y = jnp.dot(pltpu.bitcast(lhs, BF), w, preferred_element_type=F32)
            if not first:
                y = y + part_v[p, n]
            if final:
                for j in range(2):
                    ring_fill(k + j, p, y[:, 128 * j:128 * j + 128])
            else:
                part_v[p, n] = y
            w = w_next

        for j in range(b_lo, b_hi):
            if starts[j]:
                @pl.when(b == j)
                def _():
                    for cp in starts[j]:
                        cp.start()
        return carry

    for b_lo, b_hi in ((0, NP), (NP, 2 * NP), (2 * NP, 3 * NP), (3 * NP, 4 * NP)):
        quarters = functools.partial(quarter_block, b_lo, b_hi)
        lax.fori_loop(b_lo, b_hi, quarters, 0)

    def bulk_dot(i, k, never, t, md):
        w = pltpu.bitcast(wqkv_v[pl.ds(pl.multiple_of((8 * i + k) * PITCH, 8), 512), :], BF)
        cols = [hp_v[c // 2, :, pl.ds(128 * (c % 2), 128)] for c in range(8)]
        toks = {}
        for g in range(8):
            tk = relayout((t & 1) * D + 128 * k + 16 * g, t * (8 * PITCH) + 64 * k + 8 * g, 16)
            md[1] = mod_rows(md[0], 128 * k + 16 * g, 16, md[1])
            toks[10 + 6 * (g + g // 4)] = tk ^ token(md[1][:, :256] + md[1][:, 256:])
        cols[0] = tie_lhs(cols[0], never, toks)
        cols[4] = tie_lhs(cols[4], never, {j - 32: tk for j, tk in toks.items()})
        hb = pltpu.bitcast(jnp.concatenate(cols, axis=1), BF)
        y = jnp.dot(hb, w, preferred_element_type=F32)
        ring_fill(k, i, y)

    def bulk_qkv(i, carry):
        @pl.when(i < 11)
        def _():
            par = (i + 1) & 1
            stage_wait(pl.multiple_of(par * D, D), D, 4 + par)

        @pl.when(i > NP)
        def _():
            wmod_copy(i, 2 + (i & 1)).wait()

        for j in range(NP, 10):
            @pl.when(i == j)
            def _():
                piece_copy(j + 2, 4 + j % 2).start()

        t = jnp.minimum(i + 1, 11)
        never = jnp.full((8, 128), i, jnp.int32) < 0
        md = [i, None]
        for k in range(8):
            bulk_dot(i, k, never, t, md)
        macc_v[jnp.maximum(i, 4)] = md[1]

        for j in range(NP, 10):
            @pl.when(i == j)
            def _():
                wmod_copy(j + 2, 2 + j % 2).start()
                if j < 9:
                    mid_copies[j - NP + 1].start()
                else:
                    for cp in mid_copies[7:]:
                        cp.start()
        return carry
    mid_copies[0].start()
    lax.fori_loop(NP, 12, bulk_qkv, 0)

    for q in range(4):
        sh, sca = shift_scale(macc_v[q])
        mod_v[0, :, pl.ds(q * QK, QK)] = sh
        mod_v[1, :, pl.ds(q * QK, QK)] = sca
        ho_v[0, pl.ds(BULK, RIDE), pl.ds(q * QK, QK)] = modulated(q, BULK, RIDE, sh, sca)
    for k in range(4, 12):
        y = _rb(jnp.sum(macc_v[k], axis=0, keepdims=True))
        if k // 2 == 4:
            y = _rb(1.0 + y)
        mod_v[k // 2, :, pl.ds((k % 2) * 512, 512)] = jnp.broadcast_to(y, (8, 512))
    for cp in mid_copies:
        cp.wait()
    x2_copy.start()
    for cp in ffn_copies:
        cp.start()

    scale = DH ** -0.5
    kk = lax.broadcasted_iota(jnp.int32, (M + SEG, 80), 0)
    cc = lax.broadcasted_iota(jnp.int32, (M + SEG, 80), 1)
    second = ((cc >= 8) & (cc < 16)) | (cc >= 48)
    allowed = (cc < 16) | (kk <= jnp.where(second, cc - 40, cc - 8))

    def over_keys(f, fr, v):
        t = v[0:8]
        for j in range(8, M + SEG, 8):
            t = f(t, v[j:j + 8])
        return fr(t, axis=0, keepdims=True)

    def tied(u, never, toks):
        if not toks:
            return u
        parts, at = [], 0
        for j, tk in enumerate(toks):
            r = 64 * j
            if r > at:
                parts.append(u[at:r])
            parts.append(jnp.where(never, tk, u[r:r + 8]))
            at = r + 8
        return jnp.concatenate(parts + [u[at:]], axis=0)

    def w_slab(t, g, lo=0, n=512, never=None, toks=()):
        return pltpu.bitcast(
            tied(wqkv_v[pl.ds((8 * t + g) * PITCH + lo, n), :], never, toks), BF)

    def step(s, u, mem, left, att_prev, scores_out):
        odd = left is not None
        wr = 3 * lax.rem(s >> 2, NRING // 3)
        rd = lax.rem(s + NRING - BULK // SEG, NRING)

        def ring_put(g, t, y):
            if odd:
                u32 = pltpu.bitcast(y.astype(BF), U32)
                parts = [(3 * u, u32[4:8]), (3 * u + 1, u32[8:16])]
            else:
                u32 = pltpu.bitcast(y[M:].astype(BF), U32)
                parts = [(3 * u, u32[0:8]), (3 * u + 2, u32[8:12])]
            for grp, v in parts:
                ring[g][t // 2, wr + grp // 4,
                        pl.ds(16 * (t % 2) + 4 * (grp % 4), v.shape[0]), :] = v

        xin = jnp.concatenate(
            [mem, ho_v[0, pl.ds(pl.multiple_of(BULK + RIDE * s, 8), RIDE), :]], axis=0)

        prow = SEG * (s - 1) if odd else jnp.maximum(SEG * s - 40, 0)
        nrow = BULK + RIDE * jnp.minimum(s + 1, NSEG - 1)
        works = [post_work(pl.multiple_of(prow + 8 * q, 8), functools.partial(att_prev, q),
                           scores_out) for q in range(3 if odd else 5)]
        works += [ln1_work(pl.multiple_of(nrow + 8 * q, 8)) for q in range(RIDE // 8)]
        never = jnp.full((8, 128), s, jnp.int32) < 0
        gap = (SIDE_END - SIDE0 - SIDE_LAT - SIDE_DUE) // len(works)
        sched = {}
        for q, wk in enumerate(works):
            sched.setdefault(SIDE0 + gap * q, []).append(wk[0])
            for c in range(1, len(wk)):
                sched.setdefault(SIDE0 + SIDE_LAT + gap * q + ((c - 1) * gap) // 4,
                                 []).append(wk[c])

        memqkv, probs, wl, new_left, toks = {}, {}, {}, {}, {}
        acc = []
        chain = []

        ndot = [0]

        def proj(g, t_lo, t_hi):
            part = {}
            if u > 0 and ndot[0] == 0:
                for t in range(t_lo, t_lo + 6):
                    part[t] = jnp.dot(xin[:, :512], w_slab(t, g, 0, 256),
                                      preferred_element_type=F32)
            for t0 in range(t_lo, t_hi, 2):
                ys = []
                for t in (t0, t0 + 1):
                    n = ndot[0]
                    ndot[0] += 1
                    if t in part:
                        y = jnp.dot(xin[:, 512:], w_slab(t, g, 256, 256),
                                    preferred_element_type=F32) + part[t]
                    else:
                        y = jnp.dot(xin, w_slab(t, g, 0, 512, never, toks.get(n)),
                                    preferred_element_type=F32)
                    ring_put(g, t, y)
                    ys.append(y[:M])
                    for item in sched.get(n, ()):
                        tk = item((never, y[:M]))
                        if tk is not None:
                            toks.setdefault(n + SIDE_DUE, []).append(tk)
                memqkv[(t0, g)] = jnp.concatenate(ys, axis=0).astype(BF)

        def cat(t0, g):
            return jnp.concatenate(
                [memqkv[(t0, g)], pltpu.bitcast(ring[g][t0 // 2, rd], BF)], axis=0)

        def scores(g):
            for p in (0, 2):
                if len(chain) < 4:
                    qt = pltpu.bitcast(cat(p, g).T, U32)
                    qt = jnp.concatenate(
                        [jnp.where(never[:, :80], qt[8:16], qt[0:8]), qt[8:]], axis=0)
                    st = jnp.dot(cat(4 + p, g), pltpu.bitcast(qt, BF),
                                 preferred_element_type=F32)
                else:
                    st = lax.dot_general(cat(4 + p, g), cat(p, g), (((1,), (1,)), ((), ())),
                                         preferred_element_type=F32)
                st = jnp.where(second, jnp.concatenate([st[8:16], st[48:80]], axis=0),
                               jnp.concatenate([st[0:8], st[16:48]], axis=0))
                if chain:
                    st = jnp.concatenate(
                        [jnp.where(never[:, :80], chain[-1], st[0:8]), st[8:]], axis=0)
                st = jnp.where(allowed, st * scale, -1e9)
                e = jnp.exp(st - over_keys(jnp.maximum, jnp.max, st))
                l = over_keys(jnp.add, jnp.sum, e)
                chain.append(jnp.broadcast_to(l, (8, 80)))
                rc = pl.reciprocal(l, approx=True)
                e = e * (rc * (2.0 - l * rc))
                e0 = jnp.where(second, 0.0, e)
                e1 = jnp.where(second, e, 0.0)
                probs[(p, g)] = jnp.concatenate(
                    [e0[:M], e1[:M], e0[M:], e1[M:]], axis=0).astype(BF)

        def pv(g):
            for p in (0, 2):
                o = lax.dot_general(probs[(p, g)], cat(8 + p, g), (((0,), (0,)), ((), ())),
                                    preferred_element_type=F32)
                for j in range(2):
                    om, ot = o[8 * j:8 * j + 8], o[16 + 32 * j:48 + 32 * j]
                    if odd:
                        rows = [om, left[(p + j, g)], ot]
                    else:
                        rows = [om, ot[:RIDE]]
                        new_left[(p + j, g)] = ot[RIDE:]
                    wl[(p + j, g)] = jnp.concatenate(rows, axis=0).astype(BF)

        def wo(g):
            a = jnp.concatenate([wl[(o, g)] for o in range(4)], axis=1)
            w = jnp.concatenate(
                [jnp.concatenate([wo_v[n, pl.ds((8 * o + PERM[g]) * DH, DH), :]
                                  for o in range(4)], axis=0) for n in range(2)], axis=1)
            y = jnp.dot(a, w, preferred_element_type=F32)
            acc[:] = [y if not acc else y + acc[0]]

        for op in ORDER.split():
            g = int(op[1])
            if op[0] in "qkv":
                proj(g, *{"q": (0, 12), "k": (0, 8), "v": (8, 12)}[op[0]])
            else:
                {"s": scores, "p": pv, "w": wo}[op[0]](g)
        y = acc[0].astype(BF)
        return y[:M], y[M:], (None if odd else new_left)

    def out_copy(row0, n, k):
        return pltpu.make_async_copy(ho_v.at[1, pl.ds(row0, n), :],
                                     out_hbm.at[0, pl.ds(row0, n), :], sems.at[3 + k])

    OB = SEG * UNROLL

    def carried(q):
        return att_v[pl.ds(8 * q, 8), :]

    sub1 = lax.broadcasted_iota(jnp.int32, (16, 128), 0)
    slot = (sub1 // 8) * 128 + lax.broadcasted_iota(jnp.int32, (16, 128), 1)
    idx = (slot - 5) * 8 + sub1 % 8

    def guess_blocks(r):
        key = pltpu.bitcast(pltpu.bitcast(_rb(r), jnp.int32) | (S - 1 - idx), F32)
        key = jnp.where(idx >= 0, key, -jnp.inf)
        for k in range(2):
            m = jnp.max(jnp.max(key, axis=0, keepdims=True), axis=1, keepdims=True)
            r_v[2 + k] = jnp.broadcast_to(m, (8, 128))
            key = jnp.where(key >= m, -jnp.inf, key)

    def steps(i, carry):
        @pl.when(i == 16 // UNROLL)
        def _():
            x2_copy.wait()

        mem, left, att_prev, scores = mem_v[...], None, carried, []
        for u in range(UNROLL):
            mem, att, left = step(i * UNROLL + u, u, mem, left, att_prev, scores)
            att_prev = (lambda a: lambda q: a[8 * q:8 * q + 8])(att)
        mem_v[...] = mem
        att_v[...] = att
        new = jnp.broadcast_to(scores[0], (8, 128))
        for j in range(1, 16):
            new = jnp.where((slot[:8] & 15) == j, scores[j], new)
        r = jnp.where((slot >> 4) == i, jnp.concatenate([new, new], axis=0),
                      r_v[pl.ds(0, 2)].reshape(16, 128))
        r_v[pl.ds(0, 2)] = r.reshape(2, 8, 128)
        guess_blocks(r)

        @pl.when(i >= 1)
        def _():
            out_copy(pl.multiple_of((i - 1) * OB, OB), OB, 0).start()
        return carry
    lax.fori_loop(0, NSEG // UNROLL, steps, 0)

    for cp in ffn_copies:
        cp.wait()

    def two(ref, a, b):
        return jnp.concatenate([ref[pl.ds(a, 8), :], ref[pl.ds(b, 8), :]], axis=0)

    def ffn_act(h, c):
        g = _rb(jnp.dot(h, wg_v[:, pl.ds(512 * c, 512)], preferred_element_type=F32))
        u = _rb(jnp.dot(h, wu_v[:, pl.ds(512 * c, 512)], preferred_element_type=F32))
        return (_rb(g * jax.nn.sigmoid(g)) * u).astype(BF)

    def ffn_down(a, c):
        wd = jnp.concatenate([wd_v[k, pl.ds(512 * c, 512), :] for k in range(2)], axis=1)
        return jnp.dot(a, wd, preferred_element_type=F32)

    early = _rb(r_v[pl.ds(0, 2)].reshape(16, 128))

    def guessed(k):
        j = S - 1 - (pltpu.bitcast(r_v[2 + k], jnp.int32) & (S - 1))
        return pl.multiple_of(jnp.minimum(j[0, 0] >> 3, (S - 48) // 8) * 8, 8)
    gs_a, gs_b = guessed(0), guessed(1)
    h_gs = two(ho_v.at[0], gs_a, gs_b)
    acts = [ffn_act(h_gs, c) for c in range(NSPEC)]

    last, done = [], []
    never = jnp.full((8, 128), gs_a, jnp.int32) < 0
    for q in range(5):
        items = post_work(S - 40 + 8 * q, functools.partial(carried, q), last)
        items[0](None)
        for item in items[1:]:
            done.append(item((never, pltpu.bitcast(done[-2], F32)) if len(done) >= 2 else None))
    out_copy(S - OB, OB, 0).start()

    def top2(val, idx, valid):
        def reduce(f, v):
            v = f(v, axis=0, keepdims=True)
            return v if v.shape[1] == 1 else f(v, axis=1, keepdims=True)

        def argtop(ok):
            v = jnp.where(ok, val, -jnp.inf)
            m = reduce(jnp.max, v)
            return m, reduce(jnp.min, jnp.where(ok & (v >= m), idx, float(S)))
        m1, i1 = argtop(valid)
        return (m1, i1), argtop(valid & (idx != i1))

    c_a, c_b = top2(early, idx.astype(F32), idx >= 0)
    sub2 = lax.broadcasted_iota(jnp.int32, (48, 1), 0)
    val2 = jnp.concatenate([_rb(r) for r in last] + [jnp.where(sub2[:8] == 0, c_a[0], c_b[0])],
                           axis=0)
    idx2 = jnp.where(sub2 < 40, (sub2 + (S - 40)).astype(F32),
                     jnp.where(sub2 == 40, c_a[1], c_b[1]))
    (m_a, i_a), (m_b, i_b) = top2(val2, idx2, sub2 < 42)
    i_a = i_a.astype(jnp.int32)
    i_b = i_b.astype(jnp.int32)
    ia = jnp.clip(i_a[0, 0], 0, S - 1)
    ib = jnp.clip(i_b[0, 0], 0, S - 1)
    blk_a = pl.multiple_of((ia // 8) * 8, 8)
    blk_b = pl.multiple_of((ib // 8) * 8, 8)

    hs = two(ho_v.at[0], blk_a, blk_b)
    y0 = y = None
    for c in range(1, FF // 512 + 1):
        if NSPEC <= c < FF // 512:
            acts.append(ffn_act(hs, c))
        t = ffn_down(acts[c - 1], c - 1)
        if c <= NSPEC:
            y0 = t if y0 is None else t + y0
        else:
            y = t if y is None else t + y
    sub = lax.broadcasted_iota(jnp.int32, (16, 1), 0)
    rows = jnp.where(sub < 8, blk_a + sub, blk_b + sub - 8)
    gate = jnp.where(rows == ia, jax.nn.sigmoid(m_a),
                     jnp.where(rows == ib, jax.nn.sigmoid(m_b), 0.0))

    def finish(ffn):
        upd = jnp.where((rows == ia) | (rows == ib), ffn * gate, 0.0).reshape(2, 8, D)
        fin_v[...] = _b2(_f3(two(ho_v.at[1], blk_a, blk_b)) + mod_v[5] * upd)

    finish(y + y0)

    @pl.when((gs_a != blk_a) | (gs_b != blk_b))
    def _():
        redo = [ffn_act(hs, c) for c in range(NSPEC)]
        finish(functools.reduce(lambda a, c: ffn_down(redo[c], c) + a, range(NSPEC), y))

    def patch(k, blk):
        return pltpu.make_async_copy(fin_v.at[pl.ds(8 * k, 8), :],
                                     out_hbm.at[0, pl.ds(blk, 8), :], sems.at[3 + k])

    out_copy(0, S, 0).wait()
    patch(0, blk_a).start()

    @pl.when(blk_a != blk_b)
    def _():
        patch(1, blk_b).start()
        patch(1, blk_b).wait()
    patch(0, blk_a).wait()


@jax.jit
def pallas_adaLN_cond__memory_aug_recurrent_mem_tr__moe_arch_mod__prompt_kernel(
    A_x, A_mem0, A_Wq, A_Wk, A_Wv, A_Wo, A_seg_len, B_x, B_w_r, B_w_gate, B_w_up, B_w_down, c,
    w_mod,
):
    del B_x
    del A_seg_len
    assert A_x.shape == (1, S, D) and A_Wq.shape == (D, H, DH) and A_mem0.shape == (1, M, D)
    any_spec = pl.BlockSpec(memory_space=pl.ANY)
    scratch = [
        pltpu.VMEM((S, D), BF),
        pltpu.VMEM((4, X0, QK), BF),
        pltpu.VMEM((4, BULK // 2, QK), U32),
        pltpu.VMEM((40, D), BF),
        pltpu.VMEM((2, S, D), BF),
        pltpu.VMEM((100 * PITCH, 128), U32),
        pltpu.VMEM((2, H * DH, 512), BF),
        pltpu.VMEM((5 * D, 8, 128), BF),
        pltpu.VMEM((12, D, 512), BF),
        pltpu.VMEM((D, FF), BF),
        pltpu.VMEM((D, FF), BF),
        pltpu.VMEM((2, FF, 512), BF),
        pltpu.VMEM((M, D), BF),
        pltpu.VMEM((4, 1, D), BF),
        pltpu.VMEM((7, 8, D), F32),
        pltpu.VMEM((4, 8, 128), F32),
        pltpu.VMEM((D, 128), F32),
        pltpu.VMEM((12, 8, 512), F32),
        pltpu.VMEM((NP, 4, BULK, 256), F32),
        pltpu.VMEM((16, D), BF),
        pltpu.SemaphoreType.DMA((9,)),
    ] + [pltpu.VMEM((6, NRING, 32, 128), U32)] * 8
    return pl.pallas_call(
        _kernel,
        out_shape=jax.ShapeDtypeStruct((1, S, D), BF),
        in_specs=[any_spec] * 12,
        out_specs=any_spec,
        scratch_shapes=scratch,
        compiler_params=pltpu.CompilerParams(vmem_limit_bytes=120 * 1024 * 1024),
    )(A_x, A_mem0, A_Wq, A_Wk, A_Wv, A_Wo.reshape(H * DH, D), B_w_r.reshape(1, D), B_w_gate,
      B_w_up, B_w_down, c, w_mod)
```

```python
import functools

import jax
import jax.numpy as jnp
from jax import lax
import jax.experimental.pallas as pl
import jax.experimental.pallas.tpu as pltpu

BF = jnp.bfloat16
F32 = jnp.float32
U32 = jnp.uint32

S = 2048
D = 1024
H = 32
DH = 128
M = 8
SEG = 32
NSEG = S // SEG
FF = 3584
RIDE = 24
BULK = S - RIDE * NSEG
X0 = BULK + 32
NRING = 18
PITCH = 520
X1 = 1024
NP = 3
QK = D // 4
UNROLL = 4
NSPEC = 2
EPS = 1e-5
SIDE0, SIDE_LAT, SIDE_DUE, SIDE_END = 0, 6, 6, 78
NEG = -3.0e38
ORDER = ("q0 q1 q2 q3 k4 k5 k6 k7 s0 s1 s2 s3 s4 s5 s6 s7 v4 v5 v6 v7 p0 p1 p2 p3 p4 p5 p6 p7 "
         "w0 w1 w2 w3 w4 w5 w6 w7")
PERM = (0, 2, 4, 6, 1, 3, 5, 7)


def _rb(v):
    return v.astype(BF).astype(F32)


def _layernorm(xf):
    mu = jnp.mean(xf, axis=-1, keepdims=True)
    dv = xf - mu
    var = jnp.mean(dv * dv, axis=-1, keepdims=True)
    sd = _rb(jnp.sqrt(_rb(_rb(var) + EPS)))
    return _rb(_rb(xf - _rb(mu)) * (1.0 / sd))


def _f3(v):
    return v.astype(F32).reshape(v.shape[0] // 8, 8, D)


def _b2(v):
    return v.reshape(v.shape[0] * 8, D).astype(BF)


def _kernel(x_hbm, mem0_hbm, wq_hbm, wk_hbm, wv_hbm, wo_hbm, wr_hbm, wg_hbm, wu_hbm, wd_hbm,
            c_hbm, wmod_hbm, out_hbm,
            x_v, h_v, hp_v, att_v, ho_v, wqkv_v, wo_v, stage, wmod_v,
            wg_v, wu_v, wd_v, mem_v, cw_v, mod_v, r_v, sb_v, macc_v,
            part_v, fin_v, sems, *rings):
    w_hbm = (wq_hbm, wk_hbm, wv_hbm)
    ring = rings

    def piece_copy(t, sem, lo=0, n=D, dst=None):
        dst = (t % 2) * D + lo if dst is None else dst
        return pltpu.make_async_copy(
            w_hbm[t // 4].at[pl.ds(lo, n), pl.ds((t % 4) * 8, 8), :],
            stage.at[pl.ds(dst, n)], sems.at[sem])

    def unit_copy(j):
        sem = 1 if j == 1 else 6 + min(j, 10) % 3
        return piece_copy(j % NP, sem, QK * (j // NP), QK, 2 * D + QK * j)

    def stage_wait(row, n, sem):
        dst = stage.at[pl.ds(row, n)]
        pltpu.make_async_copy(dst, dst, sems.at[sem]).wait()

    def mq_copy(q, part):
        return pltpu.make_async_copy(wmod_hbm.at[:, pl.ds(part * D + q * QK, QK)],
                                     wmod_v.at[q, :, pl.ds(part * QK, QK)], sems.at[2])

    def wmod_copy(k, sem):
        col = k * 512 if isinstance(k, int) else pl.multiple_of(k * 512, 512)
        return pltpu.make_async_copy(wmod_hbm.at[:, pl.ds(col, 512)], wmod_v.at[k], sems.at[sem])

    def x_copy(lo, hi, sem):
        return pltpu.make_async_copy(x_hbm.at[0, pl.ds(lo, hi - lo), :],
                                     x_v.at[pl.ds(lo, hi - lo), :], sems.at[sem])

    def wo_copy(n):
        lo, rows = ((n // 2) * 512, 512) if n < 6 else (1536, 2560)
        return pltpu.make_async_copy(wo_hbm.at[pl.ds(lo, rows), pl.ds((n % 2) * 512, 512)],
                                     wo_v.at[n % 2, pl.ds(lo, rows)], sems.at[0])

    small_copies = [pltpu.make_async_copy(c_hbm, cw_v.at[0], sems.at[0]),
                    pltpu.make_async_copy(mem0_hbm.at[0], mem_v, sems.at[0]),
                    pltpu.make_async_copy(wr_hbm, cw_v.at[1], sems.at[0])]
    x0_copy = x_copy(0, X0, 1)
    mid_copies = ([x_copy(X0, (X0 + X1) // 2, 0), x_copy((X0 + X1) // 2, X1, 0)]
                  + [wo_copy(n) for n in range(8)])
    x2_copy = x_copy(X1, S, 1)
    ffn_copies = [pltpu.make_async_copy(wg_hbm, wg_v, sems.at[2]),
                  pltpu.make_async_copy(wu_hbm, wu_v, sems.at[2])] + [
        pltpu.make_async_copy(wd_hbm.at[:, pl.ds(k * 512, 512)], wd_v.at[k], sems.at[2])
        for k in range(2)]

    def relayout(src, base, n):
        u = pltpu.bitcast(stage[pl.ds(src, n)], U32)
        tok = None
        for i in range(n // 2):
            a = u[2 * i]
            b = u[2 * i + 1]
            even = (a & jnp.uint32(0xFFFF)) | (b << 16)
            odd = (a >> 16) | (b & jnp.uint32(0xFFFF0000))
            wqkv_v[pl.ds(base + i, 4, stride=PITCH), :] = even
            wqkv_v[pl.ds(base + 4 * PITCH + i, 4, stride=PITCH), :] = odd
            tok = even ^ odd if tok is None else tok ^ even ^ odd
        return jnp.concatenate([tok, tok], axis=0)

    CW = 256

    def ln_stats(xf):
        mu = jnp.mean(xf, axis=-1, keepdims=True)
        dv = xf - mu
        var = jnp.mean(dv * dv, axis=-1, keepdims=True)
        sd = _rb(jnp.sqrt(_rb(_rb(var) + EPS)))
        return _rb(mu), 1.0 / sd

    def mod_c(k, c):
        return mod_v[k, :, pl.ds(c * CW, CW)]

    def token(v):
        return pltpu.bitcast(v[:, :128] + v[:, 128:], U32)

    def after(v, trig):
        if trig is None:
            return v
        return jnp.concatenate([jnp.where(trig[0], trig[1], v[:, :128]), v[:, 128:]], axis=1)

    def post_work(row0, att, scores_out):
        st = {}

        def head(trig):
            a = after(att().astype(F32), trig)
            st["x2"] = _rb(x_v[pl.ds(row0, 8), :].astype(F32) + _rb(mod_v[2] * a))
            st["mu"], st["inv"] = ln_stats(st["x2"])

        def chunk(c, trig):
            xc = after(st["x2"][:, c * CW:(c + 1) * CW], trig)
            h2b = (_rb(_rb(_rb(xc - st["mu"]) * st["inv"]) * mod_c(4, c))
                   + mod_c(3, c)).astype(BF)
            h2 = h2b.astype(F32)
            ho_v[0, pl.ds(row0, 8), pl.ds(c * CW, CW)] = h2b
            o = xc + mod_c(5, c) * h2
            ho_v[1, pl.ds(row0, 8), pl.ds(c * CW, CW)] = o.astype(BF)
            rp = h2 * mod_c(6, c)
            st["r"] = rp if c == 0 else st["r"] + rp
            if c == D // CW - 1:
                scores_out.append(jnp.sum(st["r"], axis=-1, keepdims=True))
            return token(o + st["r"])
        return [head] + [functools.partial(chunk, c) for c in range(D // CW)]

    def ln1_work(row0):
        st = {}

        def head(trig):
            st["x"] = after(x_v[pl.ds(row0, 8), :].astype(F32), trig)
            st["mu"], st["inv"] = ln_stats(st["x"])

        def chunk(c, trig):
            xc = after(st["x"][:, c * CW:(c + 1) * CW], trig)
            h = _rb(_rb(_rb(xc - st["mu"]) * st["inv"]) * mod_c(1, c)) + mod_c(0, c)
            ho_v[0, pl.ds(row0, 8), pl.ds(c * CW, CW)] = h.astype(BF)
            return token(h)
        return [head] + [functools.partial(chunk, c) for c in range(D // CW)]

    for cp in small_copies:
        cp.start()
    x0_copy.start()
    mq_copy(0, 0).start()

    r_v[...] = jnp.full(r_v.shape, NEG, F32)
    att_v[...] = jnp.zeros(att_v.shape, BF)

    for cp in small_copies:
        cp.wait()
    mod_v[6] = jnp.broadcast_to(cw_v[1].astype(F32), (8, D))
    cf = cw_v[0].astype(F32)
    sil = (cf * jax.nn.sigmoid(cf)).astype(BF)
    sc = jnp.broadcast_to(sil, (16, D))
    for k in range(8):
        sb_v[pl.ds(128 * k, 128), :] = jnp.broadcast_to(
            sil[:, 128 * k:128 * k + 128].astype(F32), (128, 128)).T

    mq_copy(0, 1).start()
    x0_copy.wait()

    LNB = X0 // 4

    def ln0(i, carry):
        r0 = pl.multiple_of(i * LNB, 8)
        ln = _b2(_layernorm(_f3(x_v[pl.ds(r0, LNB), :])))
        for q in range(4):
            h_v[q, pl.ds(r0, LNB), :] = ln[:, q * QK:(q + 1) * QK]

        @pl.when(i == 1)
        def _():
            unit_copy(0).start()
        return carry
    lax.fori_loop(0, 4, ln0, 0)

    def shift_scale(acc):
        y = _rb(acc)
        return y[:, :QK], _rb(1.0 + y[:, QK:])

    def modulated(q, r0, n, sh, sca):
        ln = h_v[q, pl.ds(r0, n), :].astype(F32).reshape(n // 8, 8, QK)
        return (_rb(ln * sca) + sh).reshape(n, QK).astype(BF)

    unit_copy(1).start()
    for part in range(2):
        mq_copy(0, part).wait()
    acc0 = jnp.dot(sc, wmod_v[0], preferred_element_type=F32)[0:8]
    macc_v[0] = acc0
    hp_v[0] = pltpu.bitcast(modulated(0, 0, BULK, *shift_scale(acc0)), U32)
    unit_copy(2).start()

    def first_unit(j):
        def relayout0(i, carry):
            relayout(2 * D + QK * j + pl.multiple_of(i * 128, 128), j * 8 * PITCH + i * 64, 128)
            return carry
        unit_copy(j).wait()
        lax.fori_loop(0, QK // 128, relayout0, 0)

    first_unit(0)
    mq_copy(1, 0).start()
    mq_copy(1, 1).start()
    unit_copy(3).start()

    def mod_rows(slab, r0, n, acc):
        for r in range(r0, r0 + n, 8):
            sv = sb_v[pl.ds(r, 8), :]
            t = wmod_v[slab, pl.ds(r, 8), :].astype(F32) * jnp.concatenate([sv] * 4, axis=1)
            acc = t if acc is None else acc + t
        return acc

    def ring_fill(g, t, y):
        ring[g][t >> 1, pl.ds(NRING - BULK // SEG, BULK // SEG),
                pl.ds(pl.multiple_of(16 * (t & 1), 16), 16), :] = (
            pltpu.bitcast(y.astype(BF), U32).reshape(BULK // SEG, 16, 128))

    def tie_lhs(col, never, toks):
        return jnp.concatenate(
            [jnp.where(never, toks[j], col[8 * j:8 * j + 8]) if j in toks
             else col[8 * j:8 * j + 8] for j in range(32)], axis=0)

    def add_tok(toks, j, tk):
        toks[j] = tk if j not in toks else toks[j] ^ tk

    starts = {0: [unit_copy(4)], 1: [unit_copy(5), piece_copy(3, 5, 0, 256)],
              2: [unit_copy(6), mq_copy(2, 0), mq_copy(2, 1)],
              3: [unit_copy(7), piece_copy(3, 5, 256, 256)], 4: [unit_copy(8)],
              5: [unit_copy(9), mq_copy(3, 0), mq_copy(3, 1)],
              6: [unit_copy(10), unit_copy(11)], 7: [piece_copy(3, 3, 512, 512)],
              8: [piece_copy(4, 4)], 9: [], 10: [wmod_copy(4, 2)], 11: []}

    def quarter_block(b_lo, b_hi, b, carry):
        first, final = b_lo == 0, b_hi == 4 * NP
        q = b_lo // NP
        p = b - NP * q
        if final:
            src = jnp.where(p == 0, 2 * D + 10 * QK, D + 512 * (p - 1))
            sem = 7 - 2 * p
            stage_wait(pl.multiple_of(src, 512), 512, sem)
            b3 = 3 * 8 * PITCH + 256 * (p - 1)
            jobs = [(src, jnp.where(p == 0, 8 * PITCH + 384, b3)),
                    (src + QK, jnp.where(p == 0, 2 * 8 * PITCH + 384, b3 + 128))]
        else:
            src = 2 * D + QK * (b + 1)
            last = p == NP - 1
            dst = jnp.where(last, 128 * (q + 1), (p + 1) * (8 * PITCH) + 128 * q)

            def unit_wait():
                stage_wait(pl.multiple_of(src, QK), QK, jnp.where(last, 6, 7 + p))
            if first:
                pl.when(b == 1)(functools.partial(first_unit, 1))
                pl.when(b > 0)(unit_wait)
                jobs = [(jnp.where(b == 0, 2 * D, src), jnp.where(b == 0, 0, dst))]
            else:
                unit_wait()
                jobs = [(src, dst)]

            @pl.when(last)
            def _():
                for part in range(2):
                    mq_copy(q + 1, part).wait()
            slab = jnp.where(last, q + 1, q)
        never = jnp.full((8, 128), b, jnp.int32) < 0

        def weights(k):
            return pltpu.bitcast(jnp.concatenate(
                [wqkv_v[pl.ds(pl.multiple_of((8 * p + kk) * PITCH + 128 * q, 8), 128), :]
                 for kk in (k, k + 1)], axis=1), BF)

        groups = [(s_ + 16 * g, d_ + 8 * g) for s_, d_ in jobs for g in range(QK // 16)]
        per = len(groups) // 4
        acc = None
        w = weights(0)
        for n, k in enumerate(range(0, 8, 2)):
            w_next = weights(k + 2) if k < 6 else None
            toks = {}
            if final and n == 2:
                wu = pltpu.bitcast(w_next, U32)
                wu = wu[:, :128] ^ wu[:, 128:]
                add_tok(toks, 3, functools.reduce(
                    jnp.bitwise_xor, [wu[8 * j:8 * j + 8] for j in range(16)]))
            for g in range(per):
                add_tok(toks, 4 + (g * 24) // per, relayout(*groups[n * per + g], 16))
            if not final and n < 2:
                for g in range(16):
                    acc = mod_rows(slab, 512 * n + 32 * g, 32, acc)
                    add_tok(toks, 2 * g + (n == 0), token(acc[:, :256] + acc[:, 256:]))
            if not final and n == 2:
                tot = jnp.broadcast_to(jnp.sum(acc, axis=0, keepdims=True), (8, 512))
                macc_v[q + 1] = tot
                sh, sca = shift_scale(tot)
            if not final and n >= 2:
                for g in range(16):
                    r0 = 256 * (n - 2) + 16 * g
                    hb = pltpu.bitcast(modulated(q + 1, r0, 16, sh, sca), U32)
                    hp_v[q + 1, pl.ds(r0 // 2, 8), :] = hb
                    add_tok(toks, (8 + (g * 3) // 2) if n == 2 else 2 * g,
                            hb[:, :128] ^ hb[:, 128:])
            lhs = jnp.concatenate([tie_lhs(hp_v[q, :, pl.ds(0, 128)], never, toks),
                                   hp_v[q, :, pl.ds(128, 128)]], axis=1)
            y = jnp.dot(pltpu.bitcast(lhs, BF), w, preferred_element_type=F32)
            if not first:
                y = y + part_v[p, n]
            if final:
                for j in range(2):
                    ring_fill(k + j, p, y[:, 128 * j:128 * j + 128])
            else:
                part_v[p, n] = y
            w = w_next

        for j in range(b_lo, b_hi):
            if starts[j]:
                @pl.when(b == j)
                def _():
                    for cp in starts[j]:
                        cp.start()
        return carry

    for b_lo, b_hi in ((0, NP), (NP, 2 * NP), (2 * NP, 3 * NP), (3 * NP, 4 * NP)):
        quarters = functools.partial(quarter_block, b_lo, b_hi)
        lax.fori_loop(b_lo, b_hi, quarters, 0)

    def bulk_dot(i, k, never, t, md):
        w = pltpu.bitcast(wqkv_v[pl.ds(pl.multiple_of((8 * i + k) * PITCH, 8), 512), :], BF)
        cols = [hp_v[c // 2, :, pl.ds(128 * (c % 2), 128)] for c in range(8)]
        toks = {}
        for g in range(8):
            tk = relayout((t & 1) * D + 128 * k + 16 * g, t * (8 * PITCH) + 64 * k + 8 * g, 16)
            md[1] = mod_rows(md[0], 128 * k + 16 * g, 16, md[1])
            toks[10 + 6 * (g + g // 4)] = tk ^ token(md[1][:, :256] + md[1][:, 256:])
        cols[0] = tie_lhs(cols[0], never, toks)
        cols[4] = tie_lhs(cols[4], never, {j - 32: tk for j, tk in toks.items()})
        hb = pltpu.bitcast(jnp.concatenate(cols, axis=1), BF)
        y = jnp.dot(hb, w, preferred_element_type=F32)
        ring_fill(k, i, y)

    def bulk_qkv(i, carry):
        @pl.when(i < 11)
        def _():
            par = (i + 1) & 1
            stage_wait(pl.multiple_of(par * D, D), D, 4 + par)

        @pl.when(i > NP)
        def _():
            wmod_copy(i, 2 + (i & 1)).wait()

        for j in range(NP, 10):
            @pl.when(i == j)
            def _():
                piece_copy(j + 2, 4 + j % 2).start()

        t = jnp.minimum(i + 1, 11)
        never = jnp.full((8, 128), i, jnp.int32) < 0
        md = [i, None]
        for k in range(8):
            bulk_dot(i, k, never, t, md)
        macc_v[jnp.maximum(i, 4)] = md[1]

        for j in range(NP, 10):
            @pl.when(i == j)
            def _():
                wmod_copy(j + 2, 2 + j % 2).start()
                if j < 9:
                    mid_copies[j - NP + 1].start()
                else:
                    for cp in mid_copies[7:]:
                        cp.start()
        return carry
    mid_copies[0].start()
    lax.fori_loop(NP, 12, bulk_qkv, 0)

    for q in range(4):
        sh, sca = shift_scale(macc_v[q])
        mod_v[0, :, pl.ds(q * QK, QK)] = sh
        mod_v[1, :, pl.ds(q * QK, QK)] = sca
        ho_v[0, pl.ds(BULK, RIDE), pl.ds(q * QK, QK)] = modulated(q, BULK, RIDE, sh, sca)
    for k in range(4, 12):
        y = _rb(jnp.sum(macc_v[k], axis=0, keepdims=True))
        if k // 2 == 4:
            y = _rb(1.0 + y)
        mod_v[k // 2, :, pl.ds((k % 2) * 512, 512)] = jnp.broadcast_to(y, (8, 512))
    for cp in mid_copies:
        cp.wait()
    x2_copy.start()
    for cp in ffn_copies:
        cp.start()

    scale = DH ** -0.5
    kk = lax.broadcasted_iota(jnp.int32, (M + SEG, 80), 0)
    cc = lax.broadcasted_iota(jnp.int32, (M + SEG, 80), 1)
    second = ((cc >= 8) & (cc < 16)) | (cc >= 48)
    allowed = (cc < 16) | (kk <= jnp.where(second, cc - 40, cc - 8))

    def over_keys(f, fr, v):
        t = v[0:8]
        for j in range(8, M + SEG, 8):
            t = f(t, v[j:j + 8])
        return fr(t, axis=0, keepdims=True)

    def tied(u, never, toks):
        if not toks:
            return u
        parts, at = [], 0
        for j, tk in enumerate(toks):
            r = 64 * j
            if r > at:
                parts.append(u[at:r])
            parts.append(jnp.where(never, tk, u[r:r + 8]))
            at = r + 8
        return jnp.concatenate(parts + [u[at:]], axis=0)

    def w_slab(t, g, lo=0, n=512, never=None, toks=()):
        return pltpu.bitcast(
            tied(wqkv_v[pl.ds((8 * t + g) * PITCH + lo, n), :], never, toks), BF)

    def step(s, u, wr, rd, never, mem, left, att_prev, scores_out):
        odd = left is not None

        def ring_put(g, t, y):
            if odd:
                u32 = pltpu.bitcast(y.astype(BF), U32)
                parts = [(3 * u, u32[4:8]), (3 * u + 1, u32[8:16])]
            else:
                u32 = pltpu.bitcast(y[M:].astype(BF), U32)
                parts = [(3 * u, u32[0:8]), (3 * u + 2, u32[8:12])]
            for grp, v in parts:
                ring[g][t // 2, wr + grp // 4,
                        pl.ds(16 * (t % 2) + 4 * (grp % 4), v.shape[0]), :] = v

        xin = jnp.concatenate(
            [mem, ho_v[0, pl.ds(pl.multiple_of(BULK + RIDE * s, 8), RIDE), :]], axis=0)

        prow = SEG * (s - 1) if odd else jnp.maximum(SEG * s - 40, 0)
        nrow = BULK + RIDE * jnp.minimum(s + 1, NSEG - 1)
        works = [post_work(pl.multiple_of(prow + 8 * q, 8), functools.partial(att_prev, q),
                           scores_out) for q in range(3 if odd else 5)]
        works += [ln1_work(pl.multiple_of(nrow + 8 * q, 8)) for q in range(RIDE // 8)]
        gap = (SIDE_END - SIDE0 - SIDE_LAT - SIDE_DUE) // len(works)
        sched = {}
        for q, wk in enumerate(works):
            sched.setdefault(SIDE0 + gap * q, []).append(wk[0])
            for c in range(1, len(wk)):
                sched.setdefault(SIDE0 + SIDE_LAT + gap * q + ((c - 1) * gap) // 4,
                                 []).append(wk[c])

        memqkv, probs, wl, new_left, toks = {}, {}, {}, {}, {}
        acc = []
        chain = []

        ndot = [0]

        def proj(g, t_lo, t_hi):
            part = {}
            if u > 0 and ndot[0] == 0:
                for t in range(t_lo, t_lo + 6):
                    part[t] = jnp.dot(xin[:, :512], w_slab(t, g, 0, 256),
                                      preferred_element_type=F32)
            for t0 in range(t_lo, t_hi, 2):
                ys = []
                for t in (t0, t0 + 1):
                    n = ndot[0]
                    ndot[0] += 1
                    if t in part:
                        y = jnp.dot(xin[:, 512:], w_slab(t, g, 256, 256),
                                    preferred_element_type=F32) + part[t]
                    else:
                        y = jnp.dot(xin, w_slab(t, g, 0, 512, never, toks.get(n)),
                                    preferred_element_type=F32)
                    ring_put(g, t, y)
                    ys.append(y[:M])
                    for item in sched.get(n, ()):
                        tk = item((never, y[:M]))
                        if tk is not None:
                            toks.setdefault(n + SIDE_DUE, []).append(tk)
                memqkv[(t0, g)] = jnp.concatenate(ys, axis=0).astype(BF)

        def cat(t0, g):
            return jnp.concatenate(
                [memqkv[(t0, g)], pltpu.bitcast(ring[g][t0 // 2, rd], BF)], axis=0)

        def scores(g):
            for p in (0, 2):
                if len(chain) < 4:
                    qt = pltpu.bitcast(cat(p, g).T, U32)
                    qt = jnp.concatenate(
                        [jnp.where(never[:, :80], qt[8:16], qt[0:8]), qt[8:]], axis=0)
                    st = jnp.dot(cat(4 + p, g), pltpu.bitcast(qt, BF),
                                 preferred_element_type=F32)
                else:
                    st = lax.dot_general(cat(4 + p, g), cat(p, g), (((1,), (1,)), ((), ())),
                                         preferred_element_type=F32)
                st = jnp.where(second, jnp.concatenate([st[8:16], st[48:80]], axis=0),
                               jnp.concatenate([st[0:8], st[16:48]], axis=0))
                if chain:
                    st = jnp.concatenate(
                        [jnp.where(never[:, :80], chain[-1], st[0:8]), st[8:]], axis=0)
                st = jnp.where(allowed, st * scale, -1e9)
                e = jnp.exp(st - over_keys(jnp.maximum, jnp.max, st))
                l = over_keys(jnp.add, jnp.sum, e)
                chain.append(jnp.broadcast_to(l, (8, 80)))
                rc = pl.reciprocal(l, approx=True)
                e = e * (rc * (2.0 - l * rc))
                e0 = jnp.where(second, 0.0, e)
                e1 = jnp.where(second, e, 0.0)
                probs[(p, g)] = jnp.concatenate(
                    [e0[:M], e1[:M], e0[M:], e1[M:]], axis=0).astype(BF)

        def pv(g):
            for p in (0, 2):
                o = lax.dot_general(probs[(p, g)], cat(8 + p, g), (((0,), (0,)), ((), ())),
                                    preferred_element_type=F32)
                for j in range(2):
                    om, ot = o[8 * j:8 * j + 8], o[16 + 32 * j:48 + 32 * j]
                    if odd:
                        rows = [om, left[(p + j, g)], ot]
                    else:
                        rows = [om, ot[:RIDE]]
                        new_left[(p + j, g)] = ot[RIDE:]
                    wl[(p + j, g)] = jnp.concatenate(rows, axis=0).astype(BF)

        def wo(g):
            a = jnp.concatenate([wl[(o, g)] for o in range(4)], axis=1)
            w = jnp.concatenate(
                [jnp.concatenate([wo_v[n, pl.ds((8 * o + PERM[g]) * DH, DH), :]
                                  for o in range(4)], axis=0) for n in range(2)], axis=1)
            y = jnp.dot(a, w, preferred_element_type=F32)
            acc[:] = [y if not acc else y + acc[0]]

        for op in ORDER.split():
            g = int(op[1])
            if op[0] in "qkv":
                proj(g, *{"q": (0, 12), "k": (0, 8), "v": (8, 12)}[op[0]])
            else:
                {"s": scores, "p": pv, "w": wo}[op[0]](g)
        y = acc[0].astype(BF)
        return y[:M], y[M:], (None if odd else new_left)

    def out_copy(row0, n, k):
        return pltpu.make_async_copy(ho_v.at[1, pl.ds(row0, n), :],
                                     out_hbm.at[0, pl.ds(row0, n), :], sems.at[3 + k])

    OB = SEG * UNROLL

    def carried(q):
        return att_v[pl.ds(8 * q, 8), :]

    sub1 = lax.broadcasted_iota(jnp.int32, (16, 128), 0)
    slot = (sub1 // 8) * 128 + lax.broadcasted_iota(jnp.int32, (16, 128), 1)
    idx = (slot - 5) * 8 + sub1 % 8

    def guess_blocks(r):
        key = pltpu.bitcast(pltpu.bitcast(_rb(r), jnp.int32) | (S - 1 - idx), F32)
        key = jnp.where(idx >= 0, key, -jnp.inf)
        for k in range(2):
            m = jnp.max(jnp.max(key, axis=0, keepdims=True), axis=1, keepdims=True)
            r_v[2 + k] = jnp.broadcast_to(m, (8, 128))
            key = jnp.where(key >= m, -jnp.inf, key)

    def steps(i, carry):
        @pl.when(i == 16 // UNROLL)
        def _():
            x2_copy.wait()

        def wrap(v):
            return jnp.where(v >= NRING, v - NRING, v)

        wr, rd = carry
        never = jnp.full((8, 128), i, jnp.int32) < 0
        mem, left, att_prev, scores = mem_v[...], None, carried, []
        for u in range(UNROLL):
            mem, att, left = step(i * UNROLL + u, u, wr, wrap(rd + u), never, mem, left,
                                  att_prev, scores)
            att_prev = (lambda a: lambda q: a[8 * q:8 * q + 8])(att)
        mem_v[...] = mem
        att_v[...] = att
        new = jnp.broadcast_to(scores[0], (8, 128))
        for j in range(1, 16):
            new = jnp.where((slot[:8] & 15) == j, scores[j], new)
        r = jnp.where((slot >> 4) == i, jnp.concatenate([new, new], axis=0),
                      r_v[pl.ds(0, 2)].reshape(16, 128))
        r_v[pl.ds(0, 2)] = r.reshape(2, 8, 128)
        guess_blocks(r)

        @pl.when(i >= 1)
        def _():
            out_copy(pl.multiple_of((i - 1) * OB, OB), OB, 0).start()
        return wrap(wr + 3), wrap(rd + UNROLL)
    lax.fori_loop(0, NSEG // UNROLL, steps, (jnp.int32(0), jnp.int32(NRING - BULK // SEG)))

    for cp in ffn_copies:
        cp.wait()

    def two(ref, a, b):
        return jnp.concatenate([ref[pl.ds(a, 8), :], ref[pl.ds(b, 8), :]], axis=0)

    def ffn_act(h, c):
        g = _rb(jnp.dot(h, wg_v[:, pl.ds(512 * c, 512)], preferred_element_type=F32))
        u = _rb(jnp.dot(h, wu_v[:, pl.ds(512 * c, 512)], preferred_element_type=F32))
        return (_rb(g * jax.nn.sigmoid(g)) * u).astype(BF)

    def ffn_down(a, c):
        wd = jnp.concatenate([wd_v[k, pl.ds(512 * c, 512), :] for k in range(2)], axis=1)
        return jnp.dot(a, wd, preferred_element_type=F32)

    early = _rb(r_v[pl.ds(0, 2)].reshape(16, 128))

    def guessed(k):
        j = S - 1 - (pltpu.bitcast(r_v[2 + k], jnp.int32) & (S - 1))
        return pl.multiple_of(jnp.minimum(j[0, 0] >> 3, (S - 48) // 8) * 8, 8)
    gs_a, gs_b = guessed(0), guessed(1)
    h_gs = two(ho_v.at[0], gs_a, gs_b)
    acts = [ffn_act(h_gs, c) for c in range(NSPEC)]

    last, done = [], []
    never = jnp.full((8, 128), gs_a, jnp.int32) < 0
    for q in range(5):
        items = post_work(S - 40 + 8 * q, functools.partial(carried, q), last)
        items[0](None)
        for item in items[1:]:
            done.append(item((never, pltpu.bitcast(done[-2], F32)) if len(done) >= 2 else None))
    out_copy(S - OB, OB, 0).start()

    def top2(val, idx, valid):
        def reduce(f, v):
            v = f(v, axis=0, keepdims=True)
            return v if v.shape[1] == 1 else f(v, axis=1, keepdims=True)

        def argtop(ok):
            v = jnp.where(ok, val, -jnp.inf)
            m = reduce(jnp.max, v)
            return m, reduce(jnp.min, jnp.where(ok & (v >= m), idx, float(S)))
        m1, i1 = argtop(valid)
        return (m1, i1), argtop(valid & (idx != i1))

    c_a, c_b = top2(early, idx.astype(F32), idx >= 0)
    sub2 = lax.broadcasted_iota(jnp.int32, (48, 1), 0)
    val2 = jnp.concatenate([_rb(r) for r in last] + [jnp.where(sub2[:8] == 0, c_a[0], c_b[0])],
                           axis=0)
    idx2 = jnp.where(sub2 < 40, (sub2 + (S - 40)).astype(F32),
                     jnp.where(sub2 == 40, c_a[1], c_b[1]))
    (m_a, i_a), (m_b, i_b) = top2(val2, idx2, sub2 < 42)
    i_a = i_a.astype(jnp.int32)
    i_b = i_b.astype(jnp.int32)
    ia = jnp.clip(i_a[0, 0], 0, S - 1)
    ib = jnp.clip(i_b[0, 0], 0, S - 1)
    blk_a = pl.multiple_of((ia // 8) * 8, 8)
    blk_b = pl.multiple_of((ib // 8) * 8, 8)

    hs = two(ho_v.at[0], blk_a, blk_b)
    y0 = y = None
    for c in range(1, FF // 512 + 1):
        if NSPEC <= c < FF // 512:
            acts.append(ffn_act(hs, c))
        t = ffn_down(acts[c - 1], c - 1)
        if c <= NSPEC:
            y0 = t if y0 is None else t + y0
        else:
            y = t if y is None else t + y
    sub = lax.broadcasted_iota(jnp.int32, (16, 1), 0)
    rows = jnp.where(sub < 8, blk_a + sub, blk_b + sub - 8)
    gate = jnp.where(rows == ia, jax.nn.sigmoid(m_a),
                     jnp.where(rows == ib, jax.nn.sigmoid(m_b), 0.0))

    def finish(ffn):
        upd = jnp.where((rows == ia) | (rows == ib), ffn * gate, 0.0).reshape(2, 8, D)
        fin_v[...] = _b2(_f3(two(ho_v.at[1], blk_a, blk_b)) + mod_v[5] * upd)

    finish(y + y0)

    @pl.when((gs_a != blk_a) | (gs_b != blk_b))
    def _():
        redo = [ffn_act(hs, c) for c in range(NSPEC)]
        finish(functools.reduce(lambda a, c: ffn_down(redo[c], c) + a, range(NSPEC), y))

    def patch(k, blk):
        return pltpu.make_async_copy(fin_v.at[pl.ds(8 * k, 8), :],
                                     out_hbm.at[0, pl.ds(blk, 8), :], sems.at[3 + k])

    out_copy(0, S, 0).wait()
    patch(0, blk_a).start()

    @pl.when(blk_a != blk_b)
    def _():
        patch(1, blk_b).start()
        patch(1, blk_b).wait()
    patch(0, blk_a).wait()


@jax.jit
def pallas_adaLN_cond__memory_aug_recurrent_mem_tr__moe_arch_mod__prompt_kernel(
    A_x, A_mem0, A_Wq, A_Wk, A_Wv, A_Wo, A_seg_len, B_x, B_w_r, B_w_gate, B_w_up, B_w_down, c,
    w_mod,
):
    del B_x
    del A_seg_len
    assert A_x.shape == (1, S, D) and A_Wq.shape == (D, H, DH) and A_mem0.shape == (1, M, D)
    any_spec = pl.BlockSpec(memory_space=pl.ANY)
    scratch = [
        pltpu.VMEM((S, D), BF),
        pltpu.VMEM((4, X0, QK), BF),
        pltpu.VMEM((4, BULK // 2, QK), U32),
        pltpu.VMEM((40, D), BF),
        pltpu.VMEM((2, S, D), BF),
        pltpu.VMEM((100 * PITCH, 128), U32),
        pltpu.VMEM((2, H * DH, 512), BF),
        pltpu.VMEM((5 * D, 8, 128), BF),
        pltpu.VMEM((12, D, 512), BF),
        pltpu.VMEM((D, FF), BF),
        pltpu.VMEM((D, FF), BF),
        pltpu.VMEM((2, FF, 512), BF),
        pltpu.VMEM((M, D), BF),
        pltpu.VMEM((4, 1, D), BF),
        pltpu.VMEM((7, 8, D), F32),
        pltpu.VMEM((4, 8, 128), F32),
        pltpu.VMEM((D, 128), F32),
        pltpu.VMEM((12, 8, 512), F32),
        pltpu.VMEM((NP, 4, BULK, 256), F32),
        pltpu.VMEM((16, D), BF),
        pltpu.SemaphoreType.DMA((9,)),
    ] + [pltpu.VMEM((6, NRING, 32, 128), U32)] * 8
    return pl.pallas_call(
        _kernel,
        out_shape=jax.ShapeDtypeStruct((1, S, D), BF),
        in_specs=[any_spec] * 12,
        out_specs=any_spec,
        scratch_shapes=scratch,
        compiler_params=pltpu.CompilerParams(vmem_limit_bytes=120 * 1024 * 1024),
    )(A_x, A_mem0, A_Wq, A_Wk, A_Wv, A_Wo.reshape(H * DH, D), B_w_r.reshape(1, D), B_w_gate,
      B_w_up, B_w_down, c, w_mod)
```
